```python
import jax
import jax.numpy as jnp

def _softmax(x, axis=-1):
    return jax.nn.softmax(x, axis=axis)
def _gelu(x):
    return jax.nn.gelu(x, approximate=True)
def _silu(x):
    return jax.nn.silu(x)
def _sigmoid(x):
    return jax.nn.sigmoid(x)
def _layernorm(x, axis=-1, eps=1e-5):
    m = jnp.mean(x, axis=axis, keepdims=True)
    v = jnp.var(x, axis=axis, keepdims=True)
    return (x - m) / jnp.sqrt(v + eps)
def _scatter_add(tgt, idx, src, axis=0):
    return tgt.at[idx].add(src)
def _segment_sum(src, seg, n):
    return jax.ops.segment_sum(src, seg, n)
class _Rng:
    def __init__(self, key):
        self._k = key
    def _next(self):
        self._k, sub = jax.random.split(self._k)
        return sub
    def normal(self, shape):
        return jax.random.normal(self._next(), shape, dtype=jnp.bfloat16)
    def randint(self, lo, hi, shape):
        return jax.random.randint(self._next(), shape, lo, hi, dtype=jnp.int32)
    def uniform(self, shape, lo=0.0, hi=1.0):
        return jax.random.uniform(self._next(), shape, jnp.bfloat16, lo, hi)
    def permutation(self, n):
        return jax.random.permutation(self._next(), n)


kernel_name = 'interleave_layers__sliding_local_dilated__glu_gated_bilinear__prompt'

def setup_inputs():
    _rng = _Rng(jax.random.key(int.from_bytes(__import__("os").urandom(4), "little")))
    _w = (lambda a: (lambda t: t.astype(jnp.bfloat16) if jnp.issubdtype(t.dtype, jnp.floating) else t)(jnp.asarray(a)))
    def _A_setup():
        B, S, D = 1, 2048, 576
        return {
            "x": _w((lambda *s: _rng.normal(s) * 0.05)(B, S, D)),
            "wqkv": _w((lambda *s: _rng.normal(s) * 0.05)(D, 3 * D)),
            "wo": _w((lambda *s: _rng.normal(s) * 0.05)(D, D)),
        }
    _A_in = _A_setup()

    def _B_setup():
        B, S, D, F = 1, 2048, 576, 4608
        return {
            "x": _w((lambda *s: _rng.normal(s) * 0.05)(B, S, D)),
            "w_gate": _w((lambda *s: _rng.normal(s) * 0.05)(D, F) * (D ** -0.5)),
            "w_up": _w((lambda *s: _rng.normal(s) * 0.05)(D, F) * (D ** -0.5)),
            "w_down": _w((lambda *s: _rng.normal(s) * 0.05)(F, D) * (F ** -0.5)),
        }
    _B_in = _B_setup()

    return {
        "A_x": _A_in["x"],
        "A_wqkv": _A_in["wqkv"],
        "A_wo": _A_in["wo"],
        "B_x": _B_in["x"],
        "B_w_gate": _B_in["w_gate"],
        "B_w_up": _B_in["w_up"],
        "B_w_down": _B_in["w_down"],
    }

def reference(A_x, A_wqkv, A_wo, B_x, B_w_gate, B_w_up, B_w_down):
    def _A_ref(x, wqkv, wo):
        B, S, D = x.shape
        H = 32; Dh = D // H
        W, dil = 8, 2
        qkv = (lambda x, *d: x.transpose(*d))((x @ wqkv).reshape(B, S, 3, H, Dh), 2, 0, 3, 1, 4)
        q, k, v = qkv[0], qkv[1], qkv[2]
        scale = Dh ** -0.5
        pos = jnp.arange(S)
        off = jnp.arange(W) * dil
        idx = pos[:, None] - off[None, :]
        mask = idx >= 0
        idx_c = jnp.where(mask, idx, 0).reshape(-1)
        kg = k[:, :, idx_c, :].reshape(B, H, S, W, Dh)
        vg = v[:, :, idx_c, :].reshape(B, H, S, W, Dh)
        logits = jnp.einsum("bhsd,bhswd->bhsw", q, kg) * scale
        logits = jnp.where(mask[None, None, :, :], logits, -1e9)
        attn = _softmax(logits, axis=-1)
        o = jnp.einsum("bhsw,bhswd->bhsd", attn, vg)
        return (lambda x, *d: x.transpose(*d))(o, 0, 2, 1, 3).reshape(B, S, D) @ wo

    def _B_ref(x, w_gate, w_up, w_down):
        g = jnp.einsum("bsd,df->bsf", x, w_gate)
        u = jnp.einsum("bsd,df->bsf", x, w_up)
        h = g * u
        return jnp.einsum("bsf,fd->bsd", h, w_down)

    x = A_x
    x = x + _A_ref(_layernorm(x, axis=-1), A_wqkv, A_wo)
    x = x + _B_ref(_layernorm(x, axis=-1), B_w_gate, B_w_up, B_w_down)
    x = x + _A_ref(_layernorm(x, axis=-1), A_wqkv, A_wo)
    x = x + _B_ref(_layernorm(x, axis=-1), B_w_gate, B_w_up, B_w_down)
    return x
```

```python
import functools

import jax
import jax.numpy as jnp
import jax.experimental.pallas as pl
import jax.experimental.pallas.tpu as pltpu

S, D, F = 2048, 576, 4608
H, DH, W = 32, 18, 8
NB = 8
TM = NB * 128
HM = TM // 2
HD = D // 2
FC = 512
HC = FC // 2
NSLOT = 17
EPS = 1e-5
f32, bf16 = jnp.float32, jnp.bfloat16

_dot = functools.partial(jnp.dot, preferred_element_type=f32)


def _dot_nt(a, b):
    return jax.lax.dot_general(a, b, (((1,), (1,)), ((), ())), preferred_element_type=f32)


def _vcat(*xs):
    return jnp.concatenate(xs, axis=0)


def _layernorm_t(x):
    m = jnp.sum(x, axis=0, keepdims=True) * (1.0 / D)
    xc = x - m
    v = jnp.sum(xc * xc, axis=0, keepdims=True) * (1.0 / D)
    return xc * jax.lax.rsqrt(v + EPS)


def _kernel(x_hbm, wqkv_hbm, wo_hbm, wg_hbm, wu_hbm, wd_hbm, out_hbm,
            xin, wqkv, wo, wg, wu, wd, wqkv_t, wo_t, perm, xres, q_s, k_s, v_s,
            a_s, acc, sems):
    groups = ((0, 2048), (2048, 2048), (4096, 512))

    def small_copies():
        return [pltpu.make_async_copy(x_hbm, xin, sems.at[0]),
                pltpu.make_async_copy(wqkv_hbm, wqkv, sems.at[1]),
                pltpu.make_async_copy(wo_hbm, wo, sems.at[2])]

    def ffn_copies(g):
        off, n = groups[g]
        return [pltpu.make_async_copy(src.at[:, pl.ds(off, n)], dst.at[:, pl.ds(off, n)],
                                      sems.at[3 + 3 * g + i])
                for i, (src, dst) in enumerate(((wg_hbm, wg), (wu_hbm, wu), (wd_hbm, wd)))]

    cx, cqkv, cwo = small_copies()
    cqkv.start()
    cx.start()
    cwo.start()
    for g in range(len(groups)):
        for c in ffn_copies(g):
            c.start()

    def pad_rows(r):
        return _vcat(r, jnp.zeros((128 - r.shape[0], r.shape[1]), r.dtype))

    cqkv.wait()
    for g in range(5):
        rows = wqkv[g * 128:min((g + 1) * 128, D), :].astype(f32)
        if g == 4:
            rows = pad_rows(rows)
        perm[g, 0:3 * D, :] = rows.T

    def qkv_rows(pd, c):
        part = pd // DH
        d = pd - part * DH
        dst = pl.multiple_of(pd * H, H)
        for g in range(5):
            r = perm[g, pl.ds(part * D + d, H, stride=DH), :].astype(bf16)
            if g == 4:
                wqkv_t[pl.ds(dst, H), 512:D] = r[:, :64]
            else:
                wqkv_t[pl.ds(dst, H), g * 128:(g + 1) * 128] = r
        return c
    jax.lax.fori_loop(0, 3 * DH, qkv_rows, 0)

    cwo.wait()
    for g in range(5):
        if g == 4:
            cols = wo[:, 512:D].astype(f32)
            perm[g, 0:D, :] = jnp.concatenate([cols, jnp.zeros_like(cols)], axis=1)
        else:
            perm[g, 0:D, :] = wo[:, g * 128:(g + 1) * 128].astype(f32)
    for g in range(5):
        r = _vcat(*[perm[g, pl.ds(d, H, stride=DH), :] for d in range(DH)])
        rt = r.astype(bf16).T
        if g == 4:
            wo_t[512:D, :] = rt[:64]
        else:
            wo_t[g * 128:(g + 1) * 128, :] = rt

    cx.wait()

    def in_t1(c, carry):
        off = pl.multiple_of(c * 128, 128)
        for g in range(5):
            r = xin[g * 128:min((g + 1) * 128, D), pl.ds(off, 128)].astype(f32)
            if g == 4:
                r = pad_rows(r)
            perm[g, pl.ds(off, 128), :] = r.T
        return carry
    jax.lax.fori_loop(0, 16, in_t1, 0)

    def in_t2(jt, carry):
        t = jt % 2
        j = jt // 2
        for g in range(5):
            r = perm[g, pl.ds(jt, 128, stride=16), :].T
            if g == 4:
                xres[t, j, 512:D, :] = r[:64]
            else:
                xres[t, j, g * 128:(g + 1) * 128, :] = r
        return carry
    jax.lax.fori_loop(0, 16, in_t2, 0)
    acc[...] = jnp.zeros_like(acc)

    def combine(t, i):
        cols = pl.ds(pl.multiple_of(i * 128, 128), 128)
        m1, m2, m3, m4, m5, m6, m7 = [acc[t, n, :, cols] for n in range(7)]
        x1 = xres[t, i] + _vcat(m1 + m4 - m5 + m7, m2 + m4)
        x2 = xres[t, i + 4] + _vcat(m3 + m5, m1 - m2 + m3 + m6)
        return x1, x2

    def phase1(t, i):
        x1, x2 = combine(t, i)
        cols = pl.ds(pl.multiple_of(i * 128, 128), 128)
        for n in range(7):
            acc[t, n, :, cols] = jnp.zeros((HD, 128), f32)
        xres[t, i] = x1
        xres[t, i + 4] = x2
        xn = jnp.concatenate([_layernorm_t(x1).astype(bf16), _layernorm_t(x2).astype(bf16)], axis=1)
        qkv = _dot(wqkv_t[...], xn)
        for n, b in enumerate((i, i + 4)):
            part = qkv[:, n * 128:(n + 1) * 128]
            q_s[b] = part[0:D].reshape(DH, H, 128)
            for dst, r in ((k_s, part[D:2 * D]), (v_s, part[2 * D:3 * D])):
                dst[b + NB] = r.reshape(DH, H, 128)
                dst[b] = pltpu.roll(r, 1, 1).reshape(DH, H, 128)

    def attention(b):
        lane = jax.lax.broadcasted_iota(jnp.int32, (8, 128), 1)
        outs = []
        for g in range(H // 8):
            hs = slice(g * 8, (g + 1) * 8)
            q = q_s[b, :, hs, :]
            logits = []
            for w in range(W):
                l = jnp.sum(q * k_s[b + NB - w, :, hs, :], axis=0) * (DH ** -0.5)
                if w > 0:
                    l = jnp.where(lane < (w > b).astype(jnp.int32), -1e9, l)
                logits.append(l)
            m = functools.reduce(jnp.maximum, logits)
            e = [jnp.exp(l - m) for l in logits]
            r = 1.0 / functools.reduce(jnp.add, e)
            o = (e[0] * r)[None] * v_s[b + NB, :, hs, :]
            for w in range(1, W):
                o = o + (e[w] * r)[None] * v_s[b + NB - w, :, hs, :]
            outs.append(o)
        return jnp.concatenate(outs, axis=1).reshape(D, 128).astype(bf16)

    def phase2(t, i):
        o = jnp.concatenate([attention(i), attention(i + 4)], axis=1)
        a = _dot(wo_t[...], o)
        x1 = xres[t, i] + a[:, :128]
        x2 = xres[t, i + 4] + a[:, 128:]
        xres[t, i] = x1
        xres[t, i + 4] = x2
        n1 = _layernorm_t(x1)
        n2 = _layernorm_t(x2)
        a11, a12, a21, a22 = n1[0:192], n1[192:384], n2[0:192], n2[192:384]
        e11, e12, e21, e22 = n1[384:448], n1[448:512], n2[384:448], n2[448:512]
        r1, r2 = n1[512:D], n2[512:D]
        z = jnp.zeros((64, 128), f32)
        ops = _vcat(a11 + a22, z,
                    a21 + a22, -(e21 + e22),
                    a11, e22,
                    a22, e11,
                    a11 + a12, -(e11 + e12),
                    a21 - a11, r2,
                    a12 - a22, r1,
                    e11 + e22, z,
                    e21 - e11, r2,
                    e12 - e22, r1)
        a_s[t, pl.ds(pl.multiple_of(i * 128, 128), 128), :] = ops.astype(bf16).T

    def proj(t, w_ref, off):
        ca = pl.ds(off, HC)
        cb = pl.ds(pl.multiple_of(off + HC, HC), HC)
        b11, b12, b21, b22 = w_ref[0:192, ca], w_ref[0:192, cb], w_ref[192:384, ca], w_ref[192:384, cb]
        c11, c12, c21, c22 = w_ref[384:448, cb], w_ref[384:448, ca], w_ref[448:512, cb], w_ref[448:512, ca]
        ra, rb = w_ref[512:D, ca], w_ref[512:D, cb]
        add = lambda x, y: (x.astype(f32) + y.astype(f32)).astype(bf16)
        sub = lambda x, y: (x.astype(f32) - y.astype(f32)).astype(bf16)
        lhs = lambda s, n: a_s[t, :, s * 128:s * 128 + n]
        p1 = _dot(lhs(0, 192), add(b11, b22))
        p2 = _dot(lhs(2, 256), _vcat(b11, c11))
        p3 = _dot(lhs(4, 256), _vcat(sub(b12, b22), sub(c21, c11)))
        p4 = _dot(lhs(6, 256), _vcat(sub(b21, b11), sub(c12, c22)))
        p5 = _dot(lhs(8, 256), _vcat(b22, c22))
        p6 = _dot(lhs(10, 256), _vcat(add(b11, b12), rb))
        p7 = _dot(lhs(12, 256), _vcat(add(b21, b22), ra))
        q1 = _dot(lhs(14, 64), add(c11, c22))
        q6 = _dot(lhs(15, 128), _vcat(add(c11, c12), ra))
        q7 = _dot(lhs(16, 128), _vcat(add(c21, c22), rb))
        return (p1 + p4 - p5 + p7, q1 + p3 + p5 + q7, q1 + p2 + p4 + q6, p1 - p2 + p3 + p6)

    def ffn_chunk(t, j):
        off = pl.multiple_of(j * FC, FC)
        g = proj(t, wg, off)
        u = proj(t, wu, off)
        b11, b21, b12, b22 = [x * y for x, y in zip(g, u)]
        ca = pl.ds(off, HC)
        cb = pl.ds(pl.multiple_of(off + HC, HC), HC)
        a11, a12, a21, a22 = wd[0:HD, ca], wd[0:HD, cb], wd[HD:D, ca], wd[HD:D, cb]
        add = lambda x, y: (x.astype(f32) + y.astype(f32)).astype(bf16)
        sub = lambda x, y: (x.astype(f32) - y.astype(f32)).astype(bf16)
        acc[t, 0] += _dot_nt(add(a11, a22), add(b11, b22))
        acc[t, 1] += _dot_nt(add(a21, a22), b11.astype(bf16))
        acc[t, 2] += _dot_nt(a11, sub(b12, b22))
        acc[t, 3] += _dot_nt(a22, sub(b21, b11))
        acc[t, 4] += _dot_nt(add(a11, a12), b22.astype(bf16))
        acc[t, 5] += _dot_nt(sub(a21, a11), add(b11, b12))
        acc[t, 6] += _dot_nt(sub(a12, a22), add(b21, b22))

    def loop(n, fn):
        def body(i, c):
            fn(i)
            return c
        jax.lax.fori_loop(0, n, body, 0)

    loop(4, lambda i: phase1(0, i))
    loop(4, lambda i: phase2(0, i))

    def wait_group(k, g):
        @pl.when(k == 0)
        def _():
            for c in ffn_copies(g):
                c.wait()

    def stage(k):
        t = k % 2
        n_ab = jnp.where(k < 3, 4, 0)

        def body_a(i):
            phase1(1 - t, i)
            ffn_chunk(t, i)

        def body_b(i):
            ffn_chunk(t, 4 + i)
            phase2(1 - t, i)

        wait_group(k, 0)
        loop(n_ab, body_a)
        wait_group(k, 1)
        loop(n_ab, body_b)
        wait_group(k, 2)
        loop(9 - 2 * n_ab, lambda i: ffn_chunk(t, 2 * n_ab + i))
    loop(4, stage)

    def out_t1(ti, carry):
        t = ti // 4
        i = ti - 4 * t
        for x, b in zip(combine(t, i), (i, i + 4)):
            xb = x.astype(bf16).astype(f32)
            for g in range(5):
                r = xb[g * 128:min((g + 1) * 128, D)]
                if g == 4:
                    r = pad_rows(r)
                perm[g, pl.ds(2 * b + t, 128, stride=16), :] = r.T
        return carry
    jax.lax.fori_loop(0, 8, out_t1, 0)

    def out_t2(c, carry):
        off = pl.multiple_of(c * 128, 128)
        for g in range(5):
            r = perm[g, pl.ds(off, 128), :].astype(bf16).T
            if g == 4:
                xin[512:D, pl.ds(off, 128)] = r[:64]
            else:
                xin[g * 128:(g + 1) * 128, pl.ds(off, 128)] = r
        return carry
    jax.lax.fori_loop(0, 16, out_t2, 0)
    cout = pltpu.make_async_copy(xin, out_hbm, sems.at[0])
    cout.start()
    cout.wait()


@jax.jit
def pallas_interleave_layers__sliding_local_dilated__glu_gated_bilinear__prompt_kernel(
    A_x: jax.Array,
    A_wqkv: jax.Array,
    A_wo: jax.Array,
    B_x: jax.Array,
    B_w_gate: jax.Array,
    B_w_up: jax.Array,
    B_w_down: jax.Array,
):
    any_spec = pl.BlockSpec(memory_space=pl.ANY)
    out_t = pl.pallas_call(
        _kernel,
        in_specs=[any_spec] * 6,
        out_specs=any_spec,
        out_shape=jax.ShapeDtypeStruct((D, S), bf16),
        scratch_shapes=[
            pltpu.VMEM((D, S), bf16),
            pltpu.VMEM((D, 3 * D), bf16),
            pltpu.VMEM((D, D), bf16),
            pltpu.VMEM((D, F), bf16),
            pltpu.VMEM((D, F), bf16),
            pltpu.VMEM((D, F), bf16),
            pltpu.VMEM((3 * D, D), bf16),
            pltpu.VMEM((D, D), bf16),
            pltpu.VMEM((5, S, 128), f32),
            pltpu.VMEM((2, NB, D, 128), f32),
            pltpu.VMEM((NB, DH, H, 128), f32),
            pltpu.VMEM((2 * NB, DH, H, 128), f32),
            pltpu.VMEM((2 * NB, DH, H, 128), f32),
            pltpu.VMEM((2, HM, NSLOT * 128), bf16),
            pltpu.VMEM((2, 7, HD, HM), f32),
            pltpu.SemaphoreType.DMA((12,)),
        ],
        compiler_params=pltpu.CompilerParams(vmem_limit_bytes=110 * 1024 * 1024),
        name="fused_layers",
    )(A_x[0].T, A_wqkv, A_wo, B_w_gate, B_w_up, B_w_down.T)
    return out_t.T[None]
```

```python
import functools
import os

import jax
import jax.numpy as jnp
import jax.experimental.pallas as pl
import jax.experimental.pallas.tpu as pltpu

S, D, F = 2048, 576, 4608
H, DH, W = 32, 18, 8
NG = H // 8
GR = 8 * DH
NB = 8
TM = NB * 128
HM = TM // 2
HD = D // 2
FC = 512
HC = FC // 2
NCH = F // FC
NSLOT = 17
EPS = 1e-5
KA = int(os.environ.get("KA", 13))
KB = int(os.environ.get("KB", 13))
PAR = int(os.environ.get("PAR", 2))
PAR0 = int(os.environ.get("PAR0", 3))
ORDER_A = "s" + "m" * KA + "ss"
ORDER_B = "s" + "m" * KB + "s" + "m" * (16 - KB) + "s"
f32, bf16, u32 = jnp.float32, jnp.bfloat16, jnp.uint32

_dot = functools.partial(jnp.dot, preferred_element_type=f32)


def _dot_nt(a, b):
    return jax.lax.dot_general(a, b, (((1,), (1,)), ((), ())), preferred_element_type=f32)


def _vcat(*xs):
    return jnp.concatenate(xs, axis=0)


def _pad_rows(r):
    return _vcat(r, jnp.zeros((128 - r.shape[0], r.shape[1]), r.dtype))


def _add(x, y):
    return (x.astype(f32) + y.astype(f32)).astype(bf16)


def _sub(x, y):
    return (x.astype(f32) - y.astype(f32)).astype(bf16)


def _layernorm_t(x, zero=None):
    rows = [x[r:r + 8] for r in range(0, D, 8)]
    s = rows[0] if zero is None else rows[0] + zero
    for r in rows[1:]:
        s = s + r
    m = jnp.sum(s, axis=0, keepdims=True) * (1.0 / D)
    rows = [r - m for r in rows]
    s = rows[0] * rows[0]
    for r in rows[1:]:
        s = s + r * r
    v = jnp.sum(s, axis=0, keepdims=True) * (1.0 / D)
    return _vcat(*rows) * jax.lax.rsqrt(v + EPS)


def _drain(*gens):
    for gen in gens:
        for _ in gen:
            pass


def _weave(order, main, side):
    for c in order:
        next(main if c == "m" else side)
    _drain(main, side)


def _scope(name):
    import contextlib
    return jax.named_scope(name) if os.environ.get("SCOPES") else contextlib.nullcontext()


def _loop(n, fn):
    def body(i, c):
        with _scope("it"):
            fn(i)
        return c
    jax.lax.fori_loop(0, n, body, 0)


def _kernel(x_hbm, wqkv_hbm, wo_hbm, wg_hbm, wu_hbm, wd_hbm, out_hbm,
            xin, wqkv, wo, wg, wu, wd, wqkv_t, wo_t, wperm, operm, pin, pout, xres,
            q0, k0, v0, q_s, k_s, v_s, a_s, acc, xn_s, sems):
    groups = ((0, 5 * FC), (5 * FC, 4 * FC))
    lane = jax.lax.broadcasted_iota(jnp.int32, (8, 128), 1)

    def x_copy(t, piece, n):
        cols = pl.ds(pl.multiple_of(t * TM + piece * n, 128), n)
        return pltpu.make_async_copy(x_hbm.at[:, cols], xin.at[:, cols], sems.at[10 + t + piece])

    def wqkv_copy(g):
        rows = pl.ds(g * 128, min(128, D - g * 128))
        return pltpu.make_async_copy(wqkv_hbm.at[rows], wqkv.at[rows], sems.at[15 + g])

    def out_copy(t, half):
        cols = pl.ds(t * TM + half * HM, HM)
        return pltpu.make_async_copy(xin.at[:, cols], out_hbm.at[:, cols], sems.at[2 * t + half])

    def ffn_copies(g):
        off, n = groups[g]
        return [pltpu.make_async_copy(src.at[:, pl.ds(off, n)], dst.at[:, pl.ds(off, n)],
                                      sems.at[4 + 3 * g + i])
                for i, (src, dst) in enumerate(((wg_hbm, wg), (wu_hbm, wu), (wd_hbm, wd)))]

    cwo = pltpu.make_async_copy(wo_hbm, wo, sems.at[3])
    x_copy(0, 0, TM).start()
    for g in range(5):
        wqkv_copy(g).start()

    def head_rows(ref, g, base):
        return _vcat(*[ref[g, pl.ds(base + d, 8, stride=DH), :] for d in range(DH)])

    def prep_wqkv():
        for gs in ((0, 1), (2, 3), (4,)):
            with _scope("w_qkv"):
                for g in gs:
                    wqkv_copy(g).wait()
            for g in gs:
                rows = wqkv[g * 128:min((g + 1) * 128, D), :].astype(f32)
                wperm[g] = (_pad_rows(rows) if g == 4 else rows).T
            for g in gs:
                for hg in range(3 * NG):
                    wqkv_t[g, hg * GR:(hg + 1) * GR, :] = head_rows(wperm, g, hg * GR).astype(bf16)

    def prep_wo():
        for g in range(5):
            cols = wo[:, g * 128:min((g + 1) * 128, D)].astype(f32)
            if g == 4:
                cols = jnp.concatenate([cols, jnp.zeros_like(cols)], axis=1)
            operm[g] = cols
        for g in range(5):
            r = _vcat(*[head_rows(operm, g, hg * GR) for hg in range(NG)], jnp.zeros((64, 128), f32))
            rt = r.astype(bf16).T
            n = 64 if g == 4 else 128
            for kt in range(5):
                wo_t[kt, g * 128:g * 128 + n, :] = rt[:n, kt * 128:(kt + 1) * 128]

    def lhs_full(ref):
        return jnp.concatenate([ref[0], ref[1], ref[2], ref[3], ref[4][:, :64]], axis=1)

    def in_t1(t, c):
        w = pltpu.bitcast(xin[:, pl.ds(pl.multiple_of(t * TM + c * 128, 128), 128)], u32)
        for g in range(3):
            r = w[g * 128:min((g + 1) * 128, HD)]
            r = (_pad_rows(r) if g == 2 else r).T
            for m in range(8):
                rows = pl.ds(pl.multiple_of((c * 8 + m) * 24, 8), 16)
                pin[t, g, rows, :] = r[m * 16:(m + 1) * 16]

    def in_t2(t, j):
        parts = []
        for g in range(3):
            r = _vcat(pin[t, g, pl.ds(2 * j + t, 64, stride=24), :],
                      pin[t, g, pl.ds(2 * j + 1 - t, 64, stride=24), :]).T
            parts.append(r[:32] if g == 2 else r)
        return pltpu.bitcast(_vcat(*parts), bf16).astype(f32)

    def out_t1(t, j, x):
        w = pltpu.bitcast(x.astype(bf16), u32)
        for g in range(3):
            r = w[g * 128:min((g + 1) * 128, HD)]
            r = (_pad_rows(r) if g == 2 else r).T
            for half in range(2):
                base = (2 * j + (half ^ t)) * 72
                pout[t, g, base:base + 64, :] = r[half * 64:(half + 1) * 64]

    def out_t2(t, c):
        parts = []
        for g in range(3):
            r = _vcat(*[pout[t, g, pl.ds(c * 8 + m, 16, stride=72), :] for m in range(8)]).T
            parts.append(r[:32] if g == 2 else r)
        xin[:, t * TM + c * 128:t * TM + (c + 1) * 128] = pltpu.bitcast(_vcat(*parts), bf16)

    def combine(t, i):
        cols = pl.ds(pl.multiple_of(i * 128, 128), 128)
        m1, m2, m3, m4, m5, m6, m7 = [acc[t, n, :, cols] for n in range(7)]
        x1 = xres[t, i] + _vcat(m1 + m4 - m5 + m7, m2 + m4)
        x2 = xres[t, i + 4] + _vcat(m3 + m5, m1 - m2 + m3 + m6)
        return x1, x2

    def store_qkv(t, b, part, q, k, v, prev=None):
        q[b] = part[0:D].reshape(NG, DH, 8, 128)
        for n, (dst, r) in enumerate(((k, part[D:2 * D]), (v, part[2 * D:3 * D]))):
            dst[b + NB] = r.reshape(NG, DH, 8, 128)
            sh = pltpu.roll(r, 1, 1).reshape(NG, DH, 8, 128)
            if isinstance(t, int) and t == 0:
                dst[b] = sh
            elif prev is not None:
                dst[b] = jnp.where(((lane & 63) == 0)[None, None], prev[n][b], sh)
            else:
                keep = jnp.broadcast_to(((lane & 63) >= t)[None, None], sh.shape)
                pltpu.store(dst.at[b], sh, mask=keep)

    def phase1(t, i):
        x1, x2 = combine(t, i)
        xres[t, i] = x1
        xres[t, i + 4] = x2
        n1 = _layernorm_t(x1)
        n2 = _layernorm_t(x2, jnp.where(lane < (i < 0).astype(jnp.int32), n1[0:8], 0.0))
        yield
        qkv = _dot(lhs_full(wqkv_t), jnp.concatenate([n1.astype(bf16), n2.astype(bf16)], axis=1))
        yield
        for n, b in enumerate((i, i + 4)):
            store_qkv(t, b, qkv[:, n * 128:(n + 1) * 128], q_s, k_s, v_s)
        yield

    def first_norm(t, b):
        x = in_t2(t, b)
        xres[t, b] = x
        xn_s[t, b] = _layernorm_t(x).astype(bf16)

    def first_qkv(t, b):
        qkv = _dot(lhs_full(wqkv_t), xn_s[t, b])
        if t == 0:
            store_qkv(t, b, qkv, q0, k0, v0)
        else:
            store_qkv(t, b, qkv, q_s, k_s, v_s, prev=(k0, v0))

    def attention_group(t, b, g, q_r, k_r, v_r, links):
        par = len(links)
        never = lane < (b < 0).astype(jnp.int32)

        def start(n, v):
            if links[n % par] is None:
                return v
            return jnp.where(never, links[n % par], 0.0) + v

        q = [q_r[b, g, d] for d in range(DH)]
        logits = []
        for w in range(W):
            l = start(w, q[0] * k_r[b + NB - w, g, 0])
            for d in range(1, DH):
                l = l + q[d] * k_r[b + NB - w, g, d]
            links[w % par] = l
            l = l * (DH ** -0.5)
            if w > 0:
                edge = jnp.logical_and(w > b, t == 0).astype(jnp.int32)
                l = jnp.where((lane & 63) < edge, -1e9, l)
            logits.append(l)
        m = functools.reduce(jnp.maximum, logits)
        e = [jnp.exp(l - m) for l in logits]
        r = 1.0 / functools.reduce(jnp.add, e)
        p = [x * r for x in e]
        outs = []
        for d in range(DH):
            o = p[0] * v_r[b + NB, g, d]
            if d >= par:
                o = start(d, o)
            for w in range(1, W):
                o = o + p[w] * v_r[b + NB - w, g, d]
            links[d % par] = o
            outs.append(o)
        return _vcat(*outs).astype(bf16)

    def phase2(t, i, par, q_r, k_r, v_r):
        links = [None] * par
        halves = [_vcat(*[attention_group(t, b, g, q_r, k_r, v_r, links) for g in range(NG)])
                  for b in (i, i + 4)]
        yield
        a = _dot(lhs_full(wo_t), jnp.concatenate(halves, axis=1))
        x1 = xres[t, i] + a[:, :128]
        x2 = xres[t, i + 4] + a[:, 128:]
        xres[t, i] = x1
        xres[t, i + 4] = x2
        n1 = _layernorm_t(x1)
        n2 = _layernorm_t(x2)
        yield
        a11, a12, a21, a22 = n1[0:192], n1[192:384], n2[0:192], n2[192:384]
        e11, e12, e21, e22 = n1[384:448], n1[448:512], n2[384:448], n2[448:512]
        r1, r2 = n1[512:D], n2[512:D]
        z = jnp.zeros((64, 128), f32)
        ops = _vcat(a11 + a22, z,
                    a21 + a22, -(e21 + e22),
                    a11, e22,
                    a22, e11,
                    a11 + a12, -(e11 + e12),
                    a21 - a11, r2,
                    a12 - a22, r1,
                    e11 + e22, z,
                    e21 - e11, r2,
                    e12 - e22, r1).astype(bf16).T
        rows = pl.ds(pl.multiple_of(i * 128, 128), 128)
        for s in range(NSLOT):
            a_s[t, s, rows, :] = ops[:, s * 128:(s + 1) * 128]
        yield

    def proj(t, w_ref, off, res):
        ca = pl.ds(off, HC)
        cb = pl.ds(pl.multiple_of(off + HC, HC), HC)
        b11, b12, b21, b22 = w_ref[0:192, ca], w_ref[0:192, cb], w_ref[192:384, ca], w_ref[192:384, cb]
        c11, c12, c21, c22 = w_ref[384:448, cb], w_ref[384:448, ca], w_ref[448:512, cb], w_ref[448:512, ca]
        ra, rb = w_ref[512:D, ca], w_ref[512:D, cb]

        def lhs(s, n):
            if n <= 128:
                return a_s[t, s][:, :n]
            return jnp.concatenate([a_s[t, s], a_s[t, s + 1][:, :n - 128]], axis=1)

        p1 = _dot(lhs(0, 192), _add(b11, b22))
        yield
        p2 = _dot(lhs(2, 256), _vcat(b11, c11))
        yield
        p3 = _dot(lhs(4, 256), _vcat(_sub(b12, b22), _sub(c21, c11)))
        yield
        p4 = _dot(lhs(6, 256), _vcat(_sub(b21, b11), _sub(c12, c22)))
        yield
        p5 = _dot(lhs(8, 256), _vcat(b22, c22))
        yield
        p6 = _dot(lhs(10, 256), _vcat(_add(b11, b12), rb))
        yield
        p7 = _dot(lhs(12, 256), _vcat(_add(b21, b22), ra))
        yield
        q1 = _dot(lhs(14, 64), _add(c11, c22))
        q6 = _dot(lhs(15, 128), _vcat(_add(c11, c12), ra))
        q7 = _dot(lhs(16, 128), _vcat(_add(c21, c22), rb))
        res.extend((p1 + p4 - p5 + p7, q1 + p3 + p5 + q7, q1 + p2 + p4 + q6, p1 - p2 + p3 + p6))
        yield

    def ffn_chunk(t, j, may_init=False):
        off = pl.multiple_of(j * FC, FC)
        g, u = [], []
        yield from proj(t, wg, off, g)
        yield from proj(t, wu, off, u)
        b11, b21, b12, b22 = [x * y for x, y in zip(g, u)]
        ca = pl.ds(off, HC)
        cb = pl.ds(pl.multiple_of(off + HC, HC), HC)
        a11, a12, a21, a22 = wd[0:HD, ca], wd[0:HD, cb], wd[HD:D, ca], wd[HD:D, cb]

        def accumulate(n, v):
            old = acc[t, n]
            if may_init:
                old = jnp.where(j > 0, old, 0.0)
            acc[t, n] = old + v

        accumulate(0, _dot_nt(_add(a11, a22), _add(b11, b22)))
        yield
        accumulate(1, _dot_nt(_add(a21, a22), b11.astype(bf16)))
        yield
        accumulate(2, _dot_nt(a11, _sub(b12, b22)))
        yield
        accumulate(3, _dot_nt(a22, _sub(b21, b11)))
        yield
        accumulate(4, _dot_nt(_add(a11, a12), b22.astype(bf16)))
        yield
        accumulate(5, _dot_nt(_sub(a21, a11), _add(b11, b12)))
        yield
        accumulate(6, _dot_nt(_sub(a12, a22), _add(b21, b22)))
        yield

    with _scope("w_x0"):
        x_copy(0, 0, TM).wait()
    for i in range(4):
        x_copy(1, i, 256).start()
    cwo.start()
    for c in range(NB):
        in_t1(0, c)
    for b in range(NB):
        first_norm(0, b)
    prep_wqkv()

    def body_f(i):
        with _scope("w_x1"):
            x_copy(1, i, 256).wait()
        first_qkv(0, i)
        first_qkv(0, i + 4)
        in_t1(1, 2 * i)
        in_t1(1, 2 * i + 1)

    def body_e(i):
        p2 = phase2(0, i, PAR0, q0, k0, v0)
        next(p2)
        first_qkv(1, i)
        next(p2)
        first_qkv(1, i + 4)
        _drain(p2)
        nxt = jnp.minimum(i + 1, 3)
        first_norm(1, nxt)
        first_norm(1, nxt + 4)

    for g in range(len(groups)):
        for c in ffn_copies(g):
            c.start()
    _loop(4, body_f)
    cwo.wait()
    prep_wo()
    first_norm(1, 0)
    first_norm(1, 4)
    _loop(4, body_e)

    def wait_group(k, g):
        @pl.when(k == 0)
        def _():
            for c in ffn_copies(g):
                c.wait()

    def stage(k):
        t = k % 2
        n_a = jnp.where(jnp.logical_and(k > 0, k < 3), 4, 0)
        n_b = jnp.where(k < 3, 4, 0)
        n_c = NCH - n_a - n_b
        wait_group(k, 0)
        _loop(n_c, lambda i: _drain(ffn_chunk(t, i, True)))
        _loop(n_a, lambda i: _weave(ORDER_A, ffn_chunk(t, n_c + i), phase1(1 - t, i)))
        wait_group(k, 1)
        _loop(n_b, lambda i: _weave(ORDER_B, ffn_chunk(t, n_c + n_a + i),
                                    phase2(1 - t, i, PAR, q_s, k_s, v_s)))
    _loop(4, stage)

    def finish(t):
        for i in range(4):
            x1, x2 = combine(t, i)
            out_t1(t, i, x1)
            out_t1(t, i + 4, x2)
        for c in range(NB):
            out_t2(t, c)
            if c % 4 == 3:
                out_copy(t, c // 4).start()

    finish(0)
    finish(1)
    with _scope("w_out"):
        for t in range(2):
            for half in range(2):
                out_copy(t, half).wait()


@jax.jit
def pallas_interleave_layers__sliding_local_dilated__glu_gated_bilinear__prompt_kernel(
    A_x: jax.Array,
    A_wqkv: jax.Array,
    A_wo: jax.Array,
    B_x: jax.Array,
    B_w_gate: jax.Array,
    B_w_up: jax.Array,
    B_w_down: jax.Array,
):
    any_spec = pl.BlockSpec(memory_space=pl.ANY)
    qkv_scratch = [
        pltpu.VMEM((NB, NG, DH, 8, 128), f32),
        pltpu.VMEM((2 * NB, NG, DH, 8, 128), f32),
        pltpu.VMEM((2 * NB, NG, DH, 8, 128), f32),
    ]
    out_t = pl.pallas_call(
        _kernel,
        in_specs=[any_spec] * 6,
        out_specs=any_spec,
        out_shape=jax.ShapeDtypeStruct((D, S), bf16),
        scratch_shapes=[
            pltpu.VMEM((D, S), bf16),
            pltpu.VMEM((D, 3 * D), bf16),
            pltpu.VMEM((D, D), bf16),
            pltpu.VMEM((D, F), bf16),
            pltpu.VMEM((D, F), bf16),
            pltpu.VMEM((D, F), bf16),
            pltpu.VMEM((5, 3 * D, 128), bf16),
            pltpu.VMEM((5, D, 128), bf16),
            pltpu.VMEM((5, 3 * D, 128), f32),
            pltpu.VMEM((5, D, 128), f32),
            pltpu.VMEM((2, 3, 64 * 24, 128), u32),
            pltpu.VMEM((2, 3, 16 * 72, 128), u32),
            pltpu.VMEM((2, NB, D, 128), f32),
            *qkv_scratch,
            *qkv_scratch,
            pltpu.VMEM((2, NSLOT, HM, 128), bf16),
            pltpu.VMEM((2, 7, HD, HM), f32),
            pltpu.VMEM((2, NB, D, 128), bf16),
            pltpu.SemaphoreType.DMA((20,)),
        ],
        compiler_params=pltpu.CompilerParams(vmem_limit_bytes=120 * 1024 * 1024),
        name="fused_layers",
    )(A_x[0].T, A_wqkv, A_wo, B_w_gate, B_w_up, B_w_down.T)
    return out_t.T[None]
```

```python
import functools
import os

import jax
import jax.numpy as jnp
import jax.experimental.pallas as pl
import jax.experimental.pallas.tpu as pltpu

S, D, F = 2048, 576, 4608
H, DH, W = 32, 18, 8
NG = H // 8
GR = 8 * DH
NB = 8
TM = NB * 128
HM = TM // 2
HD = D // 2
HQ = 3 * D // 2
FC = 512
HC = FC // 2
NCH = F // FC
NSLOT = 16
NT = int(os.environ.get("NT", 128))

GROUP_ROWS = {1: (0, 128), 2: (64, 192), 4: (256, 384), 3: (320, 448), 0: (512, 512)}
T3 = 1.0 / 3.0
SLOTS = (
    ((1, (-1, -1, 0, 0), (0, 0, 0, 1)), (3, (1, 1, 0, 0), (0, 0, 1, 0))),
    ((0, (T3, 0, 0, 0), (2, 1, 0, 0)), (2, (-.5, -1, 0, 0), (0, 0, 0, 1))),
    ((4, (.5, 1, 0, 0), (0, 0, 1, 0)), (0, (-T3, 0, 0, 0), (1, 2, 0, 0))),
    ((1, (0, 1, 0, -1), (0, 0, 1, 1)), (2, (0, 2, 0, -1), (0, 0, .5, 1))),
    ((1, (0, 0, 1, 1), (1, 0, 0, 0)), (3, (0, 0, -1, -1), (0, 1, 0, 0))),
    ((0, (0, 0, T3, 0), (2, 1, 0, 0)), (2, (0, 0, .5, 1), (1, 0, 0, 0))),
    ((4, (0, 0, -.5, -1), (0, 1, 0, 0)), (0, (0, 0, -T3, 0), (1, 2, 0, 0))),
    ((1, (-1, 0, 1, 0), (1, 1, 0, 0)), (2, (-1, 0, .5, 0), (1, 2, 0, 0))),
    ((1, (0, 0, 0, 1), (-1, 0, 1, 0)), (3, (1, 0, 0, 0), (1, 0, -1, 0))),
    ((4, (.5, 0, 0, 0), (2, 0, -1, 0)), (2, (0, 0, 0, 1), (-1, 0, .5, 0))),
    ((4, (-1, 0, .5, 0), (2, 1, 0, 0)), (3, (-1, 0, 1, 0), (1, 1, 0, 0))),
    ((1, (1, 0, 0, 1), (1, 0, 0, 1)), (2, (1, 0, 0, 1), (1, 0, 0, 1))),
    ((1, (1, 0, 0, 0), (0, 1, 0, -1)), (3, (0, 0, 0, 1), (0, -1, 0, 1))),
    ((4, (0, 0, 0, 1), (0, -1, 0, .5)), (2, (.5, 0, 0, 0), (0, 2, 0, -1))),
    ((4, (0, 2, 0, -1), (0, 0, 1, .5)), (3, (0, 1, 0, -1), (0, 0, 1, 1))),
    ((4, (1, 0, 0, 1), (0, 1, 1, 0)), (3, (1, 0, 0, 1), (0, 1, 1, 0))),
)
EPS = 1e-5
KA = int(os.environ.get("KA", 13))
KB = int(os.environ.get("KB", 13))
PAR = int(os.environ.get("PAR", 2))
PAR0 = int(os.environ.get("PAR0", 3))
ORDER_A = "s" + "m" * KA + "ss"
ORDER_B = "s" + "m" * KB + "s" + "m" * (2048 // NT - KB) + "s"
ORDER_E = "s" + "m" * int(os.environ.get("KE", 3)) + "s"
f32, bf16, u32 = jnp.float32, jnp.bfloat16, jnp.uint32

_dot = functools.partial(jnp.dot, preferred_element_type=f32)


def _dot_nt(a, b):
    return jax.lax.dot_general(a, b, (((1,), (1,)), ((), ())), preferred_element_type=f32)


def _vcat(*xs):
    return jnp.concatenate(xs, axis=0)


def _pad_rows(r):
    return _vcat(r, jnp.zeros((128 - r.shape[0], r.shape[1]), r.dtype))


def _add(x, y):
    return (x.astype(f32) + y.astype(f32)).astype(bf16)


def _sub(x, y):
    return (x.astype(f32) - y.astype(f32)).astype(bf16)


def _form(coefs, blocks):
    terms = [(c, blk) for c, blk in zip(coefs, blocks) if c != 0]
    if len(terms) == 1 and terms[0][0] == 1:
        return terms[0][1]()
    terms.sort(key=lambda cb: cb[0] < 0)
    out = None
    for c, blk in terms:
        v = blk().astype(f32)
        if out is None:
            out = v if c == 1 else v * c
        else:
            v = v if abs(c) == 1 else v * abs(c)
            out = out + v if c > 0 else out - v
    return out


def _lhs_slots(x1, x2):
    out = []
    for halves in SLOTS:
        for grp, coefs, _ in halves:
            k1, k2 = GROUP_ROWS[grp]
            blocks = [lambda x=x, k=k: x[k:k + 64] for x in (x1, x2) for k in (k1, k2)]
            out.append(_form(coefs, blocks))
    return out


def _lhs_slots_lanes(x1, x2):
    low = jax.lax.broadcasted_iota(jnp.int32, x1[0].shape, 1) < 64
    out = []
    for halves in SLOTS:
        keys = [(tuple(k // 128 for k in GROUP_ROWS[grp]), coefs) for grp, coefs, _ in halves]
        vals = [_form(coefs, [lambda x=x, g=g: x[g] for x in (x1, x2) for g in tiles])
                for tiles, coefs in keys]
        out.append(vals[0] if keys[0] == keys[1] else jnp.where(low, vals[0], vals[1]))
    return out


def _fast_product(p):
    p0, p1, p2, p3 = p(0), p(1), p(2), p(3)
    r = p0 + p1 + p2
    c11 = r + p1 + p3
    c12 = r + p2
    yield None
    p0, p1, p2, p3 = p(4), p(5), p(6), p(7)
    r = p0 + p1 + p2
    c21 = r + p1
    c22 = p3 - (r + p2)
    yield None
    p0, p1, p2, p3 = p(8), p(9), p(10), p(11)
    r = p0 + p1
    c11 = c11 + (r + p3)
    c21 = c21 + (r + p1 + p2)
    c22 = c22 + p3
    yield None
    p0, p1, p2, p3 = p(12), p(13), p(14), p(15)
    r = p0 + p1
    c12 = (r + p2 + p3) - c12
    c22 = c22 + (r + p1)
    c21 = c21 + p3
    yield (c11, c12, c21, c22)


def _rhs_slot(s, get):
    parts = []
    for grp, _, coefs in SLOTS[s]:
        k1, k2 = GROUP_ROWS[grp]
        blocks = [lambda k=k, c=c: get(slice(k, k + 64), c) for k in (k1, k2) for c in (0, 1)]
        parts.append(_form(coefs, blocks).astype(bf16))
    return _vcat(*parts)


def _layernorm_t(x, zero=None):
    rows = [x[r:r + 8] for r in range(0, D, 8)]
    s = rows[0] if zero is None else rows[0] + zero
    for r in rows[1:]:
        s = s + r
    m = jnp.sum(s, axis=0, keepdims=True) * (1.0 / D)
    rows = [r - m for r in rows]
    s = rows[0] * rows[0]
    for r in rows[1:]:
        s = s + r * r
    v = jnp.sum(s, axis=0, keepdims=True) * (1.0 / D)
    return _vcat(*rows) * jax.lax.rsqrt(v + EPS)


def _drain(*gens):
    for gen in gens:
        for _ in gen:
            pass


def _weave(order, main, side):
    for c in order:
        next(main if c == "m" else side)
    _drain(main, side)


def _scope(name):
    import contextlib
    return jax.named_scope(name) if os.environ.get("SCOPES") else contextlib.nullcontext()


def _loop(n, fn):
    def body(i, c):
        with _scope("it"):
            fn(i)
        return c
    jax.lax.fori_loop(0, n, body, 0)


def _kernel(x_hbm, wqkv_hbm, wo_hbm, wg_hbm, wu_hbm, wd_hbm, out_hbm,
            xin, wqkv, wo, wg, wu, wd, wqkv_t, wo_t, wperm, operm, pin, pout, xres,
            q0, k0, v0, q_s, k_s, v_s, a_s, acc, xn_s, sems):
    groups = ((0, 5 * FC), (5 * FC, 4 * FC))
    lane = jax.lax.broadcasted_iota(jnp.int32, (8, 128), 1)

    def x_copy(t, piece, n):
        cols = pl.ds(pl.multiple_of(t * TM + piece * n, 128), n)
        return pltpu.make_async_copy(x_hbm.at[:, cols], xin.at[:, cols], sems.at[10 + t + piece])

    def wqkv_copy(g):
        rows = pl.ds(g * 128, min(128, D - g * 128))
        return pltpu.make_async_copy(wqkv_hbm.at[rows], wqkv.at[rows], sems.at[15 + g])

    def out_copy(t, half):
        cols = pl.ds(t * TM + half * HM, HM)
        return pltpu.make_async_copy(xin.at[:, cols], out_hbm.at[:, cols], sems.at[2 * t + half])

    def ffn_copies(g):
        off, n = groups[g]
        return [pltpu.make_async_copy(src.at[:, pl.ds(off, n)], dst.at[:, pl.ds(off, n)],
                                      sems.at[4 + 3 * g + i])
                for i, (src, dst) in enumerate(((wg_hbm, wg), (wu_hbm, wu), (wd_hbm, wd)))]

    cwo = pltpu.make_async_copy(wo_hbm, wo, sems.at[3])
    x_copy(0, 0, TM).start()
    for g in range(5):
        wqkv_copy(g).start()

    def head_rows(ref, g, base):
        return _vcat(*[ref[g, pl.ds(base + d, 8, stride=DH), :] for d in range(DH)])

    def prep_wqkv():
        for gs in ((0, 1), (2, 3), (4,)):
            with _scope("w_qkv"):
                for g in gs:
                    wqkv_copy(g).wait()
            for g in gs:
                rows = wqkv[g * 128:min((g + 1) * 128, D), :].astype(f32)
                wperm[g] = (_vcat(rows, rows) if g == 4 else rows).T

        def rows_of(hg):
            base = pl.multiple_of(hg * GR, 16)
            x1 = [head_rows(wperm, g, base) for g in range(5)]
            x2 = [head_rows(wperm, g, base + HQ) for g in range(5)]
            for n, v in enumerate(_lhs_slots_lanes(x1, x2)):
                wqkv_t[n, pl.ds(base, GR), :] = v.astype(bf16)
        _loop(HQ // GR, rows_of)

    def prep_wo():
        for g in range(5):
            cols = wo[:, g * 128:min((g + 1) * 128, D)].astype(f32)
            if g == 4:
                cols = jnp.concatenate([cols, jnp.zeros_like(cols)], axis=1)
            operm[g] = cols
        parts = []
        for g in range(5):
            r = _vcat(*[head_rows(operm, g, hg * GR) for hg in range(NG)])
            rt = _vcat(r, r[512:D]).astype(bf16).T
            parts.append(rt[:64] if g == 4 else rt)
        wt = _vcat(*parts).astype(f32)
        x1 = [wt[0:HD, g * 128:(g + 1) * 128] for g in range(5)]
        x2 = [wt[HD:D, g * 128:(g + 1) * 128] for g in range(5)]
        for n, v in enumerate(_lhs_slots_lanes(x1, x2)):
            wo_t[n] = v.astype(bf16)

    def in_t1(t, c):
        w = pltpu.bitcast(xin[:, pl.ds(pl.multiple_of(t * TM + c * 128, 128), 128)], u32)
        for g in range(3):
            r = w[g * 128:min((g + 1) * 128, HD)]
            r = (_pad_rows(r) if g == 2 else r).T
            for m in range(8):
                rows = pl.ds(pl.multiple_of((c * 8 + m) * 24, 8), 16)
                pin[t, g, rows, :] = r[m * 16:(m + 1) * 16]

    def in_t2(t, j):
        parts = []
        for g in range(3):
            r = _vcat(pin[t, g, pl.ds(2 * j + t, 64, stride=24), :],
                      pin[t, g, pl.ds(2 * j + 1 - t, 64, stride=24), :]).T
            parts.append(r[:32] if g == 2 else r)
        return pltpu.bitcast(_vcat(*parts), bf16).astype(f32)

    def out_t1(t, j, x):
        w = pltpu.bitcast(x.astype(bf16), u32)
        for g in range(3):
            r = w[g * 128:min((g + 1) * 128, HD)]
            r = (_pad_rows(r) if g == 2 else r).T
            for half in range(2):
                base = (2 * j + (half ^ t)) * 72
                pout[t, g, base:base + 64, :] = r[half * 64:(half + 1) * 64]

    def out_t2(t, c):
        parts = []
        for g in range(3):
            r = _vcat(*[pout[t, g, pl.ds(c * 8 + m, 16, stride=72), :] for m in range(8)]).T
            parts.append(r[:32] if g == 2 else r)
        xin[:, t * TM + c * 128:t * TM + (c + 1) * 128] = pltpu.bitcast(_vcat(*parts), bf16)

    def combine(t, i):
        cols = pl.ds(pl.multiple_of(i * 128, 128), 128)
        m1, m2, m3, m4, m5, m6, m7 = [acc[t, n, :, cols] for n in range(7)]
        x1 = xres[t, i] + _vcat(m1 + m4 - m5 + m7, m2 + m4)
        x2 = xres[t, i + 4] + _vcat(m3 + m5, m1 - m2 + m3 + m6)
        return x1, x2

    def store_qkv(t, b, part, q, k, v, prev=None):
        q[b] = part[0:D].reshape(NG, DH, 8, 128)
        for n, (dst, r) in enumerate(((k, part[D:2 * D]), (v, part[2 * D:3 * D]))):
            dst[b + NB] = r.reshape(NG, DH, 8, 128)
            sh = pltpu.roll(r, 1, 1).reshape(NG, DH, 8, 128)
            if isinstance(t, int) and t == 0:
                dst[b] = sh
            elif prev is not None:
                dst[b] = jnp.where(((lane & 63) == 0)[None, None], prev[n][b], sh)
            else:
                keep = jnp.broadcast_to(((lane & 63) >= t)[None, None], sh.shape)
                pltpu.store(dst.at[b], sh, mask=keep)

    def phase1(t, i):
        x1, x2 = combine(t, i)
        xres[t, i] = x1
        xres[t, i + 4] = x2
        n1 = _layernorm_t(x1)
        n2 = _layernorm_t(x2, jnp.where(lane < (i < 0).astype(jnp.int32), n1[0:8], 0.0))
        yield
        rhs = lambda s: _rhs_slot(s, lambda rows, c: (n1, n2)[c][rows])
        for c in _fast_product(lambda s: _dot(wqkv_t[s], rhs(s))):
            pass
        yield
        store_qkv(t, i, _vcat(c[0], c[2]), q_s, k_s, v_s)
        store_qkv(t, i + 4, _vcat(c[1], c[3]), q_s, k_s, v_s)
        yield

    def first_norm(t, i):
        ns = []
        for b in (i, i + 4):
            x = in_t2(t, b)
            xres[t, b] = x
            ns.append(_layernorm_t(x))
        for s in range(NSLOT):
            xn_s[t, i, s] = _rhs_slot(s, lambda rows, c: ns[c][rows])

    def first_qkv(t, i):
        for c in _fast_product(lambda s: _dot(wqkv_t[s], xn_s[t, i, s])):
            yield
        for b, part in ((i, _vcat(c[0], c[2])), (i + 4, _vcat(c[1], c[3]))):
            if t == 0:
                store_qkv(t, b, part, q0, k0, v0)
            else:
                store_qkv(t, b, part, q_s, k_s, v_s, prev=(k0, v0))

    def attention_group(t, b, g, q_r, k_r, v_r, links):
        par = len(links)
        never = lane < (b < 0).astype(jnp.int32)

        def start(n, v):
            if links[n % par] is None:
                return v
            return jnp.where(never, links[n % par], 0.0) + v

        q = [q_r[b, g, d] for d in range(DH)]
        logits = []
        for w in range(W):
            l = start(w, q[0] * k_r[b + NB - w, g, 0])
            for d in range(1, DH):
                l = l + q[d] * k_r[b + NB - w, g, d]
            links[w % par] = l
            l = l * (DH ** -0.5)
            if w > 0:
                edge = jnp.logical_and(w > b, t == 0).astype(jnp.int32)
                l = jnp.where((lane & 63) < edge, -1e9, l)
            logits.append(l)
        m = functools.reduce(jnp.maximum, logits)
        e = [jnp.exp(l - m) for l in logits]
        r = 1.0 / functools.reduce(jnp.add, e)
        p = [x * r for x in e]
        outs = []
        for d in range(DH):
            o = p[0] * v_r[b + NB, g, d]
            if d >= par:
                o = start(d, o)
            for w in range(1, W):
                o = o + p[w] * v_r[b + NB - w, g, d]
            links[d % par] = o
            outs.append(o)
        return _vcat(*outs)

    def phase2(t, i, par, q_r, k_r, v_r):
        links = [None] * par
        halves = [_vcat(*[attention_group(t, b, g, q_r, k_r, v_r, links) for g in range(NG)])
                  for b in (i, i + 4)]
        yield
        rhs = lambda s: _rhs_slot(s, lambda rows, c: halves[c][rows])
        for c in _fast_product(lambda s: _dot(wo_t[s], rhs(s))):
            pass
        x1 = xres[t, i] + _vcat(c[0], c[2])
        x2 = xres[t, i + 4] + _vcat(c[1], c[3])
        xres[t, i] = x1
        xres[t, i + 4] = x2
        n1 = _layernorm_t(x1)
        n2 = _layernorm_t(x2)
        yield
        ops = _vcat(*_lhs_slots(n1, n2)).astype(bf16).T
        rows = pl.ds(pl.multiple_of(i * 128, 128), 128)
        for s in range(NSLOT):
            a_s[t, s, rows, :] = ops[:, s * 128:(s + 1) * 128]
        yield

    def proj(t, w_ref, off, res):
        outs = []
        for n0 in range(0, HC, NT):
            cols = [pl.ds(pl.multiple_of(off + n0 + c * HC, NT), NT) for c in (0, 1)]
            p = lambda s: _dot(a_s[t, s], _rhs_slot(s, lambda rows, c: w_ref[rows, cols[c]]))
            for c in _fast_product(p):
                yield
            outs.append(c)
        res.extend(jnp.concatenate(x, axis=1) if len(x) > 1 else x[0] for x in zip(*outs))

    def ffn_chunk(t, j, may_init=False):
        off = pl.multiple_of(j * FC, FC)
        g, u = [], []
        yield from proj(t, wg, off, g)
        yield from proj(t, wu, off, u)
        b11, b21, b12, b22 = [x * y for x, y in zip(g, u)]
        ca = pl.ds(off, HC)
        cb = pl.ds(pl.multiple_of(off + HC, HC), HC)
        a11, a12, a21, a22 = wd[0:HD, ca], wd[0:HD, cb], wd[HD:D, ca], wd[HD:D, cb]

        def accumulate(n, v):
            old = acc[t, n]
            if may_init:
                old = jnp.where(j > 0, old, 0.0)
            acc[t, n] = old + v

        accumulate(0, _dot_nt(_add(a11, a22), _add(b11, b22)))
        yield
        accumulate(1, _dot_nt(_add(a21, a22), b11.astype(bf16)))
        yield
        accumulate(2, _dot_nt(a11, _sub(b12, b22)))
        yield
        accumulate(3, _dot_nt(a22, _sub(b21, b11)))
        yield
        accumulate(4, _dot_nt(_add(a11, a12), b22.astype(bf16)))
        yield
        accumulate(5, _dot_nt(_sub(a21, a11), _add(b11, b12)))
        yield
        accumulate(6, _dot_nt(_sub(a12, a22), _add(b21, b22)))
        yield

    with _scope("w_x0"):
        x_copy(0, 0, TM).wait()
    for i in range(4):
        x_copy(1, i, 256).start()
    cwo.start()
    for c in range(NB):
        in_t1(0, c)
    for i in range(4):
        first_norm(0, i)
    prep_wqkv()

    def body_f(i):
        with _scope("w_x1"):
            x_copy(1, i, 256).wait()
        _drain(first_qkv(0, i))
        in_t1(1, 2 * i)
        in_t1(1, 2 * i + 1)

    def body_e(i):
        p2 = phase2(0, i, PAR0, q0, k0, v0)
        _weave(ORDER_E, first_qkv(1, i), p2)
        first_norm(1, jnp.minimum(i + 1, 3))

    for g in range(len(groups)):
        for c in ffn_copies(g):
            c.start()
    _loop(4, body_f)
    cwo.wait()
    prep_wo()
    first_norm(1, 0)
    _loop(4, body_e)

    def wait_group(k, g):
        @pl.when(k == 0)
        def _():
            for c in ffn_copies(g):
                c.wait()

    def stage(k):
        t = k % 2
        n_a = jnp.where(jnp.logical_and(k > 0, k < 3), 4, 0)
        n_b = jnp.where(k < 3, 4, 0)
        n_c = NCH - n_a - n_b
        wait_group(k, 0)
        _loop(n_c, lambda i: _drain(ffn_chunk(t, i, True)))
        _loop(n_a, lambda i: _weave(ORDER_A, ffn_chunk(t, n_c + i), phase1(1 - t, i)))
        wait_group(k, 1)
        _loop(n_b, lambda i: _weave(ORDER_B, ffn_chunk(t, n_c + n_a + i),
                                    phase2(1 - t, i, PAR, q_s, k_s, v_s)))
    _loop(4, stage)

    def finish(t):
        for i in range(4):
            x1, x2 = combine(t, i)
            out_t1(t, i, x1)
            out_t1(t, i + 4, x2)
        for c in range(NB):
            out_t2(t, c)
            if c % 4 == 3:
                out_copy(t, c // 4).start()

    finish(0)
    finish(1)
    with _scope("w_out"):
        for t in range(2):
            for half in range(2):
                out_copy(t, half).wait()


@jax.jit
def pallas_interleave_layers__sliding_local_dilated__glu_gated_bilinear__prompt_kernel(
    A_x: jax.Array,
    A_wqkv: jax.Array,
    A_wo: jax.Array,
    B_x: jax.Array,
    B_w_gate: jax.Array,
    B_w_up: jax.Array,
    B_w_down: jax.Array,
):
    any_spec = pl.BlockSpec(memory_space=pl.ANY)
    qkv_scratch = [
        pltpu.VMEM((NB, NG, DH, 8, 128), f32),
        pltpu.VMEM((2 * NB, NG, DH, 8, 128), f32),
        pltpu.VMEM((2 * NB, NG, DH, 8, 128), f32),
    ]
    out_t = pl.pallas_call(
        _kernel,
        in_specs=[any_spec] * 6,
        out_specs=any_spec,
        out_shape=jax.ShapeDtypeStruct((D, S), bf16),
        scratch_shapes=[
            pltpu.VMEM((D, S), bf16),
            pltpu.VMEM((D, 3 * D), bf16),
            pltpu.VMEM((D, D), bf16),
            pltpu.VMEM((D, F), bf16),
            pltpu.VMEM((D, F), bf16),
            pltpu.VMEM((D, F), bf16),
            pltpu.VMEM((NSLOT, HQ, 128), bf16),
            pltpu.VMEM((NSLOT, HD, 128), bf16),
            pltpu.VMEM((5, 3 * D, 128), f32),
            pltpu.VMEM((5, D, 128), f32),
            pltpu.VMEM((2, 3, 64 * 24, 128), u32),
            pltpu.VMEM((2, 3, 16 * 72, 128), u32),
            pltpu.VMEM((2, NB, D, 128), f32),
            *qkv_scratch,
            *qkv_scratch,
            pltpu.VMEM((2, NSLOT, HM, 128), bf16),
            pltpu.VMEM((2, 7, HD, HM), f32),
            pltpu.VMEM((2, 4, NSLOT, 128, 128), bf16),
            pltpu.SemaphoreType.DMA((20,)),
        ],
        compiler_params=pltpu.CompilerParams(vmem_limit_bytes=120 * 1024 * 1024),
        name="fused_layers",
    )(A_x[0].T, A_wqkv, A_wo, B_w_gate, B_w_up, B_w_down.T)
    return out_t.T[None]
```

```python
import functools
import os

import jax
import jax.numpy as jnp
import jax.experimental.pallas as pl
import jax.experimental.pallas.tpu as pltpu

S, D, F = 2048, 576, 4608
H, DH, W = 32, 18, 8
NG = H // 8
GR = 8 * DH
NB = 8
TM = NB * 128
HM = TM // 2
HD = D // 2
HQ = 3 * D // 2
FC = 512
HC = FC // 2
NCH = F // FC
NSLOT = 16
NT = int(os.environ.get("NT", 128))

GROUP_ROWS = {1: (0, 128), 2: (64, 192), 4: (256, 384), 3: (320, 448), 0: (512, 512)}
T3 = 1.0 / 3.0
SLOTS = (
    ((1, (-1, -1, 0, 0), (0, 0, 0, 1)), (3, (1, 1, 0, 0), (0, 0, 1, 0))),
    ((0, (T3, 0, 0, 0), (2, 1, 0, 0)), (2, (-.5, -1, 0, 0), (0, 0, 0, 1))),
    ((4, (.5, 1, 0, 0), (0, 0, 1, 0)), (0, (-T3, 0, 0, 0), (1, 2, 0, 0))),
    ((1, (0, 1, 0, -1), (0, 0, 1, 1)), (2, (0, 2, 0, -1), (0, 0, .5, 1))),
    ((1, (0, 0, 1, 1), (1, 0, 0, 0)), (3, (0, 0, -1, -1), (0, 1, 0, 0))),
    ((0, (0, 0, T3, 0), (2, 1, 0, 0)), (2, (0, 0, .5, 1), (1, 0, 0, 0))),
    ((4, (0, 0, -.5, -1), (0, 1, 0, 0)), (0, (0, 0, -T3, 0), (1, 2, 0, 0))),
    ((1, (-1, 0, 1, 0), (1, 1, 0, 0)), (2, (-1, 0, .5, 0), (1, 2, 0, 0))),
    ((1, (0, 0, 0, 1), (-1, 0, 1, 0)), (3, (1, 0, 0, 0), (1, 0, -1, 0))),
    ((4, (.5, 0, 0, 0), (2, 0, -1, 0)), (2, (0, 0, 0, 1), (-1, 0, .5, 0))),
    ((4, (-1, 0, .5, 0), (2, 1, 0, 0)), (3, (-1, 0, 1, 0), (1, 1, 0, 0))),
    ((1, (1, 0, 0, 1), (1, 0, 0, 1)), (2, (1, 0, 0, 1), (1, 0, 0, 1))),
    ((1, (1, 0, 0, 0), (0, 1, 0, -1)), (3, (0, 0, 0, 1), (0, -1, 0, 1))),
    ((4, (0, 0, 0, 1), (0, -1, 0, .5)), (2, (.5, 0, 0, 0), (0, 2, 0, -1))),
    ((4, (0, 2, 0, -1), (0, 0, 1, .5)), (3, (0, 1, 0, -1), (0, 0, 1, 1))),
    ((4, (1, 0, 0, 1), (0, 1, 1, 0)), (3, (1, 0, 0, 1), (0, 1, 1, 0))),
)
EPS = 1e-5
KA = int(os.environ.get("KA", 6))
KB = int(os.environ.get("KB", 12))
PAR = int(os.environ.get("PAR", 2))
PAR0 = int(os.environ.get("PAR0", 3))
ORDER_A = "s" + "m" * KA + "ss"
ORDER_B = "s" + "m" * KB + "s" + "m" * (2048 // NT - KB) + "s"
ORDER_E = "s" + "m" * int(os.environ.get("KE", 2)) + "s"
f32, bf16, u32 = jnp.float32, jnp.bfloat16, jnp.uint32

_dot = functools.partial(jnp.dot, preferred_element_type=f32)


def _dot_nt(a, b):
    return jax.lax.dot_general(a, b, (((1,), (1,)), ((), ())), preferred_element_type=f32)


def _vcat(*xs):
    return jnp.concatenate(xs, axis=0)


def _pad_rows(r):
    return _vcat(r, jnp.zeros((128 - r.shape[0], r.shape[1]), r.dtype))


def _add(x, y):
    return (x.astype(f32) + y.astype(f32)).astype(bf16)


def _sub(x, y):
    return (x.astype(f32) - y.astype(f32)).astype(bf16)


def _form(coefs, blocks):
    terms = [(c, blk) for c, blk in zip(coefs, blocks) if c != 0]
    if len(terms) == 1 and terms[0][0] == 1:
        return terms[0][1]()
    terms.sort(key=lambda cb: cb[0] < 0)
    out = None
    for c, blk in terms:
        v = blk().astype(f32)
        if out is None:
            out = v if c == 1 else v * c
        else:
            v = v if abs(c) == 1 else v * abs(c)
            out = out + v if c > 0 else out - v
    return out


def _lhs_slots(x1, x2):
    out = []
    for halves in SLOTS:
        for grp, coefs, _ in halves:
            k1, k2 = GROUP_ROWS[grp]
            blocks = [lambda x=x, k=k: x[k:k + 64] for x in (x1, x2) for k in (k1, k2)]
            out.append(_form(coefs, blocks))
    return out


def _lhs_slots_lanes(x1, x2):
    low = jax.lax.broadcasted_iota(jnp.int32, x1[0].shape, 1) < 64
    out = []
    for halves in SLOTS:
        keys = [(tuple(k // 128 for k in GROUP_ROWS[grp]), coefs) for grp, coefs, _ in halves]
        vals = [_form(coefs, [lambda x=x, g=g: x[g] for x in (x1, x2) for g in tiles])
                for tiles, coefs in keys]
        out.append(vals[0] if keys[0] == keys[1] else jnp.where(low, vals[0], vals[1]))
    return out


def _fast_product(p):
    p0, p1, p2, p3 = p(0), p(1), p(2), p(3)
    r = p0 + p1 + p2
    c11 = r + p1 + p3
    c12 = r + p2
    yield None
    p0, p1, p2, p3 = p(4), p(5), p(6), p(7)
    r = p0 + p1 + p2
    c21 = r + p1
    c22 = p3 - (r + p2)
    yield None
    p0, p1, p2, p3 = p(8), p(9), p(10), p(11)
    r = p0 + p1
    c11 = c11 + (r + p3)
    c21 = c21 + (r + p1 + p2)
    c22 = c22 + p3
    yield None
    p0, p1, p2, p3 = p(12), p(13), p(14), p(15)
    r = p0 + p1
    c12 = (r + p2 + p3) - c12
    c22 = c22 + (r + p1)
    c21 = c21 + p3
    yield (c11, c12, c21, c22)


def _rhs_slot(s, get):
    parts = []
    for grp, _, coefs in SLOTS[s]:
        k1, k2 = GROUP_ROWS[grp]
        blocks = [lambda k=k, c=c: get(slice(k, k + 64), c) for k in (k1, k2) for c in (0, 1)]
        parts.append(_form(coefs, blocks).astype(f32))
    return _vcat(*parts).astype(bf16)


def _packed(ref, *idx):
    return pltpu.bitcast(ref.bitcast(u32)[idx], bf16)


def _layernorm_t(x, zero=None):
    rows = [x[r:r + 8] for r in range(0, D, 8)]
    s = rows[0] if zero is None else rows[0] + zero
    for r in rows[1:]:
        s = s + r
    m = jnp.sum(s, axis=0, keepdims=True) * (1.0 / D)
    rows = [r - m for r in rows]
    s = rows[0] * rows[0]
    for r in rows[1:]:
        s = s + r * r
    v = jnp.sum(s, axis=0, keepdims=True) * (1.0 / D)
    return _vcat(*rows) * jax.lax.rsqrt(v + EPS)


def _drain(*gens):
    for gen in gens:
        for _ in gen:
            pass


def _weave(order, main, side):
    for c in order:
        next(main if c == "m" else side)
    _drain(main, side)


def _scope(name):
    import contextlib
    return jax.named_scope(name) if os.environ.get("SCOPES") else contextlib.nullcontext()


def _loop(n, fn):
    def body(i, c):
        with _scope("it"):
            fn(i)
        return c
    jax.lax.fori_loop(0, n, body, 0)


def _kernel(x_hbm, wqkv_hbm, wo_hbm, wg_hbm, wu_hbm, wd_hbm, out_hbm,
            xin, wqkv, wo, wg, wu, wd, wqkv_t, wo_t, wperm, operm, pin, pout, xres,
            q0, k0, v0, q_s, k_s, v_s, a_s, acc, xn_s, sems):
    groups = ((0, 5 * FC), (5 * FC, 4 * FC))
    lane = jax.lax.broadcasted_iota(jnp.int32, (8, 128), 1)

    def x_copy(t, piece, n):
        cols = pl.ds(pl.multiple_of(t * TM + piece * n, 128), n)
        return pltpu.make_async_copy(x_hbm.at[:, cols], xin.at[:, cols], sems.at[10 + t + piece])

    def wqkv_copy(g):
        rows = pl.ds(g * 128, min(128, D - g * 128))
        return pltpu.make_async_copy(wqkv_hbm.at[rows], wqkv.at[rows], sems.at[15 + g])

    def out_copy(t, half):
        cols = pl.ds(t * TM + half * HM, HM)
        return pltpu.make_async_copy(xin.at[:, cols], out_hbm.at[:, cols], sems.at[2 * t + half])

    def ffn_copies(g):
        off, n = groups[g]
        return [pltpu.make_async_copy(src.at[:, pl.ds(off, n)], dst.at[:, pl.ds(off, n)],
                                      sems.at[4 + 3 * g + i])
                for i, (src, dst) in enumerate(((wg_hbm, wg), (wu_hbm, wu), (wd_hbm, wd)))]

    cwo = pltpu.make_async_copy(wo_hbm, wo, sems.at[3])
    x_copy(0, 0, TM).start()
    for g in range(5):
        wqkv_copy(g).start()

    def head_rows(ref, g, base):
        return _vcat(*[ref[g, pl.ds(base + d, 8, stride=DH), :] for d in range(DH)])

    def prep_wqkv():
        for gs in ((0, 1), (2, 3), (4,)):
            with _scope("w_qkv"):
                for g in gs:
                    wqkv_copy(g).wait()
            for g in gs:
                rows = wqkv[g * 128:min((g + 1) * 128, D), :].astype(f32)
                wperm[g] = (_vcat(rows, rows) if g == 4 else rows).T

        def rows_of(hg):
            base = pl.multiple_of(hg * GR, 16)
            x1 = [head_rows(wperm, g, base) for g in range(5)]
            x2 = [head_rows(wperm, g, base + HQ) for g in range(5)]
            for n, v in enumerate(_lhs_slots_lanes(x1, x2)):
                wqkv_t[n, pl.ds(base, GR), :] = v.astype(bf16)
        _loop(HQ // GR, rows_of)

    def prep_wo():
        for g in range(5):
            cols = wo[:, g * 128:min((g + 1) * 128, D)].astype(f32)
            if g == 4:
                cols = jnp.concatenate([cols, jnp.zeros_like(cols)], axis=1)
            operm[g] = cols
        parts = []
        for g in range(5):
            r = _vcat(*[head_rows(operm, g, hg * GR) for hg in range(NG)])
            rt = _vcat(r, r[512:D]).astype(bf16).T
            parts.append(rt[:64] if g == 4 else rt)
        wt = _vcat(*parts).astype(f32)
        x1 = [wt[0:HD, g * 128:(g + 1) * 128] for g in range(5)]
        x2 = [wt[HD:D, g * 128:(g + 1) * 128] for g in range(5)]
        for n, v in enumerate(_lhs_slots_lanes(x1, x2)):
            wo_t[n] = v.astype(bf16)

    def to_words(x):
        return [pltpu.bitcast((x[g * 128:(g + 1) * 128] if g < 4 else _pad_rows(x[512:D])).T, u32)
                for g in range(5)]

    def from_words(words):
        parts = [pltpu.bitcast(w, bf16).T for w in words]
        return _vcat(*parts[:4], parts[4][:64])

    def in_t1(t, c):
        x = xin[:, pl.ds(pl.multiple_of(t * TM + c * 128, 128), 128)]
        for g, w in enumerate(to_words(x)):
            pin[t, g, pl.ds(pl.multiple_of(c * 64, 64), 64), :] = w

    def in_t2(t, j):
        return from_words([pin[t, g, pl.ds(j, 64, stride=8), :] for g in range(5)]).astype(f32)

    def out_t1(t, j, x):
        for g, w in enumerate(to_words(x.astype(bf16))):
            pout[t, g, j * 72:j * 72 + 64, :] = w

    def out_t2(t, c):
        words = [_vcat(*[pout[t, g, pl.ds(c * 8 + m, 8, stride=72), :] for m in range(8)])
                 for g in range(5)]
        xin[:, t * TM + c * 128:t * TM + (c + 1) * 128] = from_words(words)

    def combine(t, i):
        cols = pl.ds(pl.multiple_of(i * 128, 128), 128)
        m1, m2, m3, m4, m5, m6, m7 = [acc[t, n, :, cols] for n in range(7)]
        x1 = xres[t, i] + _vcat(m1 + m4 - m5 + m7, m2 + m4)
        x2 = xres[t, i + 4] + _vcat(m3 + m5, m1 - m2 + m3 + m6)
        return x1, x2

    def store_qkv(t, b, part, q, k, v, prev=None):
        q[b] = part[0:D].reshape(NG, DH, 8, 128)
        for n, (dst, r) in enumerate(((k, part[D:2 * D]), (v, part[2 * D:3 * D]))):
            dst[b + NB] = r.reshape(NG, DH, 8, 128)
            sh = pltpu.roll(r, 2, 1).reshape(NG, DH, 8, 128)
            if isinstance(t, int) and t == 0:
                dst[b] = sh
            elif prev is not None:
                dst[b] = jnp.where((lane < 2)[None, None], prev[n][b], sh)
            else:
                keep = jnp.broadcast_to((lane >= 2 * t)[None, None], sh.shape)
                pltpu.store(dst.at[b], sh, mask=keep)

    def phase1(t, i):
        x1, x2 = combine(t, i)
        xres[t, i] = x1
        xres[t, i + 4] = x2
        n1 = _layernorm_t(x1)
        n2 = _layernorm_t(x2, jnp.where(lane < (i < 0).astype(jnp.int32), n1[0:8], 0.0))
        yield
        rhs = lambda s: _rhs_slot(s, lambda rows, c: (n1, n2)[c][rows])
        for c in _fast_product(lambda s: _dot(_packed(wqkv_t, s), rhs(s))):
            pass
        yield
        store_qkv(t, i, _vcat(c[0], c[2]), q_s, k_s, v_s)
        store_qkv(t, i + 4, _vcat(c[1], c[3]), q_s, k_s, v_s)
        yield

    def first_norm(t, i):
        ns = []
        for b in (i, i + 4):
            x = in_t2(t, b)
            xres[t, b] = x
            ns.append(_layernorm_t(x))
        for s in range(NSLOT):
            xn_s[t, i, s] = _rhs_slot(s, lambda rows, c: ns[c][rows])

    def first_qkv(t, i):
        for c in _fast_product(lambda s: _dot(_packed(wqkv_t, s), _packed(xn_s, t, i, s))):
            yield
        for b, part in ((i, _vcat(c[0], c[2])), (i + 4, _vcat(c[1], c[3]))):
            if t == 0:
                store_qkv(t, b, part, q0, k0, v0)
            else:
                store_qkv(t, b, part, q_s, k_s, v_s, prev=(k0, v0))

    def attention_group(t, b, g, q_r, k_r, v_r, links):
        par = len(links)
        never = lane < (b < 0).astype(jnp.int32)

        def start(n, v):
            if links[n % par] is None:
                return v
            return jnp.where(never, links[n % par], 0.0) + v

        q = [q_r[b, g, d] for d in range(DH)]
        logits = []
        for w in range(W):
            l = start(w, q[0] * k_r[b + NB - w, g, 0])
            for d in range(1, DH):
                l = l + q[d] * k_r[b + NB - w, g, d]
            links[w % par] = l
            l = l * (DH ** -0.5)
            if w > 0:
                edge = jnp.where(jnp.logical_and(w > b, t == 0), 2, 0)
                l = jnp.where(lane < edge, -1e9, l)
            logits.append(l)
        m = functools.reduce(jnp.maximum, logits)
        e = [jnp.exp(l - m) for l in logits]
        r = 1.0 / functools.reduce(jnp.add, e)
        p = [x * r for x in e]
        outs = []
        for d in range(DH):
            o = p[0] * v_r[b + NB, g, d]
            if d >= par:
                o = start(d, o)
            for w in range(1, W):
                o = o + p[w] * v_r[b + NB - w, g, d]
            links[d % par] = o
            outs.append(o)
        return _vcat(*outs)

    def phase2(t, i, par, q_r, k_r, v_r):
        links = [None] * par
        halves = [_vcat(*[attention_group(t, b, g, q_r, k_r, v_r, links) for g in range(NG)])
                  for b in (i, i + 4)]
        yield
        rhs = lambda s: _rhs_slot(s, lambda rows, c: halves[c][rows])
        for c in _fast_product(lambda s: _dot(_packed(wo_t, s), rhs(s))):
            pass
        x1 = xres[t, i] + _vcat(c[0], c[2])
        x2 = xres[t, i + 4] + _vcat(c[1], c[3])
        xres[t, i] = x1
        xres[t, i + 4] = x2
        n1 = _layernorm_t(x1)
        n2 = _layernorm_t(x2)
        yield
        ops = _lhs_slots(n1, n2)
        rows = pl.ds(pl.multiple_of(i * 64, 64), 64)
        for s in range(NSLOT):
            op = _vcat(ops[2 * s], ops[2 * s + 1]).astype(bf16).T
            a_s[t, s, rows, :] = pltpu.bitcast(op, u32)
        yield

    def proj(t, w_ref, off, res):
        outs = []
        for n0 in range(0, HC, NT):
            cols = [pl.ds(pl.multiple_of(off + n0 + c * HC, NT), NT) for c in (0, 1)]
            p = lambda s: _dot(pltpu.bitcast(a_s[t, s], bf16), _rhs_slot(s, lambda rows, c: w_ref[rows, cols[c]]))
            for c in _fast_product(p):
                yield
            outs.append(c)
        res.extend(jnp.concatenate(x, axis=1) if len(x) > 1 else x[0] for x in zip(*outs))

    def ffn_chunk(t, j, may_init=False):
        off = pl.multiple_of(j * FC, FC)
        g, u = [], []
        yield from proj(t, wg, off, g)
        yield from proj(t, wu, off, u)
        b11, b21, b12, b22 = [x * y for x, y in zip(g, u)]
        ca = pl.ds(off, HC)
        cb = pl.ds(pl.multiple_of(off + HC, HC), HC)
        a11, a12, a21, a22 = wd[0:HD, ca], wd[0:HD, cb], wd[HD:D, ca], wd[HD:D, cb]

        def accumulate(n, v):
            old = acc[t, n]
            if may_init:
                old = jnp.where(j > 0, old, 0.0)
            acc[t, n] = old + v

        accumulate(0, _dot_nt(_add(a11, a22), _add(b11, b22)))
        yield
        accumulate(1, _dot_nt(_add(a21, a22), b11.astype(bf16)))
        yield
        accumulate(2, _dot_nt(a11, _sub(b12, b22)))
        yield
        accumulate(3, _dot_nt(a22, _sub(b21, b11)))
        yield
        accumulate(4, _dot_nt(_add(a11, a12), b22.astype(bf16)))
        yield
        accumulate(5, _dot_nt(_sub(a21, a11), _add(b11, b12)))
        yield
        accumulate(6, _dot_nt(_sub(a12, a22), _add(b21, b22)))
        yield

    with _scope("w_x0"):
        x_copy(0, 0, TM).wait()
    for i in range(4):
        x_copy(1, i, 256).start()
    cwo.start()
    for c in range(NB):
        in_t1(0, c)
    for i in range(4):
        first_norm(0, i)
    prep_wqkv()

    def body_f(i):
        with _scope("w_x1"):
            x_copy(1, i, 256).wait()
        _drain(first_qkv(0, i))
        in_t1(1, 2 * i)
        in_t1(1, 2 * i + 1)

    def body_e(i):
        p2 = phase2(0, i, PAR0, q0, k0, v0)
        _weave(ORDER_E, first_qkv(1, i), p2)
        first_norm(1, jnp.minimum(i + 1, 3))

    for g in range(len(groups)):
        for c in ffn_copies(g):
            c.start()
    _loop(4, body_f)
    cwo.wait()
    prep_wo()
    first_norm(1, 0)
    _loop(4, body_e)

    def wait_group(k, g):
        @pl.when(k == 0)
        def _():
            for c in ffn_copies(g):
                c.wait()

    def stage(k):
        t = k % 2
        n_a = jnp.where(jnp.logical_and(k > 0, k < 3), 4, 0)
        n_b = jnp.where(k < 3, 4, 0)
        n_c = NCH - n_a - n_b
        wait_group(k, 0)
        _loop(n_c, lambda i: _drain(ffn_chunk(t, i, True)))
        _loop(n_a, lambda i: _weave(ORDER_A, ffn_chunk(t, n_c + i), phase1(1 - t, i)))
        wait_group(k, 1)
        _loop(n_b, lambda i: _weave(ORDER_B, ffn_chunk(t, n_c + n_a + i),
                                    phase2(1 - t, i, PAR, q_s, k_s, v_s)))
    _loop(4, stage)

    def finish(t):
        for i in range(4):
            x1, x2 = combine(t, i)
            out_t1(t, i, x1)
            out_t1(t, i + 4, x2)
        for c in range(NB):
            out_t2(t, c)
            if c % 4 == 3:
                out_copy(t, c // 4).start()

    finish(0)
    finish(1)
    with _scope("w_out"):
        for t in range(2):
            for half in range(2):
                out_copy(t, half).wait()


@jax.jit
def pallas_interleave_layers__sliding_local_dilated__glu_gated_bilinear__prompt_kernel(
    A_x: jax.Array,
    A_wqkv: jax.Array,
    A_wo: jax.Array,
    B_x: jax.Array,
    B_w_gate: jax.Array,
    B_w_up: jax.Array,
    B_w_down: jax.Array,
):
    any_spec = pl.BlockSpec(memory_space=pl.ANY)
    qkv_scratch = [
        pltpu.VMEM((NB, NG, DH, 8, 128), f32),
        pltpu.VMEM((2 * NB, NG, DH, 8, 128), f32),
        pltpu.VMEM((2 * NB, NG, DH, 8, 128), f32),
    ]
    out_t = pl.pallas_call(
        _kernel,
        in_specs=[any_spec] * 6,
        out_specs=any_spec,
        out_shape=jax.ShapeDtypeStruct((D, S), bf16),
        scratch_shapes=[
            pltpu.VMEM((D, S), bf16),
            pltpu.VMEM((D, 3 * D), bf16),
            pltpu.VMEM((D, D), bf16),
            pltpu.VMEM((D, F), bf16),
            pltpu.VMEM((D, F), bf16),
            pltpu.VMEM((D, F), bf16),
            pltpu.VMEM((NSLOT, HQ, 128), bf16),
            pltpu.VMEM((NSLOT, HD, 128), bf16),
            pltpu.VMEM((5, 3 * D, 128), f32),
            pltpu.VMEM((5, D, 128), f32),
            pltpu.VMEM((2, 5, HM, 128), u32),
            pltpu.VMEM((2, 5, 8 * 72, 128), u32),
            pltpu.VMEM((2, NB, D, 128), f32),
            *qkv_scratch,
            *qkv_scratch,
            pltpu.VMEM((2, NSLOT, HM // 2, 128), u32),
            pltpu.VMEM((2, 7, HD, HM), f32),
            pltpu.VMEM((2, 4, NSLOT, 128, 128), bf16),
            pltpu.SemaphoreType.DMA((20,)),
        ],
        compiler_params=pltpu.CompilerParams(vmem_limit_bytes=120 * 1024 * 1024),
        name="fused_layers",
    )(A_x[0].T, A_wqkv, A_wo, B_w_gate, B_w_up, B_w_down.T)
    return out_t.T[None]
```

```python
import functools
import os

import jax
import jax.numpy as jnp
import jax.experimental.pallas as pl
import jax.experimental.pallas.tpu as pltpu

S, D, F = 2048, 576, 4608
H, DH, W = 32, 18, 8
NG = H // 8
GR = 8 * DH
NB = 8
TM = NB * 128
HM = TM // 2
HD = D // 2
HQ = 3 * D // 2
FC = 512
HC = FC // 2
NCH = F // FC
NSLOT = 16
NT = int(os.environ.get("NT", 128))

GROUP_ROWS = {1: (0, 128), 2: (64, 192), 4: (256, 384), 3: (320, 448), 0: (512, 512)}
T3 = 1.0 / 3.0
SLOTS = (
    ((1, (-1, -1, 0, 0), (0, 0, 0, 1)), (3, (1, 1, 0, 0), (0, 0, 1, 0))),
    ((0, (T3, 0, 0, 0), (2, 1, 0, 0)), (2, (-.5, -1, 0, 0), (0, 0, 0, 1))),
    ((4, (.5, 1, 0, 0), (0, 0, 1, 0)), (0, (-T3, 0, 0, 0), (1, 2, 0, 0))),
    ((1, (0, 1, 0, -1), (0, 0, 1, 1)), (2, (0, 2, 0, -1), (0, 0, .5, 1))),
    ((1, (0, 0, 1, 1), (1, 0, 0, 0)), (3, (0, 0, -1, -1), (0, 1, 0, 0))),
    ((0, (0, 0, T3, 0), (2, 1, 0, 0)), (2, (0, 0, .5, 1), (1, 0, 0, 0))),
    ((4, (0, 0, -.5, -1), (0, 1, 0, 0)), (0, (0, 0, -T3, 0), (1, 2, 0, 0))),
    ((1, (-1, 0, 1, 0), (1, 1, 0, 0)), (2, (-1, 0, .5, 0), (1, 2, 0, 0))),
    ((1, (0, 0, 0, 1), (-1, 0, 1, 0)), (3, (1, 0, 0, 0), (1, 0, -1, 0))),
    ((4, (.5, 0, 0, 0), (2, 0, -1, 0)), (2, (0, 0, 0, 1), (-1, 0, .5, 0))),
    ((4, (-1, 0, .5, 0), (2, 1, 0, 0)), (3, (-1, 0, 1, 0), (1, 1, 0, 0))),
    ((1, (1, 0, 0, 1), (1, 0, 0, 1)), (2, (1, 0, 0, 1), (1, 0, 0, 1))),
    ((1, (1, 0, 0, 0), (0, 1, 0, -1)), (3, (0, 0, 0, 1), (0, -1, 0, 1))),
    ((4, (0, 0, 0, 1), (0, -1, 0, .5)), (2, (.5, 0, 0, 0), (0, 2, 0, -1))),
    ((4, (0, 2, 0, -1), (0, 0, 1, .5)), (3, (0, 1, 0, -1), (0, 0, 1, 1))),
    ((4, (1, 0, 0, 1), (0, 1, 1, 0)), (3, (1, 0, 0, 1), (0, 1, 1, 0))),
)
EPS = 1e-5
KA = int(os.environ.get("KA", 6))
KB = int(os.environ.get("KB", 12))
PAR = int(os.environ.get("PAR", 2))
PAR0 = int(os.environ.get("PAR0", 3))
ORDER_A = "s" + "m" * KA + "ss"
ORDER_B = "s" + "m" * KB + "s" + "m" * (2048 // NT - KB) + "s"
ORDER_E = "s" + "m" * int(os.environ.get("KE", 5)) + "s"
f32, bf16, u32 = jnp.float32, jnp.bfloat16, jnp.uint32

_dot = functools.partial(jnp.dot, preferred_element_type=f32)


def _dot_nt(a, b):
    return jax.lax.dot_general(a, b, (((1,), (1,)), ((), ())), preferred_element_type=f32)


def _vcat(*xs):
    return jnp.concatenate(xs, axis=0)


def _pad_rows(r):
    return _vcat(r, jnp.zeros((128 - r.shape[0], r.shape[1]), r.dtype))


def _add(x, y):
    return (x.astype(f32) + y.astype(f32)).astype(bf16)


def _sub(x, y):
    return (x.astype(f32) - y.astype(f32)).astype(bf16)


def _form(coefs, blocks):
    terms = [(c, blk) for c, blk in zip(coefs, blocks) if c != 0]
    if len(terms) == 1 and terms[0][0] == 1:
        return terms[0][1]()
    terms.sort(key=lambda cb: cb[0] < 0)
    out = None
    for c, blk in terms:
        v = blk().astype(f32)
        if out is None:
            out = v if c == 1 else v * c
        else:
            v = v if abs(c) == 1 else v * abs(c)
            out = out + v if c > 0 else out - v
    return out


def _lhs_slots(x1, x2):
    out = []
    for halves in SLOTS:
        for grp, coefs, _ in halves:
            k1, k2 = GROUP_ROWS[grp]
            blocks = [lambda x=x, k=k: x[k:k + 64] for x in (x1, x2) for k in (k1, k2)]
            out.append(_form(coefs, blocks))
    return out


def _lhs_slots_lanes(x1, x2):
    low = jax.lax.broadcasted_iota(jnp.int32, x1[0].shape, 1) < 64
    out = []
    for halves in SLOTS:
        keys = [(tuple(k // 128 for k in GROUP_ROWS[grp]), coefs) for grp, coefs, _ in halves]
        vals = [_form(coefs, [lambda x=x, g=g: x[g] for x in (x1, x2) for g in tiles])
                for tiles, coefs in keys]
        out.append(vals[0] if keys[0] == keys[1] else jnp.where(low, vals[0], vals[1]))
    return out


def _fast_product(p):
    p0, p1, p2, p3 = p(0), p(1), p(2), p(3)
    r = p0 + p1 + p2
    c11 = r + p1 + p3
    c12 = r + p2
    yield None
    p0, p1, p2, p3 = p(4), p(5), p(6), p(7)
    r = p0 + p1 + p2
    c21 = r + p1
    c22 = p3 - (r + p2)
    yield None
    p0, p1, p2, p3 = p(8), p(9), p(10), p(11)
    r = p0 + p1
    c11 = c11 + (r + p3)
    c21 = c21 + (r + p1 + p2)
    c22 = c22 + p3
    yield None
    p0, p1, p2, p3 = p(12), p(13), p(14), p(15)
    r = p0 + p1
    c12 = (r + p2 + p3) - c12
    c22 = c22 + (r + p1)
    c21 = c21 + p3
    yield (c11, c12, c21, c22)


def _rhs_slot(s, get):
    parts = []
    for grp, _, coefs in SLOTS[s]:
        k1, k2 = GROUP_ROWS[grp]
        blocks = [lambda k=k, c=c: get(slice(k, k + 64), c) for k in (k1, k2) for c in (0, 1)]
        parts.append(_form(coefs, blocks).astype(f32))
    return _vcat(*parts).astype(bf16)


def _packed(ref, *idx):
    return pltpu.bitcast(ref.bitcast(u32)[idx], bf16)


def _layernorm_t(x, zero=None):
    rows = [x[r:r + 8] for r in range(0, D, 8)]
    s = rows[0] if zero is None else rows[0] + zero
    for r in rows[1:]:
        s = s + r
    m = jnp.sum(s, axis=0, keepdims=True) * (1.0 / D)
    rows = [r - m for r in rows]
    s = rows[0] * rows[0]
    for r in rows[1:]:
        s = s + r * r
    v = jnp.sum(s, axis=0, keepdims=True) * (1.0 / D)
    return _vcat(*rows) * jax.lax.rsqrt(v + EPS)


def _drain(*gens):
    for gen in gens:
        for _ in gen:
            pass


def _weave(order, main, side):
    for c in order:
        next(main if c == "m" else side)
    _drain(main, side)


def _scope(name):
    import contextlib
    return jax.named_scope(name) if os.environ.get("SCOPES") else contextlib.nullcontext()


def _loop(n, fn):
    def body(i, c):
        with _scope("it"):
            fn(i)
        return c
    jax.lax.fori_loop(0, n, body, 0)


def _kernel(x_hbm, wqkv_hbm, wo_hbm, wg_hbm, wu_hbm, wd_hbm, out_hbm,
            xin, wqkv, wo, wg, wu, wd, wqkv_t, wo_t, wperm, operm, pin, pout, xres,
            q0, k0, v0, q_s, k_s, v_s, a_s, acc, xn_s, sems):
    groups = ((0, 5 * FC), (5 * FC, 4 * FC))
    lane = jax.lax.broadcasted_iota(jnp.int32, (8, 128), 1)

    def x_copy(t, piece, n):
        cols = pl.ds(pl.multiple_of(t * TM + piece * n, 128), n)
        return pltpu.make_async_copy(x_hbm.at[:, cols], xin.at[:, cols], sems.at[10 + t + piece])

    def wqkv_copy(g):
        rows = pl.ds(g * 128, min(128, D - g * 128))
        return pltpu.make_async_copy(wqkv_hbm.at[rows], wqkv.at[rows], sems.at[15 + g])

    def out_copy(t, half):
        cols = pl.ds(t * TM + half * HM, HM)
        return pltpu.make_async_copy(xin.at[:, cols], out_hbm.at[:, cols], sems.at[2 * t + half])

    def ffn_copies(g):
        off, n = groups[g]
        return [pltpu.make_async_copy(src.at[:, pl.ds(off, n)], dst.at[:, pl.ds(off, n)],
                                      sems.at[4 + 3 * g + i])
                for i, (src, dst) in enumerate(((wg_hbm, wg), (wu_hbm, wu), (wd_hbm, wd)))]

    cwo = pltpu.make_async_copy(wo_hbm, wo, sems.at[3])
    x_copy(0, 0, TM).start()
    for g in range(5):
        wqkv_copy(g).start()

    def head_rows(ref, g, base):
        return _vcat(*[ref[g, pl.ds(base + d, 8, stride=DH), :] for d in range(DH)])

    def prep_wqkv():
        for gs in ((0, 1), (2, 3), (4,)):
            with _scope("w_qkv"):
                for g in gs:
                    wqkv_copy(g).wait()
            for g in gs:
                rows = wqkv[g * 128:min((g + 1) * 128, D), :].astype(f32)
                wperm[g] = (_vcat(rows, rows) if g == 4 else rows).T

        def rows_of(hg):
            base = pl.multiple_of(hg * GR, 16)
            x1 = [head_rows(wperm, g, base) for g in range(5)]
            x2 = [head_rows(wperm, g, base + HQ) for g in range(5)]
            for n, v in enumerate(_lhs_slots_lanes(x1, x2)):
                wqkv_t[n, pl.ds(base, GR), :] = v.astype(bf16)
        _loop(HQ // GR, rows_of)

    def prep_wo():
        for g in range(5):
            cols = wo[:, g * 128:min((g + 1) * 128, D)].astype(f32)
            if g == 4:
                cols = jnp.concatenate([cols, jnp.zeros_like(cols)], axis=1)
            operm[g] = cols
        parts = []
        for g in range(5):
            r = _vcat(*[head_rows(operm, g, hg * GR) for hg in range(NG)])
            rt = _vcat(r, r[512:D]).astype(bf16).T
            parts.append(rt[:64] if g == 4 else rt)
        wt = _vcat(*parts).astype(f32)
        x1 = [wt[0:HD, g * 128:(g + 1) * 128] for g in range(5)]
        x2 = [wt[HD:D, g * 128:(g + 1) * 128] for g in range(5)]
        for n, v in enumerate(_lhs_slots_lanes(x1, x2)):
            wo_t[n] = v.astype(bf16)

    def to_words(x):
        tiles = [x[g * 128:(g + 1) * 128] for g in range(4)] + [_pad_rows(x[512:D])]
        return [pltpu.bitcast(r.astype(bf16).T, u32) for r in tiles]

    def from_words(words):
        parts = [pltpu.bitcast(w, bf16).T for w in words]
        return _vcat(*parts[:4], parts[4][:64])

    def in_t1(t, c):
        x = xin[:, pl.ds(pl.multiple_of(t * TM + c * 128, 128), 128)]
        for g, w in enumerate(to_words(x)):
            pin[t, g, pl.ds(pl.multiple_of(c * 64, 64), 64), :] = w

    def in_t2(t, j):
        return from_words([pin[t, g, pl.ds(j, 64, stride=8), :] for g in range(5)]).astype(f32)

    def out_t1(t, j, x):
        for g, w in enumerate(to_words(x)):
            pout[t, g, j * 72:j * 72 + 64, :] = w

    def out_t2(t, c):
        words = [_vcat(*[pout[t, g, pl.ds(c * 8 + m, 8, stride=72), :] for m in range(8)])
                 for g in range(5)]
        xin[:, t * TM + c * 128:t * TM + (c + 1) * 128] = from_words(words)

    def combine(t, i):
        m1, m2, m3, m4, m5, m6, m7 = [acc[t, n, i] for n in range(7)]
        x1 = xres[t, i] + _vcat(m1 + m4 - m5 + m7, m2 + m4)
        x2 = xres[t, i + 4] + _vcat(m3 + m5, m1 - m2 + m3 + m6)
        return x1, x2

    def store_qkv(t, b, part, q, k, v, prev=None):
        q[b] = part[0:D].reshape(NG, DH, 8, 128)
        for n, (dst, r) in enumerate(((k, part[D:2 * D]), (v, part[2 * D:3 * D]))):
            dst[b + NB] = r.reshape(NG, DH, 8, 128)
            sh = pltpu.roll(r, 2, 1).reshape(NG, DH, 8, 128)
            if isinstance(t, int) and t == 0:
                dst[b] = sh
            elif prev is not None:
                dst[b] = jnp.where((lane < 2)[None, None], prev[n][b], sh)
            else:
                keep = jnp.broadcast_to((lane >= 2 * t)[None, None], sh.shape)
                pltpu.store(dst.at[b], sh, mask=keep)

    def phase1(t, i):
        x1, x2 = combine(t, i)
        xres[t, i] = x1
        xres[t, i + 4] = x2
        n1 = _layernorm_t(x1)
        n2 = _layernorm_t(x2, jnp.where(lane < (i < 0).astype(jnp.int32), n1[0:8], 0.0))
        yield
        rhs = lambda s: _rhs_slot(s, lambda rows, c: (n1, n2)[c][rows])
        for c in _fast_product(lambda s: _dot(_packed(wqkv_t, s), rhs(s))):
            pass
        yield
        store_qkv(t, i, _vcat(c[0], c[2]), q_s, k_s, v_s)
        store_qkv(t, i + 4, _vcat(c[1], c[3]), q_s, k_s, v_s)
        yield

    def first_norm(t, i, link=None):
        ns = []
        for b in (i, i + 4):
            x = in_t2(t, b)
            xres[t, b] = x
            ns.append(_layernorm_t(x, None if link is None else link[0]))
            if link is not None:
                link[0] = jnp.where(link[1], ns[-1][0:8], 0.0)
        for s in range(NSLOT):
            xn_s[t, i, s] = _rhs_slot(s, lambda rows, c: ns[c][rows])

    def first_qkv(t, i):
        cs = []
        for r0 in (0, HQ // 4):
            rows = slice(r0, r0 + HQ // 4)
            for c in _fast_product(lambda s: _dot(_packed(wqkv_t, s, rows), _packed(xn_s, t, i, s))):
                yield
            cs.append(c)
        for n, b in enumerate((i, i + 4)):
            part = _vcat(cs[0][n], cs[1][n], cs[0][n + 2], cs[1][n + 2])
            if t == 0:
                store_qkv(t, b, part, q0, k0, v0)
            else:
                store_qkv(t, b, part, q_s, k_s, v_s, prev=(k0, v0))

    def attention_group(t, b, g, q_r, k_r, v_r, links):
        par = len(links)
        never = lane < (b < 0).astype(jnp.int32)

        def start(n, v):
            if links[n % par] is None:
                return v
            return jnp.where(never, links[n % par], 0.0) + v

        q = [q_r[b, g, d] for d in range(DH)]
        logits = []
        for w in range(W):
            l = start(w, q[0] * k_r[b + NB - w, g, 0])
            for d in range(1, DH):
                l = l + q[d] * k_r[b + NB - w, g, d]
            links[w % par] = l
            l = l * (DH ** -0.5)
            if w > 0:
                edge = jnp.where(jnp.logical_and(w > b, t == 0), 2, 0)
                l = jnp.where(lane < edge, -1e9, l)
            logits.append(l)
        m = functools.reduce(jnp.maximum, logits)
        e = [jnp.exp(l - m) for l in logits]
        r = 1.0 / functools.reduce(jnp.add, e)
        p = [x * r for x in e]
        outs = []
        for d in range(DH):
            o = p[0] * v_r[b + NB, g, d]
            if d >= par:
                o = start(d, o)
            for w in range(1, W):
                o = o + p[w] * v_r[b + NB - w, g, d]
            links[d % par] = o
            outs.append(o)
        return _vcat(*outs)

    def phase2(t, i, par, q_r, k_r, v_r):
        links = [None] * par
        halves = [_vcat(*[attention_group(t, b, g, q_r, k_r, v_r, links) for g in range(NG)])
                  for b in (i, i + 4)]
        yield
        rhs = lambda s: _rhs_slot(s, lambda rows, c: halves[c][rows])
        for c in _fast_product(lambda s: _dot(_packed(wo_t, s), rhs(s))):
            pass
        x1 = xres[t, i] + _vcat(c[0], c[2])
        x2 = xres[t, i + 4] + _vcat(c[1], c[3])
        xres[t, i] = x1
        xres[t, i + 4] = x2
        n1 = _layernorm_t(x1)
        n2 = _layernorm_t(x2)
        yield
        ops = _lhs_slots(n1, n2)
        rows = pl.ds(pl.multiple_of(i * 64, 64), 64)
        for s in range(NSLOT):
            op = _vcat(ops[2 * s], ops[2 * s + 1]).astype(bf16).T
            a_s[t, s, rows, :] = pltpu.bitcast(op, u32)
        yield

    def proj(t, w_ref, off, res):
        outs = []
        for n0 in range(0, HC, NT):
            cols = [pl.ds(pl.multiple_of(off + n0 + c * HC, NT), NT) for c in (0, 1)]
            p = lambda s: _dot(pltpu.bitcast(a_s[t, s], bf16), _rhs_slot(s, lambda rows, c: w_ref[rows, cols[c]]))
            for c in _fast_product(p):
                yield
            outs.append(c)
        res.extend(jnp.concatenate(x, axis=1) if len(x) > 1 else x[0] for x in zip(*outs))

    def ffn_chunk(t, j, may_init=False):
        off = pl.multiple_of(j * FC, FC)
        g, u = [], []
        yield from proj(t, wg, off, g)
        yield from proj(t, wu, off, u)
        b11, b21, b12, b22 = [x * y for x, y in zip(g, u)]
        ca = pl.ds(off, HC)
        cb = pl.ds(pl.multiple_of(off + HC, HC), HC)
        a11, a12, a21, a22 = wd[0:HD, ca], wd[0:HD, cb], wd[HD:D, ca], wd[HD:D, cb]

        def accumulate(n, v):
            for c in range(4):
                old = acc[t, n, c]
                if may_init:
                    old = jnp.where(j > 0, old, 0.0)
                acc[t, n, c] = old + v[:, c * 128:(c + 1) * 128]

        accumulate(0, _dot_nt(_add(a11, a22), _add(b11, b22)))
        yield
        accumulate(1, _dot_nt(_add(a21, a22), b11.astype(bf16)))
        yield
        accumulate(2, _dot_nt(a11, _sub(b12, b22)))
        yield
        accumulate(3, _dot_nt(a22, _sub(b21, b11)))
        yield
        accumulate(4, _dot_nt(_add(a11, a12), b22.astype(bf16)))
        yield
        accumulate(5, _dot_nt(_sub(a21, a11), _add(b11, b12)))
        yield
        accumulate(6, _dot_nt(_sub(a12, a22), _add(b21, b22)))
        yield

    with _scope("w_x0"):
        x_copy(0, 0, TM).wait()
    x_copy(1, 0, TM).start()
    cwo.start()
    for c in range(NB):
        in_t1(0, c)
    first_norm(0, 0)
    prep_wqkv()
    with _scope("w_x1"):
        x_copy(1, 0, TM).wait()
    for g in range(len(groups)):
        for c in ffn_copies(g):
            c.start()
    for c in range(NB):
        in_t1(1, c)

    def body_f(i, last):
        _drain(first_qkv(0, i))
        link = [None, lane < (i < 0).astype(jnp.int32)]
        first_norm(1, i, link)
        if last:
            prep_wo()
        else:
            first_norm(0, i + 1, link)

    _loop(3, lambda i: body_f(i, False))
    cwo.wait()
    _loop(1, lambda i: body_f(i + 3, True))
    _loop(4, lambda i: _weave(ORDER_E, first_qkv(1, i), phase2(0, i, PAR0, q0, k0, v0)))

    def wait_group(k, g):
        @pl.when(k == 0)
        def _():
            for c in ffn_copies(g):
                c.wait()

    def stage(k):
        t = k % 2
        n_a = jnp.where(jnp.logical_and(k > 0, k < 3), 4, 0)
        n_b = jnp.where(k < 3, 4, 0)
        n_c = NCH - n_a - n_b
        wait_group(k, 0)
        _loop(n_c, lambda i: _drain(ffn_chunk(t, i, True)))
        _loop(n_a, lambda i: _weave(ORDER_A, ffn_chunk(t, n_c + i), phase1(1 - t, i)))
        wait_group(k, 1)
        _loop(n_b, lambda i: _weave(ORDER_B, ffn_chunk(t, n_c + n_a + i),
                                    phase2(1 - t, i, PAR, q_s, k_s, v_s)))
    _loop(4, stage)

    def finish(t):
        for i in range(4):
            x1, x2 = combine(t, i)
            out_t1(t, i, x1)
            out_t1(t, i + 4, x2)
        for c in range(NB):
            out_t2(t, c)
            if c % 4 == 3:
                out_copy(t, c // 4).start()

    finish(0)
    finish(1)
    with _scope("w_out"):
        for t in range(2):
            for half in range(2):
                out_copy(t, half).wait()


@jax.jit
def pallas_interleave_layers__sliding_local_dilated__glu_gated_bilinear__prompt_kernel(
    A_x: jax.Array,
    A_wqkv: jax.Array,
    A_wo: jax.Array,
    B_x: jax.Array,
    B_w_gate: jax.Array,
    B_w_up: jax.Array,
    B_w_down: jax.Array,
):
    any_spec = pl.BlockSpec(memory_space=pl.ANY)
    qkv_scratch = [
        pltpu.VMEM((NB, NG, DH, 8, 128), f32),
        pltpu.VMEM((2 * NB, NG, DH, 8, 128), f32),
        pltpu.VMEM((2 * NB, NG, DH, 8, 128), f32),
    ]
    out_t = pl.pallas_call(
        _kernel,
        in_specs=[any_spec] * 6,
        out_specs=any_spec,
        out_shape=jax.ShapeDtypeStruct((D, S), bf16),
        scratch_shapes=[
            pltpu.VMEM((D, S), bf16),
            pltpu.VMEM((D, 3 * D), bf16),
            pltpu.VMEM((D, D), bf16),
            pltpu.VMEM((D, F), bf16),
            pltpu.VMEM((D, F), bf16),
            pltpu.VMEM((D, F), bf16),
            pltpu.VMEM((NSLOT, HQ, 128), bf16),
            pltpu.VMEM((NSLOT, HD, 128), bf16),
            pltpu.VMEM((5, 3 * D, 128), f32),
            pltpu.VMEM((5, D, 128), f32),
            pltpu.VMEM((2, 5, HM, 128), u32),
            pltpu.VMEM((2, 5, 8 * 72, 128), u32),
            pltpu.VMEM((2, NB, D, 128), f32),
            *qkv_scratch,
            *qkv_scratch,
            pltpu.VMEM((2, NSLOT, HM // 2, 128), u32),
            pltpu.VMEM((2, 7, 4, HD, 128), f32),
            pltpu.VMEM((2, 4, NSLOT, 128, 128), bf16),
            pltpu.SemaphoreType.DMA((20,)),
        ],
        compiler_params=pltpu.CompilerParams(vmem_limit_bytes=120 * 1024 * 1024),
        name="fused_layers",
    )(A_x[0].T, A_wqkv, A_wo, B_w_gate, B_w_up, B_w_down.T)
    return out_t.T[None]
```

```python
import functools
import os

import jax
import jax.numpy as jnp
import jax.experimental.pallas as pl
import jax.experimental.pallas.tpu as pltpu

S, D, F = 2048, 576, 4608
H, DH, W = 32, 18, 8
NG = H // 8
GR = 8 * DH
NB = 8
TM = NB * 128
HM = TM // 2
HD = D // 2
HQ = 3 * D // 2
FC = 512
HC = FC // 2
NCH = F // FC
NSLOT = 16
NT = int(os.environ.get("NT", 128))

GROUP_ROWS = {1: (0, 128), 2: (64, 192), 4: (256, 384), 3: (320, 448), 0: (512, 512)}
T3 = 1.0 / 3.0
SLOTS = (
    ((1, (-1, -1, 0, 0), (0, 0, 0, 1)), (3, (1, 1, 0, 0), (0, 0, 1, 0))),
    ((0, (T3, 0, 0, 0), (2, 1, 0, 0)), (2, (-.5, -1, 0, 0), (0, 0, 0, 1))),
    ((4, (.5, 1, 0, 0), (0, 0, 1, 0)), (0, (-T3, 0, 0, 0), (1, 2, 0, 0))),
    ((1, (0, 1, 0, -1), (0, 0, 1, 1)), (2, (0, 2, 0, -1), (0, 0, .5, 1))),
    ((1, (0, 0, 1, 1), (1, 0, 0, 0)), (3, (0, 0, -1, -1), (0, 1, 0, 0))),
    ((0, (0, 0, T3, 0), (2, 1, 0, 0)), (2, (0, 0, .5, 1), (1, 0, 0, 0))),
    ((4, (0, 0, -.5, -1), (0, 1, 0, 0)), (0, (0, 0, -T3, 0), (1, 2, 0, 0))),
    ((1, (-1, 0, 1, 0), (1, 1, 0, 0)), (2, (-1, 0, .5, 0), (1, 2, 0, 0))),
    ((1, (0, 0, 0, 1), (-1, 0, 1, 0)), (3, (1, 0, 0, 0), (1, 0, -1, 0))),
    ((4, (.5, 0, 0, 0), (2, 0, -1, 0)), (2, (0, 0, 0, 1), (-1, 0, .5, 0))),
    ((4, (-1, 0, .5, 0), (2, 1, 0, 0)), (3, (-1, 0, 1, 0), (1, 1, 0, 0))),
    ((1, (1, 0, 0, 1), (1, 0, 0, 1)), (2, (1, 0, 0, 1), (1, 0, 0, 1))),
    ((1, (1, 0, 0, 0), (0, 1, 0, -1)), (3, (0, 0, 0, 1), (0, -1, 0, 1))),
    ((4, (0, 0, 0, 1), (0, -1, 0, .5)), (2, (.5, 0, 0, 0), (0, 2, 0, -1))),
    ((4, (0, 2, 0, -1), (0, 0, 1, .5)), (3, (0, 1, 0, -1), (0, 0, 1, 1))),
    ((4, (1, 0, 0, 1), (0, 1, 1, 0)), (3, (1, 0, 0, 1), (0, 1, 1, 0))),
)
STRASSEN = (
    ((1, 0, 0, 1), (1, 0, 0, 1)),
    ((0, 0, 1, 1), (1, 0, 0, 0)),
    ((1, 0, 0, 0), (0, 1, 0, -1)),
    ((0, 0, 0, 1), (-1, 0, 1, 0)),
    ((1, 1, 0, 0), (0, 0, 0, 1)),
    ((-1, 0, 1, 0), (1, 1, 0, 0)),
    ((0, 1, 0, -1), (0, 0, 1, 1)),
)
QD = D // 4
EPS = 1e-5
PRE = int(os.environ.get("PRE", 0))
CLINK = int(os.environ.get("CLINK", 1))
KA = int(os.environ.get("KA", 6))
KB = int(os.environ.get("KB", 16))
PAR = int(os.environ.get("PAR", 1))
PAR0 = int(os.environ.get("PAR0", 3))
ORDER_A = "s" + "m" * KA + "ss"
ORDER_B = "s" + "m" * KB + "s" + "m" * (2048 // NT - KB) + "s"
ORDER_C = "s" + "m" * int(os.environ.get("KC", 6)) + "s" + "m" * int(os.environ.get("KC2", 6)) + "s"
ORDER_E = "s" + "m" * int(os.environ.get("KE", 5)) + "s"
f32, bf16, u32 = jnp.float32, jnp.bfloat16, jnp.uint32

_dot = functools.partial(jnp.dot, preferred_element_type=f32)


def _dot_nt(a, b):
    return jax.lax.dot_general(a, b, (((1,), (1,)), ((), ())), preferred_element_type=f32)


def _vcat(*xs):
    return jnp.concatenate(xs, axis=0)


def _pad_rows(r):
    return _vcat(r, jnp.zeros((128 - r.shape[0], r.shape[1]), r.dtype))


def _add(x, y):
    return (x.astype(f32) + y.astype(f32)).astype(bf16)


def _sub(x, y):
    return (x.astype(f32) - y.astype(f32)).astype(bf16)


def _form(coefs, blocks):
    terms = [(c, blk) for c, blk in zip(coefs, blocks) if c != 0]
    if len(terms) == 1 and terms[0][0] == 1:
        return terms[0][1]()
    terms.sort(key=lambda cb: cb[0] < 0)
    out = None
    for c, blk in terms:
        v = blk().astype(f32)
        if out is None:
            out = v if c == 1 else v * c
        else:
            v = v if abs(c) == 1 else v * abs(c)
            out = out + v if c > 0 else out - v
    return out


def _lhs_slots(x1, x2):
    out = []
    for halves in SLOTS:
        for grp, coefs, _ in halves:
            k1, k2 = GROUP_ROWS[grp]
            blocks = [lambda x=x, k=k: x[k:k + 64] for x in (x1, x2) for k in (k1, k2)]
            out.append(_form(coefs, blocks))
    return out


def _lhs_slots_lanes(x1, x2):
    low = jax.lax.broadcasted_iota(jnp.int32, x1[0].shape, 1) < 64
    out = []
    for halves in SLOTS:
        keys = [(tuple(k // 128 for k in GROUP_ROWS[grp]), coefs) for grp, coefs, _ in halves]
        vals = [_form(coefs, [lambda x=x, g=g: x[g] for x in (x1, x2) for g in tiles])
                for tiles, coefs in keys]
        out.append(vals[0] if keys[0] == keys[1] else jnp.where(low, vals[0], vals[1]))
    return out


def _fast_product(p):
    p0, p1, p2, p3 = p(0), p(1), p(2), p(3)
    r = p0 + p1 + p2
    c11 = r + p1 + p3
    c12 = r + p2
    yield None
    p0, p1, p2, p3 = p(4), p(5), p(6), p(7)
    r = p0 + p1 + p2
    c21 = r + p1
    c22 = p3 - (r + p2)
    yield None
    p0, p1, p2, p3 = p(8), p(9), p(10), p(11)
    r = p0 + p1
    c11 = c11 + (r + p3)
    c21 = c21 + (r + p1 + p2)
    c22 = c22 + p3
    yield None
    p0, p1, p2, p3 = p(12), p(13), p(14), p(15)
    r = p0 + p1
    c12 = (r + p2 + p3) - c12
    c22 = c22 + (r + p1)
    c21 = c21 + p3
    yield (c11, c12, c21, c22)


def _rhs_slot(s, get, anchors=()):
    parts = []
    for grp, _, coefs in SLOTS[s]:
        k1, k2 = GROUP_ROWS[grp]
        blocks = [lambda k=k, c=c: get(slice(k, k + 64), c) for k in (k1, k2) for c in (0, 1)]
        parts.append(_form(coefs, blocks).astype(f32))
    while anchors:
        parts[0] = _vcat(parts[0][:8] + anchors.pop(), parts[0][8:])
    return _vcat(*parts).astype(bf16)


def _packed(ref, *idx):
    return pltpu.bitcast(ref.bitcast(u32)[idx], bf16)


def _layernorm_t(x, zero=None):
    rows = [x[r:r + 8] for r in range(0, D, 8)]
    s = rows[0] if zero is None else rows[0] + zero
    for r in rows[1:]:
        s = s + r
    m = jnp.sum(s, axis=0, keepdims=True) * (1.0 / D)
    rows = [r - m for r in rows]
    s = rows[0] * rows[0]
    for r in rows[1:]:
        s = s + r * r
    v = jnp.sum(s, axis=0, keepdims=True) * (1.0 / D)
    return _vcat(*rows) * jax.lax.rsqrt(v + EPS)


def _aligned(x, n):
    return x if isinstance(x, int) else pl.multiple_of(x, n)


def _drain(*gens):
    for gen in gens:
        for _ in gen:
            pass


def _weave(order, main, side):
    for c in order:
        next(main if c == "m" else side)
    _drain(main, side)


def _scope(name):
    import contextlib
    return jax.named_scope(name) if os.environ.get("SCOPES") else contextlib.nullcontext()


def _loop(n, fn):
    def body(i, c):
        with _scope("it"):
            fn(i)
        return c
    jax.lax.fori_loop(0, n, body, 0)


def _kernel(x_hbm, wqkv_hbm, wo_hbm, wg_hbm, wu_hbm, wd_hbm, out_hbm,
            xin, wqkv, wo, wg, wu, wd, wqkv_t, wo_t, wperm, operm, pin, pout, xres,
            q0, k0, v0, q_s, k_s, v_s, a_s, h_s, w_s, acc, xn_s, sems):
    groups = (range(5), range(5, NCH))
    lane = jax.lax.broadcasted_iota(jnp.int32, (8, 128), 1)

    def x_copy(t, piece, n):
        cols = pl.ds(pl.multiple_of(t * TM + piece * n, 128), n)
        return pltpu.make_async_copy(x_hbm.at[:, cols], xin.at[:, cols], sems.at[10 + t + piece])

    def wqkv_copy(g):
        rows = pl.ds(g * 128, min(128, D - g * 128))
        return pltpu.make_async_copy(wqkv_hbm.at[rows], wqkv.at[rows], sems.at[15 + g])

    def out_copy(t, half):
        cols = pl.ds(t * TM + half * HM, HM)
        return pltpu.make_async_copy(xin.at[:, cols], out_hbm.at[:, cols], sems.at[2 * t + half])

    def ffn_copies(g):
        return [pltpu.make_async_copy(src.at[:, pl.ds(j * FC, FC)], dst.at[j], sems.at[20 + 3 * j + i])
                for j in groups[g]
                for i, (src, dst) in enumerate(((wg_hbm, wg), (wu_hbm, wu), (wd_hbm, wd)))]

    cwo = pltpu.make_async_copy(wo_hbm, wo, sems.at[3])
    x_copy(0, 0, TM).start()
    for g in range(5):
        wqkv_copy(g).start()

    def head_rows(ref, g, base):
        return _vcat(*[ref[g, pl.ds(base + d, 8, stride=DH), :] for d in range(DH)])

    def prep_wqkv():
        for gs in ((0, 1), (2, 3), (4,)):
            with _scope("w_qkv"):
                for g in gs:
                    wqkv_copy(g).wait()
            for g in gs:
                rows = wqkv[g * 128:min((g + 1) * 128, D), :].astype(f32)
                wperm[g] = (_vcat(rows, rows) if g == 4 else rows).T

        def rows_of(hg):
            base = pl.multiple_of(hg * GR, 16)
            x1 = [head_rows(wperm, g, base) for g in range(5)]
            x2 = [head_rows(wperm, g, base + HQ) for g in range(5)]
            for n, v in enumerate(_lhs_slots_lanes(x1, x2)):
                wqkv_t[n, pl.ds(base, GR), :] = v.astype(bf16)
        _loop(HQ // GR, rows_of)

    def prep_wo():
        for g in range(5):
            cols = wo[:, g * 128:min((g + 1) * 128, D)].astype(f32)
            if g == 4:
                cols = jnp.concatenate([cols, jnp.zeros_like(cols)], axis=1)
            operm[g] = cols
        parts = []
        for g in range(5):
            r = _vcat(*[head_rows(operm, g, hg * GR) for hg in range(NG)])
            rt = _vcat(r, r[512:D]).astype(bf16).T
            parts.append(rt[:64] if g == 4 else rt)
        wt = _vcat(*parts).astype(f32)
        x1 = [wt[0:HD, g * 128:(g + 1) * 128] for g in range(5)]
        x2 = [wt[HD:D, g * 128:(g + 1) * 128] for g in range(5)]
        for n, v in enumerate(_lhs_slots_lanes(x1, x2)):
            wo_t[n] = v.astype(bf16)

    def to_words(x):
        tiles = [x[g * 128:(g + 1) * 128] for g in range(4)] + [_pad_rows(x[512:D])]
        return [pltpu.bitcast(r.astype(bf16).T, u32) for r in tiles]

    def from_words(words):
        parts = [pltpu.bitcast(w, bf16).T for w in words]
        return _vcat(*parts[:4], parts[4][:64])

    def in_t1(t, c):
        x = xin[:, pl.ds(pl.multiple_of(t * TM + c * 128, 128), 128)]
        for g, w in enumerate(to_words(x)):
            pin[t, g, pl.ds(pl.multiple_of(c * 64, 64), 64), :] = w

    def in_t2(t, j):
        return from_words([pin[t, g, pl.ds(j, 64, stride=8), :] for g in range(5)]).astype(f32)

    def out_t1(t, j, x):
        words = to_words(x)
        for g, w in enumerate(words):
            pout[t, g, pl.ds(_aligned(j * 72, 8), 64), :] = w
        return [w[56:64] for w in words]

    def out_t2(t, c):
        words = [_vcat(*[pout[t, g, pl.ds(c * 8 + m, 8, stride=72), :] for m in range(8)])
                 for g in range(5)]
        x = from_words(words)
        xin[:, pl.ds(_aligned(t * TM + c * 128, 128), 128)] = x
        return [pltpu.bitcast(x[r - 16:r], u32) for r in (128, 256, 384, 512, D)]

    def combine(t, i, never=None):
        c, second = i % 2, i // 2
        pick = lambda lo, hi: lo + (hi - lo) * second
        outer = lambda m1, m2, m3, m4, m5, m6, m7: (
            m1 + m4 - m5 + m7, m2 + m4, m3 + m5, m1 - m2 + m3 + m6)
        strips, link = [], None
        for r in range(0, QD, 8):
            get = lambda n, m: acc[t, c, m, n * QD + r:n * QD + r + 8, :]
            four, two = [], []
            for n in range(7):
                x = get(n, pick(3, 2))
                if link is not None and n % CLINK == 0:
                    x = x + jnp.where(never, link, 0.0)
                four.append(((get(n, 0) + x) + get(n, pick(6, 5))) - get(n, pick(4, 1)))
                two.append(get(n, pick(1, 4)) + x)
                if never is not None:
                    link = four[-1]
            rows = []
            for u, v in zip(outer(*four), outer(*two)):
                if isinstance(second, int):
                    rows += [v, u] if second else [u, v]
                else:
                    rows += [jnp.where(second > 0, v, u), jnp.where(second > 0, u, v)]
            strips.append([xres[t, i + 4 * (q // 4), (q % 4) * QD + r:(q % 4) * QD + r + 8, :] + v
                           for q, v in enumerate(rows)])
        return [_vcat(*[s[q] for q in range(q0, q0 + 4) for s in strips]) for q0 in (0, 4)]

    def store_qkv(t, b, part, q, k, v, prev=None):
        q[b] = part[0:D].reshape(NG, DH, 8, 128)
        for n, (dst, r) in enumerate(((k, part[D:2 * D]), (v, part[2 * D:3 * D]))):
            dst[b + NB] = r.reshape(NG, DH, 8, 128)
            sh = pltpu.roll(r, 2, 1).reshape(NG, DH, 8, 128)
            if isinstance(t, int) and t == 0:
                dst[b] = sh
            elif prev is not None:
                dst[b] = jnp.where((lane < 2)[None, None], prev[n][b], sh)
            else:
                keep = jnp.broadcast_to((lane >= 2 * t)[None, None], sh.shape)
                pltpu.store(dst.at[b], sh, mask=keep)

    def phase1(t, i):
        never = lane < (i < 0).astype(jnp.int32)
        x1, x2 = combine(t, i, never)
        xres[t, i] = x1
        xres[t, i + 4] = x2
        n1 = _layernorm_t(x1)
        n2 = _layernorm_t(x2, jnp.where(never, n1[0:8], 0.0))
        yield
        rhs = lambda s: _rhs_slot(s, lambda rows, c: (n1, n2)[c][rows])
        for c in _fast_product(lambda s: _dot(_packed(wqkv_t, s), rhs(s))):
            pass
        yield
        store_qkv(t, i, _vcat(c[0], c[2]), q_s, k_s, v_s)
        store_qkv(t, i + 4, _vcat(c[1], c[3]), q_s, k_s, v_s)
        yield

    def first_norm(t, i, link=None):
        ns = []
        for b in (i, i + 4):
            x = in_t2(t, b)
            xres[t, b] = x
            ns.append(_layernorm_t(x, None if link is None else link[0]))
            if link is not None:
                link[0] = jnp.where(link[1], ns[-1][0:8], 0.0)
        for s in range(NSLOT):
            xn_s[t, i, s] = _rhs_slot(s, lambda rows, c: ns[c][rows])

    def first_qkv(t, i):
        cs = []
        for r0 in (0, HQ // 4):
            rows = slice(r0, r0 + HQ // 4)
            for c in _fast_product(lambda s: _dot(_packed(wqkv_t, s, rows), _packed(xn_s, t, i, s))):
                yield
            cs.append(c)
        for n, b in enumerate((i, i + 4)):
            part = _vcat(cs[0][n], cs[1][n], cs[0][n + 2], cs[1][n + 2])
            if t == 0:
                store_qkv(t, b, part, q0, k0, v0)
            else:
                store_qkv(t, b, part, q_s, k_s, v_s, prev=(k0, v0))

    def attention_group(t, b, g, q_r, k_r, v_r, links):
        par = len(links)
        never = lane < (b < 0).astype(jnp.int32)

        def start(n, v):
            if links[n % par] is None:
                return v
            return jnp.where(never, links[n % par], 0.0) + v

        q = [q_r[b, g, d] for d in range(DH)]
        logits = []
        for w in range(W):
            l = start(w, q[0] * k_r[b + NB - w, g, 0])
            for d in range(1, DH):
                l = l + q[d] * k_r[b + NB - w, g, d]
            links[w % par] = l
            l = l * (DH ** -0.5)
            if w > 0:
                edge = jnp.where(jnp.logical_and(w > b, t == 0), 2, 0)
                l = jnp.where(lane < edge, -1e9, l)
            logits.append(l)
        m = functools.reduce(jnp.maximum, logits)
        e = [jnp.exp(l - m) for l in logits]
        r = 1.0 / functools.reduce(jnp.add, e)
        p = [x * r for x in e]
        outs = []
        for d in range(DH):
            o = p[0] * v_r[b + NB, g, d]
            if d >= par:
                o = start(d, o)
            for w in range(1, W):
                o = o + p[w] * v_r[b + NB - w, g, d]
            links[d % par] = o
            outs.append(o)
        return _vcat(*outs)

    def phase2(t, i, par, q_r, k_r, v_r):
        links = [None] * par
        halves = [_vcat(*[attention_group(t, b, g, q_r, k_r, v_r, links) for g in range(NG)])
                  for b in (i, i + 4)]
        yield
        rhs = lambda s: _rhs_slot(s, lambda rows, c: halves[c][rows])
        for c in _fast_product(lambda s: _dot(_packed(wo_t, s), rhs(s))):
            pass
        x1 = xres[t, i] + _vcat(c[0], c[2])
        x2 = xres[t, i + 4] + _vcat(c[1], c[3])
        xres[t, i] = x1
        xres[t, i + 4] = x2
        n1 = _layernorm_t(x1)
        n2 = _layernorm_t(x2)
        yield
        ops = _lhs_slots(n1, n2)
        rows = pl.ds(pl.multiple_of(i * 64, 64), 64)
        for s in range(NSLOT):
            op = _vcat(ops[2 * s], ops[2 * s + 1]).astype(bf16).T
            a_s[t, s, rows, :] = pltpu.bitcast(op, u32)
        yield

    anchors = []

    def anchor(never, words):
        anchors.append(jnp.where(never, pltpu.bitcast(functools.reduce(jnp.bitwise_or, words), f32), 0.0))

    def proj(t, w_ref, off, res, side):
        cols = [pl.ds(off + c * HC, 128) for c in (0, 1)]

        def p(s):
            x = a_s[t, s]
            zero = next(side, None)
            if zero is not None:
                r = 32 + 64 * (s % 4)
                x = _vcat(x[:r], x[r:r + 8] | zero, x[r + 8:])
            return _dot(pltpu.bitcast(x, bf16), _rhs_slot(s, lambda rows, c: w_ref[rows, cols[c]], anchors))
        for c in _fast_product(p):
            yield
        res.extend(c)

    def down_lhs(j):
        cols = [pl.ds(k * 128, 128) for k in range(4)]
        zero = (j < 0).astype(jnp.int32)
        for n in range(7):
            for r0 in range(0, QD, 16):
                outer = [_form(STRASSEN[n][0],
                               [lambda r=r, k=k, r2=r2, k2=k2: wd[j, pl.ds((2 * r + r2) * QD + r0, 16), cols[2 * k + k2]]
                                for r in (0, 1) for k in (0, 1)])
                         for r2 in (0, 1) for k2 in (0, 1)]
                for m in range(7):
                    v = _form(STRASSEN[m][0], [lambda x=x: x for x in outer])
                    w_s[pl.ds((7 * n + m) * QD + r0, 16)] = v.astype(bf16)
                done = w_s.bitcast(u32)[pl.ds(pl.multiple_of(8 * j * zero, 8), 8), :]
                yield jnp.where(lane < zero, done, jnp.uint32(0))

    def ffn_chunk(t, j, may_init=False):
        side = down_lhs(j) if PRE else iter(())
        lhs = {}
        for k2 in (0, 1):
            g, u = [], []
            yield from proj(t, wg.at[j], k2 * 128, g, side)
            yield from proj(t, wu.at[j], k2 * 128, u, side)
            b11, b21, b12, b22 = [x * y for x, y in zip(g, u)]
            for n, (_, lb) in enumerate(STRASSEN):
                h_s[n, k2] = _form(lb, [lambda x=x: x for x in (b11, b12, b21, b22)])
        order = [(n, m) for n in range(7) for m in (1, 5)] + [(n, m) for n in range(7) for m in (0, 2, 3, 4, 6)]
        for q, (n, m) in enumerate(order):
            rhs = [lambda k2=k2, c2=c2: h_s[n, k2, c2 * 256:(c2 + 1) * 256, :] for k2 in (0, 1) for c2 in (0, 1)]
            if PRE:
                left = _packed(w_s, pl.ds((7 * n + m) * QD // 2, QD // 2))
            else:
                if q == 14:
                    lhs.clear()
                if n not in lhs:
                    lhs[n] = [_form(STRASSEN[n][0],
                                    [lambda r=r, k=k, r2=r2, k2=k2: wd[j, pl.ds((2 * r + r2) * QD, QD),
                                                                       pl.ds((2 * k + k2) * 128, 128)]
                                     for r in (0, 1) for k in (0, 1)])
                              for r2 in (0, 1) for k2 in (0, 1)]
                left = _form(STRASSEN[m][0], [lambda x=x: x for x in lhs[n]]).astype(bf16)
            v = _dot_nt(left, _form(STRASSEN[m][1], rhs).astype(bf16))
            for c in range(2):
                old = acc[t, c, m, n * QD:(n + 1) * QD, :]
                if may_init:
                    old = jnp.where(j > 0, old, 0.0)
                acc[t, c, m, n * QD:(n + 1) * QD, :] = old + v[:, c * 128:(c + 1) * 128]
            if q % 7 == 6:
                yield

    with _scope("w_x0"):
        x_copy(0, 0, TM).wait()
    x_copy(1, 0, TM).start()
    cwo.start()
    for c in range(NB):
        in_t1(0, c)
    first_norm(0, 0)
    prep_wqkv()
    with _scope("w_x1"):
        x_copy(1, 0, TM).wait()
    for g in range(len(groups)):
        for c in ffn_copies(g):
            c.start()
    for c in range(NB):
        in_t1(1, c)

    def body_f(i, last):
        _drain(first_qkv(0, i))
        link = [None, lane < (i < 0).astype(jnp.int32)]
        first_norm(1, i, link)
        if last:
            prep_wo()
        else:
            first_norm(0, i + 1, link)

    _loop(3, lambda i: body_f(i, False))
    cwo.wait()
    _loop(1, lambda i: body_f(i + 3, True))
    _loop(4, lambda i: _weave(ORDER_E, first_qkv(1, i), phase2(0, i, PAR0, q0, k0, v0)))

    def wait_group(k, g):
        @pl.when(k == 0)
        def _():
            for c in ffn_copies(g):
                c.wait()

    def finish_step(i):
        u = i % 4
        never = lane < (i < 0).astype(jnp.int32)
        x1, x2 = combine(0, u, never)
        done = out_t1(0, u, x1) + out_t1(0, u + 4, x2)
        yield
        anchor(never, done)
        done = out_t2(0, 2 * u) + out_t2(0, 2 * u + 1)
        yield
        anchor(never, done)
        yield

    def stage(k):
        t = k % 2
        n_a = jnp.where(jnp.logical_and(k > 0, k < 3), 4, 0)
        n_b = jnp.where(k < 3, 4, 0)
        n_c = NCH - n_a - n_b
        wait_group(k, 0)
        _loop(n_c, lambda i: _weave(ORDER_C, ffn_chunk(t, i, True), finish_step(i)))
        _loop(n_a, lambda i: _weave(ORDER_A, ffn_chunk(t, n_c + i), phase1(1 - t, i)))
        wait_group(k, 1)
        _loop(n_b, lambda i: _weave(ORDER_B, ffn_chunk(t, n_c + n_a + i),
                                    phase2(1 - t, i, PAR, q_s, k_s, v_s)))
    _loop(4, stage)

    for half in range(2):
        out_copy(0, half).start()
    for i in range(4):
        x1, x2 = combine(1, i)
        out_t1(1, i, x1)
        out_t1(1, i + 4, x2)
    for c in range(NB):
        out_t2(1, c)
        if c % 4 == 3:
            out_copy(1, c // 4).start()
    with _scope("w_out"):
        for t in range(2):
            for half in range(2):
                out_copy(t, half).wait()


@jax.jit
def pallas_interleave_layers__sliding_local_dilated__glu_gated_bilinear__prompt_kernel(
    A_x: jax.Array,
    A_wqkv: jax.Array,
    A_wo: jax.Array,
    B_x: jax.Array,
    B_w_gate: jax.Array,
    B_w_up: jax.Array,
    B_w_down: jax.Array,
):
    any_spec = pl.BlockSpec(memory_space=pl.ANY)
    qkv_scratch = [
        pltpu.VMEM((NB, NG, DH, 8, 128), f32),
        pltpu.VMEM((2 * NB, NG, DH, 8, 128), f32),
        pltpu.VMEM((2 * NB, NG, DH, 8, 128), f32),
    ]
    out_t = pl.pallas_call(
        _kernel,
        in_specs=[any_spec] * 6,
        out_specs=any_spec,
        out_shape=jax.ShapeDtypeStruct((D, S), bf16),
        scratch_shapes=[
            pltpu.VMEM((D, S), bf16),
            pltpu.VMEM((D, 3 * D), bf16),
            pltpu.VMEM((D, D), bf16),
            pltpu.VMEM((NCH, D, FC), bf16),
            pltpu.VMEM((NCH, D, FC), bf16),
            pltpu.VMEM((NCH, D, FC), bf16),
            pltpu.VMEM((NSLOT, HQ, 128), bf16),
            pltpu.VMEM((NSLOT, HD, 128), bf16),
            pltpu.VMEM((5, 3 * D, 128), f32),
            pltpu.VMEM((5, D, 128), f32),
            pltpu.VMEM((2, 5, HM, 128), u32),
            pltpu.VMEM((2, 5, 8 * 72, 128), u32),
            pltpu.VMEM((2, NB, D, 128), f32),
            *qkv_scratch,
            *qkv_scratch,
            pltpu.VMEM((2, NSLOT, HM // 2, 128), u32),
            pltpu.VMEM((7, 2, HM, 128), f32),
            pltpu.VMEM((49 * QD, 128), bf16),
            pltpu.VMEM((2, 2, 7, 1024, 128), f32),
            pltpu.VMEM((2, 4, NSLOT, 128, 128), bf16),
            pltpu.SemaphoreType.DMA((20 + 3 * NCH,)),
        ],
        compiler_params=pltpu.CompilerParams(vmem_limit_bytes=120 * 1024 * 1024),
        name="fused_layers",
    )(A_x[0].T, A_wqkv, A_wo, B_w_gate, B_w_up, B_w_down.T)
    return out_t.T[None]
```

```python
import functools
import os

import jax
import jax.numpy as jnp
import jax.experimental.pallas as pl
import jax.experimental.pallas.tpu as pltpu

S, D, F = 2048, 576, 4608
H, DH, W = 32, 18, 8
NG = H // 8
GR = 8 * DH
NB = 8
TM = NB * 128
HM = TM // 2
HD = D // 2
HQ = 3 * D // 2
FC = 512
HC = FC // 2
NCH = F // FC
NSLOT = 16
NT = int(os.environ.get("NT", 128))

GROUP_ROWS = {1: (0, 128), 2: (64, 192), 4: (256, 384), 3: (320, 448), 0: (512, 512)}
T3 = 1.0 / 3.0
SLOTS = (
    ((1, (-1, -1, 0, 0), (0, 0, 0, 1)), (3, (1, 1, 0, 0), (0, 0, 1, 0))),
    ((0, (T3, 0, 0, 0), (2, 1, 0, 0)), (2, (-.5, -1, 0, 0), (0, 0, 0, 1))),
    ((4, (.5, 1, 0, 0), (0, 0, 1, 0)), (0, (-T3, 0, 0, 0), (1, 2, 0, 0))),
    ((1, (0, 1, 0, -1), (0, 0, 1, 1)), (2, (0, 2, 0, -1), (0, 0, .5, 1))),
    ((1, (0, 0, 1, 1), (1, 0, 0, 0)), (3, (0, 0, -1, -1), (0, 1, 0, 0))),
    ((0, (0, 0, T3, 0), (2, 1, 0, 0)), (2, (0, 0, .5, 1), (1, 0, 0, 0))),
    ((4, (0, 0, -.5, -1), (0, 1, 0, 0)), (0, (0, 0, -T3, 0), (1, 2, 0, 0))),
    ((1, (-1, 0, 1, 0), (1, 1, 0, 0)), (2, (-1, 0, .5, 0), (1, 2, 0, 0))),
    ((1, (0, 0, 0, 1), (-1, 0, 1, 0)), (3, (1, 0, 0, 0), (1, 0, -1, 0))),
    ((4, (.5, 0, 0, 0), (2, 0, -1, 0)), (2, (0, 0, 0, 1), (-1, 0, .5, 0))),
    ((4, (-1, 0, .5, 0), (2, 1, 0, 0)), (3, (-1, 0, 1, 0), (1, 1, 0, 0))),
    ((1, (1, 0, 0, 1), (1, 0, 0, 1)), (2, (1, 0, 0, 1), (1, 0, 0, 1))),
    ((1, (1, 0, 0, 0), (0, 1, 0, -1)), (3, (0, 0, 0, 1), (0, -1, 0, 1))),
    ((4, (0, 0, 0, 1), (0, -1, 0, .5)), (2, (.5, 0, 0, 0), (0, 2, 0, -1))),
    ((4, (0, 2, 0, -1), (0, 0, 1, .5)), (3, (0, 1, 0, -1), (0, 0, 1, 1))),
    ((4, (1, 0, 0, 1), (0, 1, 1, 0)), (3, (1, 0, 0, 1), (0, 1, 1, 0))),
)
STRASSEN = (
    ((1, 0, 0, 1), (1, 0, 0, 1)),
    ((0, 0, 1, 1), (1, 0, 0, 0)),
    ((1, 0, 0, 0), (0, 1, 0, -1)),
    ((0, 0, 0, 1), (-1, 0, 1, 0)),
    ((1, 1, 0, 0), (0, 0, 0, 1)),
    ((-1, 0, 1, 0), (1, 1, 0, 0)),
    ((0, 1, 0, -1), (0, 0, 1, 1)),
)
QD = D // 4
EPS = 1e-5
SPLITQ = int(os.environ.get("SPLITQ", 48))
CLINK = int(os.environ.get("CLINK", 1))
KA = int(os.environ.get("KA", 7))
KB = int(os.environ.get("KB", 8))
PAR = int(os.environ.get("PAR", 2))
PAR0 = int(os.environ.get("PAR0", 3))
ORDER_A = "s" + "m" * KA + "ss"
KB0 = int(os.environ.get("KB0", 6))
ORDER_B = "s" + "m" * KB0 + "s" + "m" * (KB - KB0) + "s" + "m" * (16 - KB) + "s"
ORDER_C = "s" + "m" * int(os.environ.get("KC", 7)) + "s" + "m" * int(os.environ.get("KC2", 6)) + "s"
ORDER_E = "s" + "m" * int(os.environ.get("KE", 5)) + "s"
f32, bf16, u32 = jnp.float32, jnp.bfloat16, jnp.uint32

_dot = functools.partial(jnp.dot, preferred_element_type=f32)


def _dot_nt(a, b):
    return jax.lax.dot_general(a, b, (((1,), (1,)), ((), ())), preferred_element_type=f32)


def _vcat(*xs):
    return jnp.concatenate(xs, axis=0)


def _pad_rows(r):
    return _vcat(r, jnp.zeros((128 - r.shape[0], r.shape[1]), r.dtype))


def _add(x, y):
    return (x.astype(f32) + y.astype(f32)).astype(bf16)


def _sub(x, y):
    return (x.astype(f32) - y.astype(f32)).astype(bf16)


def _form(coefs, blocks):
    terms = [(c, blk) for c, blk in zip(coefs, blocks) if c != 0]
    if len(terms) == 1 and terms[0][0] == 1:
        return terms[0][1]()
    terms.sort(key=lambda cb: cb[0] < 0)
    out = None
    for c, blk in terms:
        v = blk().astype(f32)
        if out is None:
            out = v if c == 1 else v * c
        else:
            v = v if abs(c) == 1 else v * abs(c)
            out = out + v if c > 0 else out - v
    return out


def _lhs_slots(x1, x2):
    out = []
    for halves in SLOTS:
        for grp, coefs, _ in halves:
            k1, k2 = GROUP_ROWS[grp]
            blocks = [lambda x=x, k=k: x[k:k + 64] for x in (x1, x2) for k in (k1, k2)]
            out.append(_form(coefs, blocks))
    return out


def _lhs_slots_lanes(x1, x2):
    low = jax.lax.broadcasted_iota(jnp.int32, x1[0].shape, 1) < 64
    out = []
    for halves in SLOTS:
        keys = [(tuple(k // 128 for k in GROUP_ROWS[grp]), coefs) for grp, coefs, _ in halves]
        vals = [_form(coefs, [lambda x=x, g=g: x[g] for x in (x1, x2) for g in tiles])
                for tiles, coefs in keys]
        out.append(vals[0] if keys[0] == keys[1] else jnp.where(low, vals[0], vals[1]))
    return out


def _fast_product(p):
    p0, p1, p2, p3 = p(0), p(1), p(2), p(3)
    r = p0 + p1 + p2
    c11 = r + p1 + p3
    c12 = r + p2
    yield None
    p0, p1, p2, p3 = p(4), p(5), p(6), p(7)
    r = p0 + p1 + p2
    c21 = r + p1
    c22 = p3 - (r + p2)
    yield None
    p0, p1, p2, p3 = p(8), p(9), p(10), p(11)
    r = p0 + p1
    c11 = c11 + (r + p3)
    c21 = c21 + (r + p1 + p2)
    c22 = c22 + p3
    yield None
    p0, p1, p2, p3 = p(12), p(13), p(14), p(15)
    r = p0 + p1
    c12 = (r + p2 + p3) - c12
    c22 = c22 + (r + p1)
    c21 = c21 + p3
    yield (c11, c12, c21, c22)


def _rhs_slot(s, get, anchors=()):
    parts = []
    for grp, _, coefs in SLOTS[s]:
        k1, k2 = GROUP_ROWS[grp]
        blocks = [lambda k=k, c=c: get(slice(k, k + 64), c) for k in (k1, k2) for c in (0, 1)]
        parts.append(_form(coefs, blocks).astype(f32))
    while anchors:
        parts[0] = _vcat(parts[0][:8] + anchors.pop(), parts[0][8:])
    return _vcat(*parts).astype(bf16)


def _packed(ref, *idx):
    return pltpu.bitcast(ref.bitcast(u32)[idx], bf16)


def _layernorm_t(x, zero=None, total=None):
    rows = [x[r:r + 8] for r in range(0, D, 8)]
    s = total
    if s is None:
        s = functools.reduce(jnp.add, rows[1:], rows[0] if zero is None else rows[0] + zero)
    m = jnp.sum(s, axis=0, keepdims=True) * (1.0 / D)
    rows = [r - m for r in rows]
    s = rows[0] * rows[0]
    for r in rows[1:]:
        s = s + r * r
    v = jnp.sum(s, axis=0, keepdims=True) * (1.0 / D)
    return _vcat(*rows) * jax.lax.rsqrt(v + EPS)


def _aligned(x, n):
    return x if isinstance(x, int) else pl.multiple_of(x, n)


def _drain(*gens):
    for gen in gens:
        for _ in gen:
            pass


def _weave(order, main, side):
    for c in order:
        next(main if c == "m" else side)
    _drain(main, side)


def _scope(name):
    import contextlib
    return jax.named_scope(name) if os.environ.get("SCOPES") else contextlib.nullcontext()


def _loop(n, fn):
    def body(i, c):
        with _scope("it"):
            fn(i)
        return c
    jax.lax.fori_loop(0, n, body, 0)


def _kernel(x_hbm, wqkv_hbm, wo_hbm, wg_hbm, wu_hbm, wd_hbm, out_hbm,
            xin, wqkv, wo, wg, wu, wd, wqkv_t, wo_t, wperm, operm, pin, pout, xres,
            q0, k0, v0, q_s, k_s, v_s, a_s, h_s, acc, xn_s, sems):
    groups = (range(5), range(5, NCH))
    lane = jax.lax.broadcasted_iota(jnp.int32, (8, 128), 1)
    anchors = []

    def x_copy(t, piece, n):
        cols = pl.ds(pl.multiple_of(t * TM + piece * n, 128), n)
        return pltpu.make_async_copy(x_hbm.at[:, cols], xin.at[:, cols], sems.at[10 + t + piece])

    def wqkv_copy(g):
        rows = pl.ds(g * 128, min(128, D - g * 128))
        return pltpu.make_async_copy(wqkv_hbm.at[rows], wqkv.at[rows], sems.at[15 + g])

    def out_copy(t, half):
        cols = pl.ds(t * TM + half * HM, HM)
        return pltpu.make_async_copy(xin.at[:, cols], out_hbm.at[:, cols], sems.at[2 * t + half])

    def ffn_copies(g):
        return [pltpu.make_async_copy(src.at[:, pl.ds(j * FC, FC)], dst.at[j], sems.at[20 + 3 * j + i])
                for j in groups[g]
                for i, (src, dst) in enumerate(((wg_hbm, wg), (wu_hbm, wu), (wd_hbm, wd)))]

    cwo = pltpu.make_async_copy(wo_hbm, wo, sems.at[3])
    x_copy(0, 0, TM).start()
    for g in range(5):
        wqkv_copy(g).start()

    def head_rows(ref, g, base):
        return _vcat(*[ref[g, pl.ds(base + d, 8, stride=DH), :] for d in range(DH)])

    def prep_wqkv():
        for gs in ((0, 1), (2, 3), (4,)):
            with _scope("w_qkv"):
                for g in gs:
                    wqkv_copy(g).wait()
            for g in gs:
                rows = wqkv[g * 128:min((g + 1) * 128, D), :].astype(f32)
                wperm[g] = (_vcat(rows, rows) if g == 4 else rows).T

        def rows_of(hg):
            base = pl.multiple_of(hg * GR, 16)
            x1 = [head_rows(wperm, g, base) for g in range(5)]
            x2 = [head_rows(wperm, g, base + HQ) for g in range(5)]
            for n, v in enumerate(_lhs_slots_lanes(x1, x2)):
                wqkv_t[n, pl.ds(base, GR), :] = v.astype(bf16)
        _loop(HQ // GR, rows_of)

    def prep_wo():
        for g in range(5):
            cols = wo[:, g * 128:min((g + 1) * 128, D)].astype(f32)
            if g == 4:
                cols = jnp.concatenate([cols, jnp.zeros_like(cols)], axis=1)
            operm[g] = cols
        parts = []
        for g in range(5):
            r = _vcat(*[head_rows(operm, g, hg * GR) for hg in range(NG)])
            rt = _vcat(r, r[512:D]).astype(bf16).T
            parts.append(rt[:64] if g == 4 else rt)
        wt = _vcat(*parts).astype(f32)
        x1 = [wt[0:HD, g * 128:(g + 1) * 128] for g in range(5)]
        x2 = [wt[HD:D, g * 128:(g + 1) * 128] for g in range(5)]
        for n, v in enumerate(_lhs_slots_lanes(x1, x2)):
            wo_t[n] = v.astype(bf16)

    def to_words(x):
        tiles = [x[g * 128:(g + 1) * 128] for g in range(4)] + [_pad_rows(x[512:D])]
        return [pltpu.bitcast(r.astype(bf16).T, u32) for r in tiles]

    def from_words(words):
        parts = [pltpu.bitcast(w, bf16).T for w in words]
        return _vcat(*parts[:4], parts[4][:64])

    def in_t1(t, c):
        x = xin[:, pl.ds(pl.multiple_of(t * TM + c * 128, 128), 128)]
        for g, w in enumerate(to_words(x)):
            pin[t, g, pl.ds(pl.multiple_of(c * 64, 64), 64), :] = w

    def in_t2(t, j):
        return from_words([pin[t, g, pl.ds(j, 64, stride=8), :] for g in range(5)]).astype(f32)

    def out_t1(t, j, x):
        words = to_words(x)
        for g, w in enumerate(words):
            pout[t, g, pl.ds(_aligned(j * 72, 8), 64), :] = w
        return [w[56:64] for w in words]

    def out_t2(t, c):
        words = [_vcat(*[pout[t, g, pl.ds(c * 8 + m, 8, stride=72), :] for m in range(8)])
                 for g in range(5)]
        x = from_words(words)
        xin[:, pl.ds(_aligned(t * TM + c * 128, 128), 128)] = x
        return [pltpu.bitcast(x[r - 16:r], u32) for r in (128, 256, 384, 512, D)]

    def combine(t, i, never=None):
        c, second = i % 2, i // 2
        pick = lambda lo, hi: lo + (hi - lo) * second
        outer = lambda m1, m2, m3, m4, m5, m6, m7: (
            m1 + m4 - m5 + m7, m2 + m4, m3 + m5, m1 - m2 + m3 + m6)
        strips, sums, link = [], [], None
        for r in range(0, QD, 8):
            get = lambda n, m: acc[t, c, m, n * QD + r:n * QD + r + 8, :]
            four, two = [], []
            for n in range(7):
                x = get(n, pick(3, 2))
                if link is not None and n % CLINK == 0:
                    x = x + jnp.where(never, link, 0.0)
                four.append(((get(n, 0) + x) + get(n, pick(6, 5))) - get(n, pick(4, 1)))
                two.append(get(n, pick(1, 4)) + x)
                if never is not None:
                    link = four[-1]
            rows = []
            for u, v in zip(outer(*four), outer(*two)):
                if isinstance(second, int):
                    rows += [v, u] if second else [u, v]
                else:
                    rows += [jnp.where(second > 0, v, u), jnp.where(second > 0, u, v)]
            strips.append([xres[t, i + 4 * (q // 4), (q % 4) * QD + r:(q % 4) * QD + r + 8, :] + v
                           for q, v in enumerate(rows)])
            if never is not None:
                sums = [functools.reduce(jnp.add, sums[n:n + 1] + strips[-1][4 * n:4 * n + 4]) for n in (0, 1)]
                link = sums[0] + sums[1]
        return [_vcat(*[s[q] for q in range(q0, q0 + 4) for s in strips]) for q0 in (0, 4)] + sums

    def store_qkv(t, b, part, q, k, v, prev=None):
        q[b] = part[0:D].reshape(NG, DH, 8, 128)
        for n, (dst, r) in enumerate(((k, part[D:2 * D]), (v, part[2 * D:3 * D]))):
            dst[b + NB] = r.reshape(NG, DH, 8, 128)
            sh = pltpu.roll(r, 2, 1).reshape(NG, DH, 8, 128)
            if isinstance(t, int) and t == 0:
                dst[b] = sh
            elif prev is not None:
                dst[b] = jnp.where((lane < 2)[None, None], prev[n][b], sh)
            else:
                keep = jnp.broadcast_to((lane >= 2 * t)[None, None], sh.shape)
                pltpu.store(dst.at[b], sh, mask=keep)

    def phase1(t, i):
        never = lane < (i < 0).astype(jnp.int32)
        x1, x2, s1, s2 = combine(t, i, never)
        xres[t, i] = x1
        xres[t, i + 4] = x2
        n1 = _layernorm_t(x1, total=s1)
        n2 = _layernorm_t(x2, total=s2 + jnp.where(never, n1[0:8], 0.0))
        yield
        rhs = lambda s: _rhs_slot(s, lambda rows, c: (n1, n2)[c][rows])
        for c in _fast_product(lambda s: _dot(_packed(wqkv_t, s), rhs(s))):
            pass
        yield
        store_qkv(t, i, _vcat(c[0], c[2]), q_s, k_s, v_s)
        store_qkv(t, i + 4, _vcat(c[1], c[3]), q_s, k_s, v_s)
        yield

    def first_norm(t, i, link=None):
        ns = []
        for b in (i, i + 4):
            x = in_t2(t, b)
            xres[t, b] = x
            ns.append(_layernorm_t(x, None if link is None else link[0]))
            if link is not None:
                link[0] = jnp.where(link[1], ns[-1][0:8], 0.0)
        for s in range(NSLOT):
            xn_s[t, i, s] = _rhs_slot(s, lambda rows, c: ns[c][rows])

    def first_qkv(t, i):
        cs = []
        for r0 in (0, HQ // 4):
            rows = slice(r0, r0 + HQ // 4)
            for c in _fast_product(lambda s: _dot(_packed(wqkv_t, s, rows), _packed(xn_s, t, i, s))):
                yield
            cs.append(c)
        for n, b in enumerate((i, i + 4)):
            part = _vcat(cs[0][n], cs[1][n], cs[0][n + 2], cs[1][n + 2])
            if t == 0:
                store_qkv(t, b, part, q0, k0, v0)
            else:
                store_qkv(t, b, part, q_s, k_s, v_s, prev=(k0, v0))

    def attention_group(t, b, g, q_r, k_r, v_r, links):
        par = len(links)
        never = lane < (b < 0).astype(jnp.int32)

        def start(n, v):
            if links[n % par] is None:
                return v
            return jnp.where(never, links[n % par], 0.0) + v

        q = [q_r[b, g, d] for d in range(DH)]
        logits = []
        for w in range(W):
            l = start(w, q[0] * k_r[b + NB - w, g, 0])
            for d in range(1, DH):
                l = l + q[d] * k_r[b + NB - w, g, d]
            links[w % par] = l
            l = l * (DH ** -0.5)
            if w > 0:
                edge = jnp.where(jnp.logical_and(w > b, t == 0), 2, 0)
                l = jnp.where(lane < edge, -1e9, l)
            logits.append(l)
        m = functools.reduce(jnp.maximum, logits)
        e = [jnp.exp(l - m) for l in logits]
        r = 1.0 / functools.reduce(jnp.add, e)
        p = [x * r for x in e]
        outs = []
        for d in range(DH):
            o = p[0] * v_r[b + NB, g, d]
            if d >= par:
                o = start(d, o)
            for w in range(1, W):
                o = o + p[w] * v_r[b + NB - w, g, d]
            links[d % par] = o
            outs.append(o)
        return _vcat(*outs)

    def phase2(t, i, par, q_r, k_r, v_r):
        links = [None] * par
        halves = [_vcat(*[attention_group(t, b, g, q_r, k_r, v_r, links) for g in range(NG)])
                  for b in (i, i + 4)]
        yield
        if q_r is q_s:
            anchors.append(jnp.where(lane < (i < 0).astype(jnp.int32), functools.reduce(jnp.add, links), 0.0))
            yield
        rhs = lambda s: _rhs_slot(s, lambda rows, c: halves[c][rows])
        for c in _fast_product(lambda s: _dot(_packed(wo_t, s), rhs(s))):
            pass
        x1 = xres[t, i] + _vcat(c[0], c[2])
        x2 = xres[t, i + 4] + _vcat(c[1], c[3])
        xres[t, i] = x1
        xres[t, i + 4] = x2
        n1 = _layernorm_t(x1)
        n2 = _layernorm_t(x2, jnp.where(lane < (i < 0).astype(jnp.int32), n1[0:8], 0.0) if q_r is q_s else None)
        yield
        ops = _lhs_slots(n1, n2)
        rows = pl.ds(pl.multiple_of(i * 64, 64), 64)
        for s in range(NSLOT):
            op = _vcat(ops[2 * s], ops[2 * s + 1]).astype(bf16).T
            a_s[t, s, rows, :] = pltpu.bitcast(op, u32)
        yield

    def anchor(never, words):
        anchors.append(jnp.where(never, pltpu.bitcast(functools.reduce(jnp.bitwise_or, words), f32), 0.0))

    def proj(t, w_ref, off, res, side):
        cols = [pl.ds(off + c * HC, 128) for c in (0, 1)]

        def p(s):
            x = a_s[t, s]
            zero = next(side, None)
            if zero is not None:
                r = 32 + 64 * (s % 4)
                x = _vcat(x[:r], x[r:r + 8] | zero, x[r + 8:])
            return _dot(pltpu.bitcast(x, bf16), _rhs_slot(s, lambda rows, c: w_ref[rows, cols[c]], anchors))
        for c in _fast_product(p):
            yield
        res.extend(c)

    def ffn_chunk(t, j, may_init=False):
        side = iter(())
        lhs = {}
        for k2 in (0, 1):
            g, u = [], []
            yield from proj(t, wg.at[j], k2 * 128, g, side)
            yield from proj(t, wu.at[j], k2 * 128, u, side)
            b11, b21, b12, b22 = [x * y for x, y in zip(g, u)]
            for n, (_, lb) in enumerate(STRASSEN):
                h_s[n, k2] = _form(lb, [lambda x=x: x for x in (b11, b12, b21, b22)])
        order = [(n, m) for n in range(7) for m in (1, 5)] + [(n, m) for n in range(7) for m in (0, 2, 3, 4, 6)]
        for q, (n, m) in enumerate(order):
            rhs = [lambda k2=k2, c2=c2: h_s[n, k2, c2 * 256:(c2 + 1) * 256, :] for k2 in (0, 1) for c2 in (0, 1)]
            if q == 14:
                lhs.clear()
            if n not in lhs:
                lhs[n] = [_form(STRASSEN[n][0],
                                [lambda r=r, k=k, r2=r2, k2=k2: wd[j, pl.ds((2 * r + r2) * QD, QD),
                                                                   pl.ds((2 * k + k2) * 128, 128)]
                                 for r in (0, 1) for k in (0, 1)])
                          for r2 in (0, 1) for k2 in (0, 1)]
            left = _form(STRASSEN[m][0], [lambda x=x: x for x in lhs[n]])
            right = _form(STRASSEN[m][1], rhs).astype(bf16)
            if q == SPLITQ:
                v = _vcat(_dot_nt(left[:80].astype(bf16), right), _dot_nt(left[80:].astype(bf16), right))
            else:
                v = _dot_nt(left.astype(bf16), right)
            for c in range(2):
                old = acc[t, c, m, n * QD:(n + 1) * QD, :]
                if may_init:
                    old = jnp.where(j > 0, old, 0.0)
                acc[t, c, m, n * QD:(n + 1) * QD, :] = old + v[:, c * 128:(c + 1) * 128]
            if q % 7 == 6:
                yield

    with _scope("w_x0"):
        x_copy(0, 0, TM).wait()
    x_copy(1, 0, TM).start()
    cwo.start()
    for c in range(NB):
        in_t1(0, c)
    first_norm(0, 0)
    prep_wqkv()
    with _scope("w_x1"):
        x_copy(1, 0, TM).wait()
    for g in range(len(groups)):
        for c in ffn_copies(g):
            c.start()
    for c in range(NB):
        in_t1(1, c)

    def body_f(i, last):
        _drain(first_qkv(0, i))
        link = [None, lane < (i < 0).astype(jnp.int32)]
        first_norm(1, i, link)
        if last:
            prep_wo()
        else:
            first_norm(0, i + 1, link)

    _loop(3, lambda i: body_f(i, False))
    cwo.wait()
    _loop(1, lambda i: body_f(i + 3, True))
    _loop(4, lambda i: _weave(ORDER_E, first_qkv(1, i), phase2(0, i, PAR0, q0, k0, v0)))

    def wait_group(k, g):
        @pl.when(k == 0)
        def _():
            for c in ffn_copies(g):
                c.wait()

    def finish_step(i):
        u = i % 4
        never = lane < (i < 0).astype(jnp.int32)
        x1, x2 = combine(0, u, never)[:2]
        done = out_t1(0, u, x1) + out_t1(0, u + 4, x2)
        yield
        anchor(never, done)
        done = out_t2(0, 2 * u) + out_t2(0, 2 * u + 1)
        yield
        anchor(never, done)
        yield

    def stage(k):
        t = k % 2
        n_a = jnp.where(jnp.logical_and(k > 0, k < 3), 4, 0)
        n_b = jnp.where(k < 3, 4, 0)
        n_c = NCH - n_a - n_b
        wait_group(k, 0)
        _loop(n_c, lambda i: _weave(ORDER_C, ffn_chunk(t, i, True), finish_step(i)))
        _loop(n_a, lambda i: _weave(ORDER_A, ffn_chunk(t, n_c + i), phase1(1 - t, i)))
        wait_group(k, 1)
        _loop(n_b, lambda i: _weave(ORDER_B, ffn_chunk(t, n_c + n_a + i),
                                    phase2(1 - t, i, PAR, q_s, k_s, v_s)))
    _loop(4, stage)

    for half in range(2):
        out_copy(0, half).start()
    for i in range(4):
        x1, x2 = combine(1, i)
        out_t1(1, i, x1)
        out_t1(1, i + 4, x2)
    for c in range(NB):
        out_t2(1, c)
        if c % 4 == 3:
            out_copy(1, c // 4).start()
    with _scope("w_out"):
        for t in range(2):
            for half in range(2):
                out_copy(t, half).wait()


@jax.jit
def pallas_interleave_layers__sliding_local_dilated__glu_gated_bilinear__prompt_kernel(
    A_x: jax.Array,
    A_wqkv: jax.Array,
    A_wo: jax.Array,
    B_x: jax.Array,
    B_w_gate: jax.Array,
    B_w_up: jax.Array,
    B_w_down: jax.Array,
):
    any_spec = pl.BlockSpec(memory_space=pl.ANY)
    qkv_scratch = [
        pltpu.VMEM((NB, NG, DH, 8, 128), f32),
        pltpu.VMEM((2 * NB, NG, DH, 8, 128), f32),
        pltpu.VMEM((2 * NB, NG, DH, 8, 128), f32),
    ]
    out_t = pl.pallas_call(
        _kernel,
        in_specs=[any_spec] * 6,
        out_specs=any_spec,
        out_shape=jax.ShapeDtypeStruct((D, S), bf16),
        scratch_shapes=[
            pltpu.VMEM((D, S), bf16),
            pltpu.VMEM((D, 3 * D), bf16),
            pltpu.VMEM((D, D), bf16),
            pltpu.VMEM((NCH, D, FC), bf16),
            pltpu.VMEM((NCH, D, FC), bf16),
            pltpu.VMEM((NCH, D, FC), bf16),
            pltpu.VMEM((NSLOT, HQ, 128), bf16),
            pltpu.VMEM((NSLOT, HD, 128), bf16),
            pltpu.VMEM((5, 3 * D, 128), f32),
            pltpu.VMEM((5, D, 128), f32),
            pltpu.VMEM((2, 5, HM, 128), u32),
            pltpu.VMEM((2, 5, 8 * 72, 128), u32),
            pltpu.VMEM((2, NB, D, 128), f32),
            *qkv_scratch,
            *qkv_scratch,
            pltpu.VMEM((2, NSLOT, HM // 2, 128), u32),
            pltpu.VMEM((7, 2, HM, 128), f32),
            pltpu.VMEM((2, 2, 7, 1024, 128), f32),
            pltpu.VMEM((2, 4, NSLOT, 128, 128), bf16),
            pltpu.SemaphoreType.DMA((20 + 3 * NCH,)),
        ],
        compiler_params=pltpu.CompilerParams(vmem_limit_bytes=120 * 1024 * 1024),
        name="fused_layers",
    )(A_x[0].T, A_wqkv, A_wo, B_w_gate, B_w_up, B_w_down.T)
    return out_t.T[None]
```

```python
import functools
import os

import jax
import jax.numpy as jnp
import jax.experimental.pallas as pl
import jax.experimental.pallas.tpu as pltpu

S, D, F = 2048, 576, 4608
H, DH, W = 32, 18, 8
NG = H // 8
GR = 8 * DH
NB = 8
TM = NB * 128
HM = TM // 2
HD = D // 2
HQ = 3 * D // 2
FC = 512
HC = FC // 2
NCH = F // FC
NSLOT = 16
NT = int(os.environ.get("NT", 128))

GROUP_ROWS = {1: (0, 128), 2: (64, 192), 4: (256, 384), 3: (320, 448), 0: (512, 512)}
T3 = 1.0 / 3.0
SLOTS = (
    ((1, (-1, -1, 0, 0), (0, 0, 0, 1)), (3, (1, 1, 0, 0), (0, 0, 1, 0))),
    ((0, (T3, 0, 0, 0), (2, 1, 0, 0)), (2, (-.5, -1, 0, 0), (0, 0, 0, 1))),
    ((4, (.5, 1, 0, 0), (0, 0, 1, 0)), (0, (-T3, 0, 0, 0), (1, 2, 0, 0))),
    ((1, (0, 1, 0, -1), (0, 0, 1, 1)), (2, (0, 2, 0, -1), (0, 0, .5, 1))),
    ((1, (0, 0, 1, 1), (1, 0, 0, 0)), (3, (0, 0, -1, -1), (0, 1, 0, 0))),
    ((0, (0, 0, T3, 0), (2, 1, 0, 0)), (2, (0, 0, .5, 1), (1, 0, 0, 0))),
    ((4, (0, 0, -.5, -1), (0, 1, 0, 0)), (0, (0, 0, -T3, 0), (1, 2, 0, 0))),
    ((1, (-1, 0, 1, 0), (1, 1, 0, 0)), (2, (-1, 0, .5, 0), (1, 2, 0, 0))),
    ((1, (0, 0, 0, 1), (-1, 0, 1, 0)), (3, (1, 0, 0, 0), (1, 0, -1, 0))),
    ((4, (.5, 0, 0, 0), (2, 0, -1, 0)), (2, (0, 0, 0, 1), (-1, 0, .5, 0))),
    ((4, (-1, 0, .5, 0), (2, 1, 0, 0)), (3, (-1, 0, 1, 0), (1, 1, 0, 0))),
    ((1, (1, 0, 0, 1), (1, 0, 0, 1)), (2, (1, 0, 0, 1), (1, 0, 0, 1))),
    ((1, (1, 0, 0, 0), (0, 1, 0, -1)), (3, (0, 0, 0, 1), (0, -1, 0, 1))),
    ((4, (0, 0, 0, 1), (0, -1, 0, .5)), (2, (.5, 0, 0, 0), (0, 2, 0, -1))),
    ((4, (0, 2, 0, -1), (0, 0, 1, .5)), (3, (0, 1, 0, -1), (0, 0, 1, 1))),
    ((4, (1, 0, 0, 1), (0, 1, 1, 0)), (3, (1, 0, 0, 1), (0, 1, 1, 0))),
)
_PASSES = (
    ("+01 +10", "-04 +14 +17", "-41 -43 +70 +71 +73", "-05 +15 +16", "-51 +60 +61 +62"),
    ("+10", "-04 +14", "+40 +41 -42 +43 -70 -71 -73", "-05 +15", "+50 +51 -52 -60 -61 -62"),
    ("+02 -03", "+00 -02", "+21 +23", "+01 -03", "+31 +33"),
    ("+00 -02 +03", "+00 +08", "+81 +83", "+01 +06", "-53 +63"),
    ("+01 +02 -03", "+02 -08", "+21", "+03 -07", "+31"),
    ("+00 -01", "+06", "+60 +62", "+07", "+70"),
    ("+10 -12 +13", "+10 +18", "+00", "+11 +16", "+10"),
    ("+12 -13", "+10 -12", "+00 +02", "+11 -13", "+10 +12"),
    ("-11 -12 +13", "+12 -18", "+80 +82", "+13 -17", "+72"),
    ("+10 +12", "-12 +14", "+42", "-13 +15", "+52"),
    ("-00 +02 +13", "+00 +18", "-00 +81 +83", "+01 +16", "-10 -53 +63"),
    ("+00 -02", "+06 -16", "+53 -62 -63", "+08 -18", "+80 -81 -83"),
    ("+00 +02", "+02 -04", "+20", "+03 -05", "+30"),
    ("+02", "+02 -12", "-20 +22 +23", "+03 -13", "-30 +32 +33"),
    ("+11 -13", "-08 +18", "-80 +81 -82", "-07 +17", "+43 -72 -73"),
    ("+02 -11 +13", "+08 -12", "+21 +80 +82", "+07 -13", "+31 +72"),
    ("+02 +13", "+00 -12", "+00 +02 -21 -23", "+01 -13", "+10 +12 -31 -33"),
    ("+10 -11", "+16", "+51 -61", "+17", "+41 +43 -71 -73"),
    ("+02 +12", "+12", "+00 +02 +22 +42 +80 +82", "+13", "+10 +12 +32 +52 +72"),
    ("+00 +10", "+04", "+20 +40", "+05", "+30 +50"),
    ("-00 +02 -10 +12", "+16", "+10 +62", "+18", "+00 -80"),
    ("+02 -10", "+04 -12", "+20 +42", "+05 -13", "+30 +52"),
    ("+03 +13", "+00", "+03 +21 +23 -43 -81 -83", "+01", "+13 +31 +33 -63"),
    ("+13", "-00 +10", "+01 +02 +03", "-01 +11", "+11 +12 +13"),
    ("-01 +03", "+00 +04 +07", "+43", "+01 +05 +06", "+53"),
    ("+01", "+04 +07 -14 -17", "+70 +71 +73", "+05 +06 -15 -16", "+53 +60 +61 +62"),
    ("+01 +11", "+14 +17", "-01 +41", "+15 +16", "-11 +51"),
    ("+11 -13", "+10 +14 +17", "+01", "+11 +15 +16", "+11"),
    ("+01 +13", "+00 +14 +17", "+01 +43", "+01 +15 +16", "+11 +53"),
    ("+01 -03 +11 -13", "+08", "+21 +81", "+07", "+31 +43 -73"),
)
PASSES = [[[(int(w[0] + "1"), int(w[1]), int(w[2])) for w in col.split()] for col in row] for row in _PASSES]
NPASS = len(PASSES)
STRASSEN = (
    ((1, 0, 0, 1), (1, 0, 0, 1)),
    ((0, 0, 1, 1), (1, 0, 0, 0)),
    ((1, 0, 0, 0), (0, 1, 0, -1)),
    ((0, 0, 0, 1), (-1, 0, 1, 0)),
    ((1, 1, 0, 0), (0, 0, 0, 1)),
    ((-1, 0, 1, 0), (1, 1, 0, 0)),
    ((0, 1, 0, -1), (0, 0, 1, 1)),
)
QD = D // 4
EPS = 1e-5
SPLITQ = int(os.environ.get("SPLITQ", 48))
CLINK = int(os.environ.get("CLINK", 1))
KA = int(os.environ.get("KA", 7))
KB = int(os.environ.get("KB", 8))
PAR = int(os.environ.get("PAR", 2))
PAR0 = int(os.environ.get("PAR0", 3))
ORDER_A = "s" + "m" * KA + "ss"
KB0 = int(os.environ.get("KB0", 6))
ORDER_B = "s" + "m" * KB0 + "s" + "m" * (KB - KB0) + "s" + "m" * (15 - KB) + "s"
ORDER_C = "s" + "m" * int(os.environ.get("KC", 7)) + "s" + "m" * int(os.environ.get("KC2", 6)) + "s"
ORDER_E = "s" + "m" * int(os.environ.get("KE", 5)) + "s"
f32, bf16, u32 = jnp.float32, jnp.bfloat16, jnp.uint32

_dot = functools.partial(jnp.dot, preferred_element_type=f32)


def _dot_nt(a, b):
    return jax.lax.dot_general(a, b, (((1,), (1,)), ((), ())), preferred_element_type=f32)


def _vcat(*xs):
    return jnp.concatenate(xs, axis=0)


def _pad_rows(r):
    return _vcat(r, jnp.zeros((128 - r.shape[0], r.shape[1]), r.dtype))


def _add(x, y):
    return (x.astype(f32) + y.astype(f32)).astype(bf16)


def _sub(x, y):
    return (x.astype(f32) - y.astype(f32)).astype(bf16)


def _form(coefs, blocks):
    terms = [(c, blk) for c, blk in zip(coefs, blocks) if c != 0]
    if len(terms) == 1 and terms[0][0] == 1:
        return terms[0][1]()
    terms.sort(key=lambda cb: cb[0] < 0)
    out = None
    for c, blk in terms:
        v = blk().astype(f32)
        if out is None:
            out = v if c == 1 else v * c
        else:
            v = v if abs(c) == 1 else v * abs(c)
            out = out + v if c > 0 else out - v
    return out


def _lhs_slots(x1, x2):
    out = []
    for halves in SLOTS:
        for grp, coefs, _ in halves:
            k1, k2 = GROUP_ROWS[grp]
            blocks = [lambda x=x, k=k: x[k:k + 64] for x in (x1, x2) for k in (k1, k2)]
            out.append(_form(coefs, blocks))
    return out


def _lhs_slots_lanes(x1, x2):
    low = jax.lax.broadcasted_iota(jnp.int32, x1[0].shape, 1) < 64
    out = []
    for halves in SLOTS:
        keys = [(tuple(k // 128 for k in GROUP_ROWS[grp]), coefs) for grp, coefs, _ in halves]
        vals = [_form(coefs, [lambda x=x, g=g: x[g] for x in (x1, x2) for g in tiles])
                for tiles, coefs in keys]
        out.append(vals[0] if keys[0] == keys[1] else jnp.where(low, vals[0], vals[1]))
    return out


def _fast_product(p):
    p0, p1, p2, p3 = p(0), p(1), p(2), p(3)
    r = p0 + p1 + p2
    c11 = r + p1 + p3
    c12 = r + p2
    yield None
    p0, p1, p2, p3 = p(4), p(5), p(6), p(7)
    r = p0 + p1 + p2
    c21 = r + p1
    c22 = p3 - (r + p2)
    yield None
    p0, p1, p2, p3 = p(8), p(9), p(10), p(11)
    r = p0 + p1
    c11 = c11 + (r + p3)
    c21 = c21 + (r + p1 + p2)
    c22 = c22 + p3
    yield None
    p0, p1, p2, p3 = p(12), p(13), p(14), p(15)
    r = p0 + p1
    c12 = (r + p2 + p3) - c12
    c22 = c22 + (r + p1)
    c21 = c21 + p3
    yield (c11, c12, c21, c22)


def _rhs_slot(s, get, anchors=()):
    parts = []
    for grp, _, coefs in SLOTS[s]:
        k1, k2 = GROUP_ROWS[grp]
        blocks = [lambda k=k, c=c: get(slice(k, k + 64), c) for k in (k1, k2) for c in (0, 1)]
        parts.append(_form(coefs, blocks).astype(f32))
    while anchors:
        parts[0] = _vcat(parts[0][:8] + anchors.pop(), parts[0][8:])
    return _vcat(*parts).astype(bf16)


def _signed(terms, get):
    return _form([t[0] for t in terms], [functools.partial(get, t[1], t[2]) for t in terms])


def _feed(outs, prods):
    vals = dict(prods)
    sums = {}
    for s in prods:
        for sign, i, n in PASSES[s][0]:
            sums.setdefault((i, n), {})[s] = sign
    while True:
        pairs = {}
        for terms in sums.values():
            keys = list(terms)
            for x in range(len(keys)):
                for y in range(x):
                    key = (keys[y], keys[x], terms[keys[x]] * terms[keys[y]])
                    pairs[key] = pairs.get(key, 0) + 1
        if not pairs or max(pairs.values()) < 2:
            break
        x, y, rel = max(pairs, key=pairs.get)
        vals[x, y] = vals[x] + vals[y] if rel > 0 else vals[x] - vals[y]
        for terms in sums.values():
            if x in terms and y in terms and terms[x] * terms[y] == rel:
                terms[x, y] = terms.pop(x)
                del terms[y]
    for blk, terms in sums.items():
        items = [(sign, vals[k]) for k, sign in terms.items()]
        sign, v = items[0]
        for s2, w in items[1:] + ([outs[blk]] if blk in outs else []):
            v = v + w if s2 == sign else v - w
        outs[blk] = (sign, v)


def _packed(ref, *idx):
    return pltpu.bitcast(ref.bitcast(u32)[idx], bf16)


def _layernorm_t(x, zero=None, total=None):
    rows = [x[r:r + 8] for r in range(0, D, 8)]
    s = total
    if s is None:
        s = functools.reduce(jnp.add, rows[1:], rows[0] if zero is None else rows[0] + zero)
    m = jnp.sum(s, axis=0, keepdims=True) * (1.0 / D)
    rows = [r - m for r in rows]
    s = rows[0] * rows[0]
    for r in rows[1:]:
        s = s + r * r
    v = jnp.sum(s, axis=0, keepdims=True) * (1.0 / D)
    return _vcat(*rows) * jax.lax.rsqrt(v + EPS)


def _norm_stats(ref, total):
    m = jnp.broadcast_to(jnp.sum(total, axis=0, keepdims=True) * (1.0 / D), (8, 128))
    s = None
    for r in range(0, D, 8):
        c = ref[r:r + 8, :] - m
        s = c * c if s is None else s + c * c
    v = jnp.sum(s, axis=0, keepdims=True) * (1.0 / D)
    return m[0:1], jax.lax.rsqrt(v + EPS)


def _tile_sum(x, zero=None):
    rows = [x[r:r + 8] for r in range(0, D, 8)]
    return functools.reduce(jnp.add, rows[1:], rows[0] if zero is None else rows[0] + zero)


def _aligned(x, n):
    return x if isinstance(x, int) else pl.multiple_of(x, n)


def _drain(*gens):
    for gen in gens:
        for _ in gen:
            pass


def _weave(order, main, side):
    for c in order:
        next(main if c == "m" else side)
    _drain(main, side)


def _scope(name):
    import contextlib
    return jax.named_scope(name) if os.environ.get("SCOPES") else contextlib.nullcontext()


def _loop(n, fn):
    def body(i, c):
        with _scope("it"):
            fn(i)
        return c
    jax.lax.fori_loop(0, n, body, 0)


def _kernel(x_hbm, wqkv_hbm, wo_hbm, wg_hbm, wu_hbm, wd_hbm, out_hbm,
            xin, wqkv, wo, wg, wu, wd, wqkv_t, wo_t, wperm, operm, pin, pout, xres,
            q0, k0, v0, q_s, k_s, v_s, a_s, h_s, acc, xn_s, sems):
    groups = (range(5), range(5, NCH))
    lane = jax.lax.broadcasted_iota(jnp.int32, (8, 128), 1)
    anchors = []

    def x_copy(t, piece, n):
        cols = pl.ds(pl.multiple_of(t * TM + piece * n, 128), n)
        return pltpu.make_async_copy(x_hbm.at[:, cols], xin.at[:, cols], sems.at[10 + t + piece])

    def wqkv_copy(g):
        rows = pl.ds(g * 128, min(128, D - g * 128))
        return pltpu.make_async_copy(wqkv_hbm.at[rows], wqkv.at[rows], sems.at[15 + g])

    def out_copy(t, half):
        cols = pl.ds(t * TM + half * HM, HM)
        return pltpu.make_async_copy(xin.at[:, cols], out_hbm.at[:, cols], sems.at[2 * t + half])

    def ffn_copies(g):
        return [pltpu.make_async_copy(src.at[:, pl.ds(j * FC, FC)], dst.at[j], sems.at[20 + 3 * j + i])
                for j in groups[g]
                for i, (src, dst) in enumerate(((wg_hbm, wg), (wu_hbm, wu), (wd_hbm, wd)))]

    cwo = pltpu.make_async_copy(wo_hbm, wo, sems.at[3])
    x_copy(0, 0, TM).start()
    for g in range(5):
        wqkv_copy(g).start()

    def head_rows(ref, g, base):
        return _vcat(*[ref[g, pl.ds(base + d, 8, stride=DH), :] for d in range(DH)])

    def prep_wqkv():
        for gs in ((0, 1), (2, 3), (4,)):
            with _scope("w_qkv"):
                for g in gs:
                    wqkv_copy(g).wait()
            for g in gs:
                rows = wqkv[g * 128:min((g + 1) * 128, D), :].astype(f32)
                wperm[g] = (_vcat(rows, rows) if g == 4 else rows).T

        def rows_of(hg):
            base = pl.multiple_of(hg * GR, 16)
            x1 = [head_rows(wperm, g, base) for g in range(5)]
            x2 = [head_rows(wperm, g, base + HQ) for g in range(5)]
            for n, v in enumerate(_lhs_slots_lanes(x1, x2)):
                wqkv_t[n, pl.ds(base, GR), :] = v.astype(bf16)
        _loop(HQ // GR, rows_of)

    def prep_wo():
        for g in range(5):
            cols = wo[:, g * 128:min((g + 1) * 128, D)].astype(f32)
            if g == 4:
                cols = jnp.concatenate([cols, jnp.zeros_like(cols)], axis=1)
            operm[g] = cols
        parts = []
        for g in range(5):
            r = _vcat(*[head_rows(operm, g, hg * GR) for hg in range(NG)])
            rt = _vcat(r, r[512:D]).astype(bf16).T
            parts.append(rt[:64] if g == 4 else rt)
        wt = _vcat(*parts).astype(f32)
        x1 = [wt[0:HD, g * 128:(g + 1) * 128] for g in range(5)]
        x2 = [wt[HD:D, g * 128:(g + 1) * 128] for g in range(5)]
        for n, v in enumerate(_lhs_slots_lanes(x1, x2)):
            wo_t[n] = v.astype(bf16)

    def to_words(x):
        tiles = [x[g * 128:(g + 1) * 128] for g in range(4)] + [_pad_rows(x[512:D])]
        return [pltpu.bitcast(r.astype(bf16).T, u32) for r in tiles]

    def from_words(words):
        parts = [pltpu.bitcast(w, bf16).T for w in words]
        return _vcat(*parts[:4], parts[4][:64])

    def in_t1(t, c):
        x = xin[:, pl.ds(pl.multiple_of(t * TM + c * 128, 128), 128)]
        for g, w in enumerate(to_words(x)):
            pin[t, g, pl.ds(pl.multiple_of(c * 64, 64), 64), :] = w

    def in_t2(t, j):
        return from_words([pin[t, g, pl.ds(j, 64, stride=8), :] for g in range(5)]).astype(f32)

    def out_t1(t, j, x):
        words = to_words(x)
        for g, w in enumerate(words):
            pout[t, g, pl.ds(_aligned(j * 72, 8), 64), :] = w
        return [w[56:64] for w in words]

    def out_t2(t, c):
        words = [_vcat(*[pout[t, g, pl.ds(c * 8 + m, 8, stride=72), :] for m in range(8)])
                 for g in range(5)]
        x = from_words(words)
        xin[:, pl.ds(_aligned(t * TM + c * 128, 128), 128)] = x
        return [pltpu.bitcast(x[r - 16:r], u32) for r in (128, 256, 384, 512, D)]

    def combine(t, i, never=None):
        c, second = i % 2, i // 2
        pick = lambda lo, hi: lo + (hi - lo) * second
        outer = lambda m1, m2, m3, m4, m5, m6, m7: (
            m1 + m4 - m5 + m7, m2 + m4, m3 + m5, m1 - m2 + m3 + m6)
        strips, sums, link = [], [], None
        for r in range(0, QD, 8):
            get = lambda n, m: acc[t, c, m, n * QD + r:n * QD + r + 8, :]
            four, two = [], []
            for n in range(7):
                x = get(n, pick(3, 2))
                if link is not None and n % CLINK == 0:
                    x = x + jnp.where(never, link, 0.0)
                four.append(((get(n, 0) + x) + get(n, pick(6, 5))) - get(n, pick(4, 1)))
                two.append(get(n, pick(1, 4)) + x)
                if never is not None:
                    link = four[-1]
            rows = []
            for u, v in zip(outer(*four), outer(*two)):
                if isinstance(second, int):
                    rows += [v, u] if second else [u, v]
                else:
                    rows += [jnp.where(second > 0, v, u), jnp.where(second > 0, u, v)]
            strips.append([xres[t, i + 4 * (q // 4), (q % 4) * QD + r:(q % 4) * QD + r + 8, :] + v
                           for q, v in enumerate(rows)])
            if never is not None:
                sums = [functools.reduce(jnp.add, sums[n:n + 1] + strips[-1][4 * n:4 * n + 4]) for n in (0, 1)]
                link = sums[0] + sums[1]
        return [_vcat(*[s[q] for q in range(q0, q0 + 4) for s in strips]) for q0 in (0, 4)] + sums

    def store_qkv(t, b, part, q, k, v, prev=None):
        q[b] = part[0:D].reshape(NG, DH, 8, 128)
        for n, (dst, r) in enumerate(((k, part[D:2 * D]), (v, part[2 * D:3 * D]))):
            dst[b + NB] = r.reshape(NG, DH, 8, 128)
            sh = pltpu.roll(r, 2, 1).reshape(NG, DH, 8, 128)
            if isinstance(t, int) and t == 0:
                dst[b] = sh
            elif prev is not None:
                dst[b] = jnp.where((lane < 2)[None, None], prev[n][b], sh)
            else:
                keep = jnp.broadcast_to((lane >= 2 * t)[None, None], sh.shape)
                pltpu.store(dst.at[b], sh, mask=keep)

    def phase1(t, i):
        never = lane < (i < 0).astype(jnp.int32)
        x1, x2, s1, s2 = combine(t, i, never)
        xres[t, i] = x1
        xres[t, i + 4] = x2
        n1 = _layernorm_t(x1, total=s1)
        n2 = _layernorm_t(x2, total=s2 + jnp.where(never, n1[0:8], 0.0))
        yield
        rhs = lambda s: _rhs_slot(s, lambda rows, c: (n1, n2)[c][rows])
        for c in _fast_product(lambda s: _dot(_packed(wqkv_t, s), rhs(s))):
            pass
        yield
        store_qkv(t, i, _vcat(c[0], c[2]), q_s, k_s, v_s)
        store_qkv(t, i + 4, _vcat(c[1], c[3]), q_s, k_s, v_s)
        yield

    def first_norm(t, i, link=None):
        stats = []
        for b in (i, i + 4):
            x = in_t2(t, b)
            xres[t, b] = x
            stats.append(_norm_stats(xres.at[t, b], _tile_sum(x, None if link is None else link[0])))
            if link is not None:
                link[0] = jnp.where(link[1], stats[-1][1], 0.0)
        get = lambda rows, c: (xres[t, i + 4 * c, rows, :] - stats[c][0]) * stats[c][1]
        for s in range(NSLOT):
            xn_s[t, i, s] = _rhs_slot(s, get)

    def first_qkv(t, i):
        cs = []
        for r0 in ((HQ // 4, 0) if t == 0 else (0, HQ // 4)):
            rows = slice(r0, r0 + HQ // 4)
            for c in _fast_product(lambda s: _dot(_packed(wqkv_t, s, rows), _packed(xn_s, t, i, s))):
                yield
            cs.append(c)
        for n, b in enumerate((i, i + 4)):
            part = _vcat(cs[1 - t][n], cs[t][n], cs[1 - t][n + 2], cs[t][n + 2])
            if t == 0:
                store_qkv(t, b, part, q0, k0, v0)
            else:
                store_qkv(t, b, part, q_s, k_s, v_s, prev=(k0, v0))

    def attention_group(t, b, g, q_r, k_r, v_r, links):
        par = len(links)
        never = lane < (b < 0).astype(jnp.int32)

        def start(n, v):
            if links[n % par] is None:
                return v
            return jnp.where(never, links[n % par], 0.0) + v

        q = [q_r[b, g, d] for d in range(DH)]
        logits = []
        for w in range(W):
            l = start(w, q[0] * k_r[b + NB - w, g, 0])
            for d in range(1, DH):
                l = l + q[d] * k_r[b + NB - w, g, d]
            links[w % par] = l
            l = l * (DH ** -0.5)
            if w > 0:
                edge = jnp.where(jnp.logical_and(w > b, t == 0), 2, 0)
                l = jnp.where(lane < edge, -1e9, l)
            logits.append(l)
        m = functools.reduce(jnp.maximum, logits)
        e = [jnp.exp(l - m) for l in logits]
        r = 1.0 / functools.reduce(jnp.add, e)
        p = [x * r for x in e]
        outs = []
        for d in range(DH):
            o = p[0] * v_r[b + NB, g, d]
            if d >= par:
                o = start(d, o)
            for w in range(1, W):
                o = o + p[w] * v_r[b + NB - w, g, d]
            links[d % par] = o
            outs.append(o)
        return _vcat(*outs)

    def phase2(t, i, par, q_r, k_r, v_r):
        links = [None] * par
        halves = [_vcat(*[attention_group(t, b, g, q_r, k_r, v_r, links) for g in range(NG)])
                  for b in (i, i + 4)]
        yield
        if q_r is q_s:
            anchors.append(jnp.where(lane < (i < 0).astype(jnp.int32), functools.reduce(jnp.add, links), 0.0))
            yield
        rhs = lambda s: _rhs_slot(s, lambda rows, c: halves[c][rows])
        for c in _fast_product(lambda s: _dot(_packed(wo_t, s), rhs(s))):
            pass
        x1 = xres[t, i] + _vcat(c[0], c[2])
        x2 = xres[t, i + 4] + _vcat(c[1], c[3])
        xres[t, i] = x1
        xres[t, i + 4] = x2
        n1 = _layernorm_t(x1)
        n2 = _layernorm_t(x2, jnp.where(lane < (i < 0).astype(jnp.int32), n1[0:8], 0.0) if q_r is q_s else None)
        yield
        rows = pl.ds(pl.multiple_of(i * 64, 64), 64)
        for s, (_, lo, _, hi, _) in enumerate(PASSES):
            op = _vcat(*[_signed(x, lambda r, k: (n1, n2)[r][64 * k:64 * k + 64]) for x in (lo, hi)])
            a_s[t, s, rows, :] = pltpu.bitcast(op.astype(bf16).T, u32)
        yield

    def anchor(never, words):
        anchors.append(jnp.where(never, pltpu.bitcast(functools.reduce(jnp.bitwise_or, words), f32), 0.0))

    def ffn_pass(t, w_ref, s):
        get = lambda k, n: w_ref[64 * k:64 * k + 64, 128 * n:128 * n + 128]
        parts = [_signed(x, get).astype(f32) for x in PASSES[s][2::2]]
        while anchors:
            parts[0] = _vcat(parts[0][:8] + anchors.pop(), parts[0][8:])
        return _dot(pltpu.bitcast(a_s[t, s], bf16), _vcat(*parts).astype(bf16))

    def ffn_chunk(t, j, may_init=False):
        lhs, g, u = {}, {}, {}
        todo = [(g, wg, s) for s in list(range(2, NPASS)) + [0, 1]] + [(u, wu, s) for s in range(NPASS)]
        for q in range(0, 2 * NPASS, 4):
            prods = [(outs, s, ffn_pass(t, w.at[j], s)) for outs, w, s in todo[q:q + 4]]
            for outs in (g, u):
                _feed(outs, {s: v for o, s, v in prods if o is outs})
            if q in (2 * NPASS - 12, 2 * NPASS - 4):
                k2 = q // (2 * NPASS - 4)
                blks = [(i, 2 * k + k2) for k in (0, 1) for i in (0, 1)]
                hs = [g[b][1] * u[b][1] for b in blks]
                for n, (_, lb) in enumerate(STRASSEN):
                    coefs = [c * g[b][0] * u[b][0] for c, b in zip(lb, blks)]
                    h_s[n, k2] = _form(coefs, [lambda x=x: x for x in hs])
            yield
        order = [(n, m) for n in range(7) for m in (1, 5)] + [(n, m) for n in range(7) for m in (0, 2, 3, 4, 6)]
        for q, (n, m) in enumerate(order):
            rhs = [lambda k2=k2, c2=c2: h_s[n, k2, c2 * 256:(c2 + 1) * 256, :] for k2 in (0, 1) for c2 in (0, 1)]
            if q == 14:
                lhs.clear()
            if n not in lhs:
                lhs[n] = [_form(STRASSEN[n][0],
                                [lambda r=r, k=k, r2=r2, k2=k2: wd[j, pl.ds((2 * r + r2) * QD, QD),
                                                                   pl.ds((2 * k + k2) * 128, 128)]
                                 for r in (0, 1) for k in (0, 1)])
                          for r2 in (0, 1) for k2 in (0, 1)]
            left = _form(STRASSEN[m][0], [lambda x=x: x for x in lhs[n]])
            right = _form(STRASSEN[m][1], rhs).astype(bf16)
            if q == SPLITQ:
                v = _vcat(_dot_nt(left[:80].astype(bf16), right), _dot_nt(left[80:].astype(bf16), right))
            else:
                v = _dot_nt(left.astype(bf16), right)
            for c in range(2):
                old = acc[t, c, m, n * QD:(n + 1) * QD, :]
                if may_init:
                    old = jnp.where(j > 0, old, 0.0)
                acc[t, c, m, n * QD:(n + 1) * QD, :] = old + v[:, c * 128:(c + 1) * 128]
            if q % 7 == 6:
                yield

    with _scope("w_x0"):
        x_copy(0, 0, TM).wait()
    x_copy(1, 0, TM).start()
    cwo.start()
    for c in range(NB):
        in_t1(0, c)
    first_norm(0, 0)
    prep_wqkv()
    with _scope("w_x1"):
        x_copy(1, 0, TM).wait()
    for g in range(len(groups)):
        for c in ffn_copies(g):
            c.start()
    for c in range(NB):
        in_t1(1, c)

    def body_f(i, last):
        _drain(first_qkv(0, i))
        link = [None, lane < (i < 0).astype(jnp.int32)]
        first_norm(1, i, link)
        if last:
            prep_wo()
        else:
            first_norm(0, i + 1, link)

    _loop(3, lambda i: body_f(i, False))
    cwo.wait()
    _loop(1, lambda i: body_f(i + 3, True))
    _loop(4, lambda i: _weave(ORDER_E, first_qkv(1, i), phase2(0, i, PAR0, q0, k0, v0)))

    def wait_group(k, g):
        @pl.when(k == 0)
        def _():
            for c in ffn_copies(g):
                c.wait()

    def finish_step(i):
        u = i % 4
        never = lane < (i < 0).astype(jnp.int32)
        x1, x2 = combine(0, u, never)[:2]
        done = out_t1(0, u, x1) + out_t1(0, u + 4, x2)
        yield
        anchor(never, done)
        done = out_t2(0, 2 * u) + out_t2(0, 2 * u + 1)
        yield
        anchor(never, done)
        yield

    def stage(k):
        t = k % 2
        n_a = jnp.where(jnp.logical_and(k > 0, k < 3), 4, 0)
        n_b = jnp.where(k < 3, 4, 0)
        n_c = NCH - n_a - n_b
        wait_group(k, 0)
        _loop(n_c, lambda i: _weave(ORDER_C, ffn_chunk(t, i, True), finish_step(i)))
        _loop(n_a, lambda i: _weave(ORDER_A, ffn_chunk(t, n_c + i), phase1(1 - t, i)))
        wait_group(k, 1)
        _loop(n_b, lambda i: _weave(ORDER_B, ffn_chunk(t, n_c + n_a + i),
                                    phase2(1 - t, i, PAR, q_s, k_s, v_s)))
    _loop(4, stage)

    for half in range(2):
        out_copy(0, half).start()
    for i in range(4):
        x1, x2 = combine(1, i)
        out_t1(1, i, x1)
        out_t1(1, i + 4, x2)
    for c in range(NB):
        out_t2(1, c)
        if c % 4 == 3:
            out_copy(1, c // 4).start()
    with _scope("w_out"):
        for t in range(2):
            for half in range(2):
                out_copy(t, half).wait()


@jax.jit
def pallas_interleave_layers__sliding_local_dilated__glu_gated_bilinear__prompt_kernel(
    A_x: jax.Array,
    A_wqkv: jax.Array,
    A_wo: jax.Array,
    B_x: jax.Array,
    B_w_gate: jax.Array,
    B_w_up: jax.Array,
    B_w_down: jax.Array,
):
    any_spec = pl.BlockSpec(memory_space=pl.ANY)
    qkv_scratch = [
        pltpu.VMEM((NB, NG, DH, 8, 128), f32),
        pltpu.VMEM((2 * NB, NG, DH, 8, 128), f32),
        pltpu.VMEM((2 * NB, NG, DH, 8, 128), f32),
    ]
    out_t = pl.pallas_call(
        _kernel,
        in_specs=[any_spec] * 6,
        out_specs=any_spec,
        out_shape=jax.ShapeDtypeStruct((D, S), bf16),
        scratch_shapes=[
            pltpu.VMEM((D, S), bf16),
            pltpu.VMEM((D, 3 * D), bf16),
            pltpu.VMEM((D, D), bf16),
            pltpu.VMEM((NCH, D, FC), bf16),
            pltpu.VMEM((NCH, D, FC), bf16),
            pltpu.VMEM((NCH, D, FC), bf16),
            pltpu.VMEM((NSLOT, HQ, 128), bf16),
            pltpu.VMEM((NSLOT, HD, 128), bf16),
            pltpu.VMEM((5, 3 * D, 128), f32),
            pltpu.VMEM((5, D, 128), f32),
            pltpu.VMEM((2, 5, HM, 128), u32),
            pltpu.VMEM((2, 5, 8 * 72, 128), u32),
            pltpu.VMEM((2, NB, D, 128), f32),
            *qkv_scratch,
            *qkv_scratch,
            pltpu.VMEM((2, NPASS, HM // 2, 128), u32),
            pltpu.VMEM((7, 2, HM, 128), f32),
            pltpu.VMEM((2, 2, 7, 1024, 128), f32),
            pltpu.VMEM((2, 4, NSLOT, 128, 128), bf16),
            pltpu.SemaphoreType.DMA((20 + 3 * NCH,)),
        ],
        compiler_params=pltpu.CompilerParams(vmem_limit_bytes=120 * 1024 * 1024),
        name="fused_layers",
    )(A_x[0].T, A_wqkv, A_wo, B_w_gate, B_w_up, B_w_down.T)
    return out_t.T[None]
```

```python
import functools
import os

import jax
import jax.numpy as jnp
import jax.experimental.pallas as pl
import jax.experimental.pallas.tpu as pltpu

S, D, F = 2048, 576, 4608
H, DH, W = 32, 18, 8
NG = H // 8
GR = 8 * DH
NB = 8
TM = NB * 128
HM = TM // 2
HD = D // 2
HQ = 3 * D // 2
FC = 512
HC = FC // 2
NCH = F // FC
NSLOT = 16
NT = int(os.environ.get("NT", 128))

GROUP_ROWS = {1: (0, 128), 2: (64, 192), 4: (256, 384), 3: (320, 448), 0: (512, 512)}
T3 = 1.0 / 3.0
SLOTS = (
    ((1, (-1, -1, 0, 0), (0, 0, 0, 1)), (3, (1, 1, 0, 0), (0, 0, 1, 0))),
    ((0, (T3, 0, 0, 0), (2, 1, 0, 0)), (2, (-.5, -1, 0, 0), (0, 0, 0, 1))),
    ((4, (.5, 1, 0, 0), (0, 0, 1, 0)), (0, (-T3, 0, 0, 0), (1, 2, 0, 0))),
    ((1, (0, 1, 0, -1), (0, 0, 1, 1)), (2, (0, 2, 0, -1), (0, 0, .5, 1))),
    ((1, (0, 0, 1, 1), (1, 0, 0, 0)), (3, (0, 0, -1, -1), (0, 1, 0, 0))),
    ((0, (0, 0, T3, 0), (2, 1, 0, 0)), (2, (0, 0, .5, 1), (1, 0, 0, 0))),
    ((4, (0, 0, -.5, -1), (0, 1, 0, 0)), (0, (0, 0, -T3, 0), (1, 2, 0, 0))),
    ((1, (-1, 0, 1, 0), (1, 1, 0, 0)), (2, (-1, 0, .5, 0), (1, 2, 0, 0))),
    ((1, (0, 0, 0, 1), (-1, 0, 1, 0)), (3, (1, 0, 0, 0), (1, 0, -1, 0))),
    ((4, (.5, 0, 0, 0), (2, 0, -1, 0)), (2, (0, 0, 0, 1), (-1, 0, .5, 0))),
    ((4, (-1, 0, .5, 0), (2, 1, 0, 0)), (3, (-1, 0, 1, 0), (1, 1, 0, 0))),
    ((1, (1, 0, 0, 1), (1, 0, 0, 1)), (2, (1, 0, 0, 1), (1, 0, 0, 1))),
    ((1, (1, 0, 0, 0), (0, 1, 0, -1)), (3, (0, 0, 0, 1), (0, -1, 0, 1))),
    ((4, (0, 0, 0, 1), (0, -1, 0, .5)), (2, (.5, 0, 0, 0), (0, 2, 0, -1))),
    ((4, (0, 2, 0, -1), (0, 0, 1, .5)), (3, (0, 1, 0, -1), (0, 0, 1, 1))),
    ((4, (1, 0, 0, 1), (0, 1, 1, 0)), (3, (1, 0, 0, 1), (0, 1, 1, 0))),
)
_PASSES = (
    ("+01 +10", "-04 +14 +17", "-41 -43 +70 +71 +73", "-05 +15 +16", "-51 +60 +61 +62"),
    ("+10", "-04 +14", "+40 +41 -42 +43 -70 -71 -73", "-05 +15", "+50 +51 -52 -60 -61 -62"),
    ("+02 -03", "+00 -02", "+21 +23", "+01 -03", "+31 +33"),
    ("+00 -02 +03", "+00 +08", "+81 +83", "+01 +06", "-53 +63"),
    ("+01 +02 -03", "+02 -08", "+21", "+03 -07", "+31"),
    ("+00 -01", "+06", "+60 +62", "+07", "+70"),
    ("+10 -12 +13", "+10 +18", "+00", "+11 +16", "+10"),
    ("+12 -13", "+10 -12", "+00 +02", "+11 -13", "+10 +12"),
    ("-11 -12 +13", "+12 -18", "+80 +82", "+13 -17", "+72"),
    ("+10 +12", "-12 +14", "+42", "-13 +15", "+52"),
    ("-00 +02 +13", "+00 +18", "-00 +81 +83", "+01 +16", "-10 -53 +63"),
    ("+00 -02", "+06 -16", "+53 -62 -63", "+08 -18", "+80 -81 -83"),
    ("+00 +02", "+02 -04", "+20", "+03 -05", "+30"),
    ("+02", "+02 -12", "-20 +22 +23", "+03 -13", "-30 +32 +33"),
    ("+11 -13", "-08 +18", "-80 +81 -82", "-07 +17", "+43 -72 -73"),
    ("+02 -11 +13", "+08 -12", "+21 +80 +82", "+07 -13", "+31 +72"),
    ("+02 +13", "+00 -12", "+00 +02 -21 -23", "+01 -13", "+10 +12 -31 -33"),
    ("+10 -11", "+16", "+51 -61", "+17", "+41 +43 -71 -73"),
    ("+02 +12", "+12", "+00 +02 +22 +42 +80 +82", "+13", "+10 +12 +32 +52 +72"),
    ("+00 +10", "+04", "+20 +40", "+05", "+30 +50"),
    ("-00 +02 -10 +12", "+16", "+10 +62", "+18", "+00 -80"),
    ("+02 -10", "+04 -12", "+20 +42", "+05 -13", "+30 +52"),
    ("+03 +13", "+00", "+03 +21 +23 -43 -81 -83", "+01", "+13 +31 +33 -63"),
    ("+13", "-00 +10", "+01 +02 +03", "-01 +11", "+11 +12 +13"),
    ("-01 +03", "+00 +04 +07", "+43", "+01 +05 +06", "+53"),
    ("+01", "+04 +07 -14 -17", "+70 +71 +73", "+05 +06 -15 -16", "+53 +60 +61 +62"),
    ("+01 +11", "+14 +17", "-01 +41", "+15 +16", "-11 +51"),
    ("+11 -13", "+10 +14 +17", "+01", "+11 +15 +16", "+11"),
    ("+01 +13", "+00 +14 +17", "+01 +43", "+01 +15 +16", "+11 +53"),
    ("+01 -03 +11 -13", "+08", "+21 +81", "+07", "+31 +43 -73"),
)
PASSES = [[[(int(w[0] + "1"), int(w[1]), int(w[2])) for w in col.split()] for col in row] for row in _PASSES]
NPASS = len(PASSES)
STRASSEN = (
    ((1, 0, 0, 1), (1, 0, 0, 1)),
    ((0, 0, 1, 1), (1, 0, 0, 0)),
    ((1, 0, 0, 0), (0, 1, 0, -1)),
    ((0, 0, 0, 1), (-1, 0, 1, 0)),
    ((1, 1, 0, 0), (0, 0, 0, 1)),
    ((-1, 0, 1, 0), (1, 1, 0, 0)),
    ((0, 1, 0, -1), (0, 0, 1, 1)),
)
QD = D // 4
EPS = 1e-5
SPLITQ = int(os.environ.get("SPLITQ", 48))
CLINK = int(os.environ.get("CLINK", 1))
KA = int(os.environ.get("KA", 11))
KB = int(os.environ.get("KB", 9))
PAR = int(os.environ.get("PAR", 2))
PAR0 = int(os.environ.get("PAR0", 3))
ORDER_A = "s" + "m" * KA + "ss"
KB0 = int(os.environ.get("KB0", 1))
ORDER_B = "m" * KB0 + "sm" * 8 + "m" * (KB - KB0 - 8) + "s" + "m" * (15 - KB + int(os.environ.get("KB2", 6))) + "ms" * NPASS
ORDER_C = "s" + "m" * int(os.environ.get("KC", 6)) + "s" + "m" * int(os.environ.get("KC2", 4)) + "s"
ORDER_E = "s" + "m" * int(os.environ.get("KE", 5)) + "s"
f32, bf16, u32 = jnp.float32, jnp.bfloat16, jnp.uint32

_dot = functools.partial(jnp.dot, preferred_element_type=f32)


def _dot_nt(a, b):
    return jax.lax.dot_general(a, b, (((1,), (1,)), ((), ())), preferred_element_type=f32)


def _vcat(*xs):
    return jnp.concatenate(xs, axis=0)


def _pad_rows(r):
    return _vcat(r, jnp.zeros((128 - r.shape[0], r.shape[1]), r.dtype))


def _add(x, y):
    return (x.astype(f32) + y.astype(f32)).astype(bf16)


def _sub(x, y):
    return (x.astype(f32) - y.astype(f32)).astype(bf16)


def _form(coefs, blocks):
    terms = [(c, blk) for c, blk in zip(coefs, blocks) if c != 0]
    if len(terms) == 1 and terms[0][0] == 1:
        return terms[0][1]()
    terms.sort(key=lambda cb: cb[0] < 0)
    out = None
    for c, blk in terms:
        v = blk().astype(f32)
        if out is None:
            out = v if c == 1 else v * c
        else:
            v = v if abs(c) == 1 else v * abs(c)
            out = out + v if c > 0 else out - v
    return out


def _lhs_slots(x1, x2):
    out = []
    for halves in SLOTS:
        for grp, coefs, _ in halves:
            k1, k2 = GROUP_ROWS[grp]
            blocks = [lambda x=x, k=k: x[k:k + 64] for x in (x1, x2) for k in (k1, k2)]
            out.append(_form(coefs, blocks))
    return out


def _lhs_slots_lanes(x1, x2):
    low = jax.lax.broadcasted_iota(jnp.int32, x1[0].shape, 1) < 64
    out = []
    for halves in SLOTS:
        keys = [(tuple(k // 128 for k in GROUP_ROWS[grp]), coefs) for grp, coefs, _ in halves]
        vals = [_form(coefs, [lambda x=x, g=g: x[g] for x in (x1, x2) for g in tiles])
                for tiles, coefs in keys]
        out.append(vals[0] if keys[0] == keys[1] else jnp.where(low, vals[0], vals[1]))
    return out


def _fast_product(p):
    p0, p1, p2, p3 = p(0), p(1), p(2), p(3)
    r = p0 + p1 + p2
    c11 = r + p1 + p3
    c12 = r + p2
    yield None
    p0, p1, p2, p3 = p(4), p(5), p(6), p(7)
    r = p0 + p1 + p2
    c21 = r + p1
    c22 = p3 - (r + p2)
    yield None
    p0, p1, p2, p3 = p(8), p(9), p(10), p(11)
    r = p0 + p1
    c11 = c11 + (r + p3)
    c21 = c21 + (r + p1 + p2)
    c22 = c22 + p3
    yield None
    p0, p1, p2, p3 = p(12), p(13), p(14), p(15)
    r = p0 + p1
    c12 = (r + p2 + p3) - c12
    c22 = c22 + (r + p1)
    c21 = c21 + p3
    yield (c11, c12, c21, c22)


def _rhs_slot(s, get, anchors=()):
    parts = []
    for grp, _, coefs in SLOTS[s]:
        k1, k2 = GROUP_ROWS[grp]
        blocks = [lambda k=k, c=c: get(slice(k, k + 64), c) for k in (k1, k2) for c in (0, 1)]
        parts.append(_form(coefs, blocks).astype(f32))
    while anchors:
        parts[0] = _vcat(parts[0][:8] + anchors.pop(), parts[0][8:])
    return _vcat(*parts).astype(bf16)


def _signed(terms, get):
    return _form([t[0] for t in terms], [functools.partial(get, t[1], t[2]) for t in terms])


def _feed(outs, prods, ref, keep=()):
    vals = dict(prods)
    sums = {}
    for s in prods:
        for sign, i, n in PASSES[s][0]:
            sums.setdefault((i, n), {})[s] = sign
    while True:
        pairs = {}
        for terms in sums.values():
            keys = list(terms)
            for x in range(len(keys)):
                for y in range(x):
                    key = (keys[y], keys[x], terms[keys[x]] * terms[keys[y]])
                    pairs[key] = pairs.get(key, 0) + 1
        if not pairs or max(pairs.values()) < 2:
            break
        x, y, rel = max(pairs, key=pairs.get)
        vals[x, y] = vals[x] + vals[y] if rel > 0 else vals[x] - vals[y]
        for terms in sums.values():
            if x in terms and y in terms and terms[x] * terms[y] == rel:
                terms[x, y] = terms.pop(x)
                del terms[y]
    for blk, terms in sums.items():
        items = [(sign, vals[k]) for k, sign in terms.items()]
        sign, v = items[0]
        for s2, w in items[1:] + ([(outs[blk][0], ref[blk])] if blk in outs else []):
            v = v + w if s2 == sign else v - w
        outs[blk] = (sign, v)
        if blk not in keep:
            ref[blk] = v


def _packed(ref, *idx):
    return pltpu.bitcast(ref.bitcast(u32)[idx], bf16)


def _norm_stats(ref, total):
    m = jnp.broadcast_to(jnp.sum(total, axis=0, keepdims=True) * (1.0 / D), (8, 128))
    s = None
    for r in range(0, D, 8):
        c = ref[r:r + 8, :] - m
        s = c * c if s is None else s + c * c
    v = jnp.sum(s, axis=0, keepdims=True) * (1.0 / D)
    return m[0:1], jax.lax.rsqrt(v + EPS)


def _tile_sum(x, zero=None):
    rows = [x[r:r + 8] for r in range(0, D, 8)]
    return functools.reduce(jnp.add, rows[1:], rows[0] if zero is None else rows[0] + zero)


def _aligned(x, n):
    return x if isinstance(x, int) else pl.multiple_of(x, n)


def _drain(*gens):
    for gen in gens:
        for _ in gen:
            pass


def _weave(order, main, side):
    for c in order:
        next(main if c == "m" else side)
    _drain(main, side)


def _scope(name):
    import contextlib
    return jax.named_scope(name) if os.environ.get("SCOPES") else contextlib.nullcontext()


def _loop(n, fn):
    def body(i, c):
        with _scope("it"):
            fn(i)
        return c
    jax.lax.fori_loop(0, n, body, 0)


def _kernel(x_hbm, wqkv_hbm, wo_hbm, wg_hbm, wu_hbm, wd_hbm, out_hbm,
            xin, wqkv, wo, wg, wu, wd, wqkv_t, wo_t, wperm, operm, pin, pout, xres,
            q0, k0, v0, q_s, k_s, v_s, o_s, n_s, a_s, gu_s, h_s, acc, xn_s, sems):
    groups = (range(5), range(5, NCH))
    lane = jax.lax.broadcasted_iota(jnp.int32, (8, 128), 1)
    anchors, ticks = [], []

    def x_copy(t, piece, n):
        cols = pl.ds(pl.multiple_of(t * TM + piece * n, 128), n)
        return pltpu.make_async_copy(x_hbm.at[:, cols], xin.at[:, cols], sems.at[10 + t + piece])

    def wqkv_copy(g):
        rows = pl.ds(g * 128, min(128, D - g * 128))
        return pltpu.make_async_copy(wqkv_hbm.at[rows], wqkv.at[rows], sems.at[15 + g])

    def out_copy(t, half):
        cols = pl.ds(t * TM + half * HM, HM)
        return pltpu.make_async_copy(xin.at[:, cols], out_hbm.at[:, cols], sems.at[2 * t + half])

    def ffn_copies(g):
        return [pltpu.make_async_copy(src.at[:, pl.ds(j * FC, FC)], dst.at[j], sems.at[20 + 3 * j + i])
                for j in groups[g]
                for i, (src, dst) in enumerate(((wg_hbm, wg), (wu_hbm, wu), (wd_hbm, wd)))]

    cwo = pltpu.make_async_copy(wo_hbm, wo, sems.at[3])
    x_copy(0, 0, TM).start()
    for g in range(5):
        wqkv_copy(g).start()

    def head_rows(ref, g, base):
        return _vcat(*[ref[g, pl.ds(base + d, 8, stride=DH), :] for d in range(DH)])

    def prep_wqkv():
        for gs in ((0, 1), (2, 3), (4,)):
            with _scope("w_qkv"):
                for g in gs:
                    wqkv_copy(g).wait()
            for g in gs:
                rows = wqkv[g * 128:min((g + 1) * 128, D), :].astype(f32)
                wperm[g] = (_vcat(rows, rows) if g == 4 else rows).T

        def rows_of(hg):
            base = pl.multiple_of(hg * GR, 16)
            x1 = [head_rows(wperm, g, base) for g in range(5)]
            x2 = [head_rows(wperm, g, base + HQ) for g in range(5)]
            for n, v in enumerate(_lhs_slots_lanes(x1, x2)):
                wqkv_t[n, pl.ds(base, GR), :] = v.astype(bf16)
        _loop(HQ // GR, rows_of)

    def prep_wo():
        for g in range(5):
            cols = wo[:, g * 128:min((g + 1) * 128, D)].astype(f32)
            if g == 4:
                cols = jnp.concatenate([cols, jnp.zeros_like(cols)], axis=1)
            operm[g] = cols
        parts = []
        for g in range(5):
            r = _vcat(*[head_rows(operm, g, hg * GR) for hg in range(NG)])
            rt = _vcat(r, r[512:D]).astype(bf16).T
            parts.append(rt[:64] if g == 4 else rt)
        wt = _vcat(*parts).astype(f32)
        x1 = [wt[0:HD, g * 128:(g + 1) * 128] for g in range(5)]
        x2 = [wt[HD:D, g * 128:(g + 1) * 128] for g in range(5)]
        for n, v in enumerate(_lhs_slots_lanes(x1, x2)):
            wo_t[n] = v.astype(bf16)

    def to_words(x):
        tiles = [x[g * 128:(g + 1) * 128] for g in range(4)] + [_pad_rows(x[512:D])]
        return [pltpu.bitcast(r.astype(bf16).T, u32) for r in tiles]

    def from_words(words):
        parts = [pltpu.bitcast(w, bf16).T for w in words]
        return _vcat(*parts[:4], parts[4][:64])

    def in_t1(t, c):
        x = xin[:, pl.ds(pl.multiple_of(t * TM + c * 128, 128), 128)]
        for g, w in enumerate(to_words(x)):
            pin[t, g, pl.ds(pl.multiple_of(c * 64, 64), 64), :] = w

    def in_t2(t, j):
        return from_words([pin[t, g, pl.ds(j, 64, stride=8), :] for g in range(5)]).astype(f32)

    def out_t1(t, j, x):
        words = to_words(x)
        for g, w in enumerate(words):
            pout[t, g, pl.ds(_aligned(j * 72, 8), 64), :] = w
        return [w[56:64] for w in words]

    def out_t2(t, c):
        words = [_vcat(*[pout[t, g, pl.ds(c * 8 + m, 8, stride=72), :] for m in range(8)])
                 for g in range(5)]
        x = from_words(words)
        xin[:, pl.ds(_aligned(t * TM + c * 128, 128), 128)] = x
        return [pltpu.bitcast(x[r - 16:r], u32) for r in (128, 256, 384, 512, D)]

    def combine(t, i, never=None):
        c, second = i % 2, i // 2
        pick = lambda lo, hi: lo + (hi - lo) * second
        outer = lambda m1, m2, m3, m4, m5, m6, m7: (
            m1 + m4 - m5 + m7, m2 + m4, m3 + m5, m1 - m2 + m3 + m6)
        strips, sums, link = [], [], None
        for r in range(0, QD, 8):
            get = lambda n, m: acc[t, c, m, n * QD + r:n * QD + r + 8, :]
            four, two = [], []
            for n in range(7):
                x = get(n, pick(3, 2))
                if link is not None and n % CLINK == 0:
                    x = x + jnp.where(never, link, 0.0)
                four.append(((get(n, 0) + x) + get(n, pick(6, 5))) - get(n, pick(4, 1)))
                two.append(get(n, pick(1, 4)) + x)
                if never is not None:
                    link = four[-1]
            rows = []
            for u, v in zip(outer(*four), outer(*two)):
                if isinstance(second, int):
                    rows += [v, u] if second else [u, v]
                else:
                    rows += [jnp.where(second > 0, v, u), jnp.where(second > 0, u, v)]
            strips.append([xres[t, i + 4 * (q // 4), (q % 4) * QD + r:(q % 4) * QD + r + 8, :] + v
                           for q, v in enumerate(rows)])
            if never is not None:
                sums = [functools.reduce(jnp.add, sums[n:n + 1] + strips[-1][4 * n:4 * n + 4]) for n in (0, 1)]
                link = sums[0] + sums[1]
        return [_vcat(*[s[q] for q in range(q0, q0 + 4) for s in strips]) for q0 in (0, 4)] + sums

    def store_qkv(t, b, part, q, k, v, prev=None):
        q[b] = part[0:D].reshape(NG, DH, 8, 128)
        for n, (dst, r) in enumerate(((k, part[D:2 * D]), (v, part[2 * D:3 * D]))):
            dst[b + NB] = r.reshape(NG, DH, 8, 128)
            sh = pltpu.roll(r, 2, 1).reshape(NG, DH, 8, 128)
            if isinstance(t, int) and t == 0:
                dst[b] = sh
            elif prev is not None:
                dst[b] = jnp.where((lane < 2)[None, None], prev[n][b], sh)
            else:
                keep = jnp.broadcast_to((lane >= 2 * t)[None, None], sh.shape)
                pltpu.store(dst.at[b], sh, mask=keep)

    def normalize(t, i, s1, s2, never):
        for c, s in enumerate((s1, s2)):
            if c and never is not None:
                s = s + jnp.where(never, r, 0.0)
            m, r = _norm_stats(xres.at[t, i + 4 * c], s)
            n_s[c] = (xres[t, i + 4 * c] - m) * r

    def phase1(t, i):
        never = lane < (i < 0).astype(jnp.int32)
        x1, x2, s1, s2 = combine(t, i, never)
        xres[t, i] = x1
        xres[t, i + 4] = x2
        normalize(t, i, s1, s2, never)
        yield
        rhs = lambda s: _rhs_slot(s, lambda rows, c: n_s[c, rows, :])
        for c in _fast_product(lambda s: _dot(_packed(wqkv_t, s), rhs(s))):
            pass
        yield
        store_qkv(t, i, _vcat(c[0], c[2]), q_s, k_s, v_s)
        store_qkv(t, i + 4, _vcat(c[1], c[3]), q_s, k_s, v_s)
        yield

    def first_norm(t, i, link=None):
        stats = []
        for b in (i, i + 4):
            x = in_t2(t, b)
            xres[t, b] = x
            stats.append(_norm_stats(xres.at[t, b], _tile_sum(x, None if link is None else link[0])))
            if link is not None:
                link[0] = jnp.where(link[1], stats[-1][1], 0.0)
        get = lambda rows, c: (xres[t, i + 4 * c, rows, :] - stats[c][0]) * stats[c][1]
        for s in range(NSLOT):
            xn_s[t, i, s] = _rhs_slot(s, get)

    def first_qkv(t, i):
        cs = []
        for r0 in ((HQ // 4, 0) if t == 0 else (0, HQ // 4)):
            rows = slice(r0, r0 + HQ // 4)
            for c in _fast_product(lambda s: _dot(_packed(wqkv_t, s, rows), _packed(xn_s, t, i, s))):
                yield
            cs.append(c)
        for n, b in enumerate((i, i + 4)):
            part = _vcat(cs[1 - t][n], cs[t][n], cs[1 - t][n + 2], cs[t][n + 2])
            if t == 0:
                store_qkv(t, b, part, q0, k0, v0)
            else:
                store_qkv(t, b, part, q_s, k_s, v_s, prev=(k0, v0))

    def attention_group(t, b, g, q_r, k_r, v_r, links):
        par = len(links)
        never = lane < (b < 0).astype(jnp.int32)

        def start(n, v):
            if links[n % par] is None:
                return v
            return jnp.where(never, links[n % par], 0.0) + v

        q = [q_r[b, g, d] for d in range(DH)]
        logits = []
        for w in range(W):
            l = start(w, q[0] * k_r[b + NB - w, g, 0])
            for d in range(1, DH):
                l = l + q[d] * k_r[b + NB - w, g, d]
            links[w % par] = l
            l = l * (DH ** -0.5)
            if w > 0:
                edge = jnp.where(jnp.logical_and(w > b, t == 0), 2, 0)
                l = jnp.where(lane < edge, -1e9, l)
            logits.append(l)
        m = functools.reduce(jnp.maximum, logits)
        e = [jnp.exp(l - m) for l in logits]
        r = 1.0 / functools.reduce(jnp.add, e)
        p = [x * r for x in e]
        outs = []
        for d in range(DH):
            o = p[0] * v_r[b + NB, g, d]
            if d >= par:
                o = start(d, o)
            for w in range(1, W):
                o = o + p[w] * v_r[b + NB - w, g, d]
            links[d % par] = o
            outs.append(o)
        return _vcat(*outs)

    def phase2(t, i, par, q_r, k_r, v_r):
        links = [None] * par
        paced = q_r is q_s
        never = lane < (i < 0).astype(jnp.int32)
        for c, b in enumerate((i, i + 4)):
            for g in range(NG):
                o_s[c, g * GR:(g + 1) * GR, :] = attention_group(t, b, g, q_r, k_r, v_r, links)
                if paced:
                    anchors.append(jnp.where(never, functools.reduce(jnp.add, links), 0.0))
                    yield
        if not paced:
            yield
        rhs = lambda s: _rhs_slot(s, lambda rows, c: o_s[c, rows, :])
        for c in _fast_product(lambda s: _dot(_packed(wo_t, s), rhs(s))):
            pass
        x1 = xres[t, i] + _vcat(c[0], c[2])
        x2 = xres[t, i + 4] + _vcat(c[1], c[3])
        xres[t, i] = x1
        xres[t, i + 4] = x2
        normalize(t, i, _tile_sum(x1), _tile_sum(x2), never if paced else None)
        yield
        rows = pl.ds(pl.multiple_of(i * 64, 64), 64)
        for s, (_, lo, _, hi, _) in enumerate(PASSES):
            op = _vcat(*[_signed(x, lambda r, k: n_s[r, 64 * k:64 * k + 64, :]) for x in (lo, hi)])
            if paced:
                op = _vcat(op[:8] + jnp.where(never, ticks[-1], 0.0), op[8:])
            a_s[t, s, rows, :] = pltpu.bitcast(op.astype(bf16).T, u32)
            yield

    def anchor(never, words):
        anchors.append(jnp.where(never, pltpu.bitcast(functools.reduce(jnp.bitwise_or, words), f32), 0.0))

    def ffn_pass(t, w_ref, s):
        get = lambda k, n: w_ref[64 * k:64 * k + 64, 128 * n:128 * n + 128]
        parts = [_signed(x, get).astype(f32) for x in PASSES[s][2::2]]
        while anchors:
            parts[0] = _vcat(parts[0][:8] + anchors.pop(), parts[0][8:])
        return _dot(pltpu.bitcast(a_s[t, s], bf16), _vcat(*parts).astype(bf16))

    def ffn_chunk(t, j, may_init=False):
        lhs, g, u = {}, {}, {}
        todo = [(g, wg, s) for s in list(range(2, NPASS)) + [0, 1]] + [(u, wu, s) for s in range(NPASS)]
        for q in range(0, 2 * NPASS, 4):
            prods = [(outs, s, ffn_pass(t, w.at[j], s)) for outs, w, s in todo[q:q + 4]]
            k2 = {2 * NPASS - 12: 0, 2 * NPASS - 4: 1}.get(q)
            blks = [] if k2 is None else [(i, 2 * k + k2) for k in (0, 1) for i in (0, 1)]
            for n, outs in enumerate((g, u)):
                _feed(outs, {s: v for o, s, v in prods if o is outs}, gu_s.at[n], blks)
            if blks:
                hs = [gu_s[(0,) + b] * u[b][1] for b in blks]
                for n, (_, lb) in enumerate(STRASSEN):
                    coefs = [c * g[b][0] * u[b][0] for c, b in zip(lb, blks)]
                    h_s[n, k2] = _form(coefs, [lambda x=x: x for x in hs])
            yield
        order = [(n, m) for n in range(7) for m in (1, 5)] + [(n, m) for n in range(7) for m in (0, 2, 3, 4, 6)]
        for q, (n, m) in enumerate(order):
            rhs = [lambda k2=k2, c2=c2: h_s[n, k2, c2 * 256:(c2 + 1) * 256, :] for k2 in (0, 1) for c2 in (0, 1)]
            if q == 14:
                lhs.clear()
            if n not in lhs:
                lhs[n] = [_form(STRASSEN[n][0],
                                [lambda r=r, k=k, r2=r2, k2=k2: wd[j, pl.ds((2 * r + r2) * QD, QD),
                                                                   pl.ds((2 * k + k2) * 128, 128)]
                                 for r in (0, 1) for k in (0, 1)])
                          for r2 in (0, 1) for k2 in (0, 1)]
            left = _form(STRASSEN[m][0], [lambda x=x: x for x in lhs[n]])
            right = _form(STRASSEN[m][1], rhs).astype(bf16)
            if q == SPLITQ:
                v = _vcat(_dot_nt(left[:80].astype(bf16), right), _dot_nt(left[80:].astype(bf16), right))
            else:
                v = _dot_nt(left.astype(bf16), right)
            for c in range(2):
                old = acc[t, c, m, n * QD:(n + 1) * QD, :]
                if may_init:
                    old = jnp.where(j > 0, old, 0.0)
                acc[t, c, m, n * QD:(n + 1) * QD, :] = old + v[:, c * 128:(c + 1) * 128]
            ticks.append(v[0:8, 0:128])
            yield

    with _scope("w_x0"):
        x_copy(0, 0, TM).wait()
    x_copy(1, 0, TM).start()
    cwo.start()
    for c in range(NB):
        in_t1(0, c)
    first_norm(0, 0)
    prep_wqkv()
    with _scope("w_x1"):
        x_copy(1, 0, TM).wait()
    for g in range(len(groups)):
        for c in ffn_copies(g):
            c.start()
    for c in range(NB):
        in_t1(1, c)

    def body_f(i, last):
        _drain(first_qkv(0, i))
        link = [None, lane < (i < 0).astype(jnp.int32)]
        first_norm(1, i, link)
        if last:
            prep_wo()
        else:
            first_norm(0, i + 1, link)

    _loop(3, lambda i: body_f(i, False))
    cwo.wait()
    _loop(1, lambda i: body_f(i + 3, True))
    _loop(4, lambda i: _weave(ORDER_E, first_qkv(1, i), phase2(0, i, PAR0, q0, k0, v0)))

    def wait_group(k, g):
        @pl.when(k == 0)
        def _():
            for c in ffn_copies(g):
                c.wait()

    def finish_step(i):
        u = i % 4
        never = lane < (i < 0).astype(jnp.int32)
        x1, x2 = combine(0, u, never)[:2]
        done = out_t1(0, u, x1) + out_t1(0, u + 4, x2)
        yield
        anchor(never, done)
        done = out_t2(0, 2 * u) + out_t2(0, 2 * u + 1)
        yield
        anchor(never, done)
        yield

    def stage(k):
        t = k % 2
        n_a = jnp.where(jnp.logical_and(k > 0, k < 3), 4, 0)
        n_b = jnp.where(k < 3, 4, 0)
        n_c = NCH - n_a - n_b
        wait_group(k, 0)
        _loop(n_c, lambda i: _weave(ORDER_C, ffn_chunk(t, i, True), finish_step(i)))
        _loop(n_a, lambda i: _weave(ORDER_A, ffn_chunk(t, n_c + i), phase1(1 - t, i)))
        wait_group(k, 1)
        _loop(n_b, lambda i: _weave(ORDER_B, ffn_chunk(t, n_c + n_a + i),
                                    phase2(1 - t, i, PAR, q_s, k_s, v_s)))
    _loop(4, stage)

    for half in range(2):
        out_copy(0, half).start()
    for i in range(4):
        x1, x2 = combine(1, i)
        out_t1(1, i, x1)
        out_t1(1, i + 4, x2)
    for c in range(NB):
        out_t2(1, c)
        if c % 4 == 3:
            out_copy(1, c // 4).start()
    with _scope("w_out"):
        for t in range(2):
            for half in range(2):
                out_copy(t, half).wait()


@jax.jit
def pallas_interleave_layers__sliding_local_dilated__glu_gated_bilinear__prompt_kernel(
    A_x: jax.Array,
    A_wqkv: jax.Array,
    A_wo: jax.Array,
    B_x: jax.Array,
    B_w_gate: jax.Array,
    B_w_up: jax.Array,
    B_w_down: jax.Array,
):
    any_spec = pl.BlockSpec(memory_space=pl.ANY)
    qkv_scratch = [
        pltpu.VMEM((NB, NG, DH, 8, 128), f32),
        pltpu.VMEM((2 * NB, NG, DH, 8, 128), f32),
        pltpu.VMEM((2 * NB, NG, DH, 8, 128), f32),
    ]
    out_t = pl.pallas_call(
        _kernel,
        in_specs=[any_spec] * 6,
        out_specs=any_spec,
        out_shape=jax.ShapeDtypeStruct((D, S), bf16),
        scratch_shapes=[
            pltpu.VMEM((D, S), bf16),
            pltpu.VMEM((D, 3 * D), bf16),
            pltpu.VMEM((D, D), bf16),
            pltpu.VMEM((NCH, D, FC), bf16),
            pltpu.VMEM((NCH, D, FC), bf16),
            pltpu.VMEM((NCH, D, FC), bf16),
            pltpu.VMEM((NSLOT, HQ, 128), bf16),
            pltpu.VMEM((NSLOT, HD, 128), bf16),
            pltpu.VMEM((5, 3 * D, 128), f32),
            pltpu.VMEM((5, D, 128), f32),
            pltpu.VMEM((2, 5, HM, 128), u32),
            pltpu.VMEM((2, 5, 8 * 72, 128), u32),
            pltpu.VMEM((2, NB, D, 128), f32),
            *qkv_scratch,
            *qkv_scratch,
            pltpu.VMEM((2, D, 128), f32),
            pltpu.VMEM((2, D, 128), f32),
            pltpu.VMEM((2, NPASS, HM // 2, 128), u32),
            pltpu.VMEM((2, 2, 4, HM, 128), f32),
            pltpu.VMEM((7, 2, HM, 128), f32),
            pltpu.VMEM((2, 2, 7, 1024, 128), f32),
            pltpu.VMEM((2, 4, NSLOT, 128, 128), bf16),
            pltpu.SemaphoreType.DMA((20 + 3 * NCH,)),
        ],
        compiler_params=pltpu.CompilerParams(vmem_limit_bytes=120 * 1024 * 1024),
        name="fused_layers",
    )(A_x[0].T, A_wqkv, A_wo, B_w_gate, B_w_up, B_w_down.T)
    return out_t.T[None]
```

```python
import functools
import os

import jax
import jax.numpy as jnp
import jax.experimental.pallas as pl
import jax.experimental.pallas.tpu as pltpu

S, D, F = 2048, 576, 4608
H, DH, W = 32, 18, 8
NG = H // 8
GR = 8 * DH
NB = 8
TM = NB * 128
HM = TM // 2
HD = D // 2
HQ = 3 * D // 2
FC = 512
HC = FC // 2
NCH = F // FC
NSLOT = 16
NT = int(os.environ.get("NT", 128))

GROUP_ROWS = {1: (0, 128), 2: (64, 192), 4: (256, 384), 3: (320, 448), 0: (512, 512)}
T3 = 1.0 / 3.0
SLOTS = (
    ((1, (-1, -1, 0, 0), (0, 0, 0, 1)), (3, (1, 1, 0, 0), (0, 0, 1, 0))),
    ((0, (T3, 0, 0, 0), (2, 1, 0, 0)), (2, (-.5, -1, 0, 0), (0, 0, 0, 1))),
    ((4, (.5, 1, 0, 0), (0, 0, 1, 0)), (0, (-T3, 0, 0, 0), (1, 2, 0, 0))),
    ((1, (0, 1, 0, -1), (0, 0, 1, 1)), (2, (0, 2, 0, -1), (0, 0, .5, 1))),
    ((1, (0, 0, 1, 1), (1, 0, 0, 0)), (3, (0, 0, -1, -1), (0, 1, 0, 0))),
    ((0, (0, 0, T3, 0), (2, 1, 0, 0)), (2, (0, 0, .5, 1), (1, 0, 0, 0))),
    ((4, (0, 0, -.5, -1), (0, 1, 0, 0)), (0, (0, 0, -T3, 0), (1, 2, 0, 0))),
    ((1, (-1, 0, 1, 0), (1, 1, 0, 0)), (2, (-1, 0, .5, 0), (1, 2, 0, 0))),
    ((1, (0, 0, 0, 1), (-1, 0, 1, 0)), (3, (1, 0, 0, 0), (1, 0, -1, 0))),
    ((4, (.5, 0, 0, 0), (2, 0, -1, 0)), (2, (0, 0, 0, 1), (-1, 0, .5, 0))),
    ((4, (-1, 0, .5, 0), (2, 1, 0, 0)), (3, (-1, 0, 1, 0), (1, 1, 0, 0))),
    ((1, (1, 0, 0, 1), (1, 0, 0, 1)), (2, (1, 0, 0, 1), (1, 0, 0, 1))),
    ((1, (1, 0, 0, 0), (0, 1, 0, -1)), (3, (0, 0, 0, 1), (0, -1, 0, 1))),
    ((4, (0, 0, 0, 1), (0, -1, 0, .5)), (2, (.5, 0, 0, 0), (0, 2, 0, -1))),
    ((4, (0, 2, 0, -1), (0, 0, 1, .5)), (3, (0, 1, 0, -1), (0, 0, 1, 1))),
    ((4, (1, 0, 0, 1), (0, 1, 1, 0)), (3, (1, 0, 0, 1), (0, 1, 1, 0))),
)
_PASSES = (
    ("+01 +10", "-04 +14 +17", "-41 -43 +70 +71 +73", "-05 +15 +16", "-51 +60 +61 +62"),
    ("+10", "-04 +14", "+40 +41 -42 +43 -70 -71 -73", "-05 +15", "+50 +51 -52 -60 -61 -62"),
    ("+02 -03", "+00 -02", "+21 +23", "+01 -03", "+31 +33"),
    ("+00 -02 +03", "+00 +08", "+81 +83", "+01 +06", "-53 +63"),
    ("+01 +02 -03", "+02 -08", "+21", "+03 -07", "+31"),
    ("+00 -01", "+06", "+60 +62", "+07", "+70"),
    ("+10 -12 +13", "+10 +18", "+00", "+11 +16", "+10"),
    ("+12 -13", "+10 -12", "+00 +02", "+11 -13", "+10 +12"),
    ("-11 -12 +13", "+12 -18", "+80 +82", "+13 -17", "+72"),
    ("+10 +12", "-12 +14", "+42", "-13 +15", "+52"),
    ("-00 +02 +13", "+00 +18", "-00 +81 +83", "+01 +16", "-10 -53 +63"),
    ("+00 -02", "+06 -16", "+53 -62 -63", "+08 -18", "+80 -81 -83"),
    ("+00 +02", "+02 -04", "+20", "+03 -05", "+30"),
    ("+02", "+02 -12", "-20 +22 +23", "+03 -13", "-30 +32 +33"),
    ("+11 -13", "-08 +18", "-80 +81 -82", "-07 +17", "+43 -72 -73"),
    ("+02 -11 +13", "+08 -12", "+21 +80 +82", "+07 -13", "+31 +72"),
    ("+02 +13", "+00 -12", "+00 +02 -21 -23", "+01 -13", "+10 +12 -31 -33"),
    ("+10 -11", "+16", "+51 -61", "+17", "+41 +43 -71 -73"),
    ("+02 +12", "+12", "+00 +02 +22 +42 +80 +82", "+13", "+10 +12 +32 +52 +72"),
    ("+00 +10", "+04", "+20 +40", "+05", "+30 +50"),
    ("-00 +02 -10 +12", "+16", "+10 +62", "+18", "+00 -80"),
    ("+02 -10", "+04 -12", "+20 +42", "+05 -13", "+30 +52"),
    ("+03 +13", "+00", "+03 +21 +23 -43 -81 -83", "+01", "+13 +31 +33 -63"),
    ("+13", "-00 +10", "+01 +02 +03", "-01 +11", "+11 +12 +13"),
    ("-01 +03", "+00 +04 +07", "+43", "+01 +05 +06", "+53"),
    ("+01", "+04 +07 -14 -17", "+70 +71 +73", "+05 +06 -15 -16", "+53 +60 +61 +62"),
    ("+01 +11", "+14 +17", "-01 +41", "+15 +16", "-11 +51"),
    ("+11 -13", "+10 +14 +17", "+01", "+11 +15 +16", "+11"),
    ("+01 +13", "+00 +14 +17", "+01 +43", "+01 +15 +16", "+11 +53"),
    ("+01 -03 +11 -13", "+08", "+21 +81", "+07", "+31 +43 -73"),
)
PASSES = [[[(int(w[0] + "1"), int(w[1]), int(w[2])) for w in col.split()] for col in row] for row in _PASSES]
NPASS = len(PASSES)
STRASSEN = (
    ((1, 0, 0, 1), (1, 0, 0, 1)),
    ((0, 0, 1, 1), (1, 0, 0, 0)),
    ((1, 0, 0, 0), (0, 1, 0, -1)),
    ((0, 0, 0, 1), (-1, 0, 1, 0)),
    ((1, 1, 0, 0), (0, 0, 0, 1)),
    ((-1, 0, 1, 0), (1, 1, 0, 0)),
    ((0, 1, 0, -1), (0, 0, 1, 1)),
)
QD = D // 4
EPS = 1e-5
WG = [[int(c) for c in x] for x in os.environ.get("WG", "40,1,2,3").split(",")]
TICK = int(os.environ.get("TICK", 40))
ORDER_F = os.environ.get("OF", "mnmwwmwnmww.")
WX = int(os.environ.get("WX", 0))
SPLITQ = int(os.environ.get("SPLITQ", 48))
CLINK = int(os.environ.get("CLINK", 1))
KA = int(os.environ.get("KA", 11))
KB = int(os.environ.get("KB", 9))
PAR = int(os.environ.get("PAR", 2))
PAR0 = int(os.environ.get("PAR0", 3))
ORDER_A = "s" + "m" * KA + "ss"
KB0 = int(os.environ.get("KB0", 1))
ORDER_B = "m" * KB0 + "sm" * 8 + "m" * (KB - KB0 - 8) + "sssssf" + "m" * (15 - KB + int(os.environ.get("KB2", 6))) + "."
ORDER_C = "s" + "m" * int(os.environ.get("KC", 6)) + "s" + "m" * int(os.environ.get("KC2", 4)) + "s"
ORDER_E = os.environ.get("OE", "ssssssss!mmmmmsssssf")
f32, bf16, u32 = jnp.float32, jnp.bfloat16, jnp.uint32

_dot = functools.partial(jnp.dot, preferred_element_type=f32)


def _dot_nt(a, b):
    return jax.lax.dot_general(a, b, (((1,), (1,)), ((), ())), preferred_element_type=f32)


def _vcat(*xs):
    return jnp.concatenate(xs, axis=0)


def _pad_rows(r):
    return _vcat(r, jnp.zeros((128 - r.shape[0], r.shape[1]), r.dtype))


def _add(x, y):
    return (x.astype(f32) + y.astype(f32)).astype(bf16)


def _sub(x, y):
    return (x.astype(f32) - y.astype(f32)).astype(bf16)


def _form(coefs, blocks):
    terms = [(c, blk) for c, blk in zip(coefs, blocks) if c != 0]
    if len(terms) == 1 and terms[0][0] == 1:
        return terms[0][1]()
    terms.sort(key=lambda cb: cb[0] < 0)
    out = None
    for c, blk in terms:
        v = blk().astype(f32)
        if out is None:
            out = v if c == 1 else v * c
        else:
            v = v if abs(c) == 1 else v * abs(c)
            out = out + v if c > 0 else out - v
    return out


def _lhs_slots_lanes(x1, x2):
    low = jax.lax.broadcasted_iota(jnp.int32, x1[0].shape, 1) < 64
    out = []
    for halves in SLOTS:
        keys = [(tuple(k // 128 for k in GROUP_ROWS[grp]), coefs) for grp, coefs, _ in halves]
        vals = [_form(coefs, [lambda x=x, g=g: x[g] for x in (x1, x2) for g in tiles])
                for tiles, coefs in keys]
        out.append(vals[0] if keys[0] == keys[1] else jnp.where(low, vals[0], vals[1]))
    return out


def _fast_product(p, ref, out):
    p0, p1, p2, p3 = p(0), p(1), p(2), p(3)
    r = p0 + p1 + p2
    ref[0] = r + p1 + p3
    ref[1] = r + p2
    yield
    p0, p1, p2, p3 = p(4), p(5), p(6), p(7)
    r = p0 + p1 + p2
    ref[2] = r + p1
    ref[3] = p3 - (r + p2)
    yield
    p0, p1, p2, p3 = p(8), p(9), p(10), p(11)
    r = p0 + p1
    c11 = ref[0] + (r + p3)
    ref[2] = ref[2] + (r + p1 + p2)
    ref[3] = ref[3] + p3
    yield
    p0, p1, p2, p3 = p(12), p(13), p(14), p(15)
    r = p0 + p1
    out.append((c11, (r + p2 + p3) - ref[1], ref[2] + p3, ref[3] + (r + p1)))
    yield


def _rhs_slot(s, get, zero=None):
    parts = []
    for grp, _, coefs in SLOTS[s]:
        k1, k2 = GROUP_ROWS[grp]
        blocks = [lambda k=k, c=c: get(slice(k, k + 64), c) for k in (k1, k2) for c in (0, 1)]
        parts.append(_form(coefs, blocks).astype(f32))
    if zero is not None:
        parts[0] = _vcat(parts[0][:8] + zero, parts[0][8:])
    return _vcat(*parts).astype(bf16)


def _signed(terms, get):
    return _form([t[0] for t in terms], [functools.partial(get, t[1], t[2]) for t in terms])


def _feed(outs, prods, ref, keep=()):
    vals = dict(prods)
    sums = {}
    for s in prods:
        for sign, i, n in PASSES[s][0]:
            sums.setdefault((i, n), {})[s] = sign
    while True:
        pairs = {}
        for terms in sums.values():
            keys = list(terms)
            for x in range(len(keys)):
                for y in range(x):
                    key = (keys[y], keys[x], terms[keys[x]] * terms[keys[y]])
                    pairs[key] = pairs.get(key, 0) + 1
        if not pairs or max(pairs.values()) < 2:
            break
        x, y, rel = max(pairs, key=pairs.get)
        vals[x, y] = vals[x] + vals[y] if rel > 0 else vals[x] - vals[y]
        for terms in sums.values():
            if x in terms and y in terms and terms[x] * terms[y] == rel:
                terms[x, y] = terms.pop(x)
                del terms[y]
    for blk, terms in sums.items():
        items = [(sign, vals[k]) for k, sign in terms.items()]
        sign, v = items[0]
        for s2, w in items[1:] + ([(outs[blk][0], ref[blk])] if blk in outs else []):
            v = v + w if s2 == sign else v - w
        outs[blk] = (sign, v)
        if blk not in keep:
            ref[blk] = v


def _packed(ref, *idx):
    return pltpu.bitcast(ref.bitcast(u32)[idx], bf16)


def _norm_stats(ref, total):
    m = jnp.broadcast_to(jnp.sum(total, axis=0, keepdims=True) * (1.0 / D), (8, 128))
    s = None
    for r in range(0, D, 8):
        c = ref[r:r + 8, :] - m
        s = c * c if s is None else s + c * c
    v = jnp.sum(s, axis=0, keepdims=True) * (1.0 / D)
    return m[0:1], jax.lax.rsqrt(v + EPS)


def _tile_sum(x, zero=None):
    rows = [x[r:r + 8] for r in range(0, D, 8)]
    return functools.reduce(jnp.add, rows[1:], rows[0] if zero is None else rows[0] + zero)


def _aligned(x, n):
    return x if isinstance(x, int) else pl.multiple_of(x, n)


def _drain(*gens):
    for gen in gens:
        for _ in gen:
            pass


def _weave(order, main, side):
    for c in order:
        next(main if c == "m" else side)
    _drain(main, side)


def _scope(name):
    import contextlib
    return jax.named_scope(name) if os.environ.get("SCOPES") else contextlib.nullcontext()


def _loop(n, fn):
    def body(i, c):
        with _scope("it"):
            fn(i)
        return c
    jax.lax.fori_loop(0, n, body, 0)


def _kernel(x_hbm, wqkv_hbm, wo_hbm, wg_hbm, wu_hbm, wd_hbm, out_hbm,
            xin, wqkv, wo, wg, wu, wd, wqkv_t, wo_t, wperm, operm, wt_s, pin0, pin1, pout, xres,
            q0, k0, v0, q_s, k_s, v_s, c_s, o_s, n_s, a_s, gu_s, h_s, acc, xn_s, sems):
    groups = (range(5), range(5, NCH))
    lane = jax.lax.broadcasted_iota(jnp.int32, (8, 128), 1)
    anchors, ticks = [], []
    pin = (pin0, pin1)

    def anchor(never, words):
        anchors.append(jnp.where(never, pltpu.bitcast(functools.reduce(jnp.bitwise_or, words), f32), 0.0))

    def x_copy(t):
        cols = pl.ds(t * TM, TM)
        return pltpu.make_async_copy(x_hbm.at[:, cols], xin.at[:, cols], sems.at[10 + t])

    def wqkv_copy(g):
        rows = pl.ds(g * 128, min(128, D - g * 128))
        return pltpu.make_async_copy(wqkv_hbm.at[rows], wqkv.at[rows], sems.at[15 + g])

    def out_copy(t, half):
        cols = pl.ds(t * TM + half * HM, HM)
        return pltpu.make_async_copy(xin.at[:, cols], out_hbm.at[:, cols], sems.at[2 * t + half])

    def ffn_copies(g):
        return [pltpu.make_async_copy(src.at[:, pl.ds(j * FC, FC)], dst.at[j], sems.at[20 + 3 * j + i])
                for j in groups[g]
                for i, (src, dst) in enumerate(((wg_hbm, wg), (wu_hbm, wu), (wd_hbm, wd)))]

    cwo = pltpu.make_async_copy(wo_hbm, wo, sems.at[3])
    x_copy(0).start()
    for gs in WG:
        for g in gs:
            wqkv_copy(g).start()

    def head_rows(ref, g, base):
        return _vcat(*[ref[g, pl.ds(base + d, 8, stride=DH), :] for d in range(DH)])

    def transpose_wqkv(g):
        rows = wqkv[g * 128:min((g + 1) * 128, D), :].astype(f32)
        wperm[g] = (_vcat(rows, rows) if g == 4 else rows).T

    def wqkv_slots(hg):
        base = pl.multiple_of(hg * GR, 16)
        for d in range(0, DH, 2):
            x1, x2 = [[_vcat(*[wperm[g, pl.ds(b + e, 8, stride=DH), :] for e in (d, d + 1)]) for g in range(5)]
                      for b in (base, base + HQ)]
            for n, v in enumerate(_lhs_slots_lanes(x1, x2)):
                wqkv_t[n, pl.ds(base + 8 * d, 16), :] = v.astype(bf16)

    def widen_wo(i):
        rows = pl.ds(pl.multiple_of(i * (D // 3), 64), D // 3)
        for g in range(5):
            cols = wo[rows, g * 128:min((g + 1) * 128, D)].astype(f32)
            if g == 4:
                cols = jnp.concatenate([cols, jnp.zeros_like(cols)], axis=1)
            operm[g, rows, :] = cols

    def prep_wo(never):
        for g in range(5):
            r = _vcat(*[head_rows(operm, g, hg * GR) for hg in range(NG)])
            r = _vcat(r, r[512:D])
            tiles = [pltpu.bitcast(r[k * 128:(k + 1) * 128].astype(bf16).T, u32) for k in range(5)]
            for k, w in enumerate(tiles):
                wt_s[k, g * 64:(g + 1) * 64, :] = w
            anchor(never, [w[56:64] for w in tiles])
            yield
        for r in range(0, HD // 2, 8):
            zero = pltpu.bitcast(jnp.where(never, ticks.pop(0), 0.0), u32)
            x1, x2 = [[pltpu.bitcast(wt_s[k, r0:r0 + 8, :] | zero, bf16).astype(f32) for k in range(5)]
                      for r0 in (r, r + HD // 2)]
            for n, v in enumerate(_lhs_slots_lanes(x1, x2)):
                wo_t[n, 2 * r:2 * r + 16, :] = v.astype(bf16)
            yield

    def to_words(x):
        tiles = [x[g * 128:(g + 1) * 128] for g in range(4)] + [_pad_rows(x[512:D])]
        return [pltpu.bitcast(r.astype(bf16).T, u32) for r in tiles]

    def from_words(words):
        parts = [pltpu.bitcast(w, bf16).T for w in words]
        return _vcat(*parts[:4], parts[4][:64])

    def in_t1(t, c):
        x = xin[:, pl.ds(pl.multiple_of(t * TM + c * 128, 128), 128)]
        words = to_words(x)
        for g, w in enumerate(words):
            pin[t][g, pl.ds(pl.multiple_of(c * 64, 64), 64), :] = w
        return [w[56:64] for w in words]

    def in_t2(t, j):
        return from_words([pin[t][g, pl.ds(j, 64, stride=8), :] for g in range(5)]).astype(f32)

    def out_t1(t, j, x):
        words = to_words(x)
        for g, w in enumerate(words):
            pout[t, g, pl.ds(_aligned(j * 72, 8), 64), :] = w
        return [w[56:64] for w in words]

    def out_t2(t, c):
        words = [_vcat(*[pout[t, g, pl.ds(c * 8 + m, 8, stride=72), :] for m in range(8)])
                 for g in range(5)]
        x = from_words(words)
        xin[:, pl.ds(_aligned(t * TM + c * 128, 128), 128)] = x
        return [pltpu.bitcast(x[r - 16:r], u32) for r in (128, 256, 384, 512, D)]

    def combine(t, i, never=None):
        c, second = i % 2, i // 2
        pick = lambda lo, hi: lo + (hi - lo) * second
        outer = lambda m1, m2, m3, m4, m5, m6, m7: (
            m1 + m4 - m5 + m7, m2 + m4, m3 + m5, m1 - m2 + m3 + m6)
        strips, sums, link = [], [], None
        for r in range(0, QD, 8):
            get = lambda n, m: acc[t, c, m, n * QD + r:n * QD + r + 8, :]
            four, two = [], []
            for n in range(7):
                x = get(n, pick(3, 2))
                if link is not None and n % CLINK == 0:
                    x = x + jnp.where(never, link, 0.0)
                four.append(((get(n, 0) + x) + get(n, pick(6, 5))) - get(n, pick(4, 1)))
                two.append(get(n, pick(1, 4)) + x)
                if never is not None:
                    link = four[-1]
            rows = []
            for u, v in zip(outer(*four), outer(*two)):
                if isinstance(second, int):
                    rows += [v, u] if second else [u, v]
                else:
                    rows += [jnp.where(second > 0, v, u), jnp.where(second > 0, u, v)]
            strips.append([xres[t, i + 4 * (q // 4), (q % 4) * QD + r:(q % 4) * QD + r + 8, :] + v
                           for q, v in enumerate(rows)])
            if never is not None:
                sums = [functools.reduce(jnp.add, sums[n:n + 1] + strips[-1][4 * n:4 * n + 4]) for n in (0, 1)]
                link = sums[0] + sums[1]
        return [_vcat(*[s[q] for q in range(q0, q0 + 4) for s in strips]) for q0 in (0, 4)] + sums

    def store_qkv(t, b, part, q, k, v, prev=None):
        q[b] = part[0:D].reshape(NG, DH, 8, 128)
        for n, (dst, r) in enumerate(((k, part[D:2 * D]), (v, part[2 * D:3 * D]))):
            dst[b + NB] = r.reshape(NG, DH, 8, 128)
            sh = pltpu.roll(r, 2, 1).reshape(NG, DH, 8, 128)
            if isinstance(t, int) and t == 0:
                dst[b] = sh
            elif prev is not None:
                dst[b] = jnp.where((lane < 2)[None, None], prev[n][b], sh)
            else:
                keep = jnp.broadcast_to((lane >= 2 * t)[None, None], sh.shape)
                pltpu.store(dst.at[b], sh, mask=keep)

    def normalize(t, i, s1, s2, never):
        for c, s in enumerate((s1, s2)):
            if c and never is not None:
                s = s + jnp.where(never, r, 0.0)
            m, r = _norm_stats(xres.at[t, i + 4 * c], s)
            n_s[c] = (xres[t, i + 4 * c] - m) * r

    def phase1(t, i):
        never = lane < (i < 0).astype(jnp.int32)
        x1, x2, s1, s2 = combine(t, i, never)
        xres[t, i] = x1
        xres[t, i + 4] = x2
        normalize(t, i, s1, s2, never)
        yield
        rhs = lambda s: _rhs_slot(s, lambda rows, c: n_s[c, rows, :])
        out = []
        _drain(_fast_product(lambda s: _dot(_packed(wqkv_t, s), rhs(s)), c_s.at[:, 0:HQ], out))
        c = out[0]
        yield
        store_qkv(t, i, _vcat(c[0], c[2]), q_s, k_s, v_s)
        store_qkv(t, i + 4, _vcat(c[1], c[3]), q_s, k_s, v_s)
        yield

    def first_norm(t, i, dst, never=None):
        sums = []
        src = [xres.at[t, i + 4 * c] for c in (0, 1)]
        for c in (0, 1):
            x = in_t2(t, i + 4 * c)
            xres[t, i + 4 * c] = x
            sums.append(_tile_sum(x))
        if never is not None:
            anchors.append(jnp.where(never, sums[0] + sums[1], 0.0))
        yield
        stats = [_norm_stats(src[c], sums[c]) for c in (0, 1)]
        if never is not None:
            anchors.append(jnp.where(never, stats[0][1] + stats[1][1], 0.0))
        yield
        for s in range(NSLOT):
            mean = [st[0] for st in stats]
            if never is not None:
                zero = jnp.where(never, ticks.pop(0), 0.0)[0:1]
                mean = [m + zero for m in mean]
            dst[s] = _rhs_slot(s, lambda rows, c: (src[c][rows, :] - mean[c]) * stats[c][1])
            yield

    def first_qkv(t, i, src):
        def p(s):
            w = wqkv_t.bitcast(u32)[s, rows]
            while anchors:
                w = _vcat(w[:8] | pltpu.bitcast(anchors.pop(), u32), w[8:])
            v = _dot(pltpu.bitcast(w, bf16), _packed(src, s))
            if s % 4 == 0:
                ticks.extend(v[r:r + 8] for r in range(0, HQ // 2, TICK))
            return v

        cs = []
        for r0 in ((HQ // 4, 0) if t == 0 else (0, HQ // 4)):
            rows = slice(r0, r0 + HQ // 4)
            yield from _fast_product(p, c_s.at[:, 2 * r0:2 * r0 + HQ // 2], cs)
        for n, b in enumerate((i, i + 4)):
            part = _vcat(cs[1 - t][n], cs[t][n], cs[1 - t][n + 2], cs[t][n + 2])
            if t == 0:
                store_qkv(t, b, part, q0, k0, v0)
            else:
                store_qkv(t, b, part, q_s, k_s, v_s, prev=(k0, v0))

    def attention_group(t, b, g, q_r, k_r, v_r, links):
        par = len(links)
        never = lane < (b < 0).astype(jnp.int32)

        def start(n, v):
            if links[n % par] is None:
                return v
            return jnp.where(never, links[n % par], 0.0) + v

        q = [q_r[b, g, d] for d in range(DH)]
        logits = []
        for w in range(W):
            l = start(w, q[0] * k_r[b + NB - w, g, 0])
            for d in range(1, DH):
                l = l + q[d] * k_r[b + NB - w, g, d]
            links[w % par] = l
            l = l * (DH ** -0.5)
            if w > 0:
                edge = jnp.where(jnp.logical_and(w > b, t == 0), 2, 0)
                l = jnp.where(lane < edge, -1e9, l)
            logits.append(l)
        m = functools.reduce(jnp.maximum, logits)
        e = [jnp.exp(l - m) for l in logits]
        r = 1.0 / functools.reduce(jnp.add, e)
        p = [x * r for x in e]
        outs = []
        for d in range(DH):
            o = p[0] * v_r[b + NB, g, d]
            if d >= par:
                o = start(d, o)
            for w in range(1, W):
                o = o + p[w] * v_r[b + NB - w, g, d]
            links[d % par] = o
            outs.append(o)
        return _vcat(*outs)

    def attend(t, i, par, q_r, k_r, v_r):
        links = [None] * par
        never = lane < (i < 0).astype(jnp.int32)
        for c, b in enumerate((i, i + 4)):
            for g in range(NG):
                o_s[c, g * GR:(g + 1) * GR, :] = attention_group(t, b, g, q_r, k_r, v_r, links)
                anchors.append(jnp.where(never, functools.reduce(jnp.add, links), 0.0))
                yield
        p = lambda s: _dot(_packed(wo_t, s), _rhs_slot(s, lambda rows, c: o_s[c, rows, :]))
        out = []
        yield from _fast_product(p, c_s.at[:, HQ:HQ + HD], out)
        for n, b in enumerate((i, i + 4)):
            x = xres[t, b] + _vcat(out[0][n], out[0][n + 2])
            xres[t, b] = x
            c_s[n, HQ + HD:, :] = _tile_sum(x)
        yield

    def ffn_slots(t, i, never=None):
        normalize(t, i, c_s[0, HQ + HD:, :], c_s[1, HQ + HD:, :], never)
        yield
        rows = pl.ds(_aligned(i * 64, 64), 64)
        for s, (_, lo, _, hi, _) in enumerate(PASSES):
            op = _vcat(*[_signed(x, lambda r, k: n_s[r, 64 * k:64 * k + 64, :]) for x in (lo, hi)])
            if never is not None:
                op = _vcat(op[:8] + jnp.where(never, ticks.pop(0), 0.0), op[8:])
            a_s[t, s, rows, :] = pltpu.bitcast(op.astype(bf16).T, u32)
            yield

    def ffn_pass(t, w_ref, s):
        get = lambda k, n: w_ref[64 * k:64 * k + 64, 128 * n:128 * n + 128]
        parts = [_signed(x, get).astype(f32) for x in PASSES[s][2::2]]
        while anchors:
            parts[0] = _vcat(parts[0][:8] + anchors.pop(), parts[0][8:])
        return _dot(pltpu.bitcast(a_s[t, s], bf16), _vcat(*parts).astype(bf16))

    def ffn_chunk(t, j, may_init=False):
        lhs, g, u = {}, {}, {}
        todo = [(g, wg, s) for s in list(range(2, NPASS)) + [0, 1]] + [(u, wu, s) for s in range(NPASS)]
        for q in range(0, 2 * NPASS, 4):
            prods = [(outs, s, ffn_pass(t, w.at[j], s)) for outs, w, s in todo[q:q + 4]]
            k2 = {2 * NPASS - 12: 0, 2 * NPASS - 4: 1}.get(q)
            blks = [] if k2 is None else [(i, 2 * k + k2) for k in (0, 1) for i in (0, 1)]
            for n, outs in enumerate((g, u)):
                _feed(outs, {s: v for o, s, v in prods if o is outs}, gu_s.at[n], blks)
            if blks:
                hs = [gu_s[(0,) + b] * u[b][1] for b in blks]
                for n, (_, lb) in enumerate(STRASSEN):
                    coefs = [c * g[b][0] * u[b][0] for c, b in zip(lb, blks)]
                    h_s[n, k2] = _form(coefs, [lambda x=x: x for x in hs])
            yield
        order = [(n, m) for n in range(7) for m in (1, 5)] + [(n, m) for n in range(7) for m in (0, 2, 3, 4, 6)]
        for q, (n, m) in enumerate(order):
            rhs = [lambda k2=k2, c2=c2: h_s[n, k2, c2 * 256:(c2 + 1) * 256, :] for k2 in (0, 1) for c2 in (0, 1)]
            if q == 14:
                lhs.clear()
            if n not in lhs:
                lhs[n] = [_form(STRASSEN[n][0],
                                [lambda r=r, k=k, r2=r2, k2=k2: wd[j, pl.ds((2 * r + r2) * QD, QD),
                                                                   pl.ds((2 * k + k2) * 128, 128)]
                                 for r in (0, 1) for k in (0, 1)])
                          for r2 in (0, 1) for k2 in (0, 1)]
            left = _form(STRASSEN[m][0], [lambda x=x: x for x in lhs[n]])
            right = _form(STRASSEN[m][1], rhs).astype(bf16)
            if q == SPLITQ:
                v = _vcat(_dot_nt(left[:80].astype(bf16), right), _dot_nt(left[80:].astype(bf16), right))
            else:
                v = _dot_nt(left.astype(bf16), right)
            for c in range(2):
                old = acc[t, c, m, n * QD:(n + 1) * QD, :]
                if may_init:
                    old = jnp.where(j > 0, old, 0.0)
                acc[t, c, m, n * QD:(n + 1) * QD, :] = old + v[:, c * 128:(c + 1) * 128]
            ticks.append(v[0:8, 0:128])
            yield

    with _scope("w_x0"):
        x_copy(0).wait()
    for c in range(NB):
        in_t1(0, c)
    for gs in WG:
        with _scope("w_qkv"):
            for g in gs:
                wqkv_copy(g).wait()
        if gs == WG[0]:
            _drain(first_norm(0, 0, xn_s.at[0, 0]))
        if gs == WG[WX]:
            x_copy(1).start()
            cwo.start()
        for g in gs:
            transpose_wqkv(g)
    _loop(HQ // GR, wqkv_slots)
    with _scope("w_x1"):
        x_copy(1).wait()
    for g in range(len(groups)):
        for c in ffn_copies(g):
            c.start()
    for c in range(NB):
        in_t1(1, c)

    def run(order, gens):
        for c in order:
            if c == ".":
                ticks.clear()
            elif c == "!":
                anchors.clear()
            else:
                next(gens[c])
        _drain(*gens.values())

    def body_f(i, zero):
        never = lane < (i < 0).astype(jnp.int32)
        xn = xn_s.at[pl.ds(i, 2)]
        widen_wo(i)
        run("mamnmamn.", {"m": first_qkv(0, i, xn.at[0, 0]), "a": first_norm(1, i, xn.at[0, 1], never),
                          "n": first_norm(0, i + 1, xn.at[1, 0], never)})
        return zero + (i < 0).astype(jnp.int32)

    with _scope("w_wo"):
        cwo.wait()
    never = lane < jax.lax.fori_loop(0, 3, body_f, 0)
    run(ORDER_F, {"m": first_qkv(0, 3, xn_s.at[3, 0]), "n": first_norm(1, 3, xn_s.at[3, 1], never),
                  "w": prep_wo(never)})
    _loop(4, lambda i: run(ORDER_E, {"m": first_qkv(1, i, xn_s.at[i, 1]), "s": attend(0, i, PAR0, q0, k0, v0),
                                     "f": ffn_slots(0, i)}))

    def wait_group(k, g):
        @pl.when(k == 0)
        def _():
            for c in ffn_copies(g):
                c.wait()

    def finish_step(i):
        u = i % 4
        never = lane < (i < 0).astype(jnp.int32)
        x1, x2 = combine(0, u, never)[:2]
        done = out_t1(0, u, x1) + out_t1(0, u + 4, x2)
        yield
        anchor(never, done)
        done = out_t2(0, 2 * u) + out_t2(0, 2 * u + 1)
        yield
        anchor(never, done)
        yield

    def stage(k):
        t = k % 2
        n_a = jnp.where(jnp.logical_and(k > 0, k < 3), 4, 0)
        n_b = jnp.where(k < 3, 4, 0)
        n_c = NCH - n_a - n_b
        wait_group(k, 0)
        _loop(n_c, lambda i: _weave(ORDER_C, ffn_chunk(t, i, True), finish_step(i)))
        _loop(n_a, lambda i: _weave(ORDER_A, ffn_chunk(t, n_c + i), phase1(1 - t, i)))
        wait_group(k, 1)

        def body_b(i):
            run(ORDER_B, {"m": ffn_chunk(t, n_c + n_a + i), "s": attend(1 - t, i, PAR, q_s, k_s, v_s),
                          "f": ffn_slots(1 - t, i, lane < (i < 0).astype(jnp.int32))})
        _loop(n_b, body_b)
    _loop(4, stage)

    for half in range(2):
        out_copy(0, half).start()
    for i in range(4):
        x1, x2 = combine(1, i)
        out_t1(1, i, x1)
        out_t1(1, i + 4, x2)
    for c in range(NB):
        out_t2(1, c)
        if c % 4 == 3:
            out_copy(1, c // 4).start()
    with _scope("w_out"):
        for t in range(2):
            for half in range(2):
                out_copy(t, half).wait()


@jax.jit
def pallas_interleave_layers__sliding_local_dilated__glu_gated_bilinear__prompt_kernel(
    A_x: jax.Array,
    A_wqkv: jax.Array,
    A_wo: jax.Array,
    B_x: jax.Array,
    B_w_gate: jax.Array,
    B_w_up: jax.Array,
    B_w_down: jax.Array,
):
    any_spec = pl.BlockSpec(memory_space=pl.ANY)
    qkv_scratch = [
        pltpu.VMEM((NB, NG, DH, 8, 128), f32),
        pltpu.VMEM((2 * NB, NG, DH, 8, 128), f32),
        pltpu.VMEM((2 * NB, NG, DH, 8, 128), f32),
    ]
    out_t = pl.pallas_call(
        _kernel,
        in_specs=[any_spec] * 6,
        out_specs=any_spec,
        out_shape=jax.ShapeDtypeStruct((D, S), bf16),
        scratch_shapes=[
            pltpu.VMEM((D, S), bf16),
            pltpu.VMEM((D, 3 * D), bf16),
            pltpu.VMEM((D, D), bf16),
            pltpu.VMEM((NCH, D, FC), bf16),
            pltpu.VMEM((NCH, D, FC), bf16),
            pltpu.VMEM((NCH, D, FC), bf16),
            pltpu.VMEM((NSLOT, HQ, 128), bf16),
            pltpu.VMEM((NSLOT, HD, 128), bf16),
            pltpu.VMEM((5, 3 * D, 128), f32),
            pltpu.VMEM((5, D, 128), f32),
            pltpu.VMEM((5, 320, 128), u32),
            pltpu.VMEM((5, HM, 128), u32),
            pltpu.VMEM((5, HM, 128), u32),
            pltpu.VMEM((2, 5, 8 * 72, 128), u32),
            pltpu.VMEM((2, NB, D, 128), f32),
            *qkv_scratch,
            *qkv_scratch,
            pltpu.VMEM((4, HQ + HD + 8, 128), f32),
            pltpu.VMEM((2, D, 128), f32),
            pltpu.VMEM((2, D, 128), f32),
            pltpu.VMEM((2, NPASS, HM // 2, 128), u32),
            pltpu.VMEM((2, 2, 4, HM, 128), f32),
            pltpu.VMEM((7, 2, HM, 128), f32),
            pltpu.VMEM((2, 2, 7, 1024, 128), f32),
            pltpu.VMEM((4, 2, NSLOT, 128, 128), bf16),
            pltpu.SemaphoreType.DMA((20 + 3 * NCH,)),
        ],
        compiler_params=pltpu.CompilerParams(vmem_limit_bytes=120 * 1024 * 1024),
        name="fused_layers",
    )(A_x[0].T, A_wqkv, A_wo, B_w_gate, B_w_up, B_w_down.T)
    return out_t.T[None]
```

```python
import functools
import os

import jax
import jax.numpy as jnp
import jax.experimental.pallas as pl
import jax.experimental.pallas.tpu as pltpu

S, D, F = 2048, 576, 4608
H, DH, W = 32, 18, 8
NG = H // 8
GR = 8 * DH
NB = 8
TM = NB * 128
HM = TM // 2
HD = D // 2
HQ = 3 * D // 2
FC = 512
HC = FC // 2
NCH = F // FC
NSLOT = 16
NT = int(os.environ.get("NT", 128))

GROUP_ROWS = {1: (0, 128), 2: (64, 192), 4: (256, 384), 3: (320, 448), 0: (512, 512)}
T3 = 1.0 / 3.0
SLOTS = (
    ((1, (-1, -1, 0, 0), (0, 0, 0, 1)), (3, (1, 1, 0, 0), (0, 0, 1, 0))),
    ((0, (T3, 0, 0, 0), (2, 1, 0, 0)), (2, (-.5, -1, 0, 0), (0, 0, 0, 1))),
    ((4, (.5, 1, 0, 0), (0, 0, 1, 0)), (0, (-T3, 0, 0, 0), (1, 2, 0, 0))),
    ((1, (0, 1, 0, -1), (0, 0, 1, 1)), (2, (0, 2, 0, -1), (0, 0, .5, 1))),
    ((1, (0, 0, 1, 1), (1, 0, 0, 0)), (3, (0, 0, -1, -1), (0, 1, 0, 0))),
    ((0, (0, 0, T3, 0), (2, 1, 0, 0)), (2, (0, 0, .5, 1), (1, 0, 0, 0))),
    ((4, (0, 0, -.5, -1), (0, 1, 0, 0)), (0, (0, 0, -T3, 0), (1, 2, 0, 0))),
    ((1, (-1, 0, 1, 0), (1, 1, 0, 0)), (2, (-1, 0, .5, 0), (1, 2, 0, 0))),
    ((1, (0, 0, 0, 1), (-1, 0, 1, 0)), (3, (1, 0, 0, 0), (1, 0, -1, 0))),
    ((4, (.5, 0, 0, 0), (2, 0, -1, 0)), (2, (0, 0, 0, 1), (-1, 0, .5, 0))),
    ((4, (-1, 0, .5, 0), (2, 1, 0, 0)), (3, (-1, 0, 1, 0), (1, 1, 0, 0))),
    ((1, (1, 0, 0, 1), (1, 0, 0, 1)), (2, (1, 0, 0, 1), (1, 0, 0, 1))),
    ((1, (1, 0, 0, 0), (0, 1, 0, -1)), (3, (0, 0, 0, 1), (0, -1, 0, 1))),
    ((4, (0, 0, 0, 1), (0, -1, 0, .5)), (2, (.5, 0, 0, 0), (0, 2, 0, -1))),
    ((4, (0, 2, 0, -1), (0, 0, 1, .5)), (3, (0, 1, 0, -1), (0, 0, 1, 1))),
    ((4, (1, 0, 0, 1), (0, 1, 1, 0)), (3, (1, 0, 0, 1), (0, 1, 1, 0))),
)
_PASSES = (
    ("+01 +10", "-04 +14 +17", "-41 -43 +70 +71 +73", "-05 +15 +16", "-51 +60 +61 +62"),
    ("+10", "-04 +14", "+40 +41 -42 +43 -70 -71 -73", "-05 +15", "+50 +51 -52 -60 -61 -62"),
    ("+02 -03", "+00 -02", "+21 +23", "+01 -03", "+31 +33"),
    ("+00 -02 +03", "+00 +08", "+81 +83", "+01 +06", "-53 +63"),
    ("+01 +02 -03", "+02 -08", "+21", "+03 -07", "+31"),
    ("+00 -01", "+06", "+60 +62", "+07", "+70"),
    ("+10 -12 +13", "+10 +18", "+00", "+11 +16", "+10"),
    ("+12 -13", "+10 -12", "+00 +02", "+11 -13", "+10 +12"),
    ("-11 -12 +13", "+12 -18", "+80 +82", "+13 -17", "+72"),
    ("+10 +12", "-12 +14", "+42", "-13 +15", "+52"),
    ("-00 +02 +13", "+00 +18", "-00 +81 +83", "+01 +16", "-10 -53 +63"),
    ("+00 -02", "+06 -16", "+53 -62 -63", "+08 -18", "+80 -81 -83"),
    ("+00 +02", "+02 -04", "+20", "+03 -05", "+30"),
    ("+02", "+02 -12", "-20 +22 +23", "+03 -13", "-30 +32 +33"),
    ("+11 -13", "-08 +18", "-80 +81 -82", "-07 +17", "+43 -72 -73"),
    ("+02 -11 +13", "+08 -12", "+21 +80 +82", "+07 -13", "+31 +72"),
    ("+02 +13", "+00 -12", "+00 +02 -21 -23", "+01 -13", "+10 +12 -31 -33"),
    ("+10 -11", "+16", "+51 -61", "+17", "+41 +43 -71 -73"),
    ("+02 +12", "+12", "+00 +02 +22 +42 +80 +82", "+13", "+10 +12 +32 +52 +72"),
    ("+00 +10", "+04", "+20 +40", "+05", "+30 +50"),
    ("-00 +02 -10 +12", "+16", "+10 +62", "+18", "+00 -80"),
    ("+02 -10", "+04 -12", "+20 +42", "+05 -13", "+30 +52"),
    ("+03 +13", "+00", "+03 +21 +23 -43 -81 -83", "+01", "+13 +31 +33 -63"),
    ("+13", "-00 +10", "+01 +02 +03", "-01 +11", "+11 +12 +13"),
    ("-01 +03", "+00 +04 +07", "+43", "+01 +05 +06", "+53"),
    ("+01", "+04 +07 -14 -17", "+70 +71 +73", "+05 +06 -15 -16", "+53 +60 +61 +62"),
    ("+01 +11", "+14 +17", "-01 +41", "+15 +16", "-11 +51"),
    ("+11 -13", "+10 +14 +17", "+01", "+11 +15 +16", "+11"),
    ("+01 +13", "+00 +14 +17", "+01 +43", "+01 +15 +16", "+11 +53"),
    ("+01 -03 +11 -13", "+08", "+21 +81", "+07", "+31 +43 -73"),
)
PASSES = [[[(int(w[0] + "1"), int(w[1]), int(w[2])) for w in col.split()] for col in row] for row in _PASSES]
NPASS = len(PASSES)
STRASSEN = (
    ((1, 0, 0, 1), (1, 0, 0, 1)),
    ((0, 0, 1, 1), (1, 0, 0, 0)),
    ((1, 0, 0, 0), (0, 1, 0, -1)),
    ((0, 0, 0, 1), (-1, 0, 1, 0)),
    ((1, 1, 0, 0), (0, 0, 0, 1)),
    ((-1, 0, 1, 0), (1, 1, 0, 0)),
    ((0, 1, 0, -1), (0, 0, 1, 1)),
)
QD = D // 4
EPS = 1e-5
WG = [[int(c) for c in x] for x in os.environ.get("WG", "40,1,2,3").split(",")]
TICK = int(os.environ.get("TICK", 40))
ORDER_F = os.environ.get("OF", "mnwmwwnmww.")
WX = int(os.environ.get("WX", 0))
SPLITQ = int(os.environ.get("SPLITQ", 48))
CLINK = int(os.environ.get("CLINK", 1))
KA = int(os.environ.get("KA", 11))
KB = int(os.environ.get("KB", 9))
PAR = int(os.environ.get("PAR", 2))
PAR0 = int(os.environ.get("PAR0", 3))
ORDER_A = "s" + "m" * KA + "ss"
KB0 = int(os.environ.get("KB0", 1))
ORDER_B = "m" * KB0 + "sm" * 8 + "m" * (KB - KB0 - 8) + "sssssf" + "m" * (15 - KB + int(os.environ.get("KB2", 6))) + "."
ORDER_C = "s" + "m" * int(os.environ.get("KC", 6)) + "s" + "m" * int(os.environ.get("KC2", 4)) + "s"
ORDER_E = os.environ.get("OE", "ssssssss!mmmmsssssf")
f32, bf16, u32 = jnp.float32, jnp.bfloat16, jnp.uint32

_dot = functools.partial(jnp.dot, preferred_element_type=f32)


def _dot_nt(a, b):
    return jax.lax.dot_general(a, b, (((1,), (1,)), ((), ())), preferred_element_type=f32)


def _vcat(*xs):
    return jnp.concatenate(xs, axis=0)


def _pad_rows(r):
    return _vcat(r, jnp.zeros((128 - r.shape[0], r.shape[1]), r.dtype))


def _add(x, y):
    return (x.astype(f32) + y.astype(f32)).astype(bf16)


def _sub(x, y):
    return (x.astype(f32) - y.astype(f32)).astype(bf16)


def _form(coefs, blocks):
    terms = [(c, blk) for c, blk in zip(coefs, blocks) if c != 0]
    if len(terms) == 1 and terms[0][0] == 1:
        return terms[0][1]()
    terms.sort(key=lambda cb: cb[0] < 0)
    out = None
    for c, blk in terms:
        v = blk().astype(f32)
        if out is None:
            out = v if c == 1 else v * c
        else:
            v = v if abs(c) == 1 else v * abs(c)
            out = out + v if c > 0 else out - v
    return out


def _lhs_slots_lanes(x1, x2):
    low = jax.lax.broadcasted_iota(jnp.int32, x1[0].shape, 1) < 64
    out = []
    for halves in SLOTS:
        keys = [(tuple(k // 128 for k in GROUP_ROWS[grp]), coefs) for grp, coefs, _ in halves]
        vals = [_form(coefs, [lambda x=x, g=g: x[g] for x in (x1, x2) for g in tiles])
                for tiles, coefs in keys]
        out.append(vals[0] if keys[0] == keys[1] else jnp.where(low, vals[0], vals[1]))
    return out


def _fast_product(p, ref, out):
    p0, p1, p2, p3 = p(0), p(1), p(2), p(3)
    r = p0 + p1 + p2
    ref[0] = r + p1 + p3
    ref[1] = r + p2
    yield
    p0, p1, p2, p3 = p(4), p(5), p(6), p(7)
    r = p0 + p1 + p2
    ref[2] = r + p1
    ref[3] = p3 - (r + p2)
    yield
    p0, p1, p2, p3 = p(8), p(9), p(10), p(11)
    r = p0 + p1
    c11 = ref[0] + (r + p3)
    ref[2] = ref[2] + (r + p1 + p2)
    ref[3] = ref[3] + p3
    yield
    p0, p1, p2, p3 = p(12), p(13), p(14), p(15)
    r = p0 + p1
    out.append((c11, (r + p2 + p3) - ref[1], ref[2] + p3, ref[3] + (r + p1)))
    yield


def _rhs_slot(s, get, zero=None):
    parts = []
    for grp, _, coefs in SLOTS[s]:
        k1, k2 = GROUP_ROWS[grp]
        blocks = [lambda k=k, c=c: get(slice(k, k + 64), c) for k in (k1, k2) for c in (0, 1)]
        parts.append(_form(coefs, blocks).astype(f32))
    if zero is not None:
        parts[0] = _vcat(parts[0][:8] + zero, parts[0][8:])
    return _vcat(*parts).astype(bf16)


def _signed(terms, get):
    return _form([t[0] for t in terms], [functools.partial(get, t[1], t[2]) for t in terms])


def _feed(outs, prods, ref, keep=()):
    vals = dict(prods)
    sums = {}
    for s in prods:
        for sign, i, n in PASSES[s][0]:
            sums.setdefault((i, n), {})[s] = sign
    while True:
        pairs = {}
        for terms in sums.values():
            keys = list(terms)
            for x in range(len(keys)):
                for y in range(x):
                    key = (keys[y], keys[x], terms[keys[x]] * terms[keys[y]])
                    pairs[key] = pairs.get(key, 0) + 1
        if not pairs or max(pairs.values()) < 2:
            break
        x, y, rel = max(pairs, key=pairs.get)
        vals[x, y] = vals[x] + vals[y] if rel > 0 else vals[x] - vals[y]
        for terms in sums.values():
            if x in terms and y in terms and terms[x] * terms[y] == rel:
                terms[x, y] = terms.pop(x)
                del terms[y]
    for blk, terms in sums.items():
        items = [(sign, vals[k]) for k, sign in terms.items()]
        sign, v = items[0]
        for s2, w in items[1:] + ([(outs[blk][0], ref[blk])] if blk in outs else []):
            v = v + w if s2 == sign else v - w
        outs[blk] = (sign, v)
        if blk not in keep:
            ref[blk] = v


def _packed(ref, *idx):
    return pltpu.bitcast(ref.bitcast(u32)[idx], bf16)


def _norm_stats(ref, total):
    m = jnp.broadcast_to(jnp.sum(total, axis=0, keepdims=True) * (1.0 / D), (8, 128))
    s = None
    for r in range(0, D, 8):
        c = ref[r:r + 8, :] - m
        s = c * c if s is None else s + c * c
    v = jnp.sum(s, axis=0, keepdims=True) * (1.0 / D)
    return m[0:1], jax.lax.rsqrt(v + EPS)


def _tile_sum(x, zero=None):
    rows = [x[r:r + 8] for r in range(0, D, 8)]
    return functools.reduce(jnp.add, rows[1:], rows[0] if zero is None else rows[0] + zero)


def _aligned(x, n):
    return x if isinstance(x, int) else pl.multiple_of(x, n)


def _drain(*gens):
    for gen in gens:
        for _ in gen:
            pass


def _weave(order, main, side):
    for c in order:
        next(main if c == "m" else side)
    _drain(main, side)


def _scope(name):
    import contextlib
    return jax.named_scope(name) if os.environ.get("SCOPES") else contextlib.nullcontext()


def _loop(n, fn):
    def body(i, c):
        with _scope("it"):
            fn(i)
        return c
    jax.lax.fori_loop(0, n, body, 0)


def _kernel(x_hbm, wqkv_hbm, wo_hbm, wg_hbm, wu_hbm, wd_hbm, out_hbm,
            xin, wqkv, wo, wg, wu, wd, wqkv_t, wo_t, wperm, operm, wt_s, pin0, pin1, pout, xres,
            q0, k0, v0, q_s, k_s, v_s, c_s, o_s, n_s, a_s, gu_s, h_s, acc, xn_s, sems):
    groups = (range(5), range(5, NCH))
    lane = jax.lax.broadcasted_iota(jnp.int32, (8, 128), 1)
    anchors, ticks = [], []
    pin = (pin0, pin1)

    def anchor(never, words):
        anchors.append(jnp.where(never, pltpu.bitcast(functools.reduce(jnp.bitwise_or, words), f32), 0.0))

    def x_copy(t):
        cols = pl.ds(t * TM, TM)
        return pltpu.make_async_copy(x_hbm.at[:, cols], xin.at[:, cols], sems.at[2 + t])

    def wqkv_copy(g):
        rows = pl.ds(g * 128, min(128, D - g * 128))
        return pltpu.make_async_copy(wqkv_hbm.at[rows], wqkv.at[rows], sems.at[5 + g])

    def out_copy(t, r0, r1):
        idx = (pl.ds(r0, r1 - r0), pl.ds(t * TM, TM))
        return pltpu.make_async_copy(xin.at[idx], out_hbm.at[idx], sems.at[t])

    def ffn_copies(g):
        return [pltpu.make_async_copy(src.at[:, pl.ds(j * FC, FC)], dst.at[j], sems.at[10 + g])
                for j in groups[g]
                for src, dst in ((wg_hbm, wg), (wu_hbm, wu), (wd_hbm, wd))]

    cwo = pltpu.make_async_copy(wo_hbm, wo, sems.at[4])
    x_copy(0).start()
    for gs in WG:
        for g in gs:
            wqkv_copy(g).start()

    def head_rows(ref, g, base):
        return _vcat(*[ref[g, pl.ds(base + d, 8, stride=DH), :] for d in range(DH)])

    def transpose_wqkv(g):
        rows = wqkv[g * 128:min((g + 1) * 128, D), :].astype(f32)
        wperm[g] = (_vcat(rows, rows) if g == 4 else rows).T

    def wqkv_slots(hg):
        base = pl.multiple_of(hg * GR, 16)
        src = base + (hg // 2) * HD
        for d in range(0, DH, 2):
            x1, x2 = [[_vcat(*[wperm[g, pl.ds(b + e, 8, stride=DH), :] for e in (d, d + 1)]) for g in range(5)]
                      for b in (src, src + HD)]
            for n, v in enumerate(_lhs_slots_lanes(x1, x2)):
                wqkv_t[n, pl.ds(base + 8 * d, 16), :] = v.astype(bf16)

    def widen_wo(i):
        rows = pl.ds(pl.multiple_of(i * (D // 3), 64), D // 3)
        for g in range(5):
            cols = wo[rows, g * 128:min((g + 1) * 128, D)].astype(f32)
            if g == 4:
                cols = jnp.concatenate([cols, jnp.zeros_like(cols)], axis=1)
            operm[g, rows, :] = cols

    def prep_wo(never):
        for g in range(5):
            r = _vcat(*[head_rows(operm, g, hg * GR) for hg in range(NG)])
            r = _vcat(r, r[512:D])
            tiles = [pltpu.bitcast(r[k * 128:(k + 1) * 128].astype(bf16).T, u32) for k in range(5)]
            for k, w in enumerate(tiles):
                wt_s[k, g * 64:(g + 1) * 64, :] = w
            anchor(never, [w[56:64] for w in tiles])
            yield
        for r in range(0, HD // 2, 8):
            zero = pltpu.bitcast(jnp.where(never, ticks.pop(0), 0.0), u32)
            x1, x2 = [[pltpu.bitcast(wt_s[k, r0:r0 + 8, :] | zero, bf16).astype(f32) for k in range(5)]
                      for r0 in (r, r + HD // 2)]
            for n, v in enumerate(_lhs_slots_lanes(x1, x2)):
                wo_t[n, 2 * r:2 * r + 16, :] = v.astype(bf16)
            yield

    def to_words(x):
        tiles = [x[g * 128:(g + 1) * 128] for g in range(4)] + [_pad_rows(x[512:D])]
        return [pltpu.bitcast(r.astype(bf16).T, u32) for r in tiles]

    def from_words(words):
        parts = [pltpu.bitcast(w, bf16).T for w in words]
        return _vcat(*parts[:4], parts[4][:64])

    def in_t1(t, c):
        x = xin[:, pl.ds(pl.multiple_of(t * TM + c * 128, 128), 128)]
        words = to_words(x)
        for g, w in enumerate(words):
            pin[t][g, pl.ds(pl.multiple_of(c * 64, 64), 64), :] = w
        return [w[56:64] for w in words]

    def in_t2(t, j):
        return from_words([pin[t][g, pl.ds(j, 64, stride=8), :] for g in range(5)]).astype(f32)

    def out_t1(j, x):
        words = to_words(x)
        for g, w in enumerate(words):
            pout[g, pl.ds(pl.multiple_of(j * 72, 8), 64), :] = w
        return [w[56:64] for w in words]

    def out_words(g, c):
        return _vcat(*[pout[g, pl.ds(c * 8 + m, 8, stride=72), :] for m in range(8)])

    def out_t2(c, dst):
        x = from_words([out_words(g, c) for g in range(5)])
        xin[:, pl.ds(pl.multiple_of(dst * 128, 128), 128)] = x
        return [pltpu.bitcast(x[r - 16:r], u32) for r in (128, 256, 384, 512, D)]

    def combine(t, i, never=None, r0=0, r1=QD):
        c, second = i % 2, i // 2
        pick = lambda lo, hi: lo + (hi - lo) * second
        outer = lambda m1, m2, m3, m4, m5, m6, m7: (
            m1 + m4 - m5 + m7, m2 + m4, m3 + m5, m1 - m2 + m3 + m6)
        strips, sums, link = [], [], None
        for r in range(r0, r1, 8):
            get = lambda n, m: acc[t, c, m, n * QD + r:n * QD + r + 8, :]
            four, two = [], []
            for n in range(7):
                x = get(n, pick(3, 2))
                if link is not None and n % CLINK == 0:
                    x = x + jnp.where(never, link, 0.0)
                four.append(((get(n, 0) + x) + get(n, pick(6, 5))) - get(n, pick(4, 1)))
                two.append(get(n, pick(1, 4)) + x)
                if never is not None:
                    link = four[-1]
            rows = []
            for u, v in zip(outer(*four), outer(*two)):
                if isinstance(second, int):
                    rows += [v, u] if second else [u, v]
                else:
                    rows += [jnp.where(second > 0, v, u), jnp.where(second > 0, u, v)]
            strips.append([xres[t, i + 4 * (q // 4), (q % 4) * QD + r:(q % 4) * QD + r + 8, :] + v
                           for q, v in enumerate(rows)])
            if never is not None:
                sums = [functools.reduce(jnp.add, sums[n:n + 1] + strips[-1][4 * n:4 * n + 4]) for n in (0, 1)]
                link = sums[0] + sums[1]
        return [_vcat(*[s[q] for q in range(q0, q0 + 4) for s in strips]) for q0 in (0, 4)] + sums

    def store_qkv(t, b, c1, c2, q, k, v, prev=None):
        part = [_vcat(c1[r:r + HD], c2[r:r + HD]) for r in range(0, HQ, HD)]
        q[b] = part[0].reshape(NG, DH, 8, 128)
        for n, (dst, r) in enumerate(((k, part[1]), (v, part[2]))):
            dst[b + NB] = r.reshape(NG, DH, 8, 128)
            sh = pltpu.roll(r, 2, 1).reshape(NG, DH, 8, 128)
            if isinstance(t, int) and t == 0:
                dst[b] = sh
            elif prev is not None:
                dst[b] = jnp.where((lane < 2)[None, None], prev[n][b], sh)
            else:
                keep = jnp.broadcast_to((lane >= 2 * t)[None, None], sh.shape)
                pltpu.store(dst.at[b], sh, mask=keep)

    def normalize(t, i, s1, s2, never):
        for c, s in enumerate((s1, s2)):
            if c and never is not None:
                s = s + jnp.where(never, r, 0.0)
            m, r = _norm_stats(xres.at[t, i + 4 * c], s)
            n_s[c] = (xres[t, i + 4 * c] - m) * r

    def phase1(t, i):
        never = lane < (i < 0).astype(jnp.int32)
        x1, x2, s1, s2 = combine(t, i, never)
        xres[t, i] = x1
        xres[t, i + 4] = x2
        normalize(t, i, s1, s2, never)
        yield
        rhs = lambda s: _rhs_slot(s, lambda rows, c: n_s[c, rows, :])
        out = []
        _drain(_fast_product(lambda s: _dot(_packed(wqkv_t, s), rhs(s)), c_s.at[:, 0:HQ], out))
        c = out[0]
        yield
        store_qkv(t, i, c[0], c[2], q_s, k_s, v_s)
        store_qkv(t, i + 4, c[1], c[3], q_s, k_s, v_s)
        yield

    def first_norm(t, i, dst, never=None):
        sums = []
        src = [xres.at[t, i + 4 * c] for c in (0, 1)]
        for c in (0, 1):
            x = in_t2(t, i + 4 * c)
            xres[t, i + 4 * c] = x
            sums.append(_tile_sum(x))
        if never is not None:
            anchors.append(jnp.where(never, sums[0] + sums[1], 0.0))
        yield
        stats = [_norm_stats(src[c], sums[c]) for c in (0, 1)]
        if never is not None:
            anchors.append(jnp.where(never, stats[0][1] + stats[1][1], 0.0))
        yield
        for s in range(NSLOT):
            mean = [st[0] for st in stats]
            if never is not None:
                zero = jnp.where(never, ticks.pop(0), 0.0)[0:1]
                mean = [m + zero for m in mean]
            dst[s] = _rhs_slot(s, lambda rows, c: (src[c][rows, :] - mean[c]) * stats[c][1])
            yield

    def first_qkv(t, i, src):
        def p(s):
            w = wqkv_t.bitcast(u32)[s, rows]
            while anchors:
                w = _vcat(w[:8] | pltpu.bitcast(anchors.pop(), u32), w[8:])
            v = _dot(pltpu.bitcast(w, bf16), _packed(src, s))
            if s % 4 == 0:
                ticks.extend(v[r:r + 8] for r in range(0, v.shape[0], TICK))
            return v

        cs = []
        for r0, r1 in ((HD, HQ), (0, HD)):
            rows = slice(r0 // 2, r1 // 2)
            yield from _fast_product(p, c_s.at[:, r0:r1], cs)
        c = [_vcat(x, y) for y, x in zip(*cs)]
        for n, b in enumerate((i, i + 4)):
            if t == 0:
                store_qkv(t, b, c[n], c[n + 2], q0, k0, v0)
            else:
                store_qkv(t, b, c[n], c[n + 2], q_s, k_s, v_s, prev=(k0, v0))

    def attention_group(t, b, g, q_r, k_r, v_r, links):
        par = len(links)
        never = lane < (b < 0).astype(jnp.int32)

        def start(n, v):
            if links[n % par] is None:
                return v
            return jnp.where(never, links[n % par], 0.0) + v

        q = [q_r[b, g, d] for d in range(DH)]
        logits = []
        for w in range(W):
            l = start(w, q[0] * k_r[b + NB - w, g, 0])
            for d in range(1, DH):
                l = l + q[d] * k_r[b + NB - w, g, d]
            links[w % par] = l
            l = l * (DH ** -0.5)
            if w > 0:
                edge = jnp.where(jnp.logical_and(w > b, t == 0), 2, 0)
                l = jnp.where(lane < edge, -1e9, l)
            logits.append(l)
        m = functools.reduce(jnp.maximum, logits)
        e = [jnp.exp(l - m) for l in logits]
        r = 1.0 / functools.reduce(jnp.add, e)
        p = [x * r for x in e]
        outs = []
        for d in range(DH):
            o = p[0] * v_r[b + NB, g, d]
            if d >= par:
                o = start(d, o)
            for w in range(1, W):
                o = o + p[w] * v_r[b + NB - w, g, d]
            links[d % par] = o
            outs.append(o)
        return _vcat(*outs)

    def attend(t, i, par, q_r, k_r, v_r):
        links = [None] * par
        never = lane < (i < 0).astype(jnp.int32)
        for c, b in enumerate((i, i + 4)):
            for g in range(NG):
                o_s[c, g * GR:(g + 1) * GR, :] = attention_group(t, b, g, q_r, k_r, v_r, links)
                anchors.append(jnp.where(never, functools.reduce(jnp.add, links), 0.0))
                yield
        p = lambda s: _dot(_packed(wo_t, s), _rhs_slot(s, lambda rows, c: o_s[c, rows, :]))
        out = []
        yield from _fast_product(p, c_s.at[:, HQ:HQ + HD], out)
        for n, b in enumerate((i, i + 4)):
            x = xres[t, b] + _vcat(out[0][n], out[0][n + 2])
            xres[t, b] = x
            c_s[n, HQ + HD:, :] = _tile_sum(x)
        yield

    def ffn_slots(t, i, never=None):
        normalize(t, i, c_s[0, HQ + HD:, :], c_s[1, HQ + HD:, :], never)
        yield
        rows = pl.ds(_aligned(i * 64, 64), 64)
        for s, (_, lo, _, hi, _) in enumerate(PASSES):
            op = _vcat(*[_signed(x, lambda r, k: n_s[r, 64 * k:64 * k + 64, :]) for x in (lo, hi)])
            if never is not None:
                op = _vcat(op[:8] + jnp.where(never, ticks.pop(0), 0.0), op[8:])
            a_s[t, s, rows, :] = pltpu.bitcast(op.astype(bf16).T, u32)
            yield

    def ffn_pass(t, w_ref, s):
        get = lambda k, n: w_ref[64 * k:64 * k + 64, 128 * n:128 * n + 128]
        parts = [_signed(x, get).astype(f32) for x in PASSES[s][2::2]]
        while anchors:
            parts[0] = _vcat(parts[0][:8] + anchors.pop(), parts[0][8:])
        return _dot(pltpu.bitcast(a_s[t, s], bf16), _vcat(*parts).astype(bf16))

    def ffn_chunk(t, j, may_init=False):
        lhs, g, u = {}, {}, {}
        todo = [(g, wg, s) for s in list(range(2, NPASS)) + [0, 1]] + [(u, wu, s) for s in range(NPASS)]
        for q in range(0, 2 * NPASS, 4):
            prods = [(outs, s, ffn_pass(t, w.at[j], s)) for outs, w, s in todo[q:q + 4]]
            k2 = {2 * NPASS - 12: 0, 2 * NPASS - 4: 1}.get(q)
            blks = [] if k2 is None else [(i, 2 * k + k2) for k in (0, 1) for i in (0, 1)]
            for n, outs in enumerate((g, u)):
                _feed(outs, {s: v for o, s, v in prods if o is outs}, gu_s.at[n], blks)
            if blks:
                hs = [gu_s[(0,) + b] * u[b][1] for b in blks]
                for n, (_, lb) in enumerate(STRASSEN):
                    coefs = [c * g[b][0] * u[b][0] for c, b in zip(lb, blks)]
                    h_s[n, k2] = _form(coefs, [lambda x=x: x for x in hs])
            yield
        order = [(n, m) for n in range(7) for m in (1, 5)] + [(n, m) for n in range(7) for m in (0, 2, 3, 4, 6)]
        for q, (n, m) in enumerate(order):
            rhs = [lambda k2=k2, c2=c2: h_s[n, k2, c2 * 256:(c2 + 1) * 256, :] for k2 in (0, 1) for c2 in (0, 1)]
            if q == 14:
                lhs.clear()
            if n not in lhs:
                lhs[n] = [_form(STRASSEN[n][0],
                                [lambda r=r, k=k, r2=r2, k2=k2: wd[j, pl.ds((2 * r + r2) * QD, QD),
                                                                   pl.ds((2 * k + k2) * 128, 128)]
                                 for r in (0, 1) for k in (0, 1)])
                          for r2 in (0, 1) for k2 in (0, 1)]
            left = _form(STRASSEN[m][0], [lambda x=x: x for x in lhs[n]])
            right = _form(STRASSEN[m][1], rhs).astype(bf16)
            if q == SPLITQ:
                v = _vcat(_dot_nt(left[:80].astype(bf16), right), _dot_nt(left[80:].astype(bf16), right))
            else:
                v = _dot_nt(left.astype(bf16), right)
            for c in range(2):
                old = acc[t, c, m, n * QD:(n + 1) * QD, :]
                if may_init:
                    old = jnp.where(j > 0, old, 0.0)
                acc[t, c, m, n * QD:(n + 1) * QD, :] = old + v[:, c * 128:(c + 1) * 128]
            ticks.append(v[0:8, 0:128])
            yield

    with _scope("w_x0"):
        x_copy(0).wait()
    for c in range(NB):
        in_t1(0, c)
    for gs in WG:
        with _scope("w_qkv"):
            for g in gs:
                wqkv_copy(g).wait()
        if gs == WG[0]:
            _drain(first_norm(0, 0, xn_s.at[0, 0]))
        if gs == WG[WX]:
            x_copy(1).start()
            cwo.start()
        for g in gs:
            transpose_wqkv(g)
    _loop(HQ // GR, wqkv_slots)
    with _scope("w_x1"):
        x_copy(1).wait()
    for g in range(len(groups)):
        for c in ffn_copies(g):
            c.start()
    for c in range(NB):
        in_t1(1, c)

    def run(order, gens):
        for c in order:
            if c == ".":
                ticks.clear()
            elif c == "!":
                anchors.clear()
            else:
                next(gens[c])
        _drain(*gens.values())

    def body_f(i, zero):
        never = lane < (i < 0).astype(jnp.int32)
        xn = xn_s.at[pl.ds(i, 2)]
        widen_wo(i)
        run(os.environ.get("OF0", "mamnamn."), {"m": first_qkv(0, i, xn.at[0, 0]), "a": first_norm(1, i, xn.at[0, 1], never),
                          "n": first_norm(0, i + 1, xn.at[1, 0], never)})
        return zero + (i < 0).astype(jnp.int32)

    with _scope("w_wo"):
        cwo.wait()
    never = lane < jax.lax.fori_loop(0, 3, body_f, 0)
    run(ORDER_F, {"m": first_qkv(0, 3, xn_s.at[3, 0]), "n": first_norm(1, 3, xn_s.at[3, 1], never),
                  "w": prep_wo(never)})
    _loop(4, lambda i: run(ORDER_E, {"m": first_qkv(1, i, xn_s.at[i, 1]), "s": attend(0, i, PAR0, q0, k0, v0),
                                     "f": ffn_slots(0, i)}))

    def wait_group(k, g):
        @pl.when(k == 0)
        def _():
            for c in ffn_copies(g):
                c.wait()

    def finish_step(i):
        u = i % 4
        never = lane < (i < 0).astype(jnp.int32)
        x1, x2 = combine(0, u, never)[:2]
        done = out_t1(u, x1) + out_t1(u + 4, x2)
        yield
        anchor(never, done)
        dst = 2 * u + (i // 8) * NB
        done = out_t2(2 * u, dst) + out_t2(2 * u + 1, dst + 1)
        yield
        anchor(never, done)
        yield

    def stage(k):
        t = k % 2
        n_a = jnp.where(jnp.logical_and(k > 0, k < 3), 4, 0)
        n_b = jnp.where(k < 3, 4, 0)
        n_c = NCH - n_a - n_b
        wait_group(k, 0)

        def body_c(i):
            pl.when(i == NCH - 1)(out_copy(0, 0, D).start)
            _weave(ORDER_C, ffn_chunk(t, i, True), finish_step(i))
        _loop(n_c, body_c)
        _loop(n_a, lambda i: _weave(ORDER_A, ffn_chunk(t, n_c + i), phase1(1 - t, i)))
        wait_group(k, 1)

        def body_b(i):
            run(ORDER_B, {"m": ffn_chunk(t, n_c + n_a + i), "s": attend(1 - t, i, PAR, q_s, k_s, v_s),
                          "f": ffn_slots(1 - t, i, lane < (i < 0).astype(jnp.int32))})
        _loop(n_b, body_b)
    _loop(4, stage)

    copies = [out_copy(0, 0, D)]
    for g in range(5):
        r0, r1 = 32 * g, min(32 * g + 32, QD)
        for i in (0, 2, 1, 3):
            for j, x in zip((i, i + 4), combine(1, i, None, r0, r1)):
                x = _pad_rows(x) if g == 4 else x
                pout[g, j * 72:j * 72 + 64, :] = pltpu.bitcast(x.astype(bf16).T, u32)
        for c in range(NB):
            x = pltpu.bitcast(out_words(g, c), bf16).T
            for q in range(4):
                xin[q * QD + r0:q * QD + r1, TM + c * 128:TM + (c + 1) * 128] = x[q * (r1 - r0):(q + 1) * (r1 - r0)]
        for q in range(4):
            copies.append(out_copy(1, q * QD + r0, q * QD + r1))
            copies[-1].start()
    with _scope("w_out"):
        for c in copies:
            c.wait()


@jax.jit
def pallas_interleave_layers__sliding_local_dilated__glu_gated_bilinear__prompt_kernel(
    A_x: jax.Array,
    A_wqkv: jax.Array,
    A_wo: jax.Array,
    B_x: jax.Array,
    B_w_gate: jax.Array,
    B_w_up: jax.Array,
    B_w_down: jax.Array,
):
    any_spec = pl.BlockSpec(memory_space=pl.ANY)
    qkv_scratch = [
        pltpu.VMEM((NB, NG, DH, 8, 128), f32),
        pltpu.VMEM((2 * NB, NG, DH, 8, 128), f32),
        pltpu.VMEM((2 * NB, NG, DH, 8, 128), f32),
    ]
    out_t = pl.pallas_call(
        _kernel,
        in_specs=[any_spec] * 6,
        out_specs=any_spec,
        out_shape=jax.ShapeDtypeStruct((D, S), bf16),
        scratch_shapes=[
            pltpu.VMEM((D, S), bf16),
            pltpu.VMEM((D, 3 * D), bf16),
            pltpu.VMEM((D, D), bf16),
            pltpu.VMEM((NCH, D, FC), bf16),
            pltpu.VMEM((NCH, D, FC), bf16),
            pltpu.VMEM((NCH, D, FC), bf16),
            pltpu.VMEM((NSLOT, HQ, 128), bf16),
            pltpu.VMEM((NSLOT, HD, 128), bf16),
            pltpu.VMEM((5, 3 * D, 128), f32),
            pltpu.VMEM((5, D, 128), f32),
            pltpu.VMEM((5, 320, 128), u32),
            pltpu.VMEM((5, HM, 128), u32),
            pltpu.VMEM((5, HM, 128), u32),
            pltpu.VMEM((5, 8 * 72, 128), u32),
            pltpu.VMEM((2, NB, D, 128), f32),
            *qkv_scratch,
            *qkv_scratch,
            pltpu.VMEM((4, HQ + HD + 8, 128), f32),
            pltpu.VMEM((2, D, 128), f32),
            pltpu.VMEM((2, D, 128), f32),
            pltpu.VMEM((2, NPASS, HM // 2, 128), u32),
            pltpu.VMEM((2, 2, 4, HM, 128), f32),
            pltpu.VMEM((7, 2, HM, 128), f32),
            pltpu.VMEM((2, 2, 7, 1024, 128), f32),
            pltpu.VMEM((4, 2, NSLOT, 128, 128), bf16),
            pltpu.SemaphoreType.DMA((12,)),
        ],
        compiler_params=pltpu.CompilerParams(vmem_limit_bytes=120 * 1024 * 1024),
        name="fused_layers",
    )(A_x[0].T, A_wqkv, A_wo, B_w_gate, B_w_up, B_w_down.T)
    return out_t.T[None]
```

```python
import functools
import os

import jax
import jax.numpy as jnp
import jax.experimental.pallas as pl
import jax.experimental.pallas.tpu as pltpu

S, D, F = 2048, 576, 4608
H, DH, W = 32, 18, 8
NG = H // 8
GR = 8 * DH
NB = 8
TM = NB * 128
HM = TM // 2
HD = D // 2
HQ = 3 * D // 2
FC = 512
HC = FC // 2
NCH = F // FC
NSLOT = 16
NT = int(os.environ.get("NT", 128))

GROUP_ROWS = {1: (0, 128), 2: (64, 192), 4: (256, 384), 3: (320, 448), 0: (512, 512)}
T3 = 1.0 / 3.0
SLOTS = (
    ((1, (-1, -1, 0, 0), (0, 0, 0, 1)), (3, (1, 1, 0, 0), (0, 0, 1, 0))),
    ((0, (T3, 0, 0, 0), (2, 1, 0, 0)), (2, (-.5, -1, 0, 0), (0, 0, 0, 1))),
    ((4, (.5, 1, 0, 0), (0, 0, 1, 0)), (0, (-T3, 0, 0, 0), (1, 2, 0, 0))),
    ((1, (0, 1, 0, -1), (0, 0, 1, 1)), (2, (0, 2, 0, -1), (0, 0, .5, 1))),
    ((1, (0, 0, 1, 1), (1, 0, 0, 0)), (3, (0, 0, -1, -1), (0, 1, 0, 0))),
    ((0, (0, 0, T3, 0), (2, 1, 0, 0)), (2, (0, 0, .5, 1), (1, 0, 0, 0))),
    ((4, (0, 0, -.5, -1), (0, 1, 0, 0)), (0, (0, 0, -T3, 0), (1, 2, 0, 0))),
    ((1, (-1, 0, 1, 0), (1, 1, 0, 0)), (2, (-1, 0, .5, 0), (1, 2, 0, 0))),
    ((1, (0, 0, 0, 1), (-1, 0, 1, 0)), (3, (1, 0, 0, 0), (1, 0, -1, 0))),
    ((4, (.5, 0, 0, 0), (2, 0, -1, 0)), (2, (0, 0, 0, 1), (-1, 0, .5, 0))),
    ((4, (-1, 0, .5, 0), (2, 1, 0, 0)), (3, (-1, 0, 1, 0), (1, 1, 0, 0))),
    ((1, (1, 0, 0, 1), (1, 0, 0, 1)), (2, (1, 0, 0, 1), (1, 0, 0, 1))),
    ((1, (1, 0, 0, 0), (0, 1, 0, -1)), (3, (0, 0, 0, 1), (0, -1, 0, 1))),
    ((4, (0, 0, 0, 1), (0, -1, 0, .5)), (2, (.5, 0, 0, 0), (0, 2, 0, -1))),
    ((4, (0, 2, 0, -1), (0, 0, 1, .5)), (3, (0, 1, 0, -1), (0, 0, 1, 1))),
    ((4, (1, 0, 0, 1), (0, 1, 1, 0)), (3, (1, 0, 0, 1), (0, 1, 1, 0))),
)
_PASSES = (
    ("+01 +10", "-04 +14 +17", "-41 -43 +70 +71 +73", "-05 +15 +16", "-51 +60 +61 +62"),
    ("+10", "-04 +14", "+40 +41 -42 +43 -70 -71 -73", "-05 +15", "+50 +51 -52 -60 -61 -62"),
    ("+02 -03", "+00 -02", "+21 +23", "+01 -03", "+31 +33"),
    ("+00 -02 +03", "+00 +08", "+81 +83", "+01 +06", "-53 +63"),
    ("+01 +02 -03", "+02 -08", "+21", "+03 -07", "+31"),
    ("+00 -01", "+06", "+60 +62", "+07", "+70"),
    ("+10 -12 +13", "+10 +18", "+00", "+11 +16", "+10"),
    ("+12 -13", "+10 -12", "+00 +02", "+11 -13", "+10 +12"),
    ("-11 -12 +13", "+12 -18", "+80 +82", "+13 -17", "+72"),
    ("+10 +12", "-12 +14", "+42", "-13 +15", "+52"),
    ("-00 +02 +13", "+00 +18", "-00 +81 +83", "+01 +16", "-10 -53 +63"),
    ("+00 -02", "+06 -16", "+53 -62 -63", "+08 -18", "+80 -81 -83"),
    ("+00 +02", "+02 -04", "+20", "+03 -05", "+30"),
    ("+02", "+02 -12", "-20 +22 +23", "+03 -13", "-30 +32 +33"),
    ("+11 -13", "-08 +18", "-80 +81 -82", "-07 +17", "+43 -72 -73"),
    ("+02 -11 +13", "+08 -12", "+21 +80 +82", "+07 -13", "+31 +72"),
    ("+02 +13", "+00 -12", "+00 +02 -21 -23", "+01 -13", "+10 +12 -31 -33"),
    ("+10 -11", "+16", "+51 -61", "+17", "+41 +43 -71 -73"),
    ("+02 +12", "+12", "+00 +02 +22 +42 +80 +82", "+13", "+10 +12 +32 +52 +72"),
    ("+00 +10", "+04", "+20 +40", "+05", "+30 +50"),
    ("-00 +02 -10 +12", "+16", "+10 +62", "+18", "+00 -80"),
    ("+02 -10", "+04 -12", "+20 +42", "+05 -13", "+30 +52"),
    ("+03 +13", "+00", "+03 +21 +23 -43 -81 -83", "+01", "+13 +31 +33 -63"),
    ("+13", "-00 +10", "+01 +02 +03", "-01 +11", "+11 +12 +13"),
    ("-01 +03", "+00 +04 +07", "+43", "+01 +05 +06", "+53"),
    ("+01", "+04 +07 -14 -17", "+70 +71 +73", "+05 +06 -15 -16", "+53 +60 +61 +62"),
    ("+01 +11", "+14 +17", "-01 +41", "+15 +16", "-11 +51"),
    ("+11 -13", "+10 +14 +17", "+01", "+11 +15 +16", "+11"),
    ("+01 +13", "+00 +14 +17", "+01 +43", "+01 +15 +16", "+11 +53"),
    ("+01 -03 +11 -13", "+08", "+21 +81", "+07", "+31 +43 -73"),
)
PASSES = [[[(int(w[0] + "1"), int(w[1]), int(w[2])) for w in col.split()] for col in row] for row in _PASSES]
NPASS = len(PASSES)
STRASSEN = (
    ((1, 0, 0, 1), (1, 0, 0, 1)),
    ((0, 0, 1, 1), (1, 0, 0, 0)),
    ((1, 0, 0, 0), (0, 1, 0, -1)),
    ((0, 0, 0, 1), (-1, 0, 1, 0)),
    ((1, 1, 0, 0), (0, 0, 0, 1)),
    ((-1, 0, 1, 0), (1, 1, 0, 0)),
    ((0, 1, 0, -1), (0, 0, 1, 1)),
)
QD = D // 4
EPS = 1e-5
WG = [[int(c) for c in x] for x in os.environ.get("WG", "40,1,2,3").split(",")]
TICK = int(os.environ.get("TICK", 40))
ORDER_F = os.environ.get("OF", "mnwmwwnmww.")
WX = int(os.environ.get("WX", 0))
SPLITQ = int(os.environ.get("SPLITQ", 48))
CLINK = int(os.environ.get("CLINK", 1))
KA = int(os.environ.get("KA", 11))
KB = int(os.environ.get("KB", 9))
PAR = int(os.environ.get("PAR", 2))
PAR0 = int(os.environ.get("PAR0", 3))
CSEG = int(os.environ.get("CSEG", 3))
ORDER_A = os.environ.get("OA", "sssssss!mmmmmmmmmmmss")
KB0 = int(os.environ.get("KB0", 1))
ORDER_B = "m" * KB0 + "sm" * 8 + "m" * (KB - KB0 - 8) + "sssssf" + "m" * (15 - KB + int(os.environ.get("KB2", 6))) + "."
ORDER_C = os.environ.get("OC", "msmsmsmsmsmsmsmmsmms")
ORDER_E = os.environ.get("OE", "ssssssss!mmmmsssssf")
f32, bf16, u32 = jnp.float32, jnp.bfloat16, jnp.uint32

_dot = functools.partial(jnp.dot, preferred_element_type=f32)


def _dot_nt(a, b):
    return jax.lax.dot_general(a, b, (((1,), (1,)), ((), ())), preferred_element_type=f32)


def _vcat(*xs):
    return jnp.concatenate(xs, axis=0)


def _pad_rows(r):
    return _vcat(r, jnp.zeros((128 - r.shape[0], r.shape[1]), r.dtype))


def _add(x, y):
    return (x.astype(f32) + y.astype(f32)).astype(bf16)


def _sub(x, y):
    return (x.astype(f32) - y.astype(f32)).astype(bf16)


def _form(coefs, blocks):
    terms = [(c, blk) for c, blk in zip(coefs, blocks) if c != 0]
    if len(terms) == 1 and terms[0][0] == 1:
        return terms[0][1]()
    terms.sort(key=lambda cb: cb[0] < 0)
    out = None
    for c, blk in terms:
        v = blk().astype(f32)
        if out is None:
            out = v if c == 1 else v * c
        else:
            v = v if abs(c) == 1 else v * abs(c)
            out = out + v if c > 0 else out - v
    return out


def _lhs_slots_lanes(x1, x2):
    low = jax.lax.broadcasted_iota(jnp.int32, x1[0].shape, 1) < 64
    out = []
    for halves in SLOTS:
        keys = [(tuple(k // 128 for k in GROUP_ROWS[grp]), coefs) for grp, coefs, _ in halves]
        vals = [_form(coefs, [lambda x=x, g=g: x[g] for x in (x1, x2) for g in tiles])
                for tiles, coefs in keys]
        out.append(vals[0] if keys[0] == keys[1] else jnp.where(low, vals[0], vals[1]))
    return out


def _fast_product(p, ref, out):
    p0, p1, p2, p3 = p(0), p(1), p(2), p(3)
    r = p0 + p1 + p2
    ref[0] = r + p1 + p3
    ref[1] = r + p2
    yield
    p0, p1, p2, p3 = p(4), p(5), p(6), p(7)
    r = p0 + p1 + p2
    ref[2] = r + p1
    ref[3] = p3 - (r + p2)
    yield
    p0, p1, p2, p3 = p(8), p(9), p(10), p(11)
    r = p0 + p1
    c11 = ref[0] + (r + p3)
    ref[2] = ref[2] + (r + p1 + p2)
    ref[3] = ref[3] + p3
    yield
    p0, p1, p2, p3 = p(12), p(13), p(14), p(15)
    r = p0 + p1
    out.append((c11, (r + p2 + p3) - ref[1], ref[2] + p3, ref[3] + (r + p1)))
    yield


def _rhs_slot(s, get, zero=None):
    parts = []
    for grp, _, coefs in SLOTS[s]:
        k1, k2 = GROUP_ROWS[grp]
        blocks = [lambda k=k, c=c: get(slice(k, k + 64), c) for k in (k1, k2) for c in (0, 1)]
        parts.append(_form(coefs, blocks).astype(f32))
    if zero is not None:
        parts[0] = _vcat(parts[0][:8] + zero, parts[0][8:])
    return _vcat(*parts).astype(bf16)


def _signed(terms, get):
    return _form([t[0] for t in terms], [functools.partial(get, t[1], t[2]) for t in terms])


def _feed(outs, prods, ref, keep=()):
    vals = dict(prods)
    sums = {}
    for s in prods:
        for sign, i, n in PASSES[s][0]:
            sums.setdefault((i, n), {})[s] = sign
    while True:
        pairs = {}
        for terms in sums.values():
            keys = list(terms)
            for x in range(len(keys)):
                for y in range(x):
                    key = (keys[y], keys[x], terms[keys[x]] * terms[keys[y]])
                    pairs[key] = pairs.get(key, 0) + 1
        if not pairs or max(pairs.values()) < 2:
            break
        x, y, rel = max(pairs, key=pairs.get)
        vals[x, y] = vals[x] + vals[y] if rel > 0 else vals[x] - vals[y]
        for terms in sums.values():
            if x in terms and y in terms and terms[x] * terms[y] == rel:
                terms[x, y] = terms.pop(x)
                del terms[y]
    for blk, terms in sums.items():
        items = [(sign, vals[k]) for k, sign in terms.items()]
        sign, v = items[0]
        for s2, w in items[1:] + ([(outs[blk][0], ref[blk])] if blk in outs else []):
            v = v + w if s2 == sign else v - w
        outs[blk] = (sign, v)
        if blk not in keep:
            ref[blk] = v


def _packed(ref, *idx):
    return pltpu.bitcast(ref.bitcast(u32)[idx], bf16)


def _norm_stats(ref, total):
    m = jnp.broadcast_to(jnp.sum(total, axis=0, keepdims=True) * (1.0 / D), (8, 128))
    s = None
    for r in range(0, D, 8):
        c = ref[r:r + 8, :] - m
        s = c * c if s is None else s + c * c
    v = jnp.sum(s, axis=0, keepdims=True) * (1.0 / D)
    return m[0:1], jax.lax.rsqrt(v + EPS)


def _tile_sum(x, zero=None):
    rows = [x[r:r + 8] for r in range(0, D, 8)]
    return functools.reduce(jnp.add, rows[1:], rows[0] if zero is None else rows[0] + zero)


def _aligned(x, n):
    return x if isinstance(x, int) else pl.multiple_of(x, n)


def _drain(*gens):
    for gen in gens:
        for _ in gen:
            pass


def _scope(name):
    import contextlib
    return jax.named_scope(name) if os.environ.get("SCOPES") else contextlib.nullcontext()


def _loop(n, fn):
    def body(i, c):
        with _scope("it"):
            fn(i)
        return c
    jax.lax.fori_loop(0, n, body, 0)


def _kernel(x_hbm, wqkv_hbm, wo_hbm, wg_hbm, wu_hbm, wd_hbm, out_hbm,
            xin, wqkv, wo, wg, wu, wd, wqkv_t, wo_t, wperm, operm, wt_s, pin0, pin1, pout, xres,
            q0, k0, v0, q_s, k_s, v_s, c_s, o_s, n_s, a_s, gu_s, h_s, acc, xn_s, sems):
    groups = (range(5), range(5, NCH))
    lane = jax.lax.broadcasted_iota(jnp.int32, (8, 128), 1)
    anchors, ticks = [], []
    pin = (pin0, pin1)

    def anchor(never, words):
        anchors.append(jnp.where(never, pltpu.bitcast(functools.reduce(jnp.bitwise_or, words), f32), 0.0))

    def x_copy(t):
        cols = pl.ds(t * TM, TM)
        return pltpu.make_async_copy(x_hbm.at[:, cols], xin.at[:, cols], sems.at[2 + t])

    def wqkv_copy(g):
        rows = pl.ds(g * 128, min(128, D - g * 128))
        return pltpu.make_async_copy(wqkv_hbm.at[rows], wqkv.at[rows], sems.at[5 + g])

    def out_copy(t, r0, r1):
        idx = (pl.ds(r0, r1 - r0), pl.ds(t * TM, TM))
        return pltpu.make_async_copy(xin.at[idx], out_hbm.at[idx], sems.at[t])

    def ffn_copies(g):
        return [pltpu.make_async_copy(src.at[:, pl.ds(j * FC, FC)], dst.at[j], sems.at[10 + g])
                for j in groups[g]
                for src, dst in ((wg_hbm, wg), (wu_hbm, wu), (wd_hbm, wd))]

    cwo = pltpu.make_async_copy(wo_hbm, wo, sems.at[4])
    x_copy(0).start()
    for gs in WG:
        for g in gs:
            wqkv_copy(g).start()

    def head_rows(ref, g, base):
        return _vcat(*[ref[g, pl.ds(base + d, 8, stride=DH), :] for d in range(DH)])

    def transpose_wqkv(g):
        rows = wqkv[g * 128:min((g + 1) * 128, D), :].astype(f32)
        wperm[g] = (_vcat(rows, rows) if g == 4 else rows).T

    def wqkv_slots(hg):
        base = pl.multiple_of(hg * GR, 16)
        src = base + (hg // 2) * HD
        for d in range(0, DH, 2):
            x1, x2 = [[_vcat(*[wperm[g, pl.ds(b + e, 8, stride=DH), :] for e in (d, d + 1)]) for g in range(5)]
                      for b in (src, src + HD)]
            for n, v in enumerate(_lhs_slots_lanes(x1, x2)):
                wqkv_t[n, pl.ds(base + 8 * d, 16), :] = v.astype(bf16)

    def widen_wo(i):
        rows = pl.ds(pl.multiple_of(i * (D // 3), 64), D // 3)
        for g in range(5):
            cols = wo[rows, g * 128:min((g + 1) * 128, D)].astype(f32)
            if g == 4:
                cols = jnp.concatenate([cols, jnp.zeros_like(cols)], axis=1)
            operm[g, rows, :] = cols

    def prep_wo(never):
        for g in range(5):
            r = _vcat(*[head_rows(operm, g, hg * GR) for hg in range(NG)])
            r = _vcat(r, r[512:D])
            tiles = [pltpu.bitcast(r[k * 128:(k + 1) * 128].astype(bf16).T, u32) for k in range(5)]
            for k, w in enumerate(tiles):
                wt_s[k, g * 64:(g + 1) * 64, :] = w
            anchor(never, [w[56:64] for w in tiles])
            yield
        for r in range(0, HD // 2, 8):
            zero = pltpu.bitcast(jnp.where(never, ticks.pop(0), 0.0), u32)
            x1, x2 = [[pltpu.bitcast(wt_s[k, r0:r0 + 8, :] | zero, bf16).astype(f32) for k in range(5)]
                      for r0 in (r, r + HD // 2)]
            for n, v in enumerate(_lhs_slots_lanes(x1, x2)):
                wo_t[n, 2 * r:2 * r + 16, :] = v.astype(bf16)
            yield

    def to_words(x):
        tiles = [x[g * 128:(g + 1) * 128] for g in range(4)] + [_pad_rows(x[512:D])]
        return [pltpu.bitcast(r.astype(bf16).T, u32) for r in tiles]

    def from_words(words):
        parts = [pltpu.bitcast(w, bf16).T for w in words]
        return _vcat(*parts[:4], parts[4][:64])

    def in_t1(t, c):
        x = xin[:, pl.ds(pl.multiple_of(t * TM + c * 128, 128), 128)]
        words = to_words(x)
        for g, w in enumerate(words):
            pin[t][g, pl.ds(pl.multiple_of(c * 64, 64), 64), :] = w
        return [w[56:64] for w in words]

    def in_t2(t, j):
        return from_words([pin[t][g, pl.ds(j, 64, stride=8), :] for g in range(5)]).astype(f32)

    def out_t1(j, x):
        words = to_words(x)
        for g, w in enumerate(words):
            pout[g, pl.ds(pl.multiple_of(j * 72, 8), 64), :] = w
        return [w[56:64] for w in words]

    def out_words(g, c):
        return _vcat(*[pout[g, pl.ds(c * 8 + m, 8, stride=72), :] for m in range(8)])

    def out_t2(c, dst):
        x = from_words([out_words(g, c) for g in range(5)])
        xin[:, pl.ds(pl.multiple_of(dst * 128, 128), 128)] = x
        return [pltpu.bitcast(x[r - 16:r], u32) for r in (128, 256, 384, 512, D)]

    def combine(t, i, never=None, r0=0, r1=QD):
        c, second = i % 2, i // 2
        pick = lambda lo, hi: lo + (hi - lo) * second
        outer = lambda m1, m2, m3, m4, m5, m6, m7: (
            m1 + m4 - m5 + m7, m2 + m4, m3 + m5, m1 - m2 + m3 + m6)
        strips, sums, link = [], [], None
        for r in range(r0, r1, 8):
            get = lambda n, m: acc[t, c, m, n * QD + r:n * QD + r + 8, :]
            four, two = [], []
            for n in range(7):
                x = get(n, pick(3, 2))
                if link is not None and n % CLINK == 0:
                    x = x + jnp.where(never, link, 0.0)
                four.append(((get(n, 0) + x) + get(n, pick(6, 5))) - get(n, pick(4, 1)))
                two.append(get(n, pick(1, 4)) + x)
                if never is not None:
                    link = four[-1]
            rows = []
            for u, v in zip(outer(*four), outer(*two)):
                if isinstance(second, int):
                    rows += [v, u] if second else [u, v]
                else:
                    rows += [jnp.where(second > 0, v, u), jnp.where(second > 0, u, v)]
            strips.append([xres[t, i + 4 * (q // 4), (q % 4) * QD + r:(q % 4) * QD + r + 8, :] + v
                           for q, v in enumerate(rows)])
            if never is not None:
                sums = [functools.reduce(jnp.add, sums[n:n + 1] + strips[-1][4 * n:4 * n + 4]) for n in (0, 1)]
                link = sums[0] + sums[1]
                if len(strips) % CSEG == 0:
                    anchors.append(jnp.where(never, link, 0.0))
                    yield
        return [_vcat(*[s[q] for q in range(q0, q0 + 4) for s in strips]) for q0 in (0, 4)] + sums

    def store_qkv(t, b, c1, c2, q, k, v, prev=None):
        part = [_vcat(c1[r:r + HD], c2[r:r + HD]) for r in range(0, HQ, HD)]
        q[b] = part[0].reshape(NG, DH, 8, 128)
        for n, (dst, r) in enumerate(((k, part[1]), (v, part[2]))):
            dst[b + NB] = r.reshape(NG, DH, 8, 128)
            sh = pltpu.roll(r, 2, 1).reshape(NG, DH, 8, 128)
            if isinstance(t, int) and t == 0:
                dst[b] = sh
            elif prev is not None:
                dst[b] = jnp.where((lane < 2)[None, None], prev[n][b], sh)
            else:
                keep = jnp.broadcast_to((lane >= 2 * t)[None, None], sh.shape)
                pltpu.store(dst.at[b], sh, mask=keep)

    def normalize(t, i, s1, s2, never):
        for c, s in enumerate((s1, s2)):
            if c and never is not None:
                s = s + jnp.where(never, r, 0.0)
            m, r = _norm_stats(xres.at[t, i + 4 * c], s)
            n_s[c] = (xres[t, i + 4 * c] - m) * r

    def phase1(t, i):
        never = lane < (i < 0).astype(jnp.int32)
        x1, x2, s1, s2 = yield from combine(t, i, never)
        xres[t, i] = x1
        xres[t, i + 4] = x2
        normalize(t, i, s1, s2, never)
        yield
        rhs = lambda s: _rhs_slot(s, lambda rows, c: n_s[c, rows, :])
        out = []
        _drain(_fast_product(lambda s: _dot(_packed(wqkv_t, s), rhs(s)), c_s.at[:, 0:HQ], out))
        c = out[0]
        yield
        store_qkv(t, i, c[0], c[2], q_s, k_s, v_s)
        store_qkv(t, i + 4, c[1], c[3], q_s, k_s, v_s)
        yield

    def first_norm(t, i, dst, never=None):
        sums = []
        src = [xres.at[t, i + 4 * c] for c in (0, 1)]
        for c in (0, 1):
            x = in_t2(t, i + 4 * c)
            xres[t, i + 4 * c] = x
            sums.append(_tile_sum(x))
        if never is not None:
            anchors.append(jnp.where(never, sums[0] + sums[1], 0.0))
        yield
        stats = [_norm_stats(src[c], sums[c]) for c in (0, 1)]
        if never is not None:
            anchors.append(jnp.where(never, stats[0][1] + stats[1][1], 0.0))
        yield
        for s in range(NSLOT):
            mean = [st[0] for st in stats]
            if never is not None:
                zero = jnp.where(never, ticks.pop(0), 0.0)[0:1]
                mean = [m + zero for m in mean]
            dst[s] = _rhs_slot(s, lambda rows, c: (src[c][rows, :] - mean[c]) * stats[c][1])
            yield

    def first_qkv(t, i, src):
        def p(s):
            w = wqkv_t.bitcast(u32)[s, rows]
            while anchors:
                w = _vcat(w[:8] | pltpu.bitcast(anchors.pop(), u32), w[8:])
            v = _dot(pltpu.bitcast(w, bf16), _packed(src, s))
            if s % 4 == 0:
                ticks.extend(v[r:r + 8] for r in range(0, v.shape[0], TICK))
            return v

        cs = []
        for r0, r1 in ((HD, HQ), (0, HD)):
            rows = slice(r0 // 2, r1 // 2)
            yield from _fast_product(p, c_s.at[:, r0:r1], cs)
        c = [_vcat(x, y) for y, x in zip(*cs)]
        for n, b in enumerate((i, i + 4)):
            if t == 0:
                store_qkv(t, b, c[n], c[n + 2], q0, k0, v0)
            else:
                store_qkv(t, b, c[n], c[n + 2], q_s, k_s, v_s, prev=(k0, v0))

    def attention_group(t, b, g, q_r, k_r, v_r, links):
        par = len(links)
        never = lane < (b < 0).astype(jnp.int32)

        def start(n, v):
            if links[n % par] is None:
                return v
            return jnp.where(never, links[n % par], 0.0) + v

        q = [q_r[b, g, d] for d in range(DH)]
        logits = []
        for w in range(W):
            l = start(w, q[0] * k_r[b + NB - w, g, 0])
            for d in range(1, DH):
                l = l + q[d] * k_r[b + NB - w, g, d]
            links[w % par] = l
            l = l * (DH ** -0.5)
            if w > 0:
                edge = jnp.where(jnp.logical_and(w > b, t == 0), 2, 0)
                l = jnp.where(lane < edge, -1e9, l)
            logits.append(l)
        m = functools.reduce(jnp.maximum, logits)
        e = [jnp.exp(l - m) for l in logits]
        r = 1.0 / functools.reduce(jnp.add, e)
        p = [x * r for x in e]
        outs = []
        for d in range(DH):
            o = p[0] * v_r[b + NB, g, d]
            if d >= par:
                o = start(d, o)
            for w in range(1, W):
                o = o + p[w] * v_r[b + NB - w, g, d]
            links[d % par] = o
            outs.append(o)
        return _vcat(*outs)

    def attend(t, i, par, q_r, k_r, v_r):
        links = [None] * par
        never = lane < (i < 0).astype(jnp.int32)
        for c, b in enumerate((i, i + 4)):
            for g in range(NG):
                o_s[c, g * GR:(g + 1) * GR, :] = attention_group(t, b, g, q_r, k_r, v_r, links)
                anchors.append(jnp.where(never, functools.reduce(jnp.add, links), 0.0))
                yield
        p = lambda s: _dot(_packed(wo_t, s), _rhs_slot(s, lambda rows, c: o_s[c, rows, :]))
        out = []
        yield from _fast_product(p, c_s.at[:, HQ:HQ + HD], out)
        for n, b in enumerate((i, i + 4)):
            x = xres[t, b] + _vcat(out[0][n], out[0][n + 2])
            xres[t, b] = x
            c_s[n, HQ + HD:, :] = _tile_sum(x)
        yield

    def ffn_slots(t, i, never=None):
        normalize(t, i, c_s[0, HQ + HD:, :], c_s[1, HQ + HD:, :], never)
        yield
        rows = pl.ds(_aligned(i * 64, 64), 64)
        for s, (_, lo, _, hi, _) in enumerate(PASSES):
            op = _vcat(*[_signed(x, lambda r, k: n_s[r, 64 * k:64 * k + 64, :]) for x in (lo, hi)])
            if never is not None:
                op = _vcat(op[:8] + jnp.where(never, ticks.pop(0), 0.0), op[8:])
            a_s[t, s, rows, :] = pltpu.bitcast(op.astype(bf16).T, u32)
            yield

    def ffn_pass(t, w_ref, s):
        get = lambda k, n: w_ref[64 * k:64 * k + 64, 128 * n:128 * n + 128]
        parts = [_signed(x, get).astype(f32) for x in PASSES[s][2::2]]
        while anchors:
            parts[0] = _vcat(parts[0][:8] + anchors.pop(), parts[0][8:])
        return _dot(pltpu.bitcast(a_s[t, s], bf16), _vcat(*parts).astype(bf16))

    def ffn_chunk(t, j, may_init=False):
        lhs, g, u = {}, {}, {}
        todo = [(g, wg, s) for s in list(range(2, NPASS)) + [0, 1]] + [(u, wu, s) for s in range(NPASS)]
        for q in range(0, 2 * NPASS, 4):
            prods = [(outs, s, ffn_pass(t, w.at[j], s)) for outs, w, s in todo[q:q + 4]]
            k2 = {2 * NPASS - 12: 0, 2 * NPASS - 4: 1}.get(q)
            blks = [] if k2 is None else [(i, 2 * k + k2) for k in (0, 1) for i in (0, 1)]
            for n, outs in enumerate((g, u)):
                _feed(outs, {s: v for o, s, v in prods if o is outs}, gu_s.at[n], blks)
            if blks:
                hs = [gu_s[(0,) + b] * u[b][1] for b in blks]
                for n, (_, lb) in enumerate(STRASSEN):
                    coefs = [c * g[b][0] * u[b][0] for c, b in zip(lb, blks)]
                    h_s[n, k2] = _form(coefs, [lambda x=x: x for x in hs])
            yield
        order = [(n, m) for n in range(7) for m in (1, 5)] + [(n, m) for n in range(7) for m in (0, 2, 3, 4, 6)]
        for q, (n, m) in enumerate(order):
            rhs = [lambda k2=k2, c2=c2: h_s[n, k2, c2 * 256:(c2 + 1) * 256, :] for k2 in (0, 1) for c2 in (0, 1)]
            if q == 14:
                lhs.clear()
            if n not in lhs:
                lhs[n] = [_form(STRASSEN[n][0],
                                [lambda r=r, k=k, r2=r2, k2=k2: wd[j, pl.ds((2 * r + r2) * QD, QD),
                                                                   pl.ds((2 * k + k2) * 128, 128)]
                                 for r in (0, 1) for k in (0, 1)])
                          for r2 in (0, 1) for k2 in (0, 1)]
            left = _form(STRASSEN[m][0], [lambda x=x: x for x in lhs[n]])
            right = _form(STRASSEN[m][1], rhs).astype(bf16)
            if q == SPLITQ:
                v = _vcat(_dot_nt(left[:80].astype(bf16), right), _dot_nt(left[80:].astype(bf16), right))
            else:
                v = _dot_nt(left.astype(bf16), right)
            for c in range(2):
                old = acc[t, c, m, n * QD:(n + 1) * QD, :]
                if may_init:
                    old = jnp.where(j > 0, old, 0.0)
                acc[t, c, m, n * QD:(n + 1) * QD, :] = old + v[:, c * 128:(c + 1) * 128]
            ticks.append(v[0:8, 0:128])
            yield

    with _scope("w_x0"):
        x_copy(0).wait()
    for c in range(NB):
        in_t1(0, c)
    for gs in WG:
        with _scope("w_qkv"):
            for g in gs:
                wqkv_copy(g).wait()
        if gs == WG[0]:
            _drain(first_norm(0, 0, xn_s.at[0, 0]))
        if gs == WG[WX]:
            x_copy(1).start()
            cwo.start()
        for g in gs:
            transpose_wqkv(g)
    _loop(HQ // GR, wqkv_slots)
    with _scope("w_x1"):
        x_copy(1).wait()
    for g in range(len(groups)):
        for c in ffn_copies(g):
            c.start()
    for c in range(NB):
        in_t1(1, c)

    def run(order, gens):
        for c in order:
            if c == ".":
                ticks.clear()
            elif c == "!":
                anchors.clear()
            else:
                next(gens[c])
        _drain(*gens.values())

    def body_f(i, zero):
        never = lane < (i < 0).astype(jnp.int32)
        xn = xn_s.at[pl.ds(i, 2)]
        widen_wo(i)
        run(os.environ.get("OF0", "mamnamn."), {"m": first_qkv(0, i, xn.at[0, 0]), "a": first_norm(1, i, xn.at[0, 1], never),
                          "n": first_norm(0, i + 1, xn.at[1, 0], never)})
        return zero + (i < 0).astype(jnp.int32)

    with _scope("w_wo"):
        cwo.wait()
    never = lane < jax.lax.fori_loop(0, 3, body_f, 0)
    run(ORDER_F, {"m": first_qkv(0, 3, xn_s.at[3, 0]), "n": first_norm(1, 3, xn_s.at[3, 1], never),
                  "w": prep_wo(never)})
    _loop(4, lambda i: run(ORDER_E, {"m": first_qkv(1, i, xn_s.at[i, 1]), "s": attend(0, i, PAR0, q0, k0, v0),
                                     "f": ffn_slots(0, i)}))

    def wait_group(k, g):
        @pl.when(k == 0)
        def _():
            for c in ffn_copies(g):
                c.wait()

    def finish_step(i):
        u = i % 4
        never = lane < (i < 0).astype(jnp.int32)
        x1, x2 = (yield from combine(0, u, never))[:2]
        done = out_t1(u, x1) + out_t1(u + 4, x2)
        yield
        anchor(never, done)
        dst = 2 * u + (i // 8) * NB
        done = out_t2(2 * u, dst) + out_t2(2 * u + 1, dst + 1)
        yield
        anchor(never, done)
        yield

    def stage(k):
        t = k % 2
        n_a = jnp.where(jnp.logical_and(k > 0, k < 3), 4, 0)
        n_b = jnp.where(k < 3, 4, 0)
        n_c = NCH - n_a - n_b
        wait_group(k, 0)

        def body_c(i):
            pl.when(i == NCH - 1)(out_copy(0, 0, D).start)
            run(ORDER_C, {"m": ffn_chunk(t, i, True), "s": finish_step(i)})
        _loop(n_c, body_c)
        _loop(n_a, lambda i: run(ORDER_A, {"m": ffn_chunk(t, n_c + i), "s": phase1(1 - t, i)}))
        wait_group(k, 1)

        def body_b(i):
            run(ORDER_B, {"m": ffn_chunk(t, n_c + n_a + i), "s": attend(1 - t, i, PAR, q_s, k_s, v_s),
                          "f": ffn_slots(1 - t, i, lane < (i < 0).astype(jnp.int32))})
        _loop(n_b, body_b)
    _loop(4, stage)

    copies = [out_copy(0, 0, D)]

    def last_t1(g):
        for i in (0, 2, 1, 3):
            xs = yield from combine(1, i, None, 32 * g, min(32 * g + 32, QD))
            for j, x in zip((i, i + 4), xs):
                x = _pad_rows(x) if g == 4 else x
                pout[g, j * 72:j * 72 + 64, :] = pltpu.bitcast(x.astype(bf16).T, u32)

    def last_t2(g):
        r0, r1 = 32 * g, min(32 * g + 32, QD)
        for c in range(NB):
            x = pltpu.bitcast(out_words(g, c), bf16).T
            for q in range(4):
                xin[q * QD + r0:q * QD + r1, TM + c * 128:TM + (c + 1) * 128] = x[q * (r1 - r0):(q + 1) * (r1 - r0)]
        for q in range(4):
            copies.append(out_copy(1, q * QD + r0, q * QD + r1))
            copies[-1].start()

    for c in os.environ.get("OZ", "abAcBdCeDE"):
        if c.islower():
            _drain(last_t1(ord(c) - 97))
        else:
            last_t2(ord(c) - 65)
    with _scope("w_out"):
        for c in copies:
            c.wait()


@jax.jit
def pallas_interleave_layers__sliding_local_dilated__glu_gated_bilinear__prompt_kernel(
    A_x: jax.Array,
    A_wqkv: jax.Array,
    A_wo: jax.Array,
    B_x: jax.Array,
    B_w_gate: jax.Array,
    B_w_up: jax.Array,
    B_w_down: jax.Array,
):
    any_spec = pl.BlockSpec(memory_space=pl.ANY)
    qkv_scratch = [
        pltpu.VMEM((NB, NG, DH, 8, 128), f32),
        pltpu.VMEM((2 * NB, NG, DH, 8, 128), f32),
        pltpu.VMEM((2 * NB, NG, DH, 8, 128), f32),
    ]
    out_t = pl.pallas_call(
        _kernel,
        in_specs=[any_spec] * 6,
        out_specs=any_spec,
        out_shape=jax.ShapeDtypeStruct((D, S), bf16),
        scratch_shapes=[
            pltpu.VMEM((D, S), bf16),
            pltpu.VMEM((D, 3 * D), bf16),
            pltpu.VMEM((D, D), bf16),
            pltpu.VMEM((NCH, D, FC), bf16),
            pltpu.VMEM((NCH, D, FC), bf16),
            pltpu.VMEM((NCH, D, FC), bf16),
            pltpu.VMEM((NSLOT, HQ, 128), bf16),
            pltpu.VMEM((NSLOT, HD, 128), bf16),
            pltpu.VMEM((5, 3 * D, 128), f32),
            pltpu.VMEM((5, D, 128), f32),
            pltpu.VMEM((5, 320, 128), u32),
            pltpu.VMEM((5, HM, 128), u32),
            pltpu.VMEM((5, HM, 128), u32),
            pltpu.VMEM((5, 8 * 72, 128), u32),
            pltpu.VMEM((2, NB, D, 128), f32),
            *qkv_scratch,
            *qkv_scratch,
            pltpu.VMEM((4, HQ + HD + 8, 128), f32),
            pltpu.VMEM((2, D, 128), f32),
            pltpu.VMEM((2, D, 128), f32),
            pltpu.VMEM((2, NPASS, HM // 2, 128), u32),
            pltpu.VMEM((2, 2, 4, HM, 128), f32),
            pltpu.VMEM((7, 2, HM, 128), f32),
            pltpu.VMEM((2, 2, 7, 1024, 128), f32),
            pltpu.VMEM((4, 2, NSLOT, 128, 128), bf16),
            pltpu.SemaphoreType.DMA((12,)),
        ],
        compiler_params=pltpu.CompilerParams(vmem_limit_bytes=120 * 1024 * 1024),
        name="fused_layers",
    )(A_x[0].T, A_wqkv, A_wo, B_w_gate, B_w_up, B_w_down.T)
    return out_t.T[None]
```

```python
import functools
import os

import jax
import jax.numpy as jnp
import jax.experimental.pallas as pl
import jax.experimental.pallas.tpu as pltpu

S, D, F = 2048, 576, 4608
H, DH, W = 32, 18, 8
NG = H // 8
GR = 8 * DH
NB = 8
TM = NB * 128
HM = TM // 2
HD = D // 2
HQ = 3 * D // 2
FC = 512
HC = FC // 2
NCH = F // FC
NSLOT = 16
NT = int(os.environ.get("NT", 128))

GROUP_ROWS = {1: (0, 128), 2: (64, 192), 4: (256, 384), 3: (320, 448), 0: (512, 512)}
T3 = 1.0 / 3.0
SLOTS = (
    ((1, (-1, -1, 0, 0), (0, 0, 0, 1)), (3, (1, 1, 0, 0), (0, 0, 1, 0))),
    ((0, (T3, 0, 0, 0), (2, 1, 0, 0)), (2, (-.5, -1, 0, 0), (0, 0, 0, 1))),
    ((4, (.5, 1, 0, 0), (0, 0, 1, 0)), (0, (-T3, 0, 0, 0), (1, 2, 0, 0))),
    ((1, (0, 1, 0, -1), (0, 0, 1, 1)), (2, (0, 2, 0, -1), (0, 0, .5, 1))),
    ((1, (0, 0, 1, 1), (1, 0, 0, 0)), (3, (0, 0, -1, -1), (0, 1, 0, 0))),
    ((0, (0, 0, T3, 0), (2, 1, 0, 0)), (2, (0, 0, .5, 1), (1, 0, 0, 0))),
    ((4, (0, 0, -.5, -1), (0, 1, 0, 0)), (0, (0, 0, -T3, 0), (1, 2, 0, 0))),
    ((1, (-1, 0, 1, 0), (1, 1, 0, 0)), (2, (-1, 0, .5, 0), (1, 2, 0, 0))),
    ((1, (0, 0, 0, 1), (-1, 0, 1, 0)), (3, (1, 0, 0, 0), (1, 0, -1, 0))),
    ((4, (.5, 0, 0, 0), (2, 0, -1, 0)), (2, (0, 0, 0, 1), (-1, 0, .5, 0))),
    ((4, (-1, 0, .5, 0), (2, 1, 0, 0)), (3, (-1, 0, 1, 0), (1, 1, 0, 0))),
    ((1, (1, 0, 0, 1), (1, 0, 0, 1)), (2, (1, 0, 0, 1), (1, 0, 0, 1))),
    ((1, (1, 0, 0, 0), (0, 1, 0, -1)), (3, (0, 0, 0, 1), (0, -1, 0, 1))),
    ((4, (0, 0, 0, 1), (0, -1, 0, .5)), (2, (.5, 0, 0, 0), (0, 2, 0, -1))),
    ((4, (0, 2, 0, -1), (0, 0, 1, .5)), (3, (0, 1, 0, -1), (0, 0, 1, 1))),
    ((4, (1, 0, 0, 1), (0, 1, 1, 0)), (3, (1, 0, 0, 1), (0, 1, 1, 0))),
)
_PASSES = (
    ("+01 +10", "-04 +14 +17", "-41 -43 +70 +71 +73", "-05 +15 +16", "-51 +60 +61 +62"),
    ("+10", "-04 +14", "+40 +41 -42 +43 -70 -71 -73", "-05 +15", "+50 +51 -52 -60 -61 -62"),
    ("+02 -03", "+00 -02", "+21 +23", "+01 -03", "+31 +33"),
    ("+00 -02 +03", "+00 +08", "+81 +83", "+01 +06", "-53 +63"),
    ("+01 +02 -03", "+02 -08", "+21", "+03 -07", "+31"),
    ("+00 -01", "+06", "+60 +62", "+07", "+70"),
    ("+10 -12 +13", "+10 +18", "+00", "+11 +16", "+10"),
    ("+12 -13", "+10 -12", "+00 +02", "+11 -13", "+10 +12"),
    ("-11 -12 +13", "+12 -18", "+80 +82", "+13 -17", "+72"),
    ("+10 +12", "-12 +14", "+42", "-13 +15", "+52"),
    ("-00 +02 +13", "+00 +18", "-00 +81 +83", "+01 +16", "-10 -53 +63"),
    ("+00 -02", "+06 -16", "+53 -62 -63", "+08 -18", "+80 -81 -83"),
    ("+00 +02", "+02 -04", "+20", "+03 -05", "+30"),
    ("+02", "+02 -12", "-20 +22 +23", "+03 -13", "-30 +32 +33"),
    ("+11 -13", "-08 +18", "-80 +81 -82", "-07 +17", "+43 -72 -73"),
    ("+02 -11 +13", "+08 -12", "+21 +80 +82", "+07 -13", "+31 +72"),
    ("+02 +13", "+00 -12", "+00 +02 -21 -23", "+01 -13", "+10 +12 -31 -33"),
    ("+10 -11", "+16", "+51 -61", "+17", "+41 +43 -71 -73"),
    ("+02 +12", "+12", "+00 +02 +22 +42 +80 +82", "+13", "+10 +12 +32 +52 +72"),
    ("+00 +10", "+04", "+20 +40", "+05", "+30 +50"),
    ("-00 +02 -10 +12", "+16", "+10 +62", "+18", "+00 -80"),
    ("+02 -10", "+04 -12", "+20 +42", "+05 -13", "+30 +52"),
    ("+03 +13", "+00", "+03 +21 +23 -43 -81 -83", "+01", "+13 +31 +33 -63"),
    ("+13", "-00 +10", "+01 +02 +03", "-01 +11", "+11 +12 +13"),
    ("-01 +03", "+00 +04 +07", "+43", "+01 +05 +06", "+53"),
    ("+01", "+04 +07 -14 -17", "+70 +71 +73", "+05 +06 -15 -16", "+53 +60 +61 +62"),
    ("+01 +11", "+14 +17", "-01 +41", "+15 +16", "-11 +51"),
    ("+11 -13", "+10 +14 +17", "+01", "+11 +15 +16", "+11"),
    ("+01 +13", "+00 +14 +17", "+01 +43", "+01 +15 +16", "+11 +53"),
    ("+01 -03 +11 -13", "+08", "+21 +81", "+07", "+31 +43 -73"),
)
PASSES = [[[(int(w[0] + "1"), int(w[1]), int(w[2])) for w in col.split()] for col in row] for row in _PASSES]
NPASS = len(PASSES)
STRASSEN = (
    ((1, 0, 0, 1), (1, 0, 0, 1)),
    ((0, 0, 1, 1), (1, 0, 0, 0)),
    ((1, 0, 0, 0), (0, 1, 0, -1)),
    ((0, 0, 0, 1), (-1, 0, 1, 0)),
    ((1, 1, 0, 0), (0, 0, 0, 1)),
    ((-1, 0, 1, 0), (1, 1, 0, 0)),
    ((0, 1, 0, -1), (0, 0, 1, 1)),
)
QD = D // 4
EPS = 1e-5
WG = [[int(c) for c in x] for x in os.environ.get("WG", "40,1,2,3").split(",")]
TICK = int(os.environ.get("TICK", 40))
ORDER_F = os.environ.get("OF", "mnwmwwnmww.")
WX = int(os.environ.get("WX", 0))
SPLITQ = int(os.environ.get("SPLITQ", 48))
CLINK = int(os.environ.get("CLINK", 1))
KA = int(os.environ.get("KA", 11))
KB = int(os.environ.get("KB", 9))
PAR = int(os.environ.get("PAR", 2))
PAR0 = int(os.environ.get("PAR0", 3))
CSEG = int(os.environ.get("CSEG", 3))
ORDER_A = os.environ.get("OA", "sssssss!mmmmmmmmmmmss")
KB0 = int(os.environ.get("KB0", 1))
ORDER_B = "m" * KB0 + "sm" * 8 + "m" * (KB - KB0 - 8) + "sssssf" + "m" * (15 - KB + int(os.environ.get("KB2", 6))) + "."
ORDER_C = os.environ.get("OC", "msmsmsmsmsmsmsmmsmms")
ORDER_E = os.environ.get("OE", "ssssssss!mmmmsssssf")
f32, bf16, u32 = jnp.float32, jnp.bfloat16, jnp.uint32

_dot = functools.partial(jnp.dot, preferred_element_type=f32)


def _dot_nt(a, b):
    return jax.lax.dot_general(a, b, (((1,), (1,)), ((), ())), preferred_element_type=f32)


def _vcat(*xs):
    return jnp.concatenate(xs, axis=0)


def _pad_rows(r):
    return _vcat(r, jnp.zeros((128 - r.shape[0], r.shape[1]), r.dtype))


def _add(x, y):
    return (x.astype(f32) + y.astype(f32)).astype(bf16)


def _sub(x, y):
    return (x.astype(f32) - y.astype(f32)).astype(bf16)


def _form(coefs, blocks):
    terms = [(c, blk) for c, blk in zip(coefs, blocks) if c != 0]
    if len(terms) == 1 and terms[0][0] == 1:
        return terms[0][1]()
    terms.sort(key=lambda cb: cb[0] < 0)
    out = None
    for c, blk in terms:
        v = blk().astype(f32)
        if out is None:
            out = v if c == 1 else v * c
        else:
            v = v if abs(c) == 1 else v * abs(c)
            out = out + v if c > 0 else out - v
    return out


def _lhs_slots_lanes(x1, x2):
    low = jax.lax.broadcasted_iota(jnp.int32, x1[0].shape, 1) < 64
    out = []
    for halves in SLOTS:
        keys = [(tuple(k // 128 for k in GROUP_ROWS[grp]), coefs) for grp, coefs, _ in halves]
        vals = [_form(coefs, [lambda x=x, g=g: x[g] for x in (x1, x2) for g in tiles])
                for tiles, coefs in keys]
        out.append(vals[0] if keys[0] == keys[1] else jnp.where(low, vals[0], vals[1]))
    return out


def _fast_product(p, ref, out):
    p0, p1, p2, p3 = p(0), p(1), p(2), p(3)
    r = p0 + p1 + p2
    ref[0] = r + p1 + p3
    ref[1] = r + p2
    yield
    p0, p1, p2, p3 = p(4), p(5), p(6), p(7)
    r = p0 + p1 + p2
    ref[2] = r + p1
    ref[3] = p3 - (r + p2)
    yield
    p0, p1, p2, p3 = p(8), p(9), p(10), p(11)
    r = p0 + p1
    c11 = ref[0] + (r + p3)
    ref[2] = ref[2] + (r + p1 + p2)
    ref[3] = ref[3] + p3
    yield
    p0, p1, p2, p3 = p(12), p(13), p(14), p(15)
    r = p0 + p1
    out.append((c11, (r + p2 + p3) - ref[1], ref[2] + p3, ref[3] + (r + p1)))
    yield


def _rhs_slot(s, get, zero=None):
    parts = []
    for grp, _, coefs in SLOTS[s]:
        k1, k2 = GROUP_ROWS[grp]
        blocks = [lambda k=k, c=c: get(slice(k, k + 64), c) for k in (k1, k2) for c in (0, 1)]
        parts.append(_form(coefs, blocks).astype(f32))
    if zero is not None:
        parts[0] = _vcat(parts[0][:8] + zero, parts[0][8:])
    return _vcat(*parts).astype(bf16)


def _signed(terms, get):
    return _form([t[0] for t in terms], [functools.partial(get, t[1], t[2]) for t in terms])


def _feed(outs, prods, ref, keep=()):
    vals = dict(prods)
    sums = {}
    for s in prods:
        for sign, i, n in PASSES[s][0]:
            sums.setdefault((i, n), {})[s] = sign
    while True:
        pairs = {}
        for terms in sums.values():
            keys = list(terms)
            for x in range(len(keys)):
                for y in range(x):
                    key = (keys[y], keys[x], terms[keys[x]] * terms[keys[y]])
                    pairs[key] = pairs.get(key, 0) + 1
        if not pairs or max(pairs.values()) < 2:
            break
        x, y, rel = max(pairs, key=pairs.get)
        vals[x, y] = vals[x] + vals[y] if rel > 0 else vals[x] - vals[y]
        for terms in sums.values():
            if x in terms and y in terms and terms[x] * terms[y] == rel:
                terms[x, y] = terms.pop(x)
                del terms[y]
    for blk, terms in sums.items():
        items = [(sign, vals[k]) for k, sign in terms.items()]
        sign, v = items[0]
        for s2, w in items[1:] + ([(outs[blk][0], ref[blk])] if blk in outs else []):
            v = v + w if s2 == sign else v - w
        outs[blk] = (sign, v)
        if blk not in keep:
            ref[blk] = v


def _packed(ref, *idx):
    return pltpu.bitcast(ref.bitcast(u32)[idx], bf16)


def _norm_stats(ref, total):
    m = jnp.broadcast_to(jnp.sum(total, axis=0, keepdims=True) * (1.0 / D), (8, 128))
    s = None
    for r in range(0, D, 8):
        c = ref[r:r + 8, :] - m
        s = c * c if s is None else s + c * c
    v = jnp.sum(s, axis=0, keepdims=True) * (1.0 / D)
    return m[0:1], jax.lax.rsqrt(v + EPS)


def _tile_sum(x, zero=None):
    rows = [x[r:r + 8] for r in range(0, D, 8)]
    return functools.reduce(jnp.add, rows[1:], rows[0] if zero is None else rows[0] + zero)


def _aligned(x, n):
    return x if isinstance(x, int) else pl.multiple_of(x, n)


def _drain(*gens):
    for gen in gens:
        for _ in gen:
            pass


def _scope(name):
    import contextlib
    return jax.named_scope(name) if os.environ.get("SCOPES") else contextlib.nullcontext()


def _loop(n, fn):
    def body(i, c):
        with _scope("it"):
            fn(i)
        return c
    jax.lax.fori_loop(0, n, body, 0)


def _kernel(x_hbm, wqkv_hbm, wo_hbm, wg_hbm, wu_hbm, wd_hbm, out_hbm,
            xin, wqkv, wo, wg, wu, wd, wqkv_t, wo_t, wperm, operm, wt_s, pin0, pin1, pout, xres,
            q0, k0, v0, q_s, k_s, v_s, c_s, o_s, n_s, a_s, gu_s, h_s, acc, xn_s, sems):
    groups = (range(5), range(5, NCH))
    lane = jax.lax.broadcasted_iota(jnp.int32, (8, 128), 1)
    anchors, ticks = [], []
    pin = (pin0, pin1)

    def anchor(never, words):
        anchors.append(jnp.where(never, pltpu.bitcast(functools.reduce(jnp.bitwise_or, words), f32), 0.0))

    def x_copy(t):
        cols = pl.ds(t * TM, TM)
        return pltpu.make_async_copy(x_hbm.at[:, cols], xin.at[:, cols], sems.at[2 + t])

    def wqkv_copy(g):
        rows = pl.ds(g * 128, min(128, D - g * 128))
        return pltpu.make_async_copy(wqkv_hbm.at[rows], wqkv.at[rows], sems.at[5 + g])

    def out_copy(t, r0, r1):
        idx = (pl.ds(r0, r1 - r0), pl.ds(t * TM, TM))
        return pltpu.make_async_copy(xin.at[idx], out_hbm.at[idx], sems.at[t])

    def ffn_copies(g):
        return [pltpu.make_async_copy(src.at[:, pl.ds(j * FC, FC)], dst.at[j], sems.at[10 + g])
                for j in groups[g]
                for src, dst in ((wg_hbm, wg), (wu_hbm, wu), (wd_hbm, wd))]

    cwo = pltpu.make_async_copy(wo_hbm, wo, sems.at[4])
    x_copy(0).start()
    for gs in WG:
        for g in gs:
            wqkv_copy(g).start()

    def head_rows(ref, g, base):
        return _vcat(*[ref[g, pl.ds(base + d, 8, stride=DH), :] for d in range(DH)])

    def transpose_wqkv(g):
        rows = wqkv[g * 128:min((g + 1) * 128, D), :].astype(f32)
        wperm[g] = (_vcat(rows, rows) if g == 4 else rows).T

    def wqkv_slots(hg):
        base = pl.multiple_of(hg * GR, 16)
        src = base + (hg // 2) * HD
        for d in range(0, DH, 2):
            x1, x2 = [[_vcat(*[wperm[g, pl.ds(b + e, 8, stride=DH), :] for e in (d, d + 1)]) for g in range(5)]
                      for b in (src, src + HD)]
            for n, v in enumerate(_lhs_slots_lanes(x1, x2)):
                wqkv_t[n, pl.ds(base + 8 * d, 16), :] = v.astype(bf16)

    def widen_wo(i):
        rows = pl.ds(pl.multiple_of(i * (D // 3), 64), D // 3)
        for g in range(5):
            cols = wo[rows, g * 128:min((g + 1) * 128, D)].astype(f32)
            if g == 4:
                cols = jnp.concatenate([cols, jnp.zeros_like(cols)], axis=1)
            operm[g, rows, :] = cols

    def prep_wo(never):
        for g in range(5):
            r = _vcat(*[head_rows(operm, g, hg * GR) for hg in range(NG)])
            r = _vcat(r, r[512:D])
            tiles = [pltpu.bitcast(r[k * 128:(k + 1) * 128].astype(bf16).T, u32) for k in range(5)]
            for k, w in enumerate(tiles):
                wt_s[k, g * 64:(g + 1) * 64, :] = w
            anchor(never, [w[56:64] for w in tiles])
            yield
        for r in range(0, HD // 2, 8):
            zero = pltpu.bitcast(jnp.where(never, ticks.pop(0), 0.0), u32)
            x1, x2 = [[pltpu.bitcast(wt_s[k, r0:r0 + 8, :] | zero, bf16).astype(f32) for k in range(5)]
                      for r0 in (r, r + HD // 2)]
            for n, v in enumerate(_lhs_slots_lanes(x1, x2)):
                wo_t[n, 2 * r:2 * r + 16, :] = v.astype(bf16)
            yield

    def to_words(x):
        tiles = [x[g * 128:(g + 1) * 128] for g in range(4)] + [_pad_rows(x[512:D])]
        return [pltpu.bitcast(r.astype(bf16).T, u32) for r in tiles]

    def from_words(words):
        parts = [pltpu.bitcast(w, bf16).T for w in words]
        return _vcat(*parts[:4], parts[4][:64])

    def in_t1(t, c):
        x = xin[:, pl.ds(pl.multiple_of(t * TM + c * 128, 128), 128)]
        words = to_words(x)
        for g, w in enumerate(words):
            pin[t][g, pl.ds(pl.multiple_of(c * 64, 64), 64), :] = w
        return [w[56:64] for w in words]

    def in_t2(t, j):
        return from_words([pin[t][g, pl.ds(j, 64, stride=8), :] for g in range(5)]).astype(f32)

    def out_t1(j, x):
        words = to_words(x)
        for g, w in enumerate(words):
            pout[g, pl.ds(pl.multiple_of(j * 72, 8), 64), :] = w
        return [w[56:64] for w in words]

    def out_words(g, c):
        return _vcat(*[pout[g, pl.ds(c * 8 + m, 8, stride=72), :] for m in range(8)])

    def out_t2(c, dst):
        x = from_words([out_words(g, c) for g in range(5)])
        xin[:, pl.ds(pl.multiple_of(dst * 128, 128), 128)] = x
        return [pltpu.bitcast(x[r - 16:r], u32) for r in (128, 256, 384, 512, D)]

    def combine(t, i, never=None, r0=0, r1=QD):
        c, second = i % 2, i // 2
        pick = lambda lo, hi: lo + (hi - lo) * second
        outer = lambda m1, m2, m3, m4, m5, m6, m7: (
            m1 + m4 - m5 + m7, m2 + m4, m3 + m5, m1 - m2 + m3 + m6)
        strips, sums, link = [], [], None
        for r in range(r0, r1, 8):
            get = lambda n, m: acc[t, c, m, n * QD + r:n * QD + r + 8, :]
            four, two = [], []
            for n in range(7):
                x = get(n, pick(3, 2))
                if link is not None and n % CLINK == 0:
                    x = x + jnp.where(never, link, 0.0)
                four.append(((get(n, 0) + x) + get(n, pick(6, 5))) - get(n, pick(4, 1)))
                two.append(get(n, pick(1, 4)) + x)
                if never is not None:
                    link = four[-1]
            rows = []
            for u, v in zip(outer(*four), outer(*two)):
                if isinstance(second, int):
                    rows += [v, u] if second else [u, v]
                else:
                    rows += [jnp.where(second > 0, v, u), jnp.where(second > 0, u, v)]
            strips.append([xres[t, i + 4 * (q // 4), (q % 4) * QD + r:(q % 4) * QD + r + 8, :] + v
                           for q, v in enumerate(rows)])
            if never is not None:
                sums = [functools.reduce(jnp.add, sums[n:n + 1] + strips[-1][4 * n:4 * n + 4]) for n in (0, 1)]
                link = sums[0] + sums[1]
                if len(strips) % CSEG == 0:
                    anchors.append(jnp.where(never, link, 0.0))
                    yield
        return [_vcat(*[s[q] for q in range(q0, q0 + 4) for s in strips]) for q0 in (0, 4)] + sums

    def store_qkv(t, b, c1, c2, q, k, v, prev=None):
        part = [_vcat(c1[r:r + HD], c2[r:r + HD]) for r in range(0, HQ, HD)]
        q[b] = part[0].reshape(NG, DH, 8, 128)
        for n, (dst, r) in enumerate(((k, part[1]), (v, part[2]))):
            dst[b + NB] = r.reshape(NG, DH, 8, 128)
            sh = pltpu.roll(r, 2, 1).reshape(NG, DH, 8, 128)
            if isinstance(t, int) and t == 0:
                dst[b] = sh
            elif prev is not None:
                dst[b] = jnp.where((lane < 2)[None, None], prev[n][b], sh)
            else:
                keep = jnp.broadcast_to((lane >= 2 * t)[None, None], sh.shape)
                pltpu.store(dst.at[b], sh, mask=keep)

    def normalize(t, i, s1, s2, never):
        for c, s in enumerate((s1, s2)):
            if c and never is not None:
                s = s + jnp.where(never, r, 0.0)
            m, r = _norm_stats(xres.at[t, i + 4 * c], s)
            n_s[c] = (xres[t, i + 4 * c] - m) * r

    def phase1(t, i):
        never = lane < (i < 0).astype(jnp.int32)
        x1, x2, s1, s2 = yield from combine(t, i, never)
        xres[t, i] = x1
        xres[t, i + 4] = x2
        normalize(t, i, s1, s2, never)
        yield
        rhs = lambda s: _rhs_slot(s, lambda rows, c: n_s[c, rows, :])
        out = []
        _drain(_fast_product(lambda s: _dot(_packed(wqkv_t, s), rhs(s)), c_s.at[:, 0:HQ], out))
        c = out[0]
        yield
        store_qkv(t, i, c[0], c[2], q_s, k_s, v_s)
        store_qkv(t, i + 4, c[1], c[3], q_s, k_s, v_s)
        yield

    def first_norm(t, i, dst, never=None):
        sums = []
        src = [xres.at[t, i + 4 * c] for c in (0, 1)]
        for c in (0, 1):
            x = in_t2(t, i + 4 * c)
            xres[t, i + 4 * c] = x
            sums.append(_tile_sum(x))
        if never is not None:
            anchors.append(jnp.where(never, sums[0] + sums[1], 0.0))
        yield
        stats = [_norm_stats(src[c], sums[c]) for c in (0, 1)]
        if never is not None:
            anchors.append(jnp.where(never, stats[0][1] + stats[1][1], 0.0))
        yield
        for s in range(NSLOT):
            mean = [st[0] for st in stats]
            if never is not None:
                zero = jnp.where(never, ticks.pop(0), 0.0)[0:1]
                mean = [m + zero for m in mean]
            dst[s] = _rhs_slot(s, lambda rows, c: (src[c][rows, :] - mean[c]) * stats[c][1])
            yield

    def first_qkv(t, i, src):
        def p(s):
            w = wqkv_t.bitcast(u32)[s, rows]
            while anchors:
                w = _vcat(w[:8] | pltpu.bitcast(anchors.pop(), u32), w[8:])
            v = _dot(pltpu.bitcast(w, bf16), _packed(src, s))
            if s % 4 == 0:
                ticks.extend(v[r:r + 8] for r in range(0, v.shape[0], TICK))
            return v

        cs = []
        for r0, r1 in ((HD, HQ), (0, HD)):
            rows = slice(r0 // 2, r1 // 2)
            yield from _fast_product(p, c_s.at[:, r0:r1], cs)
        c = [_vcat(x, y) for y, x in zip(*cs)]
        for n, b in enumerate((i, i + 4)):
            if t == 0:
                store_qkv(t, b, c[n], c[n + 2], q0, k0, v0)
            else:
                store_qkv(t, b, c[n], c[n + 2], q_s, k_s, v_s, prev=(k0, v0))

    def attention_group(t, b, g, q_r, k_r, v_r, links):
        par = len(links)
        never = lane < (b < 0).astype(jnp.int32)

        def start(n, v):
            if links[n % par] is None:
                return v
            return jnp.where(never, links[n % par], 0.0) + v

        q = [q_r[b, g, d] for d in range(DH)]
        logits = []
        for w in range(W):
            l = start(w, q[0] * k_r[b + NB - w, g, 0])
            for d in range(1, DH):
                l = l + q[d] * k_r[b + NB - w, g, d]
            links[w % par] = l
            l = l * (DH ** -0.5)
            if w > 0:
                edge = jnp.where(jnp.logical_and(w > b, t == 0), 2, 0)
                l = jnp.where(lane < edge, -1e9, l)
            logits.append(l)
        m = functools.reduce(jnp.maximum, logits)
        e = [jnp.exp(l - m) for l in logits]
        r = 1.0 / functools.reduce(jnp.add, e)
        p = [x * r for x in e]
        outs = []
        for d in range(DH):
            o = p[0] * v_r[b + NB, g, d]
            if d >= par:
                o = start(d, o)
            for w in range(1, W):
                o = o + p[w] * v_r[b + NB - w, g, d]
            links[d % par] = o
            outs.append(o)
        return _vcat(*outs)

    def attend(t, i, par, q_r, k_r, v_r):
        links = [None] * par
        never = lane < (i < 0).astype(jnp.int32)
        for c, b in enumerate((i, i + 4)):
            for g in range(NG):
                o_s[c, g * GR:(g + 1) * GR, :] = attention_group(t, b, g, q_r, k_r, v_r, links)
                anchors.append(jnp.where(never, functools.reduce(jnp.add, links), 0.0))
                yield
        p = lambda s: _dot(_packed(wo_t, s), _rhs_slot(s, lambda rows, c: o_s[c, rows, :]))
        out = []
        yield from _fast_product(p, c_s.at[:, HQ:HQ + HD], out)
        for n, b in enumerate((i, i + 4)):
            x = xres[t, b] + _vcat(out[0][n], out[0][n + 2])
            xres[t, b] = x
            c_s[n, HQ + HD:, :] = _tile_sum(x)
        yield

    def ffn_slots(t, i, never=None):
        stats = []
        for c in (0, 1):
            s = c_s[c, HQ + HD:, :]
            if c and never is not None:
                s = s + jnp.where(never, stats[0][1], 0.0)
            stats.append(_norm_stats(xres.at[t, i + 4 * c], s))
        yield

        def form(terms, zero):
            out = []
            for c in (0, 1):
                sub = [w for w in terms if w[1] == c]
                if sub:
                    sign = max(w[0] for w in sub)
                    v = _signed([(w[0] * sign,) + w[1:] for w in sub],
                                lambda _, k: xres[t, i + 4 * c, 64 * k:64 * k + 64, :])
                    count = sign * sum(w[0] for w in sub)
                    if count:
                        v = v - stats[c][0] * count
                    out.append(v * (stats[c][1] * sign + zero))
            return functools.reduce(jnp.add, out)

        rows = pl.ds(_aligned(i * 64, 64), 64)
        for s, (_, lo, _, hi, _) in enumerate(PASSES):
            zero = 0.0 if never is None else jnp.where(never, ticks.pop(0), 0.0)[0:1]
            op = _vcat(form(lo, zero), form(hi, zero))
            a_s[t, s, rows, :] = pltpu.bitcast(op.astype(bf16).T, u32)
            yield

    def ffn_pass(t, w_ref, s):
        get = lambda k, n: w_ref[64 * k:64 * k + 64, 128 * n:128 * n + 128]
        parts = [_signed(x, get).astype(f32) for x in PASSES[s][2::2]]
        while anchors:
            parts[0] = _vcat(parts[0][:8] + anchors.pop(), parts[0][8:])
        return _dot(pltpu.bitcast(a_s[t, s], bf16), _vcat(*parts).astype(bf16))

    def ffn_chunk(t, j, may_init=False):
        lhs, g, u = {}, {}, {}
        todo = [(g, wg, s) for s in list(range(2, NPASS)) + [0, 1]] + [(u, wu, s) for s in range(NPASS)]
        for q in range(0, 2 * NPASS, 4):
            prods = [(outs, s, ffn_pass(t, w.at[j], s)) for outs, w, s in todo[q:q + 4]]
            k2 = {2 * NPASS - 12: 0, 2 * NPASS - 4: 1}.get(q)
            blks = [] if k2 is None else [(i, 2 * k + k2) for k in (0, 1) for i in (0, 1)]
            for n, outs in enumerate((g, u)):
                _feed(outs, {s: v for o, s, v in prods if o is outs}, gu_s.at[n], blks)
            if blks:
                hs = [gu_s[(0,) + b] * u[b][1] for b in blks]
                for n, (_, lb) in enumerate(STRASSEN):
                    coefs = [c * g[b][0] * u[b][0] for c, b in zip(lb, blks)]
                    h_s[n, k2] = _form(coefs, [lambda x=x: x for x in hs])
            yield
        order = [(n, m) for n in range(7) for m in (1, 5)] + [(n, m) for n in range(7) for m in (0, 2, 3, 4, 6)]
        for q, (n, m) in enumerate(order):
            rhs = [lambda k2=k2, c2=c2: h_s[n, k2, c2 * 256:(c2 + 1) * 256, :] for k2 in (0, 1) for c2 in (0, 1)]
            if q == 14:
                lhs.clear()
            if n not in lhs:
                lhs[n] = [_form(STRASSEN[n][0],
                                [lambda r=r, k=k, r2=r2, k2=k2: wd[j, pl.ds((2 * r + r2) * QD, QD),
                                                                   pl.ds((2 * k + k2) * 128, 128)]
                                 for r in (0, 1) for k in (0, 1)])
                          for r2 in (0, 1) for k2 in (0, 1)]
            left = _form(STRASSEN[m][0], [lambda x=x: x for x in lhs[n]])
            right = _form(STRASSEN[m][1], rhs).astype(bf16)
            if q == SPLITQ:
                v = _vcat(_dot_nt(left[:80].astype(bf16), right), _dot_nt(left[80:].astype(bf16), right))
            else:
                v = _dot_nt(left.astype(bf16), right)
            for c in range(2):
                old = acc[t, c, m, n * QD:(n + 1) * QD, :]
                if may_init:
                    old = jnp.where(j > 0, old, 0.0)
                acc[t, c, m, n * QD:(n + 1) * QD, :] = old + v[:, c * 128:(c + 1) * 128]
            ticks.append(v[0:8, 0:128])
            yield

    with _scope("w_x0"):
        x_copy(0).wait()
    for c in range(NB):
        in_t1(0, c)
    for gs in WG:
        with _scope("w_qkv"):
            for g in gs:
                wqkv_copy(g).wait()
        if gs == WG[0]:
            _drain(first_norm(0, 0, xn_s.at[0, 0]))
        if gs == WG[WX]:
            x_copy(1).start()
            cwo.start()
        for g in gs:
            transpose_wqkv(g)
    _loop(HQ // GR, wqkv_slots)
    with _scope("w_x1"):
        x_copy(1).wait()
    for g in range(len(groups)):
        for c in ffn_copies(g):
            c.start()
    for c in range(NB):
        in_t1(1, c)

    def run(order, gens):
        for c in order:
            if c == ".":
                ticks.clear()
            elif c == "!":
                anchors.clear()
            else:
                next(gens[c])
        _drain(*gens.values())

    def body_f(i, zero):
        never = lane < (i < 0).astype(jnp.int32)
        xn = xn_s.at[pl.ds(i, 2)]
        widen_wo(i)
        run(os.environ.get("OF0", "mamnamn."), {"m": first_qkv(0, i, xn.at[0, 0]), "a": first_norm(1, i, xn.at[0, 1], never),
                          "n": first_norm(0, i + 1, xn.at[1, 0], never)})
        return zero + (i < 0).astype(jnp.int32)

    with _scope("w_wo"):
        cwo.wait()
    never = lane < jax.lax.fori_loop(0, 3, body_f, 0)
    run(ORDER_F, {"m": first_qkv(0, 3, xn_s.at[3, 0]), "n": first_norm(1, 3, xn_s.at[3, 1], never),
                  "w": prep_wo(never)})
    _loop(4, lambda i: run(ORDER_E, {"m": first_qkv(1, i, xn_s.at[i, 1]), "s": attend(0, i, PAR0, q0, k0, v0),
                                     "f": ffn_slots(0, i)}))

    def wait_group(k, g):
        @pl.when(k == 0)
        def _():
            for c in ffn_copies(g):
                c.wait()

    def finish_step(i):
        u = i % 4
        never = lane < (i < 0).astype(jnp.int32)
        x1, x2 = (yield from combine(0, u, never))[:2]
        done = out_t1(u, x1) + out_t1(u + 4, x2)
        yield
        anchor(never, done)
        dst = 2 * u + (i // 8) * NB
        done = out_t2(2 * u, dst) + out_t2(2 * u + 1, dst + 1)
        yield
        anchor(never, done)
        yield

    def stage(k):
        t = k % 2
        n_a = jnp.where(jnp.logical_and(k > 0, k < 3), 4, 0)
        n_b = jnp.where(k < 3, 4, 0)
        n_c = NCH - n_a - n_b
        wait_group(k, 0)

        def body_c(i):
            pl.when(i == NCH - 1)(out_copy(0, 0, D).start)
            run(ORDER_C, {"m": ffn_chunk(t, i, True), "s": finish_step(i)})
        _loop(n_c, body_c)
        _loop(n_a, lambda i: run(ORDER_A, {"m": ffn_chunk(t, n_c + i), "s": phase1(1 - t, i)}))
        wait_group(k, 1)

        def body_b(i):
            run(ORDER_B, {"m": ffn_chunk(t, n_c + n_a + i), "s": attend(1 - t, i, PAR, q_s, k_s, v_s),
                          "f": ffn_slots(1 - t, i, lane < (i < 0).astype(jnp.int32))})
        _loop(n_b, body_b)
    _loop(4, stage)

    copies = [out_copy(0, 0, D)]

    def last_t1(g):
        for i in (0, 2, 1, 3):
            xs = yield from combine(1, i, None, 32 * g, min(32 * g + 32, QD))
            for j, x in zip((i, i + 4), xs):
                x = _pad_rows(x) if g == 4 else x
                pout[g, j * 72:j * 72 + 64, :] = pltpu.bitcast(x.astype(bf16).T, u32)

    def last_t2(g):
        r0, r1 = 32 * g, min(32 * g + 32, QD)
        for c in range(NB):
            x = pltpu.bitcast(out_words(g, c), bf16).T
            for q in range(4):
                xin[q * QD + r0:q * QD + r1, TM + c * 128:TM + (c + 1) * 128] = x[q * (r1 - r0):(q + 1) * (r1 - r0)]
        for q in range(4):
            copies.append(out_copy(1, q * QD + r0, q * QD + r1))
            copies[-1].start()

    for c in os.environ.get("OZ", "abAcBdCeDE"):
        if c.islower():
            _drain(last_t1(ord(c) - 97))
        else:
            last_t2(ord(c) - 65)
    with _scope("w_out"):
        for c in copies:
            c.wait()


@jax.jit
def pallas_interleave_layers__sliding_local_dilated__glu_gated_bilinear__prompt_kernel(
    A_x: jax.Array,
    A_wqkv: jax.Array,
    A_wo: jax.Array,
    B_x: jax.Array,
    B_w_gate: jax.Array,
    B_w_up: jax.Array,
    B_w_down: jax.Array,
):
    any_spec = pl.BlockSpec(memory_space=pl.ANY)
    qkv_scratch = [
        pltpu.VMEM((NB, NG, DH, 8, 128), f32),
        pltpu.VMEM((2 * NB, NG, DH, 8, 128), f32),
        pltpu.VMEM((2 * NB, NG, DH, 8, 128), f32),
    ]
    out_t = pl.pallas_call(
        _kernel,
        in_specs=[any_spec] * 6,
        out_specs=any_spec,
        out_shape=jax.ShapeDtypeStruct((D, S), bf16),
        scratch_shapes=[
            pltpu.VMEM((D, S), bf16),
            pltpu.VMEM((D, 3 * D), bf16),
            pltpu.VMEM((D, D), bf16),
            pltpu.VMEM((NCH, D, FC), bf16),
            pltpu.VMEM((NCH, D, FC), bf16),
            pltpu.VMEM((NCH, D, FC), bf16),
            pltpu.VMEM((NSLOT, HQ, 128), bf16),
            pltpu.VMEM((NSLOT, HD, 128), bf16),
            pltpu.VMEM((5, 3 * D, 128), f32),
            pltpu.VMEM((5, D, 128), f32),
            pltpu.VMEM((5, 320, 128), u32),
            pltpu.VMEM((5, HM, 128), u32),
            pltpu.VMEM((5, HM, 128), u32),
            pltpu.VMEM((5, 8 * 72, 128), u32),
            pltpu.VMEM((2, NB, D, 128), f32),
            *qkv_scratch,
            *qkv_scratch,
            pltpu.VMEM((4, HQ + HD + 8, 128), f32),
            pltpu.VMEM((2, D, 128), f32),
            pltpu.VMEM((2, D, 128), f32),
            pltpu.VMEM((2, NPASS, HM // 2, 128), u32),
            pltpu.VMEM((2, 2, 4, HM, 128), f32),
            pltpu.VMEM((7, 2, HM, 128), f32),
            pltpu.VMEM((2, 2, 7, 1024, 128), f32),
            pltpu.VMEM((4, 2, NSLOT, 128, 128), bf16),
            pltpu.SemaphoreType.DMA((12,)),
        ],
        compiler_params=pltpu.CompilerParams(vmem_limit_bytes=120 * 1024 * 1024),
        name="fused_layers",
    )(A_x[0].T, A_wqkv, A_wo, B_w_gate, B_w_up, B_w_down.T)
    return out_t.T[None]
```

```python
import functools
import os

import jax
import jax.numpy as jnp
import jax.experimental.pallas as pl
import jax.experimental.pallas.tpu as pltpu

S, D, F = 2048, 576, 4608
H, DH, W = 32, 18, 8
NG = H // 8
GR = 8 * DH
NB = 8
TM = NB * 128
HM = TM // 2
HD = D // 2
HQ = 3 * D // 2
FC = 512
HC = FC // 2
NCH = F // FC

_PASSES = (
    ("+01 +10", "-04 +14 +17", "-41 -43 +70 +71 +73", "-05 +15 +16", "-51 +60 +61 +62"),
    ("+10", "-04 +14", "+40 +41 -42 +43 -70 -71 -73", "-05 +15", "+50 +51 -52 -60 -61 -62"),
    ("+02 -03", "+00 -02", "+21 +23", "+01 -03", "+31 +33"),
    ("+00 -02 +03", "+00 +08", "+81 +83", "+01 +06", "-53 +63"),
    ("+01 +02 -03", "+02 -08", "+21", "+03 -07", "+31"),
    ("+00 -01", "+07", "+70", "+06", "+60 +62"),
    ("+10 -12 +13", "+10 +18", "+00", "+11 +16", "+10"),
    ("+12 -13", "+10 -12", "+00 +02", "+11 -13", "+10 +12"),
    ("-11 -12 +13", "+12 -18", "+80 +82", "+13 -17", "+72"),
    ("+10 +12", "-12 +14", "+42", "-13 +15", "+52"),
    ("-00 +02 +13", "+00 +18", "-00 +81 +83", "+01 +16", "-10 -53 +63"),
    ("+00 -02", "+08 -18", "+80 -81 -83", "+06 -16", "+53 -62 -63"),
    ("+00 +02", "+02 -04", "+20", "+03 -05", "+30"),
    ("+02", "+02 -12", "-20 +22 +23", "+03 -13", "-30 +32 +33"),
    ("+11 -13", "-08 +18", "-80 +81 -82", "-07 +17", "+43 -72 -73"),
    ("+02 -11 +13", "+08 -12", "+21 +80 +82", "+07 -13", "+31 +72"),
    ("+02 +13", "+00 -12", "+00 +02 -21 -23", "+01 -13", "+10 +12 -31 -33"),
    ("+10 -11", "+17", "+41 +43 -71 -73", "+16", "+51 -61"),
    ("+02 +12", "+12", "+00 +02 +22 +42 +80 +82", "+13", "+10 +12 +32 +52 +72"),
    ("+00 +10", "+04", "+20 +40", "+05", "+30 +50"),
    ("-00 +02 -10 +12", "+18", "+00 -80", "+16", "+10 +62"),
    ("+02 -10", "+04 -12", "+20 +42", "+05 -13", "+30 +52"),
    ("+03 +13", "+00", "+03 +21 +23 -43 -81 -83", "+01", "+13 +31 +33 -63"),
    ("+13", "-00 +10", "+01 +02 +03", "-01 +11", "+11 +12 +13"),
    ("-01 +03", "+00 +04 +07", "+43", "+01 +05 +06", "+53"),
    ("+01", "+04 +07 -14 -17", "+70 +71 +73", "+05 +06 -15 -16", "+53 +60 +61 +62"),
    ("+01 +11", "+14 +17", "-01 +41", "+15 +16", "-11 +51"),
    ("+11 -13", "+10 +14 +17", "+01", "+11 +15 +16", "+11"),
    ("+01 +13", "+00 +14 +17", "+01 +43", "+01 +15 +16", "+11 +53"),
    ("+01 -03 +11 -13", "+08", "+21 +81", "+07", "+31 +43 -73"),
)
PASSES = [[[(int(w[0] + "1"), int(w[1]), int(w[2])) for w in col.split()] for col in row] for row in _PASSES]
NPASS = len(PASSES)
LANE_TILES = ((0, 1), (2, 3), (4, 5), (7, 6), (8, 7), (5, 4))
RQ = 3 * GR
STRASSEN = (
    ((1, 0, 0, 1), (1, 0, 0, 1)),
    ((0, 0, 1, 1), (1, 0, 0, 0)),
    ((1, 0, 0, 0), (0, 1, 0, -1)),
    ((0, 0, 0, 1), (-1, 0, 1, 0)),
    ((1, 1, 0, 0), (0, 0, 0, 1)),
    ((-1, 0, 1, 0), (1, 1, 0, 0)),
    ((0, 1, 0, -1), (0, 0, 1, 1)),
)
QD = D // 4
EPS = 1e-5
WG = [[int(c) for c in x] for x in os.environ.get("WG", "34,0,1,2").split(",")]
TICK = int(os.environ.get("TICK", 24))
ORDER_F = os.environ.get("OF", "mmnwmwmwnmwmw.")
WX = int(os.environ.get("WX", 0))
SPLITQ = int(os.environ.get("SPLITQ", 48))
CLINK = int(os.environ.get("CLINK", 1))
KA = int(os.environ.get("KA", 11))
KB = int(os.environ.get("KB", 9))
PAR = int(os.environ.get("PAR", 2))
PAR0 = int(os.environ.get("PAR0", 3))
CSEG = int(os.environ.get("CSEG", 3))
ORDER_A = os.environ.get("OA", "sssssss!mmmmmmmmmmms")
KB0 = int(os.environ.get("KB0", 1))
ORDER_B = "m" * KB0 + "sm" * 8 + "m" * (KB - KB0 - 8) + "sf" + "m" * (15 - KB + int(os.environ.get("KB2", 6))) + "."
ORDER_C = os.environ.get("OC", "msmsmsmsmsmsmsmmsmms")
ORDER_E = os.environ.get("OE", "ssssssss!mmmmmmmmsf")
f32, bf16, u32 = jnp.float32, jnp.bfloat16, jnp.uint32

_dot = functools.partial(jnp.dot, preferred_element_type=f32)


def _dot_nt(a, b):
    return jax.lax.dot_general(a, b, (((1,), (1,)), ((), ())), preferred_element_type=f32)


def _vcat(*xs):
    return jnp.concatenate(xs, axis=0)


def _pad_rows(r):
    return _vcat(r, jnp.zeros((128 - r.shape[0], r.shape[1]), r.dtype))


def _add(x, y):
    return (x.astype(f32) + y.astype(f32)).astype(bf16)


def _sub(x, y):
    return (x.astype(f32) - y.astype(f32)).astype(bf16)


def _form(coefs, blocks):
    terms = [(c, blk) for c, blk in zip(coefs, blocks) if c != 0]
    if len(terms) == 1 and terms[0][0] == 1:
        return terms[0][1]()
    terms.sort(key=lambda cb: cb[0] < 0)
    out = None
    for c, blk in terms:
        v = blk().astype(f32)
        if out is None:
            out = v if c == 1 else v * c
        else:
            v = v if abs(c) == 1 else v * abs(c)
            out = out + v if c > 0 else out - v
    return out


def _signed(terms, get):
    return _form([t[0] for t in terms], [functools.partial(get, t[1], t[2]) for t in terms])


def _feed(outs, prods, ref, keep=()):
    vals = dict(prods)
    sums = {}
    for s in prods:
        for sign, i, n in PASSES[s][0]:
            sums.setdefault((i, n), {})[s] = sign
    while True:
        pairs = {}
        for terms in sums.values():
            keys = list(terms)
            for x in range(len(keys)):
                for y in range(x):
                    key = (keys[y], keys[x], terms[keys[x]] * terms[keys[y]])
                    pairs[key] = pairs.get(key, 0) + 1
        if not pairs or max(pairs.values()) < 2:
            break
        x, y, rel = max(pairs, key=pairs.get)
        vals[x, y] = vals[x] + vals[y] if rel > 0 else vals[x] - vals[y]
        for terms in sums.values():
            if x in terms and y in terms and terms[x] * terms[y] == rel:
                terms[x, y] = terms.pop(x)
                del terms[y]
    for blk, terms in sums.items():
        items = [(sign, vals[k]) for k, sign in terms.items()]
        items += [(outs[blk][0], ref[blk])] if blk in outs else []
        sign, v = items.pop(max(range(len(items)), key=lambda x: items[x][0]))
        for s2, w in items:
            v = v + w if s2 == sign else v - w
        outs[blk] = (sign, v)
        if blk not in keep:
            ref[blk] = v


def _lane_forms(get):
    get = functools.lru_cache(None)(get)
    tile = lambda g, n: pltpu.roll(get(2, n), 64, 1) if g == 5 else get(g, n)
    low = jax.lax.broadcasted_iota(jnp.int32, get(0, 0).shape, 1) < 64
    for row in PASSES:
        lo, hi = [[(c, [t[h] for t in LANE_TILES].index(k), n) for c, k, n in row[2 + 2 * h]] for h in (0, 1)]
        both = [w for w in lo if w in hi]
        rest = [[w for w in x if w not in both] for x in (lo, hi)]
        out = [_signed(both, tile)] if both else []
        if rest[0] or rest[1]:
            out.append(jnp.where(low, *[_signed(x, tile) if x else 0.0 for x in rest]))
        yield functools.reduce(jnp.add, out)


def _product_t(dot, rows, ref, emit):
    groups = [range(q, q + 4) for q in range(2, NPASS, 4)]
    groups.insert(4, range(2))
    last = {w[1:]: g for g, grp in enumerate(groups) for s in grp for w in PASSES[s][0]}
    mid = (rows + 16) // 32 * 16
    outs = {}
    for g, grp in enumerate(groups):
        prods = {s: dot(s, 0, rows) if len(grp) == 4 else _vcat(dot(s, 0, mid), dot(s, mid, rows)) for s in grp}
        done = [b for b in last if last[b] == g]
        _feed(outs, prods, ref, done)
        for b in done:
            emit(*b, outs[b][1] if outs[b][0] > 0 else -outs[b][1])
        yield


def _packed(ref, *idx):
    return pltpu.bitcast(ref.bitcast(u32)[idx], bf16)


def _norm_stats(ref, total):
    m = jnp.broadcast_to(jnp.sum(total, axis=0, keepdims=True) * (1.0 / D), (8, 128))
    s = None
    for r in range(0, D, 8):
        c = ref[r:r + 8, :] - m
        s = c * c if s is None else s + c * c
    v = jnp.sum(s, axis=0, keepdims=True) * (1.0 / D)
    return m[0:1], jax.lax.rsqrt(v + EPS)


def _tile_sum(x, zero=None):
    rows = [x[r:r + 8] for r in range(0, x.shape[0], 8)]
    return functools.reduce(jnp.add, rows[1:], rows[0] if zero is None else rows[0] + zero)


def _aligned(x, n):
    return x if isinstance(x, int) else pl.multiple_of(x, n)


def _drain(*gens):
    for gen in gens:
        for _ in gen:
            pass


def _scope(name):
    import contextlib
    return jax.named_scope(name) if os.environ.get("SCOPES") else contextlib.nullcontext()


def _loop(n, fn):
    def body(i, c):
        with _scope("it"):
            fn(i)
        return c
    jax.lax.fori_loop(0, n, body, 0)


def _kernel(x_hbm, wqkv_hbm, wo_hbm, wg_hbm, wu_hbm, wd_hbm, out_hbm,
            xin, wqkv, wo, wg, wu, wd, wqkv_t, wo_t, wperm, operm, wt_s, pin0, pin1, pout, xres,
            q0, k0, v0, q_s, k_s, v_s, c_s, o_s, n_s, a_s, gu_s, h_s, acc, xn_s, sems):
    groups = (range(5), range(5, NCH))
    lane = jax.lax.broadcasted_iota(jnp.int32, (8, 128), 1)
    anchors, ticks = [], []
    pin = (pin0, pin1)

    def anchor(never, words):
        anchors.append(jnp.where(never, pltpu.bitcast(functools.reduce(jnp.bitwise_or, words), f32), 0.0))

    def x_copy(t):
        cols = pl.ds(t * TM, TM)
        return pltpu.make_async_copy(x_hbm.at[:, cols], xin.at[:, cols], sems.at[2 + t])

    def wqkv_copy(g):
        rows = pl.ds(g * 128, min(128, D - g * 128))
        return pltpu.make_async_copy(wqkv_hbm.at[rows], wqkv.at[rows], sems.at[5 + g])

    def out_copy(t, r0, r1):
        idx = (pl.ds(r0, r1 - r0), pl.ds(t * TM, TM))
        return pltpu.make_async_copy(xin.at[idx], out_hbm.at[idx], sems.at[t])

    def ffn_copies(g):
        return [pltpu.make_async_copy(src.at[:, pl.ds(j * FC, FC)], dst.at[j], sems.at[10 + g])
                for j in groups[g]
                for src, dst in ((wg_hbm, wg), (wu_hbm, wu), (wd_hbm, wd))]

    cwo = pltpu.make_async_copy(wo_hbm, wo, sems.at[4])
    x_copy(0).start()
    for gs in WG:
        for g in gs:
            wqkv_copy(g).start()

    def head_rows(ref, g, base):
        return _vcat(*[ref[g, pl.ds(base + d, 8, stride=DH), :] for d in range(DH)])

    def transpose_wqkv(g):
        wperm[g] = _vcat(*[wqkv[64 * k:64 * k + 64, :].astype(f32) for k in LANE_TILES[g]]).T

    def wqkv_slots(u):
        for e in range(0, 6, 2):
            src = (u // 3) * D + (u % 3) * 6 + e
            get = lambda g, n: _vcat(*[wperm[g, pl.ds(src + n * GR + x, 8, stride=DH), :] for x in (0, 1)])
            for s, v in enumerate(_lane_forms(get)):
                wqkv_t[s, pl.ds(pl.multiple_of(u * 48, 16) + 8 * e, 16), :] = v.astype(bf16)

    def widen_wo(i):
        rows = pl.ds(pl.multiple_of(i * (D // 3), 64), D // 3)
        for g in range(5):
            cols = wo[rows, g * 128:min((g + 1) * 128, D)].astype(f32)
            if g == 4:
                cols = jnp.concatenate([cols, jnp.zeros_like(cols)], axis=1)
            operm[g, rows, :] = cols

    def prep_wo(never):
        for g in range(5):
            r = _vcat(*[head_rows(operm, g, hg * GR) for hg in range(NG)])
            tiles = [pltpu.bitcast(_vcat(*[r[64 * k:64 * k + 64] for k in ks]).astype(bf16).T, u32)
                     for ks in LANE_TILES[:5]]
            for k, w in enumerate(tiles):
                wt_s[k, g * 64:(g + 1) * 64, :] = w
            anchor(never, [w[56:64] for w in tiles])
            yield
        for r in range(0, QD // 2, 8):
            zero = pltpu.bitcast(jnp.where(never, ticks.pop(0), 0.0), u32)
            get = lambda g, n: pltpu.bitcast(wt_s[g, pl.ds(n * QD // 2 + r, 8), :] | zero, bf16).astype(f32)
            for s, v in enumerate(_lane_forms(get)):
                wo_t[s, 2 * r:2 * r + 16, :] = v.astype(bf16)
            ticks.pop(0)
            yield

    def to_words(x):
        tiles = [x[g * 128:(g + 1) * 128] for g in range(4)] + [_pad_rows(x[512:D])]
        return [pltpu.bitcast(r.astype(bf16).T, u32) for r in tiles]

    def from_words(words):
        parts = [pltpu.bitcast(w, bf16).T for w in words]
        return _vcat(*parts[:4], parts[4][:64])

    def in_t1(t, c):
        x = xin[:, pl.ds(pl.multiple_of(t * TM + c * 128, 128), 128)]
        words = to_words(x)
        for g, w in enumerate(words):
            pin[t][g, pl.ds(pl.multiple_of(c * 64, 64), 64), :] = w
        return [w[56:64] for w in words]

    def in_t2(t, j):
        return from_words([pin[t][g, pl.ds(j, 64, stride=8), :] for g in range(5)]).astype(f32)

    def out_t1(j, x):
        words = to_words(x)
        for g, w in enumerate(words):
            pout[g, pl.ds(pl.multiple_of(j * 72, 8), 64), :] = w
        return [w[56:64] for w in words]

    def out_words(g, c):
        return _vcat(*[pout[g, pl.ds(c * 8 + m, 8, stride=72), :] for m in range(8)])

    def out_t2(c, dst):
        x = from_words([out_words(g, c) for g in range(5)])
        xin[:, pl.ds(pl.multiple_of(dst * 128, 128), 128)] = x
        return [pltpu.bitcast(x[r - 16:r], u32) for r in (128, 256, 384, 512, D)]

    def combine(t, i, never=None, r0=0, r1=QD):
        c, second = i % 2, i // 2
        pick = lambda lo, hi: lo + (hi - lo) * second
        outer = lambda m1, m2, m3, m4, m5, m6, m7: (
            m1 + m4 - m5 + m7, m2 + m4, m3 + m5, m1 - m2 + m3 + m6)
        strips, sums, link = [], [], None
        for r in range(r0, r1, 8):
            get = lambda n, m: acc[t, c, m, n * QD + r:n * QD + r + 8, :]
            four, two = [], []
            for n in range(7):
                x = get(n, pick(3, 2))
                if link is not None and n % CLINK == 0:
                    x = x + jnp.where(never, link, 0.0)
                four.append(((get(n, 0) + x) + get(n, pick(6, 5))) - get(n, pick(4, 1)))
                two.append(get(n, pick(1, 4)) + x)
                if never is not None:
                    link = four[-1]
            rows = []
            for u, v in zip(outer(*four), outer(*two)):
                if isinstance(second, int):
                    rows += [v, u] if second else [u, v]
                else:
                    rows += [jnp.where(second > 0, v, u), jnp.where(second > 0, u, v)]
            strips.append([xres[t, i + 4 * (q // 4), (q % 4) * QD + r:(q % 4) * QD + r + 8, :] + v
                           for q, v in enumerate(rows)])
            if never is not None:
                sums = [functools.reduce(jnp.add, sums[n:n + 1] + strips[-1][4 * n:4 * n + 4]) for n in (0, 1)]
                link = sums[0] + sums[1]
                if len(strips) % CSEG == 0:
                    anchors.append(jnp.where(never, link, 0.0))
                    yield
        return [_vcat(*[s[q] for q in range(q0, q0 + 4) for s in strips]) for q0 in (0, 4)] + sums

    def store_qkv(t, i, r0, q, k, v, prev=None):
        def emit(c, g, x):
            b = i + 4 * c
            for r in range(0, x.shape[0], GR):
                n = (r0 + r) // GR
                y = x[r:r + GR]
                if n == 0:
                    q[b, g] = y.reshape(DH, 8, 128)
                    continue
                dst = (k, v)[n - 1]
                dst[b + NB, g] = y.reshape(DH, 8, 128)
                sh = pltpu.roll(y, 2, 1).reshape(DH, 8, 128)
                if isinstance(t, int) and t == 0:
                    dst[b, g] = sh
                elif prev is not None:
                    dst[b, g] = jnp.where((lane < 2)[None], prev[n - 1][b, g], sh)
                else:
                    pltpu.store(dst.at[b, g], sh, mask=jnp.broadcast_to((lane >= 2 * t)[None], sh.shape))
        return emit

    def plain_rhs(ref):
        get = lambda c, k: ref[c, 64 * k:64 * k + 64, :]
        return functools.lru_cache(None)(
            lambda s: _vcat(*[_signed(x, get) for x in PASSES[s][1::2]]).astype(bf16))

    def normed_lhs(t, i, stats, s, zero):
        parts = []
        for terms in PASSES[s][1::2]:
            out = []
            for c in (0, 1):
                sub = [w for w in terms if w[1] == c]
                if sub:
                    sign = max(w[0] for w in sub)
                    v = _signed([(w[0] * sign,) + w[1:] for w in sub],
                                lambda _, k: xres[t, i + 4 * c, 64 * k:64 * k + 64, :])
                    count = sign * sum(w[0] for w in sub)
                    if count:
                        v = v - stats[c][0] * count
                    out.append(v * (stats[c][1] * sign + zero))
            parts.append(functools.reduce(jnp.add, out))
        return _vcat(*parts).astype(bf16)

    def normalize(t, i, s1, s2, never):
        for c, s in enumerate((s1, s2)):
            if c and never is not None:
                s = s + jnp.where(never, r, 0.0)
            m, r = _norm_stats(xres.at[t, i + 4 * c], s)
            n_s[c] = (xres[t, i + 4 * c] - m) * r

    def phase1(t, i):
        never = lane < (i < 0).astype(jnp.int32)
        x1, x2, s1, s2 = yield from combine(t, i, never)
        xres[t, i] = x1
        xres[t, i + 4] = x2
        normalize(t, i, s1, s2, never)
        yield
        rhs = plain_rhs(n_s)
        dot = lambda s, r0, r1: _dot(_packed(wqkv_t, s, slice(r0 // 2, r1 // 2)), rhs(s))
        _drain(_product_t(dot, RQ, c_s.at[:, :, 0:RQ], store_qkv(t, i, 0, q_s, k_s, v_s)))
        yield

    def first_norm(t, i, dst, never=None):
        sums = []
        src = [xres.at[t, i + 4 * c] for c in (0, 1)]
        for c in (0, 1):
            x = in_t2(t, i + 4 * c)
            xres[t, i + 4 * c] = x
            sums.append(_tile_sum(x))
        if never is not None:
            anchors.append(jnp.where(never, sums[0] + sums[1], 0.0))
        yield
        stats = [_norm_stats(src[c], sums[c]) for c in (0, 1)]
        if never is not None:
            anchors.append(jnp.where(never, stats[0][1] + stats[1][1], 0.0))
        yield
        for s in range(NPASS):
            zero = 0.0 if never is None else jnp.where(never, ticks.pop(0), 0.0)[0:1]
            dst[s] = normed_lhs(t, i, stats, s, zero)
            yield

    def first_qkv(t, i, src):
        def dot(s, r0, r1):
            w = wqkv_t.bitcast(u32)[s, (base + r0) // 2:(base + r1) // 2]
            while anchors:
                w = _vcat(w[:8] | pltpu.bitcast(anchors.pop(), u32), w[8:])
            v = _dot(pltpu.bitcast(w, bf16), _packed(src, s))
            if s % 4 == 2:
                ticks.extend(v[r:r + 8] for r in range(0, v.shape[0], TICK))
            return v

        dsts = (q0, k0, v0) if t == 0 else (q_s, k_s, v_s, (k0, v0))
        for base, end in ((GR, RQ), (0, GR)):
            yield from _product_t(dot, end - base, c_s.at[:, :, base:end], store_qkv(t, i, base, *dsts))

    def attention_group(t, b, g, q_r, k_r, v_r, links):
        par = len(links)
        never = lane < (b < 0).astype(jnp.int32)

        def start(n, v):
            if links[n % par] is None:
                return v
            return jnp.where(never, links[n % par], 0.0) + v

        q = [q_r[b, g, d] for d in range(DH)]
        logits = []
        for w in range(W):
            l = start(w, q[0] * k_r[b + NB - w, g, 0])
            for d in range(1, DH):
                l = l + q[d] * k_r[b + NB - w, g, d]
            links[w % par] = l
            l = l * (DH ** -0.5)
            if w > 0:
                edge = jnp.where(jnp.logical_and(w > b, t == 0), 2, 0)
                l = jnp.where(lane < edge, -1e9, l)
            logits.append(l)
        m = functools.reduce(jnp.maximum, logits)
        e = [jnp.exp(l - m) for l in logits]
        r = 1.0 / functools.reduce(jnp.add, e)
        p = [x * r for x in e]
        outs = []
        for d in range(DH):
            o = p[0] * v_r[b + NB, g, d]
            if d >= par:
                o = start(d, o)
            for w in range(1, W):
                o = o + p[w] * v_r[b + NB - w, g, d]
            links[d % par] = o
            outs.append(o)
        return _vcat(*outs)

    def attend(t, i, par, q_r, k_r, v_r):
        links = [None] * par
        never = lane < (i < 0).astype(jnp.int32)
        for c, b in enumerate((i, i + 4)):
            for g in range(NG):
                o_s[c, g * GR:(g + 1) * GR, :] = attention_group(t, b, g, q_r, k_r, v_r, links)
                anchors.append(jnp.where(never, functools.reduce(jnp.add, links), 0.0))
                yield
        sums = [[], []]

        def emit(c, n, y):
            x = xres[t, i + 4 * c, n * QD:(n + 1) * QD, :] + y
            xres[t, i + 4 * c, n * QD:(n + 1) * QD, :] = x
            sums[c].append(_tile_sum(x))

        rhs = plain_rhs(o_s)
        dot = lambda s, r0, r1: _dot(_packed(wo_t, s, slice(r0 // 2, r1 // 2)), rhs(s))
        _drain(_product_t(dot, QD, c_s.at[:, :, RQ:RQ + QD], emit))
        for c in (0, 1):
            c_s[c, 0, RQ + QD:, :] = functools.reduce(jnp.add, sums[c])
        yield

    def ffn_slots(t, i, never=None):
        stats = []
        for c in (0, 1):
            s = c_s[c, 0, RQ + QD:, :]
            if c and never is not None:
                s = s + jnp.where(never, stats[0][1], 0.0)
            stats.append(_norm_stats(xres.at[t, i + 4 * c], s))
        yield
        rows = pl.ds(_aligned(i * 64, 64), 64)
        for s in range(NPASS):
            zero = 0.0 if never is None else jnp.where(never, ticks.pop(0), 0.0)[0:1]
            a_s[t, s, rows, :] = pltpu.bitcast(normed_lhs(t, i, stats, s, zero).T, u32)
            yield

    def ffn_pass(t, w_ref, s):
        get = lambda k, n: w_ref[64 * k:64 * k + 64, 128 * n:128 * n + 128]
        parts = [_signed(x, get).astype(f32) for x in PASSES[s][2::2]]
        while anchors:
            parts[0] = _vcat(parts[0][:8] + anchors.pop(), parts[0][8:])
        return _dot(pltpu.bitcast(a_s[t, s], bf16), _vcat(*parts).astype(bf16))

    def ffn_chunk(t, j, may_init=False):
        lhs, g, u = {}, {}, {}
        todo = [(g, wg, s) for s in list(range(2, NPASS)) + [0, 1]] + [(u, wu, s) for s in range(NPASS)]
        for q in range(0, 2 * NPASS, 4):
            prods = [(outs, s, ffn_pass(t, w.at[j], s)) for outs, w, s in todo[q:q + 4]]
            k2 = {2 * NPASS - 12: 0, 2 * NPASS - 4: 1}.get(q)
            blks = [] if k2 is None else [(i, 2 * k + k2) for k in (0, 1) for i in (0, 1)]
            for n, outs in enumerate((g, u)):
                _feed(outs, {s: v for o, s, v in prods if o is outs}, gu_s.at[n], blks)
            if blks:
                hs = [gu_s[(0,) + b] * u[b][1] for b in blks]
                for n, (_, lb) in enumerate(STRASSEN):
                    coefs = [c * g[b][0] * u[b][0] for c, b in zip(lb, blks)]
                    h_s[n, k2] = _form(coefs, [lambda x=x: x for x in hs])
            yield
        order = [(n, m) for n in range(7) for m in (1, 5)] + [(n, m) for n in range(7) for m in (0, 2, 3, 4, 6)]
        for q, (n, m) in enumerate(order):
            rhs = [lambda k2=k2, c2=c2: h_s[n, k2, c2 * 256:(c2 + 1) * 256, :] for k2 in (0, 1) for c2 in (0, 1)]
            if q == 14:
                lhs.clear()
            if n not in lhs:
                lhs[n] = [_form(STRASSEN[n][0],
                                [lambda r=r, k=k, r2=r2, k2=k2: wd[j, pl.ds((2 * r + r2) * QD, QD),
                                                                   pl.ds((2 * k + k2) * 128, 128)]
                                 for r in (0, 1) for k in (0, 1)])
                          for r2 in (0, 1) for k2 in (0, 1)]
            left = _form(STRASSEN[m][0], [lambda x=x: x for x in lhs[n]])
            right = _form(STRASSEN[m][1], rhs).astype(bf16)
            if q == SPLITQ:
                v = _vcat(_dot_nt(left[:80].astype(bf16), right), _dot_nt(left[80:].astype(bf16), right))
            else:
                v = _dot_nt(left.astype(bf16), right)
            for c in range(2):
                old = acc[t, c, m, n * QD:(n + 1) * QD, :]
                if may_init:
                    old = jnp.where(j > 0, old, 0.0)
                acc[t, c, m, n * QD:(n + 1) * QD, :] = old + v[:, c * 128:(c + 1) * 128]
            ticks.append(v[0:8, 0:128])
            yield

    with _scope("w_x0"):
        x_copy(0).wait()
    for c in range(NB):
        in_t1(0, c)
    for gs in WG:
        with _scope("w_qkv"):
            for g in gs:
                wqkv_copy(g).wait()
        if gs == WG[0]:
            _drain(first_norm(0, 0, xn_s.at[0, 0]))
        if gs == WG[WX]:
            x_copy(1).start()
            cwo.start()
        for g in gs:
            transpose_wqkv(g)
    _loop(9, wqkv_slots)
    with _scope("w_x1"):
        x_copy(1).wait()
    for g in range(len(groups)):
        for c in ffn_copies(g):
            c.start()
    for c in range(NB):
        in_t1(1, c)

    def run(order, gens):
        for c in order:
            if c == ".":
                ticks.clear()
            elif c == "!":
                anchors.clear()
            else:
                next(gens[c])
        _drain(*gens.values())

    def body_f(i, zero):
        never = lane < (i < 0).astype(jnp.int32)
        xn = xn_s.at[pl.ds(i, 2)]
        widen_wo(i)
        run(os.environ.get("OF0", "mmamnmamn."), {"m": first_qkv(0, i, xn.at[0, 0]), "a": first_norm(1, i, xn.at[0, 1], never),
                          "n": first_norm(0, i + 1, xn.at[1, 0], never)})
        return zero + (i < 0).astype(jnp.int32)

    with _scope("w_wo"):
        cwo.wait()
    never = lane < jax.lax.fori_loop(0, 3, body_f, 0)
    run(ORDER_F, {"m": first_qkv(0, 3, xn_s.at[3, 0]), "n": first_norm(1, 3, xn_s.at[3, 1], never),
                  "w": prep_wo(never)})
    _loop(4, lambda i: run(ORDER_E, {"m": first_qkv(1, i, xn_s.at[i, 1]), "s": attend(0, i, PAR0, q0, k0, v0),
                                     "f": ffn_slots(0, i)}))

    def wait_group(k, g):
        @pl.when(k == 0)
        def _():
            for c in ffn_copies(g):
                c.wait()

    def finish_step(i):
        u = i % 4
        never = lane < (i < 0).astype(jnp.int32)
        x1, x2 = (yield from combine(0, u, never))[:2]
        done = out_t1(u, x1) + out_t1(u + 4, x2)
        yield
        anchor(never, done)
        dst = 2 * u + (i // 8) * NB
        done = out_t2(2 * u, dst) + out_t2(2 * u + 1, dst + 1)
        yield
        anchor(never, done)
        yield

    def stage(k):
        t = k % 2
        n_a = jnp.where(jnp.logical_and(k > 0, k < 3), 4, 0)
        n_b = jnp.where(k < 3, 4, 0)
        n_c = NCH - n_a - n_b
        wait_group(k, 0)

        def body_c(i):
            pl.when(i == NCH - 1)(out_copy(0, 0, D).start)
            run(ORDER_C, {"m": ffn_chunk(t, i, True), "s": finish_step(i)})
        _loop(n_c, body_c)
        _loop(n_a, lambda i: run(ORDER_A, {"m": ffn_chunk(t, n_c + i), "s": phase1(1 - t, i)}))
        wait_group(k, 1)

        def body_b(i):
            run(ORDER_B, {"m": ffn_chunk(t, n_c + n_a + i), "s": attend(1 - t, i, PAR, q_s, k_s, v_s),
                          "f": ffn_slots(1 - t, i, lane < (i < 0).astype(jnp.int32))})
        _loop(n_b, body_b)
    _loop(4, stage)

    copies = [out_copy(0, 0, D)]

    def last_t1(g):
        for i in (0, 2, 1, 3):
            xs = yield from combine(1, i, None, 32 * g, min(32 * g + 32, QD))
            for j, x in zip((i, i + 4), xs):
                x = _pad_rows(x) if g == 4 else x
                pout[g, j * 72:j * 72 + 64, :] = pltpu.bitcast(x.astype(bf16).T, u32)

    def last_t2(g):
        r0, r1 = 32 * g, min(32 * g + 32, QD)
        for c in range(NB):
            x = pltpu.bitcast(out_words(g, c), bf16).T
            for q in range(4):
                xin[q * QD + r0:q * QD + r1, TM + c * 128:TM + (c + 1) * 128] = x[q * (r1 - r0):(q + 1) * (r1 - r0)]
        for q in range(4):
            copies.append(out_copy(1, q * QD + r0, q * QD + r1))
            copies[-1].start()

    for c in os.environ.get("OZ", "abAcBdCeDE"):
        if c.islower():
            _drain(last_t1(ord(c) - 97))
        else:
            last_t2(ord(c) - 65)
    with _scope("w_out"):
        for c in copies:
            c.wait()


@jax.jit
def pallas_interleave_layers__sliding_local_dilated__glu_gated_bilinear__prompt_kernel(
    A_x: jax.Array,
    A_wqkv: jax.Array,
    A_wo: jax.Array,
    B_x: jax.Array,
    B_w_gate: jax.Array,
    B_w_up: jax.Array,
    B_w_down: jax.Array,
):
    any_spec = pl.BlockSpec(memory_space=pl.ANY)
    qkv_scratch = [
        pltpu.VMEM((NB, NG, DH, 8, 128), f32),
        pltpu.VMEM((2 * NB, NG, DH, 8, 128), f32),
        pltpu.VMEM((2 * NB, NG, DH, 8, 128), f32),
    ]
    out_t = pl.pallas_call(
        _kernel,
        in_specs=[any_spec] * 6,
        out_specs=any_spec,
        out_shape=jax.ShapeDtypeStruct((D, S), bf16),
        scratch_shapes=[
            pltpu.VMEM((D, S), bf16),
            pltpu.VMEM((D, 3 * D), bf16),
            pltpu.VMEM((D, D), bf16),
            pltpu.VMEM((NCH, D, FC), bf16),
            pltpu.VMEM((NCH, D, FC), bf16),
            pltpu.VMEM((NCH, D, FC), bf16),
            pltpu.VMEM((NPASS, RQ, 128), bf16),
            pltpu.VMEM((NPASS, QD, 128), bf16),
            pltpu.VMEM((5, 3 * D, 128), f32),
            pltpu.VMEM((5, D, 128), f32),
            pltpu.VMEM((5, 320, 128), u32),
            pltpu.VMEM((5, HM, 128), u32),
            pltpu.VMEM((5, HM, 128), u32),
            pltpu.VMEM((5, 8 * 72, 128), u32),
            pltpu.VMEM((2, NB, D, 128), f32),
            *qkv_scratch,
            *qkv_scratch,
            pltpu.VMEM((2, 4, RQ + QD + 8, 128), f32),
            pltpu.VMEM((2, D, 128), f32),
            pltpu.VMEM((2, D, 128), f32),
            pltpu.VMEM((2, NPASS, HM // 2, 128), u32),
            pltpu.VMEM((2, 2, 4, HM, 128), f32),
            pltpu.VMEM((7, 2, HM, 128), f32),
            pltpu.VMEM((2, 2, 7, 1024, 128), f32),
            pltpu.VMEM((4, 2, NPASS, 128, 128), bf16),
            pltpu.SemaphoreType.DMA((12,)),
        ],
        compiler_params=pltpu.CompilerParams(vmem_limit_bytes=120 * 1024 * 1024),
        name="fused_layers",
    )(A_x[0].T, A_wqkv, A_wo, B_w_gate, B_w_up, B_w_down.T)
    return out_t.T[None]
```

```python
import functools
import os

import jax
import jax.numpy as jnp
import jax.experimental.pallas as pl
import jax.experimental.pallas.tpu as pltpu

S, D, F = 2048, 576, 4608
H, DH, W = 32, 18, 8
NG = H // 8
GR = 8 * DH
NB = 8
TM = NB * 128
HM = TM // 2
HD = D // 2
HQ = 3 * D // 2
FC = 512
HC = FC // 2
NCH = F // FC

_PASSES = (
    ("+01 +10", "-04 +14 +17", "-41 -43 +70 +71 +73", "-05 +15 +16", "-51 +60 +61 +62"),
    ("+10", "-04 +14", "+40 +41 -42 +43 -70 -71 -73", "-05 +15", "+50 +51 -52 -60 -61 -62"),
    ("+02 -03", "+00 -02", "+21 +23", "+01 -03", "+31 +33"),
    ("+00 -02 +03", "+00 +08", "+81 +83", "+01 +06", "-53 +63"),
    ("+01 +02 -03", "+02 -08", "+21", "+03 -07", "+31"),
    ("+00 -01", "+07", "+70", "+06", "+60 +62"),
    ("+10 -12 +13", "+10 +18", "+00", "+11 +16", "+10"),
    ("+12 -13", "+10 -12", "+00 +02", "+11 -13", "+10 +12"),
    ("-11 -12 +13", "+12 -18", "+80 +82", "+13 -17", "+72"),
    ("+10 +12", "-12 +14", "+42", "-13 +15", "+52"),
    ("-00 +02 +13", "+00 +18", "-00 +81 +83", "+01 +16", "-10 -53 +63"),
    ("+00 -02", "+08 -18", "+80 -81 -83", "+06 -16", "+53 -62 -63"),
    ("+00 +02", "+02 -04", "+20", "+03 -05", "+30"),
    ("+02", "+02 -12", "-20 +22 +23", "+03 -13", "-30 +32 +33"),
    ("+11 -13", "-08 +18", "-80 +81 -82", "-07 +17", "+43 -72 -73"),
    ("+02 -11 +13", "+08 -12", "+21 +80 +82", "+07 -13", "+31 +72"),
    ("+02 +13", "+00 -12", "+00 +02 -21 -23", "+01 -13", "+10 +12 -31 -33"),
    ("+10 -11", "+17", "+41 +43 -71 -73", "+16", "+51 -61"),
    ("+02 +12", "+12", "+00 +02 +22 +42 +80 +82", "+13", "+10 +12 +32 +52 +72"),
    ("+00 +10", "+04", "+20 +40", "+05", "+30 +50"),
    ("-00 +02 -10 +12", "+18", "+00 -80", "+16", "+10 +62"),
    ("+02 -10", "+04 -12", "+20 +42", "+05 -13", "+30 +52"),
    ("+03 +13", "+00", "+03 +21 +23 -43 -81 -83", "+01", "+13 +31 +33 -63"),
    ("+13", "-00 +10", "+01 +02 +03", "-01 +11", "+11 +12 +13"),
    ("-01 +03", "+00 +04 +07", "+43", "+01 +05 +06", "+53"),
    ("+01", "+04 +07 -14 -17", "+70 +71 +73", "+05 +06 -15 -16", "+53 +60 +61 +62"),
    ("+01 +11", "+14 +17", "-01 +41", "+15 +16", "-11 +51"),
    ("+11 -13", "+10 +14 +17", "+01", "+11 +15 +16", "+11"),
    ("+01 +13", "+00 +14 +17", "+01 +43", "+01 +15 +16", "+11 +53"),
    ("+01 -03 +11 -13", "+08", "+21 +81", "+07", "+31 +43 -73"),
)
PASSES = [[[(int(w[0] + "1"), int(w[1]), int(w[2])) for w in col.split()] for col in row] for row in _PASSES]
NPASS = len(PASSES)
LANE_TILES = ((0, 1), (2, 3), (4, 5), (7, 6), (8, 7), (5, 4))
RQ = 3 * GR
STRASSEN = (
    ((1, 0, 0, 1), (1, 0, 0, 1)),
    ((0, 0, 1, 1), (1, 0, 0, 0)),
    ((1, 0, 0, 0), (0, 1, 0, -1)),
    ((0, 0, 0, 1), (-1, 0, 1, 0)),
    ((1, 1, 0, 0), (0, 0, 0, 1)),
    ((-1, 0, 1, 0), (1, 1, 0, 0)),
    ((0, 1, 0, -1), (0, 0, 1, 1)),
)
QD = D // 4
EPS = 1e-5
WG = [[int(c) for c in x] for x in os.environ.get("WG", "34,0,1,2").split(",")]
TICK = int(os.environ.get("TICK", 32))
ORDER_F = os.environ.get("OF", "mmnwmwmwnmwmw.")
XS = int(os.environ.get("XS", 4))
NS1 = int(os.environ.get("NS1", 4))
NS2 = int(os.environ.get("NS2", 8))
SPLITQ = int(os.environ.get("SPLITQ", 48))
CLINK = int(os.environ.get("CLINK", 1))
KA = int(os.environ.get("KA", 11))
KB = int(os.environ.get("KB", 9))
PAR = int(os.environ.get("PAR", 2))
PAR0 = int(os.environ.get("PAR0", 3))
CSEG = int(os.environ.get("CSEG", 3))
ORDER_A = os.environ.get("OA", "sssssss!mmmmmmmmmmms")
KB0 = int(os.environ.get("KB0", 1))
ORDER_B = "m" * KB0 + "sm" * 8 + "m" * (KB - KB0 - 8) + "sf" + "m" * (15 - KB + int(os.environ.get("KB2", 6))) + "."
ORDER_C = os.environ.get("OC", "msmsmsmsmsmsmsmmsmms")
ORDER_E = os.environ.get("OE", "ssssssss!mmmmmmmmsf")
f32, bf16, u32 = jnp.float32, jnp.bfloat16, jnp.uint32

_dot = functools.partial(jnp.dot, preferred_element_type=f32)


def _dot_nt(a, b):
    return jax.lax.dot_general(a, b, (((1,), (1,)), ((), ())), preferred_element_type=f32)


def _vcat(*xs):
    return jnp.concatenate(xs, axis=0)


def _pad_rows(r):
    return _vcat(r, jnp.zeros((128 - r.shape[0], r.shape[1]), r.dtype))


def _add(x, y):
    return (x.astype(f32) + y.astype(f32)).astype(bf16)


def _sub(x, y):
    return (x.astype(f32) - y.astype(f32)).astype(bf16)


def _form(coefs, blocks):
    terms = [(c, blk) for c, blk in zip(coefs, blocks) if c != 0]
    if len(terms) == 1 and terms[0][0] == 1:
        return terms[0][1]()
    terms.sort(key=lambda cb: cb[0] < 0)
    out = None
    for c, blk in terms:
        v = blk().astype(f32)
        if out is None:
            out = v if c == 1 else v * c
        else:
            v = v if abs(c) == 1 else v * abs(c)
            out = out + v if c > 0 else out - v
    return out


def _signed(terms, get):
    return _form([t[0] for t in terms], [functools.partial(get, t[1], t[2]) for t in terms])


def _feed(outs, prods, ref, keep=()):
    vals = dict(prods)
    sums = {}
    for s in prods:
        for sign, i, n in PASSES[s][0]:
            sums.setdefault((i, n), {})[s] = sign
    while True:
        pairs = {}
        for terms in sums.values():
            keys = list(terms)
            for x in range(len(keys)):
                for y in range(x):
                    key = (keys[y], keys[x], terms[keys[x]] * terms[keys[y]])
                    pairs[key] = pairs.get(key, 0) + 1
        if not pairs or max(pairs.values()) < 2:
            break
        x, y, rel = max(pairs, key=pairs.get)
        vals[x, y] = vals[x] + vals[y] if rel > 0 else vals[x] - vals[y]
        for terms in sums.values():
            if x in terms and y in terms and terms[x] * terms[y] == rel:
                terms[x, y] = terms.pop(x)
                del terms[y]
    for blk, terms in sums.items():
        items = [(sign, vals[k]) for k, sign in terms.items()]
        items += [(outs[blk][0], ref[blk])] if blk in outs else []
        sign, v = items.pop(max(range(len(items)), key=lambda x: items[x][0]))
        for s2, w in items:
            v = v + w if s2 == sign else v - w
        outs[blk] = (sign, v)
        if blk not in keep:
            ref[blk] = v


def _lane_forms(get):
    get = functools.lru_cache(None)(get)
    tile = lambda g, n: pltpu.roll(get(2, n), 64, 1) if g == 5 else get(g, n)
    low = jax.lax.broadcasted_iota(jnp.int32, get(0, 0).shape, 1) < 64
    for row in PASSES:
        lo, hi = [[(c, [t[h] for t in LANE_TILES].index(k), n) for c, k, n in row[2 + 2 * h]] for h in (0, 1)]
        both = [w for w in lo if w in hi]
        rest = [[w for w in x if w not in both] for x in (lo, hi)]
        out = [_signed(both, tile)] if both else []
        if rest[0] or rest[1]:
            out.append(jnp.where(low, *[_signed(x, tile) if x else 0.0 for x in rest]))
        yield functools.reduce(jnp.add, out)


def _product_t(dot, rows, ref, emit):
    groups = [range(q, q + 4) for q in range(2, NPASS, 4)]
    groups.insert(4, range(2))
    last = {w[1:]: g for g, grp in enumerate(groups) for s in grp for w in PASSES[s][0]}
    mid = (rows + 16) // 32 * 16
    outs = {}
    for g, grp in enumerate(groups):
        prods = {s: dot(s, 0, rows) if len(grp) == 4 else _vcat(dot(s, 0, mid), dot(s, mid, rows)) for s in grp}
        done = [b for b in last if last[b] == g]
        _feed(outs, prods, ref, done)
        for b in done:
            emit(*b, outs[b][1] if outs[b][0] > 0 else -outs[b][1])
        yield


def _packed(ref, *idx):
    return pltpu.bitcast(ref.bitcast(u32)[idx], bf16)


def _norm_stats(ref, total):
    m = jnp.broadcast_to(jnp.sum(total, axis=0, keepdims=True) * (1.0 / D), (8, 128))
    s = None
    for r in range(0, D, 8):
        c = ref[r:r + 8, :] - m
        s = c * c if s is None else s + c * c
    v = jnp.sum(s, axis=0, keepdims=True) * (1.0 / D)
    return m[0:1], jax.lax.rsqrt(v + EPS)


def _tile_sum(x, zero=None):
    rows = [x[r:r + 8] for r in range(0, x.shape[0], 8)]
    return functools.reduce(jnp.add, rows[1:], rows[0] if zero is None else rows[0] + zero)


def _aligned(x, n):
    return x if isinstance(x, int) else pl.multiple_of(x, n)


def _drain(*gens):
    for gen in gens:
        for _ in gen:
            pass


def _scope(name):
    import contextlib
    return jax.named_scope(name) if os.environ.get("SCOPES") else contextlib.nullcontext()


def _loop(n, fn):
    def body(i, c):
        with _scope("it"):
            fn(i)
        return c
    jax.lax.fori_loop(0, n, body, 0)


def _kernel(x_hbm, wqkv_hbm, wo_hbm, wg_hbm, wu_hbm, wd_hbm, out_hbm,
            xin, wqkv, wo, wg, wu, wd, wqkv_t, wo_t, wperm, operm, wt_s, pin0, pin1, pout, xres,
            q0, k0, v0, q_s, k_s, v_s, c_s, o_s, n_s, a_s, gu_s, h_s, acc, xn_s, sems):
    groups = (range(5), range(5, NCH))
    lane = jax.lax.broadcasted_iota(jnp.int32, (8, 128), 1)
    anchors, ticks = [], []
    pin = (pin0, pin1)

    def anchor(never, words):
        anchors.append(jnp.where(never, pltpu.bitcast(functools.reduce(jnp.bitwise_or, words), f32), 0.0))

    def x_copy(c0, c1, sem):
        cols = pl.ds(c0 * 128, (c1 - c0) * 128)
        return pltpu.make_async_copy(x_hbm.at[:, cols], xin.at[:, cols], sems.at[sem])

    x0 = x_copy(0, NB, 2)
    x1 = [x_copy(NB, NB + XS, 2), x_copy(NB + XS, 2 * NB, 3)]

    def wqkv_copy(g):
        rows = pl.ds(g * 128, min(128, D - g * 128))
        return pltpu.make_async_copy(wqkv_hbm.at[rows], wqkv.at[rows], sems.at[4 + g])

    def out_copy(t, r0, r1):
        idx = (pl.ds(r0, r1 - r0), pl.ds(t * TM, TM))
        return pltpu.make_async_copy(xin.at[idx], out_hbm.at[idx], sems.at[t])

    def ffn_copies(g):
        return [pltpu.make_async_copy(src.at[:, pl.ds(j * FC, FC)], dst.at[j], sems.at[9 + g])
                for j in groups[g]
                for src, dst in ((wg_hbm, wg), (wu_hbm, wu), (wd_hbm, wd))]

    def wo_copy(i):
        rows = pl.ds(pl.multiple_of(i * (D // 3), 64), D // 3)
        return pltpu.make_async_copy(wo_hbm.at[rows], wo.at[rows], sems.at[4 + i])

    x0.start()
    for gs in WG:
        for g in gs:
            wqkv_copy(g).start()

    def head_rows(ref, g, base):
        return _vcat(*[ref[g, pl.ds(base + d, 8, stride=DH), :] for d in range(DH)])

    def transpose_wqkv(g):
        wperm[g] = _vcat(*[wqkv[64 * k:64 * k + 64, :].astype(f32) for k in LANE_TILES[g]]).T

    def wqkv_slots(u):
        for e in range(0, 6, 2):
            src = (u // 3) * D + (u % 3) * 6 + e
            get = lambda g, n: _vcat(*[wperm[g, pl.ds(src + n * GR + x, 8, stride=DH), :] for x in (0, 1)])
            for s, v in enumerate(_lane_forms(get)):
                wqkv_t[s, pl.ds(pl.multiple_of(u * 48, 16) + 8 * e, 16), :] = v.astype(bf16)

    def widen_wo(i):
        rows = pl.ds(pl.multiple_of(i * (D // 3), 64), D // 3)
        for g in range(5):
            cols = wo[rows, g * 128:min((g + 1) * 128, D)].astype(f32)
            if g == 4:
                cols = jnp.concatenate([cols, jnp.zeros_like(cols)], axis=1)
            operm[g, rows, :] = cols

    def prep_wo(never):
        for g in range(5):
            r = _vcat(*[head_rows(operm, g, hg * GR) for hg in range(NG)])
            tiles = [pltpu.bitcast(_vcat(*[r[64 * k:64 * k + 64] for k in ks]).astype(bf16).T, u32)
                     for ks in LANE_TILES[:5]]
            for k, w in enumerate(tiles):
                wt_s[k, g * 64:(g + 1) * 64, :] = w
            anchor(never, [w[56:64] for w in tiles])
            yield
        for r in range(0, QD // 2, 8):
            zero = pltpu.bitcast(jnp.where(never, ticks.pop(0), 0.0), u32)
            get = lambda g, n: pltpu.bitcast(wt_s[g, pl.ds(n * QD // 2 + r, 8), :] | zero, bf16).astype(f32)
            for s, v in enumerate(_lane_forms(get)):
                wo_t[s, 2 * r:2 * r + 16, :] = v.astype(bf16)
            ticks.pop(0)
            yield

    def to_words(x):
        tiles = [x[g * 128:(g + 1) * 128] for g in range(4)] + [_pad_rows(x[512:D])]
        return [pltpu.bitcast(r.astype(bf16).T, u32) for r in tiles]

    def from_words(words):
        parts = [pltpu.bitcast(w, bf16).T for w in words]
        return _vcat(*parts[:4], parts[4][:64])

    def in_t1(t, c):
        x = xin[:, pl.ds(pl.multiple_of(t * TM + c * 128, 128), 128)]
        words = to_words(x)
        for g, w in enumerate(words):
            pin[t][g, pl.ds(pl.multiple_of(c * 64, 64), 64), :] = w
        return [w[56:64] for w in words]

    def in_t2(t, j):
        return from_words([pin[t][g, pl.ds(j, 64, stride=8), :] for g in range(5)]).astype(f32)

    def out_t1(j, x):
        words = to_words(x)
        for g, w in enumerate(words):
            pout[g, pl.ds(pl.multiple_of(j * 72, 8), 64), :] = w
        return [w[56:64] for w in words]

    def out_words(g, c):
        return _vcat(*[pout[g, pl.ds(c * 8 + m, 8, stride=72), :] for m in range(8)])

    def out_t2(c, dst):
        x = from_words([out_words(g, c) for g in range(5)])
        xin[:, pl.ds(pl.multiple_of(dst * 128, 128), 128)] = x
        return [pltpu.bitcast(x[r - 16:r], u32) for r in (128, 256, 384, 512, D)]

    def combine(t, i, never=None, r0=0, r1=QD):
        c, second = i % 2, i // 2
        pick = lambda lo, hi: lo + (hi - lo) * second
        outer = lambda m1, m2, m3, m4, m5, m6, m7: (
            m1 + m4 - m5 + m7, m2 + m4, m3 + m5, m1 - m2 + m3 + m6)
        strips, sums, link = [], [], None
        for r in range(r0, r1, 8):
            get = lambda n, m: acc[t, c, m, n * QD + r:n * QD + r + 8, :]
            four, two = [], []
            for n in range(7):
                x = get(n, pick(3, 2))
                if link is not None and n % CLINK == 0:
                    x = x + jnp.where(never, link, 0.0)
                four.append(((get(n, 0) + x) + get(n, pick(6, 5))) - get(n, pick(4, 1)))
                two.append(get(n, pick(1, 4)) + x)
                if never is not None:
                    link = four[-1]
            rows = []
            for u, v in zip(outer(*four), outer(*two)):
                if isinstance(second, int):
                    rows += [v, u] if second else [u, v]
                else:
                    rows += [jnp.where(second > 0, v, u), jnp.where(second > 0, u, v)]
            strips.append([xres[t, i + 4 * (q // 4), (q % 4) * QD + r:(q % 4) * QD + r + 8, :] + v
                           for q, v in enumerate(rows)])
            if never is not None:
                sums = [functools.reduce(jnp.add, sums[n:n + 1] + strips[-1][4 * n:4 * n + 4]) for n in (0, 1)]
                link = sums[0] + sums[1]
                if len(strips) % CSEG == 0:
                    anchors.append(jnp.where(never, link, 0.0))
                    yield
        return [_vcat(*[s[q] for q in range(q0, q0 + 4) for s in strips]) for q0 in (0, 4)] + sums

    def store_qkv(t, i, r0, q, k, v, prev=None):
        def emit(c, g, x):
            b = i + 4 * c
            for r in range(0, x.shape[0], GR):
                n = (r0 + r) // GR
                y = x[r:r + GR]
                if n == 0:
                    q[b, g] = y.reshape(DH, 8, 128)
                    continue
                dst = (k, v)[n - 1]
                dst[b + NB, g] = y.reshape(DH, 8, 128)
                sh = pltpu.roll(y, 2, 1).reshape(DH, 8, 128)
                if isinstance(t, int) and t == 0:
                    dst[b, g] = sh
                elif prev is not None:
                    dst[b, g] = jnp.where((lane < 2)[None], prev[n - 1][b, g], sh)
                else:
                    pltpu.store(dst.at[b, g], sh, mask=jnp.broadcast_to((lane >= 2 * t)[None], sh.shape))
        return emit

    def plain_rhs(ref):
        get = lambda c, k: ref[c, 64 * k:64 * k + 64, :]
        return functools.lru_cache(None)(
            lambda s: _vcat(*[_signed(x, get) for x in PASSES[s][1::2]]).astype(bf16))

    def normed_lhs(t, i, stats, s, zero):
        parts = []
        for terms in PASSES[s][1::2]:
            out = []
            for c in (0, 1):
                sub = [w for w in terms if w[1] == c]
                if sub:
                    sign = max(w[0] for w in sub)
                    v = _signed([(w[0] * sign,) + w[1:] for w in sub],
                                lambda _, k: xres[t, i + 4 * c, 64 * k:64 * k + 64, :])
                    count = sign * sum(w[0] for w in sub)
                    if count:
                        v = v - stats[c][0] * count
                    out.append(v * (stats[c][1] * sign + zero))
            parts.append(functools.reduce(jnp.add, out))
        return _vcat(*parts).astype(bf16)

    def normalize(t, i, s1, s2, never):
        for c, s in enumerate((s1, s2)):
            if c and never is not None:
                s = s + jnp.where(never, r, 0.0)
            m, r = _norm_stats(xres.at[t, i + 4 * c], s)
            n_s[c] = (xres[t, i + 4 * c] - m) * r

    def phase1(t, i):
        never = lane < (i < 0).astype(jnp.int32)
        x1, x2, s1, s2 = yield from combine(t, i, never)
        xres[t, i] = x1
        xres[t, i + 4] = x2
        normalize(t, i, s1, s2, never)
        yield
        rhs = plain_rhs(n_s)
        dot = lambda s, r0, r1: _dot(_packed(wqkv_t, s, slice(r0 // 2, r1 // 2)), rhs(s))
        _drain(_product_t(dot, RQ, c_s.at[:, :, 0:RQ], store_qkv(t, i, 0, q_s, k_s, v_s)))
        yield

    def first_norm(t, i, dst, never=None):
        sums = []
        src = [xres.at[t, i + 4 * c] for c in (0, 1)]
        for c in (0, 1):
            x = in_t2(t, i + 4 * c)
            xres[t, i + 4 * c] = x
            sums.append(_tile_sum(x))
        if never is not None:
            anchors.append(jnp.where(never, sums[0] + sums[1], 0.0))
        yield
        stats = [_norm_stats(src[c], sums[c]) for c in (0, 1)]
        if never is not None:
            anchors.append(jnp.where(never, stats[0][1] + stats[1][1], 0.0))
        yield
        for s in range(NPASS):
            zero = 0.0 if never is None else jnp.where(never, ticks.pop(0), 0.0)[0:1]
            dst[s] = normed_lhs(t, i, stats, s, zero)
            yield

    def first_qkv(t, i, src):
        def dot(s, r0, r1):
            w = wqkv_t.bitcast(u32)[s, (base + r0) // 2:(base + r1) // 2]
            while anchors:
                w = _vcat(w[:8] | pltpu.bitcast(anchors.pop(), u32), w[8:])
            v = _dot(pltpu.bitcast(w, bf16), _packed(src, s))
            if s % 4 == 2:
                ticks.extend(v[r:r + 8] for r in range(0, v.shape[0], TICK))
            return v

        dsts = (q0, k0, v0) if t == 0 else (q_s, k_s, v_s, (k0, v0))
        for base, end in ((GR, RQ), (0, GR)):
            yield from _product_t(dot, end - base, c_s.at[:, :, base:end], store_qkv(t, i, base, *dsts))

    def attention_group(t, b, g, q_r, k_r, v_r, links):
        par = len(links)
        never = lane < (b < 0).astype(jnp.int32)

        def start(n, v):
            if links[n % par] is None:
                return v
            return jnp.where(never, links[n % par], 0.0) + v

        q = [q_r[b, g, d] for d in range(DH)]
        logits = []
        for w in range(W):
            l = start(w, q[0] * k_r[b + NB - w, g, 0])
            for d in range(1, DH):
                l = l + q[d] * k_r[b + NB - w, g, d]
            links[w % par] = l
            l = l * (DH ** -0.5)
            if w > 0:
                edge = jnp.where(jnp.logical_and(w > b, t == 0), 2, 0)
                l = jnp.where(lane < edge, -1e9, l)
            logits.append(l)
        m = functools.reduce(jnp.maximum, logits)
        e = [jnp.exp(l - m) for l in logits]
        r = 1.0 / functools.reduce(jnp.add, e)
        p = [x * r for x in e]
        outs = []
        for d in range(DH):
            o = p[0] * v_r[b + NB, g, d]
            if d >= par:
                o = start(d, o)
            for w in range(1, W):
                o = o + p[w] * v_r[b + NB - w, g, d]
            links[d % par] = o
            outs.append(o)
        return _vcat(*outs)

    def attend(t, i, par, q_r, k_r, v_r):
        links = [None] * par
        never = lane < (i < 0).astype(jnp.int32)
        for c, b in enumerate((i, i + 4)):
            for g in range(NG):
                o_s[c, g * GR:(g + 1) * GR, :] = attention_group(t, b, g, q_r, k_r, v_r, links)
                anchors.append(jnp.where(never, functools.reduce(jnp.add, links), 0.0))
                yield
        sums = [[], []]

        def emit(c, n, y):
            x = xres[t, i + 4 * c, n * QD:(n + 1) * QD, :] + y
            xres[t, i + 4 * c, n * QD:(n + 1) * QD, :] = x
            sums[c].append(_tile_sum(x))

        rhs = plain_rhs(o_s)
        dot = lambda s, r0, r1: _dot(_packed(wo_t, s, slice(r0 // 2, r1 // 2)), rhs(s))
        _drain(_product_t(dot, QD, c_s.at[:, :, RQ:RQ + QD], emit))
        for c in (0, 1):
            c_s[c, 0, RQ + QD:, :] = functools.reduce(jnp.add, sums[c])
        yield

    def ffn_slots(t, i, never=None):
        stats = []
        for c in (0, 1):
            s = c_s[c, 0, RQ + QD:, :]
            if c and never is not None:
                s = s + jnp.where(never, stats[0][1], 0.0)
            stats.append(_norm_stats(xres.at[t, i + 4 * c], s))
        yield
        rows = pl.ds(_aligned(i * 64, 64), 64)
        for s in range(NPASS):
            zero = 0.0 if never is None else jnp.where(never, ticks.pop(0), 0.0)[0:1]
            a_s[t, s, rows, :] = pltpu.bitcast(normed_lhs(t, i, stats, s, zero).T, u32)
            yield

    def ffn_pass(t, w_ref, s):
        get = lambda k, n: w_ref[64 * k:64 * k + 64, 128 * n:128 * n + 128]
        parts = [_signed(x, get).astype(f32) for x in PASSES[s][2::2]]
        while anchors:
            parts[0] = _vcat(parts[0][:8] + anchors.pop(), parts[0][8:])
        return _dot(pltpu.bitcast(a_s[t, s], bf16), _vcat(*parts).astype(bf16))

    def ffn_chunk(t, j, may_init=False):
        lhs, g, u = {}, {}, {}
        todo = [(g, wg, s) for s in list(range(2, NPASS)) + [0, 1]] + [(u, wu, s) for s in range(NPASS)]
        for q in range(0, 2 * NPASS, 4):
            prods = [(outs, s, ffn_pass(t, w.at[j], s)) for outs, w, s in todo[q:q + 4]]
            k2 = {2 * NPASS - 12: 0, 2 * NPASS - 4: 1}.get(q)
            blks = [] if k2 is None else [(i, 2 * k + k2) for k in (0, 1) for i in (0, 1)]
            for n, outs in enumerate((g, u)):
                _feed(outs, {s: v for o, s, v in prods if o is outs}, gu_s.at[n], blks)
            if blks:
                hs = [gu_s[(0,) + b] * u[b][1] for b in blks]
                for n, (_, lb) in enumerate(STRASSEN):
                    coefs = [c * g[b][0] * u[b][0] for c, b in zip(lb, blks)]
                    h_s[n, k2] = _form(coefs, [lambda x=x: x for x in hs])
            yield
        order = [(n, m) for n in range(7) for m in (1, 5)] + [(n, m) for n in range(7) for m in (0, 2, 3, 4, 6)]
        for q, (n, m) in enumerate(order):
            rhs = [lambda k2=k2, c2=c2: h_s[n, k2, c2 * 256:(c2 + 1) * 256, :] for k2 in (0, 1) for c2 in (0, 1)]
            if q == 14:
                lhs.clear()
            if n not in lhs:
                lhs[n] = [_form(STRASSEN[n][0],
                                [lambda r=r, k=k, r2=r2, k2=k2: wd[j, pl.ds((2 * r + r2) * QD, QD),
                                                                   pl.ds((2 * k + k2) * 128, 128)]
                                 for r in (0, 1) for k in (0, 1)])
                          for r2 in (0, 1) for k2 in (0, 1)]
            left = _form(STRASSEN[m][0], [lambda x=x: x for x in lhs[n]])
            right = _form(STRASSEN[m][1], rhs).astype(bf16)
            if q == SPLITQ:
                v = _vcat(_dot_nt(left[:80].astype(bf16), right), _dot_nt(left[80:].astype(bf16), right))
            else:
                v = _dot_nt(left.astype(bf16), right)
            for c in range(2):
                old = acc[t, c, m, n * QD:(n + 1) * QD, :]
                if may_init:
                    old = jnp.where(j > 0, old, 0.0)
                acc[t, c, m, n * QD:(n + 1) * QD, :] = old + v[:, c * 128:(c + 1) * 128]
            ticks.append(v[0:8, 0:128])
            yield

    with _scope("w_x0"):
        x0.wait()
    for c in range(NB):
        in_t1(0, c)
    for gs in WG:
        with _scope("w_qkv"):
            for g in gs:
                wqkv_copy(g).wait()
        if gs == WG[0]:
            for c in x1:
                c.start()
            _drain(first_norm(0, 0, xn_s.at[0, 0]))
        for g in gs:
            transpose_wqkv(g)
    for u in range(NS1):
        wqkv_slots(u)
    for i in range(3):
        wo_copy(i).start()
    for c, blocks, slots in zip(x1, (range(XS), range(XS, NB)), (range(NS1, NS2), range(NS2, 9))):
        with _scope("w_x1"):
            c.wait()
        for b in blocks:
            in_t1(1, b)
        for u in slots:
            wqkv_slots(u)
    for g in range(len(groups)):
        for c in ffn_copies(g):
            c.start()

    def run(order, gens):
        for c in order:
            if c == ".":
                ticks.clear()
            elif c == "!":
                anchors.clear()
            else:
                next(gens[c])
        _drain(*gens.values())

    def body_f(i, zero):
        never = lane < (i < 0).astype(jnp.int32)
        xn = xn_s.at[pl.ds(i, 2)]
        wo_copy(i).wait()
        widen_wo(i)
        run(os.environ.get("OF0", "mmamnmamn."), {"m": first_qkv(0, i, xn.at[0, 0]), "a": first_norm(1, i, xn.at[0, 1], never),
                          "n": first_norm(0, i + 1, xn.at[1, 0], never)})
        return zero + (i < 0).astype(jnp.int32)

    never = lane < jax.lax.fori_loop(0, 3, body_f, 0)
    run(ORDER_F, {"m": first_qkv(0, 3, xn_s.at[3, 0]), "n": first_norm(1, 3, xn_s.at[3, 1], never),
                  "w": prep_wo(never)})
    _loop(4, lambda i: run(ORDER_E, {"m": first_qkv(1, i, xn_s.at[i, 1]), "s": attend(0, i, PAR0, q0, k0, v0),
                                     "f": ffn_slots(0, i)}))

    def wait_group(k, g):
        @pl.when(k == 0)
        def _():
            for c in ffn_copies(g):
                c.wait()

    def finish_step(i):
        u = i % 4
        never = lane < (i < 0).astype(jnp.int32)
        x1, x2 = (yield from combine(0, u, never))[:2]
        done = out_t1(u, x1) + out_t1(u + 4, x2)
        yield
        anchor(never, done)
        dst = 2 * u + (i // 8) * NB
        done = out_t2(2 * u, dst) + out_t2(2 * u + 1, dst + 1)
        yield
        anchor(never, done)
        yield

    def stage(k):
        t = k % 2
        n_a = jnp.where(jnp.logical_and(k > 0, k < 3), 4, 0)
        n_b = jnp.where(k < 3, 4, 0)
        n_c = NCH - n_a - n_b
        wait_group(k, 0)

        def body_c(i):
            pl.when(i == NCH - 1)(out_copy(0, 0, D).start)
            run(ORDER_C, {"m": ffn_chunk(t, i, True), "s": finish_step(i)})
        _loop(n_c, body_c)
        _loop(n_a, lambda i: run(ORDER_A, {"m": ffn_chunk(t, n_c + i), "s": phase1(1 - t, i)}))
        wait_group(k, 1)

        def body_b(i):
            run(ORDER_B, {"m": ffn_chunk(t, n_c + n_a + i), "s": attend(1 - t, i, PAR, q_s, k_s, v_s),
                          "f": ffn_slots(1 - t, i, lane < (i < 0).astype(jnp.int32))})
        _loop(n_b, body_b)
    _loop(4, stage)

    copies = [out_copy(0, 0, D)]

    def last_t1(g):
        for i in (0, 2, 1, 3):
            xs = yield from combine(1, i, None, 32 * g, min(32 * g + 32, QD))
            for j, x in zip((i, i + 4), xs):
                x = _pad_rows(x) if g == 4 else x
                pout[g, j * 72:j * 72 + 64, :] = pltpu.bitcast(x.astype(bf16).T, u32)

    def last_t2(g):
        r0, r1 = 32 * g, min(32 * g + 32, QD)
        for c in range(NB):
            x = pltpu.bitcast(out_words(g, c), bf16).T
            for q in range(4):
                xin[q * QD + r0:q * QD + r1, TM + c * 128:TM + (c + 1) * 128] = x[q * (r1 - r0):(q + 1) * (r1 - r0)]
        for q in range(4):
            copies.append(out_copy(1, q * QD + r0, q * QD + r1))
            copies[-1].start()

    for c in os.environ.get("OZ", "abAcBdCeDE"):
        if c.islower():
            _drain(last_t1(ord(c) - 97))
        else:
            last_t2(ord(c) - 65)
    with _scope("w_out"):
        for c in copies:
            c.wait()


@jax.jit
def pallas_interleave_layers__sliding_local_dilated__glu_gated_bilinear__prompt_kernel(
    A_x: jax.Array,
    A_wqkv: jax.Array,
    A_wo: jax.Array,
    B_x: jax.Array,
    B_w_gate: jax.Array,
    B_w_up: jax.Array,
    B_w_down: jax.Array,
):
    any_spec = pl.BlockSpec(memory_space=pl.ANY)
    qkv_scratch = [
        pltpu.VMEM((NB, NG, DH, 8, 128), f32),
        pltpu.VMEM((2 * NB, NG, DH, 8, 128), f32),
        pltpu.VMEM((2 * NB, NG, DH, 8, 128), f32),
    ]
    out_t = pl.pallas_call(
        _kernel,
        in_specs=[any_spec] * 6,
        out_specs=any_spec,
        out_shape=jax.ShapeDtypeStruct((D, S), bf16),
        scratch_shapes=[
            pltpu.VMEM((D, S), bf16),
            pltpu.VMEM((D, 3 * D), bf16),
            pltpu.VMEM((D, D), bf16),
            pltpu.VMEM((NCH, D, FC), bf16),
            pltpu.VMEM((NCH, D, FC), bf16),
            pltpu.VMEM((NCH, D, FC), bf16),
            pltpu.VMEM((NPASS, RQ, 128), bf16),
            pltpu.VMEM((NPASS, QD, 128), bf16),
            pltpu.VMEM((5, 3 * D, 128), f32),
            pltpu.VMEM((5, D, 128), f32),
            pltpu.VMEM((5, 320, 128), u32),
            pltpu.VMEM((5, HM, 128), u32),
            pltpu.VMEM((5, HM, 128), u32),
            pltpu.VMEM((5, 8 * 72, 128), u32),
            pltpu.VMEM((2, NB, D, 128), f32),
            *qkv_scratch,
            *qkv_scratch,
            pltpu.VMEM((2, 4, RQ + QD + 8, 128), f32),
            pltpu.VMEM((2, D, 128), f32),
            pltpu.VMEM((2, D, 128), f32),
            pltpu.VMEM((2, NPASS, HM // 2, 128), u32),
            pltpu.VMEM((2, 2, 4, HM, 128), f32),
            pltpu.VMEM((7, 2, HM, 128), f32),
            pltpu.VMEM((2, 2, 7, 1024, 128), f32),
            pltpu.VMEM((4, 2, NPASS, 128, 128), bf16),
            pltpu.SemaphoreType.DMA((11,)),
        ],
        compiler_params=pltpu.CompilerParams(vmem_limit_bytes=120 * 1024 * 1024),
        name="fused_layers",
    )(A_x[0].T, A_wqkv, A_wo, B_w_gate, B_w_up, B_w_down.T)
    return out_t.T[None]
```

```python
import functools

import jax
import jax.numpy as jnp
import jax.experimental.pallas as pl
import jax.experimental.pallas.tpu as pltpu

S, D, F = 2048, 576, 4608
H, DH, W = 32, 18, 8
NG = H // 8
GR = 8 * DH
NB = 8
TM = NB * 128
HM = TM // 2
FC = 512
NCH = F // FC

_PASSES = (
    ("+01 +10", "-04 +14 +17", "-41 -43 +70 +71 +73", "-05 +15 +16", "-51 +60 +61 +62"),
    ("+10", "-04 +14", "+40 +41 -42 +43 -70 -71 -73", "-05 +15", "+50 +51 -52 -60 -61 -62"),
    ("+02 -03", "+00 -02", "+21 +23", "+01 -03", "+31 +33"),
    ("+00 -02 +03", "+00 +08", "+81 +83", "+01 +06", "-53 +63"),
    ("+01 +02 -03", "+02 -08", "+21", "+03 -07", "+31"),
    ("+00 -01", "+07", "+70", "+06", "+60 +62"),
    ("+10 -12 +13", "+10 +18", "+00", "+11 +16", "+10"),
    ("+12 -13", "+10 -12", "+00 +02", "+11 -13", "+10 +12"),
    ("-11 -12 +13", "+12 -18", "+80 +82", "+13 -17", "+72"),
    ("+10 +12", "-12 +14", "+42", "-13 +15", "+52"),
    ("-00 +02 +13", "+00 +18", "-00 +81 +83", "+01 +16", "-10 -53 +63"),
    ("+00 -02", "+08 -18", "+80 -81 -83", "+06 -16", "+53 -62 -63"),
    ("+00 +02", "+02 -04", "+20", "+03 -05", "+30"),
    ("+02", "+02 -12", "-20 +22 +23", "+03 -13", "-30 +32 +33"),
    ("+11 -13", "-08 +18", "-80 +81 -82", "-07 +17", "+43 -72 -73"),
    ("+02 -11 +13", "+08 -12", "+21 +80 +82", "+07 -13", "+31 +72"),
    ("+02 +13", "+00 -12", "+00 +02 -21 -23", "+01 -13", "+10 +12 -31 -33"),
    ("+10 -11", "+17", "+41 +43 -71 -73", "+16", "+51 -61"),
    ("+02 +12", "+12", "+00 +02 +22 +42 +80 +82", "+13", "+10 +12 +32 +52 +72"),
    ("+00 +10", "+04", "+20 +40", "+05", "+30 +50"),
    ("-00 +02 -10 +12", "+18", "+00 -80", "+16", "+10 +62"),
    ("+02 -10", "+04 -12", "+20 +42", "+05 -13", "+30 +52"),
    ("+03 +13", "+00", "+03 +21 +23 -43 -81 -83", "+01", "+13 +31 +33 -63"),
    ("+13", "-00 +10", "+01 +02 +03", "-01 +11", "+11 +12 +13"),
    ("-01 +03", "+00 +04 +07", "+43", "+01 +05 +06", "+53"),
    ("+01", "+04 +07 -14 -17", "+70 +71 +73", "+05 +06 -15 -16", "+53 +60 +61 +62"),
    ("+01 +11", "+14 +17", "-01 +41", "+15 +16", "-11 +51"),
    ("+11 -13", "+10 +14 +17", "+01", "+11 +15 +16", "+11"),
    ("+01 +13", "+00 +14 +17", "+01 +43", "+01 +15 +16", "+11 +53"),
    ("+01 -03 +11 -13", "+08", "+21 +81", "+07", "+31 +43 -73"),
)
PASSES = [[[(int(w[0] + "1"), int(w[1]), int(w[2])) for w in col.split()] for col in row] for row in _PASSES]
NPASS = len(PASSES)
LANE_TILES = ((0, 1), (2, 3), (4, 5), (7, 6), (8, 7), (5, 4))
RQ = 3 * GR
STRASSEN = (
    ((1, 0, 0, 1), (1, 0, 0, 1)),
    ((0, 0, 1, 1), (1, 0, 0, 0)),
    ((1, 0, 0, 0), (0, 1, 0, -1)),
    ((0, 0, 0, 1), (-1, 0, 1, 0)),
    ((1, 1, 0, 0), (0, 0, 0, 1)),
    ((-1, 0, 1, 0), (1, 1, 0, 0)),
    ((0, 1, 0, -1), (0, 0, 1, 1)),
)
QD = D // 4
EPS = 1e-5

WQKV_GROUPS = ((3, 4), (0,), (1,), (2,))
TICK = 32
PAR = 2
ORDER_F = "mmamnmamn."
ORDER_F_LAST = "mmnwmwmwnmwmw."
ORDER_E = "mmsmsmsmmsmsmmsmmsmmsmf.mm" + "fffffs" * 5
ORDER_A = "sssssss!mmmmmmmmmmms"
ORDER_B = "mm" + "smsmm" * 3 + "smsm" + "sf" + "m" * 13 + "."
ORDER_C = "msmsmsmsmsmsmsmmsmms"
ORDER_Z = "abAcBdCeDE"
f32, bf16, u32 = jnp.float32, jnp.bfloat16, jnp.uint32

_dot = functools.partial(jnp.dot, preferred_element_type=f32)


def _dot_nt(a, b):
    return jax.lax.dot_general(a, b, (((1,), (1,)), ((), ())), preferred_element_type=f32)


def _vcat(*xs):
    return jnp.concatenate(xs, axis=0)


def _pad_rows(r):
    return _vcat(r, jnp.zeros((128 - r.shape[0], r.shape[1]), r.dtype))


def _form(coefs, blocks):
    terms = [(c, blk) for c, blk in zip(coefs, blocks) if c != 0]
    if len(terms) == 1 and terms[0][0] == 1:
        return terms[0][1]()
    terms.sort(key=lambda cb: cb[0] < 0)
    out = None
    for c, blk in terms:
        v = blk().astype(f32)
        if out is None:
            out = v if c == 1 else v * c
        else:
            v = v if abs(c) == 1 else v * abs(c)
            out = out + v if c > 0 else out - v
    return out


def _signed(terms, get):
    return _form([t[0] for t in terms], [functools.partial(get, t[1], t[2]) for t in terms])


def _feed(outs, prods, ref, keep=()):
    vals = dict(prods)
    sums = {}
    for s in prods:
        for sign, i, n in PASSES[s][0]:
            sums.setdefault((i, n), {})[s] = sign
    while True:
        pairs = {}
        for terms in sums.values():
            keys = list(terms)
            for x in range(len(keys)):
                for y in range(x):
                    key = (keys[y], keys[x], terms[keys[x]] * terms[keys[y]])
                    pairs[key] = pairs.get(key, 0) + 1
        if not pairs or max(pairs.values()) < 2:
            break
        x, y, rel = max(pairs, key=pairs.get)
        vals[x, y] = vals[x] + vals[y] if rel > 0 else vals[x] - vals[y]
        for terms in sums.values():
            if x in terms and y in terms and terms[x] * terms[y] == rel:
                terms[x, y] = terms.pop(x)
                del terms[y]
    for blk, terms in sums.items():
        items = [(sign, vals[k]) for k, sign in terms.items()]
        items += [(outs[blk][0], ref[blk])] if blk in outs else []
        sign, v = items.pop(max(range(len(items)), key=lambda x: items[x][0]))
        for s2, w in items:
            v = v + w if s2 == sign else v - w
        outs[blk] = (sign, v)
        if blk not in keep:
            ref[blk] = v


def _lane_forms(get):
    get = functools.lru_cache(None)(get)
    tile = lambda g, n: pltpu.roll(get(2, n), 64, 1) if g == 5 else get(g, n)
    low = jax.lax.broadcasted_iota(jnp.int32, get(0, 0).shape, 1) < 64
    for row in PASSES:
        lo, hi = [[(c, [t[h] for t in LANE_TILES].index(k), n) for c, k, n in row[2 + 2 * h]] for h in (0, 1)]
        both = [w for w in lo if w in hi]
        rest = [[w for w in x if w not in both] for x in (lo, hi)]
        out = [_signed(both, tile)] if both else []
        if rest[0] or rest[1]:
            out.append(jnp.where(low, *[_signed(x, tile) if x else 0.0 for x in rest]))
        yield functools.reduce(jnp.add, out)


def _product_t(dot, rows, ref, emit):
    groups = [range(q, q + 4) for q in range(2, NPASS, 4)]
    groups.insert(4, range(2))
    last = {w[1:]: g for g, grp in enumerate(groups) for s in grp for w in PASSES[s][0]}
    mid = (rows + 16) // 32 * 16
    outs = {}
    for g, grp in enumerate(groups):
        prods = {s: dot(s, 0, rows) if len(grp) == 4 else _vcat(dot(s, 0, mid), dot(s, mid, rows)) for s in grp}
        done = [b for b in last if last[b] == g]
        _feed(outs, prods, ref, done)
        for b in done:
            emit(*b, outs[b][1] if outs[b][0] > 0 else -outs[b][1])
        yield


def _packed(ref, *idx):
    return pltpu.bitcast(ref.bitcast(u32)[idx], bf16)


def _norm_stats(ref, total):
    m = jnp.broadcast_to(jnp.sum(total, axis=0, keepdims=True) * (1.0 / D), (8, 128))
    s = None
    for r in range(0, D, 8):
        c = ref[r:r + 8, :] - m
        s = c * c if s is None else s + c * c
    v = jnp.sum(s, axis=0, keepdims=True) * (1.0 / D)
    return m[0:1], jax.lax.rsqrt(v + EPS)


def _tile_sum(x):
    return functools.reduce(jnp.add, [x[r:r + 8] for r in range(0, x.shape[0], 8)])


def _aligned(x, n):
    return x if isinstance(x, int) else pl.multiple_of(x, n)


def _drain(*gens):
    for gen in gens:
        for _ in gen:
            pass


def _loop(n, fn):
    def body(i, c):
        fn(i)
        return c
    jax.lax.fori_loop(0, n, body, 0)


def _kernel(x_hbm, wqkv_hbm, wo_hbm, wg_hbm, wu_hbm, wd_hbm, out_hbm,
            xin, wqkv, wo, wg, wu, wd, wqkv_t, wo_t, wperm, operm, wt_s, pin0, pin1, pout, xres,
            q0, k0, v0, q_s, k_s, v_s, c_s, o_s, n_s, a_s, gu_s, h_s, acc, xn_s, sems):
    groups = (range(5), range(5, NCH))
    lane = jax.lax.broadcasted_iota(jnp.int32, (8, 128), 1)
    anchors, ticks = [], []
    pin = (pin0, pin1)

    def anchor(never, words):
        anchors.append(jnp.where(never, pltpu.bitcast(functools.reduce(jnp.bitwise_or, words), f32), 0.0))

    def x_copy(c0, c1, sem):
        cols = pl.ds(c0 * 128, (c1 - c0) * 128)
        return pltpu.make_async_copy(x_hbm.at[:, cols], xin.at[:, cols], sems.at[sem])

    x0 = x_copy(0, NB, 2)
    x1 = [x_copy(NB, NB + 4, 2), x_copy(NB + 4, 2 * NB, 3)]

    def wqkv_copy(g):
        rows = pl.ds(g * 128, min(128, D - g * 128))
        return pltpu.make_async_copy(wqkv_hbm.at[rows], wqkv.at[rows], sems.at[4 + g])

    def out_copy(t, r0, r1):
        idx = (pl.ds(r0, r1 - r0), pl.ds(t * TM, TM))
        return pltpu.make_async_copy(xin.at[idx], out_hbm.at[idx], sems.at[t])

    def ffn_copies(g):
        return [pltpu.make_async_copy(src.at[:, pl.ds(j * FC, FC)], dst.at[j], sems.at[9 + g])
                for j in groups[g]
                for src, dst in ((wg_hbm, wg), (wu_hbm, wu), (wd_hbm, wd))]

    def wo_copy(i):
        rows = pl.ds(pl.multiple_of(i * (D // 3), 64), D // 3)
        return pltpu.make_async_copy(wo_hbm.at[rows], wo.at[rows], sems.at[4 + i])

    x0.start()
    for gs in WQKV_GROUPS:
        for g in gs:
            wqkv_copy(g).start()

    def head_rows(ref, g, base):
        return _vcat(*[ref[g, pl.ds(base + d, 8, stride=DH), :] for d in range(DH)])

    def transpose_wqkv(g):
        wperm[g] = _vcat(*[wqkv[64 * k:64 * k + 64, :].astype(f32) for k in LANE_TILES[g]]).T

    def wqkv_slots(u):
        for e in range(0, 6, 2):
            src = (u // 3) * D + (u % 3) * 6 + e
            get = lambda g, n: _vcat(*[wperm[g, pl.ds(src + n * GR + x, 8, stride=DH), :] for x in (0, 1)])
            for s, v in enumerate(_lane_forms(get)):
                wqkv_t[s, pl.ds(pl.multiple_of(u * 48, 16) + 8 * e, 16), :] = v.astype(bf16)

    def widen_wo(i):
        rows = pl.ds(pl.multiple_of(i * (D // 3), 64), D // 3)
        for g in range(5):
            cols = wo[rows, g * 128:min((g + 1) * 128, D)].astype(f32)
            if g == 4:
                cols = jnp.concatenate([cols, jnp.zeros_like(cols)], axis=1)
            operm[g, rows, :] = cols

    def prep_wo(never):
        for g in range(5):
            r = _vcat(*[head_rows(operm, g, hg * GR) for hg in range(NG)])
            tiles = [pltpu.bitcast(_vcat(*[r[64 * k:64 * k + 64] for k in ks]).astype(bf16).T, u32)
                     for ks in LANE_TILES[:5]]
            for k, w in enumerate(tiles):
                wt_s[k, g * 64:(g + 1) * 64, :] = w
            anchor(never, [w[56:64] for w in tiles])
            yield
        for r in range(0, QD // 2, 8):
            zero = pltpu.bitcast(jnp.where(never, ticks.pop(0), 0.0), u32)
            get = lambda g, n: pltpu.bitcast(wt_s[g, pl.ds(n * QD // 2 + r, 8), :] | zero, bf16).astype(f32)
            for s, v in enumerate(_lane_forms(get)):
                wo_t[s, 2 * r:2 * r + 16, :] = v.astype(bf16)
            ticks.pop(0)
            yield

    def to_words(x):
        tiles = [x[g * 128:(g + 1) * 128] for g in range(4)] + [_pad_rows(x[512:D])]
        return [pltpu.bitcast(r.astype(bf16).T, u32) for r in tiles]

    def from_words(words):
        parts = [pltpu.bitcast(w, bf16).T for w in words]
        return _vcat(*parts[:4], parts[4][:64])

    def in_t1(t, c):
        x = xin[:, pl.ds(pl.multiple_of(t * TM + c * 128, 128), 128)]
        words = to_words(x)
        for g, w in enumerate(words):
            pin[t][g, pl.ds(pl.multiple_of(c * 64, 64), 64), :] = w
        return [w[56:64] for w in words]

    def in_t2(t, j):
        return from_words([pin[t][g, pl.ds(j, 64, stride=8), :] for g in range(5)]).astype(f32)

    def out_t1(j, x):
        words = to_words(x)
        for g, w in enumerate(words):
            pout[g, pl.ds(pl.multiple_of(j * 72, 8), 64), :] = w
        return [w[56:64] for w in words]

    def out_words(g, c):
        return _vcat(*[pout[g, pl.ds(c * 8 + m, 8, stride=72), :] for m in range(8)])

    def out_t2(c, dst):
        x = from_words([out_words(g, c) for g in range(5)])
        xin[:, pl.ds(pl.multiple_of(dst * 128, 128), 128)] = x
        return [pltpu.bitcast(x[r - 16:r], u32) for r in (128, 256, 384, 512, D)]

    def combine(t, i, never=None, r0=0, r1=QD):
        c, second = i % 2, i // 2
        pick = lambda lo, hi: lo + (hi - lo) * second
        outer = lambda m1, m2, m3, m4, m5, m6, m7: (
            m1 + m4 - m5 + m7, m2 + m4, m3 + m5, m1 - m2 + m3 + m6)
        strips, sums, link = [], [], None
        for r in range(r0, r1, 8):
            get = lambda n, m: acc[t, c, m, n * QD + r:n * QD + r + 8, :]
            four, two = [], []
            for n in range(7):
                x = get(n, pick(3, 2))
                if link is not None:
                    x = x + jnp.where(never, link, 0.0)
                four.append(((get(n, 0) + x) + get(n, pick(6, 5))) - get(n, pick(4, 1)))
                two.append(get(n, pick(1, 4)) + x)
                if never is not None:
                    link = four[-1]
            rows = []
            for u, v in zip(outer(*four), outer(*two)):
                if isinstance(second, int):
                    rows += [v, u] if second else [u, v]
                else:
                    rows += [jnp.where(second > 0, v, u), jnp.where(second > 0, u, v)]
            strips.append([xres[t, i + 4 * (q // 4), (q % 4) * QD + r:(q % 4) * QD + r + 8, :] + v
                           for q, v in enumerate(rows)])
            if never is not None:
                sums = [functools.reduce(jnp.add, sums[n:n + 1] + strips[-1][4 * n:4 * n + 4]) for n in (0, 1)]
                link = sums[0] + sums[1]
                if len(strips) % 3 == 0:
                    anchors.append(jnp.where(never, link, 0.0))
                    yield
        return [_vcat(*[s[q] for q in range(q0, q0 + 4) for s in strips]) for q0 in (0, 4)] + sums

    def store_qkv(t, i, r0, q, k, v, prev=None):
        def emit(c, g, x):
            b = i + 4 * c
            for r in range(0, x.shape[0], GR):
                n = (r0 + r) // GR
                y = x[r:r + GR]
                if n == 0:
                    q[b, g] = y.reshape(DH, 8, 128)
                    continue
                dst = (k, v)[n - 1]
                dst[b + NB, g] = y.reshape(DH, 8, 128)
                sh = pltpu.roll(y, 2, 1).reshape(DH, 8, 128)
                if isinstance(t, int) and t == 0:
                    dst[b, g] = sh
                elif prev is not None:
                    dst[b, g] = jnp.where((lane < 2)[None], prev[n - 1][b, g], sh)
                else:
                    pltpu.store(dst.at[b, g], sh, mask=jnp.broadcast_to((lane >= 2 * t)[None], sh.shape))
        return emit

    def plain_rhs(ref):
        get = lambda c, k: ref[c, 64 * k:64 * k + 64, :]
        return functools.lru_cache(None)(
            lambda s: _vcat(*[_signed(x, get) for x in PASSES[s][1::2]]).astype(bf16))

    def normed_lhs(t, i, stats, s, zero):
        parts = []
        for terms in PASSES[s][1::2]:
            out = []
            for c in (0, 1):
                sub = [w for w in terms if w[1] == c]
                if sub:
                    sign = max(w[0] for w in sub)
                    v = _signed([(w[0] * sign,) + w[1:] for w in sub],
                                lambda _, k: xres[t, i + 4 * c, 64 * k:64 * k + 64, :])
                    count = sign * sum(w[0] for w in sub)
                    if count:
                        v = v - stats[c][0] * count
                    out.append(v * (stats[c][1] * sign + zero))
            parts.append(functools.reduce(jnp.add, out))
        return _vcat(*parts).astype(bf16)

    def normalize(t, i, s1, s2, never):
        for c, s in enumerate((s1, s2)):
            if c and never is not None:
                s = s + jnp.where(never, r, 0.0)
            m, r = _norm_stats(xres.at[t, i + 4 * c], s)
            n_s[c] = (xres[t, i + 4 * c] - m) * r

    def phase1(t, i):
        never = lane < (i < 0).astype(jnp.int32)
        x1, x2, s1, s2 = yield from combine(t, i, never)
        xres[t, i] = x1
        xres[t, i + 4] = x2
        normalize(t, i, s1, s2, never)
        yield
        rhs = plain_rhs(n_s)
        dot = lambda s, r0, r1: _dot(_packed(wqkv_t, s, slice(r0 // 2, r1 // 2)), rhs(s))
        _drain(_product_t(dot, RQ, c_s.at[:, :, 0:RQ], store_qkv(t, i, 0, q_s, k_s, v_s)))
        yield

    def first_norm(t, i, dst, never=None):
        sums = []
        src = [xres.at[t, i + 4 * c] for c in (0, 1)]
        for c in (0, 1):
            x = in_t2(t, i + 4 * c)
            xres[t, i + 4 * c] = x
            sums.append(_tile_sum(x))
        if never is not None:
            anchors.append(jnp.where(never, sums[0] + sums[1], 0.0))
        yield
        stats = [_norm_stats(src[c], sums[c]) for c in (0, 1)]
        if never is not None:
            anchors.append(jnp.where(never, stats[0][1] + stats[1][1], 0.0))
        yield
        for s in range(NPASS):
            zero = 0.0 if never is None else jnp.where(never, ticks.pop(0), 0.0)[0:1]
            dst[s] = normed_lhs(t, i, stats, s, zero)
            yield

    def first_qkv(t, i, src):
        def dot(s, r0, r1):
            w = wqkv_t.bitcast(u32)[s, (base + r0) // 2:(base + r1) // 2]
            while anchors:
                w = _vcat(w[:8] | pltpu.bitcast(anchors.pop(), u32), w[8:])
            v = _dot(pltpu.bitcast(w, bf16), _packed(src, s))
            if s % 4 == 2:
                ticks.extend(v[r:r + 8] for r in range(0, v.shape[0], TICK))
            return v

        dsts = (q0, k0, v0) if t == 0 else (q_s, k_s, v_s, (k0, v0))
        for base, end in ((GR, RQ), (0, GR)):
            yield from _product_t(dot, end - base, c_s.at[:, :, base:end], store_qkv(t, i, base, *dsts))

    def attention_group(t, b, g, q_r, k_r, v_r, links):
        par = len(links)
        never = lane < (b < 0).astype(jnp.int32)

        def start(n, v):
            if links[n % par] is None:
                return v
            return jnp.where(never, links[n % par], 0.0) + v

        q = [q_r[b, g, d] for d in range(DH)]
        logits = []
        for w in range(W):
            l = start(w, q[0] * k_r[b + NB - w, g, 0])
            for d in range(1, DH):
                l = l + q[d] * k_r[b + NB - w, g, d]
            links[w % par] = l
            l = l * (DH ** -0.5)
            if w > 0:
                edge = jnp.where(jnp.logical_and(w > b, t == 0), 2, 0)
                l = jnp.where(lane < edge, -1e9, l)
            logits.append(l)
        m = functools.reduce(jnp.maximum, logits)
        e = [jnp.exp(l - m) for l in logits]
        r = 1.0 / functools.reduce(jnp.add, e)
        p = [x * r for x in e]
        outs = []
        for d in range(DH):
            o = p[0] * v_r[b + NB, g, d]
            if d >= par:
                o = start(d, o)
            for w in range(1, W):
                o = o + p[w] * v_r[b + NB - w, g, d]
            links[d % par] = o
            outs.append(o)
        return _vcat(*outs)

    def attend(t, i, q_r, k_r, v_r, fine=False):
        links = [None] * PAR
        never = lane < (i < 0).astype(jnp.int32)
        for c, b in enumerate((i, i + 4)):
            for g in range(NG):
                o_s[c, g * GR:(g + 1) * GR, :] = attention_group(t, b, g, q_r, k_r, v_r, links)
                anchors.append(jnp.where(never, functools.reduce(jnp.add, links), 0.0))
                yield
        sums = [[], []]

        def emit(c, n, y):
            x = xres[t, i + 4 * c, n * QD:(n + 1) * QD, :] + y
            xres[t, i + 4 * c, n * QD:(n + 1) * QD, :] = x
            sums[c].append(_tile_sum(x))

        rhs = plain_rhs(o_s)

        def dot(s, r0, r1):
            v = _dot(_packed(wo_t, s, slice(r0 // 2, r1 // 2)), rhs(s))
            if fine and s % 4 == 2:
                ticks.extend(v[r:r + 8] for r in range(0, v.shape[0], TICK))
            return v

        steps = _product_t(dot, QD, c_s.at[:, :, RQ:RQ + QD], emit)
        if fine:
            yield from steps
        _drain(steps)
        for c in (0, 1):
            c_s[c, 0, RQ + QD:, :] = functools.reduce(jnp.add, sums[c])
        yield

    def ffn_slots(t, i, never=None):
        stats = []
        for c in (0, 1):
            s = c_s[c, 0, RQ + QD:, :]
            if c and never is not None:
                s = s + jnp.where(never, stats[0][1], 0.0)
            stats.append(_norm_stats(xres.at[t, i + 4 * c], s))
        yield
        rows = pl.ds(_aligned(i * 64, 64), 64)
        for s in range(NPASS):
            zero = 0.0 if never is None else jnp.where(never, ticks.pop(0), 0.0)[0:1]
            a_s[t, s, rows, :] = pltpu.bitcast(normed_lhs(t, i, stats, s, zero).T, u32)
            yield

    def ffn_pass(t, w_ref, s):
        get = lambda k, n: w_ref[64 * k:64 * k + 64, 128 * n:128 * n + 128]
        parts = [_signed(x, get).astype(f32) for x in PASSES[s][2::2]]
        while anchors:
            parts[0] = _vcat(parts[0][:8] + anchors.pop(), parts[0][8:])
        return _dot(pltpu.bitcast(a_s[t, s], bf16), _vcat(*parts).astype(bf16))

    def ffn_chunk(t, j, may_init=False):
        lhs, g, u = {}, {}, {}
        todo = [(g, wg, s) for s in list(range(2, NPASS)) + [0, 1]] + [(u, wu, s) for s in range(NPASS)]
        for q in range(0, 2 * NPASS, 4):
            prods = [(outs, s, ffn_pass(t, w.at[j], s)) for outs, w, s in todo[q:q + 4]]
            k2 = {2 * NPASS - 12: 0, 2 * NPASS - 4: 1}.get(q)
            blks = [] if k2 is None else [(i, 2 * k + k2) for k in (0, 1) for i in (0, 1)]
            for n, outs in enumerate((g, u)):
                _feed(outs, {s: v for o, s, v in prods if o is outs}, gu_s.at[n], blks)
            if blks:
                hs = [gu_s[(0,) + b] * u[b][1] for b in blks]
                for n, (_, lb) in enumerate(STRASSEN):
                    coefs = [c * g[b][0] * u[b][0] for c, b in zip(lb, blks)]
                    h_s[n, k2] = _form(coefs, [lambda x=x: x for x in hs])
            yield
        order = [(n, m) for n in range(7) for m in (1, 5)] + [(n, m) for n in range(7) for m in (0, 2, 3, 4, 6)]
        for q, (n, m) in enumerate(order):
            rhs = [lambda k2=k2, c2=c2: h_s[n, k2, c2 * 256:(c2 + 1) * 256, :] for k2 in (0, 1) for c2 in (0, 1)]
            if q == 14:
                lhs.clear()
            if n not in lhs:
                lhs[n] = [_form(STRASSEN[n][0],
                                [lambda r=r, k=k, r2=r2, k2=k2: wd[j, pl.ds((2 * r + r2) * QD, QD),
                                                                   pl.ds((2 * k + k2) * 128, 128)]
                                 for r in (0, 1) for k in (0, 1)])
                          for r2 in (0, 1) for k2 in (0, 1)]
            left = _form(STRASSEN[m][0], [lambda x=x: x for x in lhs[n]])
            right = _form(STRASSEN[m][1], rhs).astype(bf16)
            if q == 48:
                v = _vcat(_dot_nt(left[:80].astype(bf16), right), _dot_nt(left[80:].astype(bf16), right))
            else:
                v = _dot_nt(left.astype(bf16), right)
            for c in range(2):
                old = acc[t, c, m, n * QD:(n + 1) * QD, :]
                if may_init:
                    old = jnp.where(j > 0, old, 0.0)
                acc[t, c, m, n * QD:(n + 1) * QD, :] = old + v[:, c * 128:(c + 1) * 128]
            ticks.append(v[0:8, 0:128])
            yield

    x0.wait()
    for c in range(NB):
        in_t1(0, c)
    for gs in WQKV_GROUPS:
        for g in gs:
            wqkv_copy(g).wait()
        if gs == WQKV_GROUPS[0]:
            for c in x1:
                c.start()
            _drain(first_norm(0, 0, xn_s.at[0, 0]))
        for g in gs:
            transpose_wqkv(g)
    for u in range(4):
        wqkv_slots(u)
    for i in range(3):
        wo_copy(i).start()
    for c, blocks, slots in zip(x1, (range(4), range(4, NB)), (range(4, 8), range(8, 9))):
        c.wait()
        for b in blocks:
            in_t1(1, b)
        for u in slots:
            wqkv_slots(u)
    for g in range(len(groups)):
        for c in ffn_copies(g):
            c.start()

    def run(order, gens):
        for c in order:
            if c == ".":
                ticks.clear()
            elif c == "!":
                anchors.clear()
            else:
                next(gens[c])
        _drain(*gens.values())

    def body_f(i, zero):
        never = lane < (i < 0).astype(jnp.int32)
        xn = xn_s.at[pl.ds(i, 2)]
        wo_copy(i).wait()
        widen_wo(i)
        run(ORDER_F, {"m": first_qkv(0, i, xn.at[0, 0]), "a": first_norm(1, i, xn.at[0, 1], never),
                      "n": first_norm(0, i + 1, xn.at[1, 0], never)})
        return zero + (i < 0).astype(jnp.int32)

    never = lane < jax.lax.fori_loop(0, 3, body_f, 0)
    run(ORDER_F_LAST, {"m": first_qkv(0, 3, xn_s.at[3, 0]), "n": first_norm(1, 3, xn_s.at[3, 1], never),
                       "w": prep_wo(never)})

    def body_e(i):
        never = lane < (i < 0).astype(jnp.int32)
        run(ORDER_E, {"m": first_qkv(1, i, xn_s.at[i, 1]), "f": ffn_slots(0, jnp.maximum(i - 1, 0), never),
                      "s": attend(0, i, q0, k0, v0, True)})
    _loop(4, body_e)
    _drain(ffn_slots(0, 3))

    def wait_group(k, g):
        @pl.when(k == 0)
        def _():
            for c in ffn_copies(g):
                c.wait()

    def finish_step(i):
        u = i % 4
        never = lane < (i < 0).astype(jnp.int32)
        x1, x2 = (yield from combine(0, u, never))[:2]
        done = out_t1(u, x1) + out_t1(u + 4, x2)
        yield
        anchor(never, done)
        dst = 2 * u + (i // 8) * NB
        done = out_t2(2 * u, dst) + out_t2(2 * u + 1, dst + 1)
        yield
        anchor(never, done)
        yield

    def stage(k):
        t = k % 2
        n_a = jnp.where(jnp.logical_and(k > 0, k < 3), 4, 0)
        n_b = jnp.where(k < 3, 4, 0)
        n_c = NCH - n_a - n_b
        wait_group(k, 0)

        def body_c(i):
            pl.when(i == NCH - 1)(out_copy(0, 0, D).start)
            run(ORDER_C, {"m": ffn_chunk(t, i, True), "s": finish_step(i)})
        _loop(n_c, body_c)
        _loop(n_a, lambda i: run(ORDER_A, {"m": ffn_chunk(t, n_c + i), "s": phase1(1 - t, i)}))
        wait_group(k, 1)

        def body_b(i):
            run(ORDER_B, {"m": ffn_chunk(t, n_c + n_a + i), "s": attend(1 - t, i, q_s, k_s, v_s),
                          "f": ffn_slots(1 - t, i, lane < (i < 0).astype(jnp.int32))})
        _loop(n_b, body_b)
    _loop(4, stage)

    copies = [out_copy(0, 0, D)]

    def last_t1(g):
        for i in (0, 2, 1, 3):
            xs = yield from combine(1, i, None, 32 * g, min(32 * g + 32, QD))
            for j, x in zip((i, i + 4), xs):
                x = _pad_rows(x) if g == 4 else x
                pout[g, j * 72:j * 72 + 64, :] = pltpu.bitcast(x.astype(bf16).T, u32)

    def last_t2(g):
        r0, r1 = 32 * g, min(32 * g + 32, QD)
        for c in range(NB):
            x = pltpu.bitcast(out_words(g, c), bf16).T
            for q in range(4):
                xin[q * QD + r0:q * QD + r1, TM + c * 128:TM + (c + 1) * 128] = x[q * (r1 - r0):(q + 1) * (r1 - r0)]
        for q in range(4):
            copies.append(out_copy(1, q * QD + r0, q * QD + r1))
            copies[-1].start()

    for c in ORDER_Z:
        if c.islower():
            _drain(last_t1(ord(c) - 97))
        else:
            last_t2(ord(c) - 65)
    for c in copies:
        c.wait()


@jax.jit
def pallas_interleave_layers__sliding_local_dilated__glu_gated_bilinear__prompt_kernel(
    A_x: jax.Array,
    A_wqkv: jax.Array,
    A_wo: jax.Array,
    B_x: jax.Array,
    B_w_gate: jax.Array,
    B_w_up: jax.Array,
    B_w_down: jax.Array,
):
    any_spec = pl.BlockSpec(memory_space=pl.ANY)
    qkv_scratch = [
        pltpu.VMEM((NB, NG, DH, 8, 128), f32),
        pltpu.VMEM((2 * NB, NG, DH, 8, 128), f32),
        pltpu.VMEM((2 * NB, NG, DH, 8, 128), f32),
    ]
    out_t = pl.pallas_call(
        _kernel,
        in_specs=[any_spec] * 6,
        out_specs=any_spec,
        out_shape=jax.ShapeDtypeStruct((D, S), bf16),
        scratch_shapes=[
            pltpu.VMEM((D, S), bf16),
            pltpu.VMEM((D, 3 * D), bf16),
            pltpu.VMEM((D, D), bf16),
            pltpu.VMEM((NCH, D, FC), bf16),
            pltpu.VMEM((NCH, D, FC), bf16),
            pltpu.VMEM((NCH, D, FC), bf16),
            pltpu.VMEM((NPASS, RQ, 128), bf16),
            pltpu.VMEM((NPASS, QD, 128), bf16),
            pltpu.VMEM((5, 3 * D, 128), f32),
            pltpu.VMEM((5, D, 128), f32),
            pltpu.VMEM((5, 320, 128), u32),
            pltpu.VMEM((5, HM, 128), u32),
            pltpu.VMEM((5, HM, 128), u32),
            pltpu.VMEM((5, 8 * 72, 128), u32),
            pltpu.VMEM((2, NB, D, 128), f32),
            *qkv_scratch,
            *qkv_scratch,
            pltpu.VMEM((2, 4, RQ + QD + 8, 128), f32),
            pltpu.VMEM((2, D, 128), f32),
            pltpu.VMEM((2, D, 128), f32),
            pltpu.VMEM((2, NPASS, HM // 2, 128), u32),
            pltpu.VMEM((2, 2, 4, HM, 128), f32),
            pltpu.VMEM((7, 2, HM, 128), f32),
            pltpu.VMEM((2, 2, 7, 1024, 128), f32),
            pltpu.VMEM((4, 2, NPASS, 128, 128), bf16),
            pltpu.SemaphoreType.DMA((11,)),
        ],
        compiler_params=pltpu.CompilerParams(vmem_limit_bytes=120 * 1024 * 1024),
        name="fused_layers",
    )(A_x[0].T, A_wqkv, A_wo, B_w_gate, B_w_up, B_w_down.T)
    return out_t.T[None]
```
